```python
import jax
import jax.numpy as jnp

def _softmax(x, axis=-1):
    return jax.nn.softmax(x, axis=axis)

def _gelu(x):
    return jax.nn.gelu(x, approximate=True)

def _silu(x):
    return jax.nn.silu(x)

def _sigmoid(x):
    return jax.nn.sigmoid(x)

def _layernorm(x, axis=-1, eps=1e-05):
    m = jnp.mean(x, axis=axis, keepdims=True)
    v = jnp.var(x, axis=axis, keepdims=True)
    return (x - m) / jnp.sqrt(v + eps)

def _scatter_add(tgt, idx, src, axis=0):
    return tgt.at[idx].add(src)

def _segment_sum(src, seg, n):
    return jax.ops.segment_sum(src, seg, n)

class _Rng:

    def __init__(self, key):
        self._k = key

    def _next(self):
        self._k, sub = jax.random.split(self._k)
        return sub

    def normal(self, shape):
        return jax.random.normal(self._next(), shape, dtype=jnp.bfloat16)

    def randint(self, lo, hi, shape):
        return jax.random.randint(self._next(), shape, lo, hi, dtype=jnp.int32)

    def uniform(self, shape, lo=0.0, hi=1.0):
        return jax.random.uniform(self._next(), shape, jnp.bfloat16, lo, hi)

    def permutation(self, n):
        return jax.random.permutation(self._next(), n)
kernel_name = 'concat_heads__memory_aug_recurrent_mem_tr__ssm_conv_s4__prompt'

def setup_inputs():
    _rng = _Rng(jax.random.key(int.from_bytes(__import__("os").urandom(4), "little")))
    _w = lambda a: (lambda t: t.astype(jnp.bfloat16) if jnp.issubdtype(t.dtype, jnp.floating) else t)(jnp.asarray(a))

    def _A_setup():
        B, S, Dm = (1, 2048, 1024)
        H, Dh = (32, 128)
        M, seg = (8, 32)
        seg = min(seg, S)
        S = S // seg * seg
        return {'x': _w((lambda *s: _rng.normal(s) * 0.05)(B, S, Dm)), 'mem0': _w((lambda *s: _rng.normal(s) * 0.05)(B, M, Dm)), 'Wq': _w((lambda *s: _rng.normal(s) * 0.05)(Dm, H, Dh) * Dm ** (-0.5)), 'Wk': _w((lambda *s: _rng.normal(s) * 0.05)(Dm, H, Dh) * Dm ** (-0.5)), 'Wv': _w((lambda *s: _rng.normal(s) * 0.05)(Dm, H, Dh) * Dm ** (-0.5)), 'Wo': _w((lambda *s: _rng.normal(s) * 0.05)(H, Dh, Dm) * (H * Dh) ** (-0.5)), 'seg_len': seg}
    _A_in = _A_setup()

    def _B_setup():
        B, L, D, N = (1, 2048, 1024, 128)
        A_re = -jnp.exp((lambda *s: _rng.normal(s) * 0.05)(D, N))
        A_im = jnp.pi * (lambda *s: _rng.normal(s) * 0.05)(D, N)
        B_re = (lambda *s: _rng.normal(s) * 0.05)(D, N)
        B_im = (lambda *s: _rng.normal(s) * 0.05)(D, N)
        C_re = (lambda *s: _rng.normal(s) * 0.05)(D, N)
        C_im = (lambda *s: _rng.normal(s) * 0.05)(D, N)
        log_dt = (lambda *s: _rng.normal(s) * 0.05)(D) * 0.5 - 4.0
        Dskip = (lambda *s: _rng.normal(s) * 0.05)(D)
        return {'u': _w((lambda *s: _rng.normal(s) * 0.05)(B, L, D)), 'A_re': _w(A_re), 'A_im': _w(A_im), 'B_re': _w(B_re), 'B_im': _w(B_im), 'C_re': _w(C_re), 'C_im': _w(C_im), 'log_dt': _w(log_dt), 'Dskip': _w(Dskip)}
    _B_in = _B_setup()
    return {'A_x': _A_in['x'], 'A_mem0': _A_in['mem0'], 'A_Wq': _A_in['Wq'], 'A_Wk': _A_in['Wk'], 'A_Wv': _A_in['Wv'], 'A_Wo': _A_in['Wo'], 'A_seg_len': _A_in['seg_len'], 'B_u': _B_in['u'], 'B_A_re': _B_in['A_re'], 'B_A_im': _B_in['A_im'], 'B_B_re': _B_in['B_re'], 'B_B_im': _B_in['B_im'], 'B_C_re': _B_in['C_re'], 'B_C_im': _B_in['C_im'], 'B_log_dt': _B_in['log_dt'], 'B_Dskip': _B_in['Dskip']}

def reference(A_x, A_mem0, A_Wq, A_Wk, A_Wv, A_Wo, A_seg_len, B_u, B_A_re, B_A_im, B_B_re, B_B_im, B_C_re, B_C_im, B_log_dt, B_Dskip):

    def _A_ref(x, mem0, Wq, Wk, Wv, Wo, seg_len):
        B, S, Dm = x.shape
        H, Dh = (Wq.shape[1], Wq.shape[2])
        M = mem0.shape[1]
        scale = Dh ** (-0.5)
        n_seg = S // seg_len
        L = M + seg_len
        idx = jnp.arange(L)
        mask = (idx[:, None] < M) | (idx[:, None] >= idx[None, :])
        mem = mem0
        outs = []
        for s in range(n_seg):
            xs = x[:, s * seg_len:(s + 1) * seg_len, :].copy()
            h = jnp.concatenate([mem, xs], axis=1)
            q = jnp.einsum('btd,dhe->bhte', h, Wq)
            k = jnp.einsum('btd,dhe->bhte', h, Wk)
            v = jnp.einsum('btd,dhe->bhte', h, Wv)
            scores = jnp.einsum('bhqe,bhke->bhqk', q, k) * scale
            scores = jnp.where(mask[None, None], scores, -1000000000.0)
            p = _softmax(scores, axis=-1)
            o = jnp.einsum('bhqk,bhke->bhqe', p, v)
            o = jnp.einsum('bhte,hed->btd', o, Wo)
            mem = o[:, :M, :].copy()
            outs.append(o[:, M:, :])
        return jnp.concatenate(outs, axis=1)

    def _B_ref(u, A_re, A_im, B_re, B_im, C_re, C_im, log_dt, Dskip):
        Bsz, L, D = u.shape
        dt = jnp.exp(log_dt)[:, None]
        A = A_re + 1j * A_im
        Bc = B_re + 1j * B_im
        Cc = C_re + 1j * C_im
        logdA = dt * A
        dB = dt * Bc
        l = (lambda x, dt: x.astype(dt))(jnp.arange(L), A_re.dtype)
        P = jnp.exp(logdA[:, :, None] * l[None, None, :])
        K = jnp.einsum('dn,dnl,dn->dl', Cc, P, dB).real
        L2 = 2 * L
        Kp = jnp.pad(K, ((0, 0), (0, L)))
        up = (lambda x, *d: x.transpose(*d))(u, 0, 2, 1)
        up = jnp.pad(up, ((0, 0), (0, 0), (0, L)))
        Kf = (lambda x, axes=(-2, -1): jnp.fft.rfft2(x.astype(jnp.float32), axes=axes))(Kp[:, None, :], axes=(-2, -1))
        Uf = (lambda x, axes=(-2, -1): jnp.fft.rfft2(x.astype(jnp.float32), axes=axes))(up[:, :, None, :], axes=(-2, -1))
        Yf = Uf * Kf[None, :, :, :]
        y = (lambda x, s, axes=(-2, -1): jnp.fft.irfft2(x, s=s, axes=axes).astype(jnp.bfloat16))(Yf, (1, L2), axes=(-2, -1))[:, :, 0, :L]
        y = (lambda x, *d: x.transpose(*d))(y, 0, 2, 1) + u * Dskip[None, None, :]
        return y
    a = _A_ref(A_x, A_mem0, A_Wq, A_Wk, A_Wv, A_Wo, A_seg_len)
    b = _B_ref(B_u, B_A_re, B_A_im, B_B_re, B_B_im, B_C_re, B_C_im, B_log_dt, B_Dskip)
    return jnp.concatenate([a, b], axis=-1)
```

```python
import functools

import numpy as np
import jax
import jax.numpy as jnp
from jax import lax
import jax.experimental.pallas as pl
import jax.experimental.pallas.tpu as pltpu

bf16, f32, u32 = jnp.bfloat16, jnp.float32, jnp.uint32

S, DM, H, E, M, SEG = 2048, 1024, 32, 128, 8, 32
NSEG = S // SEG
TOK = 24
T0 = S - TOK * NSEG
RING = 576
QOFF = 64
NP = H // 2
L, D, N = 2048, 1024, 128
BLK = 128
NBLK = L // BLK
NT = D // 128
TAPROWS = 656
WINDOWS = ((0, 128, 0, 1), (128, 128, 1, 1), (256, 128, 2, 1), (320, 80, 3, 1),
           (384, 128, 4, 3), (480, 48, 7, 1), (512, 128, 8, 7), (624, 32, 15, 1))


def _bf16_round_int(l):
    u = np.asarray(l, np.float32).view(np.uint32)
    r = (u + 0x7FFF + ((u >> 16) & 1)) & 0xFFFF0000
    return r.astype(np.uint32).view(np.float32).astype(np.int64)


def _tap_row(lp):
    return np.where(lp < 256, lp, np.where(lp < 512, 256 + (lp - 256) // 2,
                    np.where(lp < 1024, 384 + (lp - 512) // 4, 512 + (lp - 1024) // 8)))


@functools.lru_cache(maxsize=None)
def _dft_consts():
    t = np.arange(BLK)
    F = np.zeros((8, 32, BLK))
    G = np.zeros((BLK, 8, 32))
    for r in range(8):
        f = np.concatenate([16 * r + 2 * np.arange(8), 16 * r + 2 * np.arange(8) + 1])
        th = 2 * np.pi * (f + 0.5) / (2 * BLK)
        F[r, :16] = np.cos(th[:, None] * t[None])
        F[r, 16:] = -np.sin(th[:, None] * t[None])
        G[:, r, 0::2] = np.cos(th[None] * t[:, None]) / BLK
        G[:, r, 1::2] = -np.sin(th[None] * t[:, None]) / BLK
    FS = np.zeros((8, NBLK, 32, 128))
    for (w0, wn, b0, nb) in WINDOWS:
        for j in range(b0, b0 + nb):
            rows = _tap_row(_bf16_round_int(BLK * j + t)) - w0
            assert rows.min() >= 0 and rows.max() < wn
            sel = np.zeros((BLK, 128))
            sel[t, rows] = 1.0
            FS[:, j] = F @ sel
    return (FS.reshape(8, NBLK * 32, 128).astype(np.float32),
            G.reshape(BLK, 256).astype(np.float32))


def _cmul(a, b):
    return (a[0] * b[0] - a[1] * b[1], a[0] * b[1] + a[1] * b[0])


def _csq(a):
    return (a[0] * a[0] - a[1] * a[1], 2.0 * (a[0] * a[1]))


def _cexp(lr, li):
    m = jnp.exp(lr)
    return (m * jnp.cos(li), m * jnp.sin(li))


def _prep_tile(c, praw, vec, par):
    rows = pl.ds(pl.multiple_of(c * 128, 128), 128)
    tr = lambda k: praw[k, rows, :].astype(f32).T
    dt = jnp.exp(vec[0, pl.ds(c, 1), :]).astype(bf16).astype(f32)
    par[c, 0] = dt * tr(0)
    par[c, 1] = dt * tr(1)
    cc = _cmul((tr(4), tr(5)), (dt * tr(2), dt * tr(3)))
    par[c, 2] = cc[0]
    par[c, 3] = cc[1]


def _kgen_pieces(c, r, par, ytab, taps, tslot):
    st = {}

    def setup():
        rows = pl.ds(pl.multiple_of(r * 16, 16), 16)
        lr = par[c, 0, rows, :]
        li = par[c, 1, rows, :]
        cf = (par[c, 2, rows, :], par[c, 3, rows, :])
        z1 = _cexp(lr, li)
        z2 = _csq(z1)
        z4 = _csq(z2)
        z8 = _csq(z4)
        z16 = _csq(z8)
        z32 = _csq(z16)
        z64 = _csq(z32)
        z128 = _cexp(lr * 128.0, li * 128.0)
        z256 = _csq(z128)
        z512 = _csq(z256)
        z1024 = _csq(z512)
        st['start'] = [cf, _cmul(cf, z128), _cmul(cf, z256), _cmul(cf, z512), _cmul(cf, z1024)]
        st['step'] = [z8, z8, z16, z32, z64]
        s = lax.broadcasted_iota(jnp.int32, (16, 128), 0) & 7
        fs = [(jnp.where((s >> k) & 1 == 1, z[0], 1.0), jnp.where((s >> k) & 1 == 1, z[1], 0.0))
              for k, z in enumerate((z1, z2, z4))]
        y = _cmul(_cmul(fs[0], fs[1]), fs[2])
        for k in range(8):
            ytab[k, 0] = y[0]
            ytab[k, 1] = y[1]
            if k < 7:
                y = _cmul(y, z1)
                y = (jnp.where(s == 7 - k, 1.0, y[0]), jnp.where(s == 7 - k, 0.0, y[1]))

    def square():
        for k in range(8):
            y = _csq((ytab[k, 0], ytab[k, 1]))
            ytab[k, 0] = y[0]
            ytab[k, 1] = y[1]

    def rows_of(g, i0, ni):
        n_i = 16 + (g == 4)

        def fn():
            x = st.pop('x') if i0 > 0 else st['start'][g]
            xs = []
            for t in range(ni):
                xs.append(x)
                if i0 + t + 1 < n_i:
                    x = _cmul(x, st['step'][g])
            if i0 + ni < n_i:
                st['x'] = x
            acc = [None] * ni
            for k in range(8):
                yr = ytab[k, 0]
                yi = ytab[k, 1]
                for t in range(ni):
                    v = xs[t][0] * yr - xs[t][1] * yi
                    v = v[:8] + v[8:]
                    if k:
                        v = pltpu.roll(v, k, 0)
                    acc[t] = v if acc[t] is None else acc[t] + v
            for t in range(ni):
                row = 128 * g + 8 * (i0 + t)
                a = acc[t]
                if row == 640:
                    a = jnp.where(lax.broadcasted_iota(jnp.int32, (8, 128), 0) == 0, a, 0.0)
                taps[tslot, pl.ds(row, 8), :] = taps[tslot, pl.ds(row, 8), :] + a
        return fn

    pieces = [setup]
    for g in range(5):
        if g >= 2:
            pieces.append(square)
        for i0 in range(0, 16, 2):
            pieces.append(rows_of(g, i0, 2))
        if g == 4:
            pieces.append(rows_of(g, 16, 1))
    return pieces


def _conv_pieces(c, r, buf, fs_ref, us, taps, uf, kf, yf):
    st = {}

    def fwd_u(b0, b1):
        def fn():
            lhs = fs_ref[r, pl.ds(0, 32), :]
            for b in range(b0, b1):
                w = pltpu.bitcast(us[c, pl.ds(b * 64, 64), :], bf16)
                res = jnp.dot(lhs, w, preferred_element_type=f32)
                if b == 0:
                    uf[b] = res
                else:
                    p = st['prev']
                    uf[b, pl.ds(0, 8), :] = res[0:8] - p[16:24]
                    uf[b, pl.ds(8, 8), :] = res[8:16] + p[24:32]
                    uf[b, pl.ds(16, 8), :] = res[16:24] + p[0:8]
                    uf[b, pl.ds(24, 8), :] = res[24:32] - p[8:16]
                st['prev'] = res
        return fn

    def fwd_k(w_lo, w_hi):
        def fn():
            for (w0, wn, b0, nb) in WINDOWS[w_lo:w_hi]:
                lhs = fs_ref[r, pl.ds(b0 * 32, nb * 32), pl.ds(0, wn)]
                w = taps[c, pl.ds(w0, wn), :].astype(bf16)
                res = jnp.dot(lhs, w, preferred_element_type=f32)
                for t in range(nb):
                    kf[b0 + t] = res[t * 32:(t + 1) * 32]
        return fn

    def mac(q, i0, ni):
        def fn():
            re = pl.ds(8 * q, 8)
            im = pl.ds(16 + 8 * q, 8)
            zr = {}
            zi = {}
            ucache = {}
            for j in range(i0 + ni):
                kr = kf[j, re, :]
                ki = kf[j, im, :]
                for i in range(max(i0, j), i0 + ni):
                    if i - j not in ucache:
                        ucache[i - j] = (uf[i - j, re, :], uf[i - j, im, :])
                    ur, ui = ucache[i - j]
                    if i not in zr:
                        zr[i] = kr * ur - ki * ui
                        zi[i] = kr * ui + ki * ur
                    else:
                        zr[i] = zr[i] + kr * ur - ki * ui
                        zi[i] = zi[i] + kr * ui + ki * ur
            row = pl.multiple_of(r * 16 + q * 8, 8)
            for i in range(i0, i0 + ni):
                yf[buf, i, pl.ds(row, 8), :] = pltpu.pack_elementwise([zr[i], zi[i]], packed_dtype=bf16)
        return fn

    fwd = [fwd_u(0, 8), fwd_u(8, 16), fwd_k(0, 5), fwd_k(5, 8)]
    macs = [mac(q, i0, 4) for i0 in range(0, 16, 4) for q in range(2)]
    return fwd, macs


def _inv_piece(c, b, buf, g_ref, us, vec, yf, outb):
    rows = pl.ds(pl.multiple_of(b * 64, 64), 64)
    w = pltpu.bitcast(yf[buf, b], bf16)
    y = jnp.dot(g_ref[...], w, preferred_element_type=f32)
    u = pltpu.bitcast(us[c, rows, :], bf16).astype(f32)
    sk = (u * vec[1, pl.ds(c, 1), :]).astype(bf16).astype(f32)
    o = (y.astype(bf16).astype(f32) + sk).astype(bf16)
    outb[c, rows, :] = pltpu.bitcast(o, u32)


def _attn_fill():
    n = 2 * (SEG + M)
    r = lax.broadcasted_iota(jnp.int32, (n, n), 0)
    c = lax.broadcasted_iota(jnp.int32, (n, n), 1)
    head = lambda i: jnp.where(i < 2 * SEG, i // SEG, (i - 2 * SEG) // M)
    same = head(r) == head(c)
    allowed = same & ((r >= 2 * SEG) | (c >= 2 * SEG) | (r >= c))
    return jnp.where(allowed, 0.0, jnp.where(same, -1e9, -jnp.inf)).astype(f32)


def _kernel(x_hbm, mem0_ref, wq_hbm, wk_hbm, wv_hbm, wo_hbm,
            u_hbm, p0, p1, p2, p3, p4, p5, ldt_ref, dsk_ref, fs_hbm, g_hbm,
            out_hbm,
            wqkv, wo, xs, h_ref, outs, fill_ref,
            praw, par, us, taps, ytab, uf, kf, yf, outb, vec, fs_ref, g_ref,
            sem_w, sem_o, sem_x, sem_p, sem_u, sem_out, *rings):
    ring = rings[:NP]
    oring = rings[NP:2 * NP]
    lo_ref = rings[2 * NP:3 * NP]
    scale = E ** -0.5

    whbm = [w.bitcast(u32) for w in (wq_hbm, wk_hbm, wv_hbm)]

    def wcp(j, m, p):
        return pltpu.make_async_copy(whbm[m].at[:, p, j, :], wqkv.at[m, p, j], sem_w.at[(j * 3 + m) * 2 + p])

    def start_w(j):
        for m in range(3):
            for p in range(2):
                wcp(j, m, p).start()

    xcp0 = pltpu.make_async_copy(x_hbm.at[pl.ds(0, T0)], xs.at[pl.ds(0, T0)], sem_x.at[0])
    xcp1 = pltpu.make_async_copy(x_hbm.at[pl.ds(T0, S - T0)], xs.at[pl.ds(T0, S - T0)], sem_x.at[1])
    pcs = [pltpu.make_async_copy(p, praw.at[k], sem_p.at[k]) for k, p in enumerate((p0, p1, p2, p3, p4, p5))]
    ccs = [pltpu.make_async_copy(fs_hbm, fs_ref, sem_p.at[6]), pltpu.make_async_copy(g_hbm, g_ref, sem_p.at[7])]
    wou = wo_hbm.bitcast(u32)
    ocs = [pltpu.make_async_copy(wou.at[:, pl.ds(c * 128, 128)], wo.at[c], sem_o.at[c]) for c in range(8)]
    uu = u_hbm.bitcast(u32)
    ucs = [pltpu.make_async_copy(uu.at[:, pl.ds(c * 128, 128)], us.at[c], sem_u.at[c]) for c in range(NT)]

    for cp in pcs:
        cp.start()
    xcp0.start()
    start_w(0)
    vec[0] = ldt_ref[...].astype(f32)
    vec[1] = dsk_ref[...].astype(f32)
    taps[...] = jnp.zeros(taps.shape, f32)
    yf[1] = jnp.zeros(yf.shape[1:], u32)
    fill_ref[...] = _attn_fill()
    h_ref[pl.ds(0, M), :] = mem0_ref[...]
    for cp in pcs:
        cp.wait()
    start_w(1)

    with jax.named_scope("prep"):
        def prep(c, carry):
            _prep_tile(c, praw, vec, par)
            return carry
        lax.fori_loop(0, NT, prep, 0)

        def kg(r, carry):
            for p in _kgen_pieces(0, r, par, ytab, taps, 0):
                p()
            return carry
        lax.fori_loop(0, 8, kg, 0)
    xcp0.wait()

    later = [[] for _ in range(NP)]
    for c in range(8):
        later[2 + c].append(ocs[c])
        later[2 + c].append(ucs[c])
    later[10].append(xcp1)
    later[11].extend(ccs)
    with jax.named_scope("bulk"):
        for j in range(NP):
            if j + 2 < NP:
                start_w(j + 2)
            for cp in later[j]:
                cp.start()

            def bulk(m, carry, j=j):
                for p in range(2):
                    pltpu.make_async_copy(wqkv.at[m, p, j], wqkv.at[m, p, j], sem_w.at[(j * 3 + m) * 2 + p]).wait()
                a = wqkv[m, 0, j]
                b = wqkv[m, 1, j]
                lo = (a & u32(0xFFFF)) | (b << 16)
                hi = (a >> 16) | (b & u32(0xFFFF0000))
                wqkv[m, 0, j] = lo
                wqkv[m, 1, j] = hi
                xb = xs[pl.ds(0, T0), :]
                for p, w in enumerate((lo, hi)):
                    r = jnp.dot(xb, pltpu.bitcast(w, bf16), preferred_element_type=f32)
                    ring[j][m, p, pl.ds(QOFF, T0), :] = r.astype(bf16)
                return carry
            lax.fori_loop(0, 3, bulk, 0)
    for cp in ocs + ucs + ccs + [xcp1]:
        cp.wait()

    ou = out_hbm.bitcast(u32)

    def outa_cp(row, n):
        return pltpu.make_async_copy(outs.at[pl.ds(row, n)], out_hbm.at[pl.ds(row, n), pl.ds(0, DM)], sem_out.at[0])

    def outb_cp(c, row, n):
        return pltpu.make_async_copy(outb.at[c, pl.ds(row, n)], ou.at[pl.ds(row, n), pl.ds(DM + c * 128, 128)],
                                     sem_out.at[1])

    def step(s, carry):
        tok0 = pl.multiple_of(T0 + TOK * s, 8)
        h_ref[pl.ds(M, TOK), :] = xs[pl.ds(tok0, TOK), :]
        h = h_ref[...]
        ppos = pl.multiple_of(lax.rem(TOK * s, RING), 8)
        cpos = pl.multiple_of(lax.rem(QOFF + SEG * s, RING), 32)
        opos = pl.multiple_of(lax.rem(SEG * s, RING), 32)
        orow = pl.multiple_of(TOK * s, 8)
        mem_rows = {}
        probs = {}

        ct = s // 8
        r = s % 8
        buf = ct % 2
        cprev = (ct + NT - 1) % NT
        fwd, macs = _conv_pieces(ct, r, buf, fs_ref, us, taps, uf, kf, yf)
        kgen = _kgen_pieces((ct + 1) % NT, r, par, ytab, taps, ct + 1)

        def stage_a(j):
            for m in range(3):
                mm = []
                for p in range(2):
                    w = pltpu.bitcast(wqkv[m, p, j], bf16)
                    res = jnp.dot(h, w, preferred_element_type=f32)
                    ring[j][m, p, pl.ds(ppos, TOK), :] = res[M:].astype(bf16)
                    mm.append(res[:M])
                mem_rows[m, j] = jnp.concatenate(mm, axis=0).astype(bf16)

        def gather(m, j):
            return jnp.concatenate([ring[j][m, 0, pl.ds(cpos, SEG), :], ring[j][m, 1, pl.ds(cpos, SEG), :],
                                    mem_rows[m, j]], axis=0)

        def stage_b(j):
            sc = lax.dot_general(gather(0, j), gather(1, j), (((1,), (1,)), ((), ())),
                                 preferred_element_type=f32)
            fl = fill_ref[...]
            sc = jnp.where(fl == 0.0, sc * scale, fl)
            mx = jnp.max(sc, axis=-1, keepdims=True)
            e = jnp.exp(sc - mx)
            den = jnp.sum(e, axis=-1, keepdims=True)
            r0 = pl.reciprocal(den, approx=True)
            r1 = r0 * (2.0 - den * r0)
            probs[j] = (e * r1).astype(bf16)

        def stage_c(j):
            o = jnp.dot(probs[j], gather(2, j), preferred_element_type=f32)
            for p in range(2):
                oring[j][p, pl.ds(opos, SEG), :] = o[p * SEG:(p + 1) * SEG].astype(bf16)
                lo_ref[j][p, pl.ds(0, M), :] = o[2 * SEG + p * M:2 * SEG + (p + 1) * M].astype(bf16)
                lo_ref[j][p, pl.ds(M, TOK), :] = oring[j][p, pl.ds(ppos, TOK), :]

        acc = [None] * 8

        def stage_d(h0, h1, last=False):
            lhs = jnp.concatenate([lo_ref[hh // 2][hh % 2] for hh in range(h0, h1)], axis=1)
            for c in range(8):
                w = pltpu.bitcast(wo[c, pl.ds(h0 * 64, (h1 - h0) * 64), :], bf16)
                res = jnp.dot(lhs, w, preferred_element_type=f32)
                acc[c] = res if acc[c] is None else acc[c] + res
                if last:
                    rb = acc[c].astype(bf16)
                    h_ref[pl.ds(0, M), pl.ds(c * 128, 128)] = rb[:M]
                    outs[pl.ds(orow, TOK), pl.ds(c * 128, 128)] = rb[M:]

        for t in range(2):
            _inv_piece(cprev, 2 * r + t, 1 - buf, g_ref, us, vec, yf, outb)
        for p in fwd:
            p()
        vpu = kgen + macs
        nv = len(vpu)
        for j in range(NP):
            stage_a(j)
            if j >= 1:
                stage_b(j - 1)
            if j >= 2:
                stage_c(j - 2)
            for p in vpu[j * nv // NP:(j + 1) * nv // NP]:
                p()
        stage_d(0, 8)
        stage_b(15)
        stage_c(14)
        stage_d(8, 20)
        stage_c(15)
        stage_d(20, 28)
        stage_d(28, 32, last=True)

        outa_cp(orow, TOK).start()

        @pl.when(s >= 8)
        def _():
            outb_cp(cprev, pl.multiple_of(r * 128, 128), 128).start()
        return carry

    with jax.named_scope("steps"):
        lax.fori_loop(0, NSEG, step, 0)

    with jax.named_scope("flush"):
        for b in range(NBLK):
            _inv_piece(NT - 1, b, (NT - 1) % 2, g_ref, us, vec, yf, outb)
        outb_cp(NT - 1, 0, L // 2).start()
        done = TOK * NSEG
        p0_ = done % RING
        n0 = RING - p0_
        for (rp, n, t) in ((p0_, n0, done), (0, S - done - n0, done + n0)):
            lhs = jnp.concatenate([oring[hh // 2][hh % 2, pl.ds(rp, n), :] for hh in range(H)], axis=1)
            for c in range(8):
                outs[pl.ds(t, n), pl.ds(c * 128, 128)] = jnp.dot(
                    lhs, pltpu.bitcast(wo[c], bf16), preferred_element_type=f32).astype(bf16)
            outa_cp(t, n).start()
    outa_cp(0, S).wait()
    pltpu.make_async_copy(outb, outb, sem_out.at[1]).wait()


@functools.partial(jax.jit, static_argnames=("A_seg_len",))
def pallas_concat_heads__memory_aug_recurrent_mem_tr__ssm_conv_s4__prompt_kernel(
    A_x, A_mem0, A_Wq, A_Wk, A_Wv, A_Wo, A_seg_len,
    B_u, B_A_re, B_A_im, B_B_re, B_B_im, B_C_re, B_C_im, B_log_dt, B_Dskip,
):
    assert A_seg_len == SEG and A_x.shape == (1, S, DM) and B_u.shape == (1, L, D)
    fs, g = _dft_consts()
    w4 = lambda w: w.reshape(DM // 2, 2, H, E)
    any_ = pl.BlockSpec(memory_space=pl.ANY)
    vm = pl.BlockSpec(memory_space=pltpu.VMEM)
    V = pltpu.VMEM
    out = pl.pallas_call(
        _kernel,
        out_shape=jax.ShapeDtypeStruct((S, DM + D), bf16),
        in_specs=[any_, vm, any_, any_, any_, any_] + [any_] * 7 + [vm, vm, any_, any_],
        out_specs=any_,
        scratch_shapes=[
            V((3, 2, NP, DM // 2, E), u32),
            V((8, H * E // 2, 128), u32),
            V((S, DM), bf16),
            V((M + TOK, DM), bf16),
            V((S, DM), bf16),
            V((2 * (SEG + M), 2 * (SEG + M)), f32),
            V((6, D, N), bf16),
            V((NT, 4, N, 128), f32),
            V((NT, L // 2, 128), u32),
            V((NT + 1, TAPROWS, 128), f32),
            V((8, 2, 16, 128), f32),
            V((NBLK, 32, 128), f32),
            V((NBLK, 32, 128), f32),
            V((2, NBLK, 128, 128), u32),
            V((NT, L // 2, 128), u32),
            V((2, 8, 128), f32),
            V((8, NBLK * 32, 128), bf16),
            V((BLK, 256), bf16),
            pltpu.SemaphoreType.DMA((6 * NP,)),
            pltpu.SemaphoreType.DMA((8,)),
            pltpu.SemaphoreType.DMA((2,)),
            pltpu.SemaphoreType.DMA((8,)),
            pltpu.SemaphoreType.DMA((NT,)),
            pltpu.SemaphoreType.DMA((2,)),
        ] + [V((3, 2, RING, E), bf16)] * NP + [V((2, RING, E), bf16)] * NP + [V((2, M + TOK, E), bf16)] * NP,
        compiler_params=pltpu.CompilerParams(vmem_limit_bytes=110 * 1024 * 1024),
    )(A_x.reshape(S, DM), A_mem0.reshape(M, DM), w4(A_Wq), w4(A_Wk), w4(A_Wv), A_Wo.reshape(H * E, DM),
      B_u.reshape(L, D), B_A_re, B_A_im, B_B_re, B_B_im, B_C_re, B_C_im,
      B_log_dt.reshape(8, 128), B_Dskip.reshape(8, 128),
      jnp.asarray(fs, bf16), jnp.asarray(g, bf16))
    return out.reshape(1, S, DM + D)
```

```python
import functools

import numpy as np
import jax
import jax.numpy as jnp
from jax import lax
import jax.experimental.pallas as pl
import jax.experimental.pallas.tpu as pltpu

bf16, f32, u32 = jnp.bfloat16, jnp.float32, jnp.uint32

S, DM, H, E, M, SEG = 2048, 1024, 32, 128, 8, 32
NSEG = S // SEG
TOK = 24
T0 = S - TOK * NSEG
RING = 576
QOFF = 64
NP = H // 2
KNI = 1
MACJ = 6
NSLOT = 118
L, D, N = 2048, 1024, 128
BLK = 128
NBLK = L // BLK
NT = D // 128
TAPROWS = 656
WINDOWS = ((0, 128, 0, 1), (128, 128, 1, 1), (256, 128, 2, 1), (320, 80, 3, 1),
           (384, 128, 4, 3), (480, 48, 7, 1), (512, 128, 8, 7), (624, 32, 15, 1))

V_FENCE = 0
V_YTAB = 8
V_START = V_YTAB + 256
V_STEP = V_START + 160
V_UF = V_STEP + 128
V_KF = V_UF + NBLK * 32
V_ROWS = V_KF + NBLK * 32


def _bf16_round_int(l):
    u = np.asarray(l, np.float32).view(np.uint32)
    r = (u + 0x7FFF + ((u >> 16) & 1)) & 0xFFFF0000
    return r.astype(np.uint32).view(np.float32).astype(np.int64)


def _tap_row(lp):
    return np.where(lp < 256, lp, np.where(lp < 512, 256 + (lp - 256) // 2,
                    np.where(lp < 1024, 384 + (lp - 512) // 4, 512 + (lp - 1024) // 8)))


@functools.lru_cache(maxsize=None)
def _dft_consts():
    t = np.arange(BLK)
    F = np.zeros((8, 32, BLK))
    G = np.zeros((BLK, 8, 32))
    for r in range(8):
        f = np.concatenate([16 * r + 2 * np.arange(8), 16 * r + 2 * np.arange(8) + 1])
        th = 2 * np.pi * (f + 0.5) / (2 * BLK)
        F[r, :16] = np.cos(th[:, None] * t[None])
        F[r, 16:] = -np.sin(th[:, None] * t[None])
        G[:, r, 0::2] = np.cos(th[None] * t[:, None]) / BLK
        G[:, r, 1::2] = -np.sin(th[None] * t[:, None]) / BLK
    FS = np.zeros((8, NBLK, 32, 128))
    for (w0, wn, b0, nb) in WINDOWS:
        for j in range(b0, b0 + nb):
            rows = _tap_row(_bf16_round_int(BLK * j + t)) - w0
            assert rows.min() >= 0 and rows.max() < wn
            sel = np.zeros((BLK, 128))
            sel[t, rows] = 1.0
            FS[:, j] = F @ sel
    return (FS.reshape(8, NBLK * 32, 128).astype(np.float32),
            G.reshape(BLK, 256).astype(np.float32))


def _cmul(a, b):
    return (a[0] * b[0] - a[1] * b[1], a[0] * b[1] + a[1] * b[0])


def _csq(a):
    return (a[0] * a[0] - a[1] * a[1], 2.0 * (a[0] * a[1]))


def _cexp(lr, li):
    m = jnp.exp(lr)
    return (m * jnp.cos(li), m * jnp.sin(li))


def _prep_tile(c, praw, vec, par):
    rows = pl.ds(pl.multiple_of(c * 128, 128), 128)
    tr = lambda k: praw[k, rows, :].astype(f32).T
    dt = jnp.exp(vec[0, pl.ds(c, 1), :]).astype(bf16).astype(f32)
    par[c, 0] = dt * tr(0)
    par[c, 1] = dt * tr(1)
    cc = _cmul((tr(4), tr(5)), (dt * tr(2), dt * tr(3)))
    par[c, 2] = cc[0]
    par[c, 3] = cc[1]


def _kgen_pieces(c, r, par, vb, taps, tslot):
    st = {}

    def put(row, z, h=None):
        if h is None:
            vb[pl.ds(row, 16), :] = z[0]
            vb[pl.ds(row + 16, 16), :] = z[1]
        else:
            vb[pl.ds(row + 8 * h, 8), :] = z[0]
            vb[pl.ds(row + 16 + 8 * h, 8), :] = z[1]

    def get(row, h=None):
        if h is None:
            return (vb[pl.ds(row, 16), :], vb[pl.ds(row + 16, 16), :])
        return (vb[pl.ds(row + 8 * h, 8), :], vb[pl.ds(row + 16 + 8 * h, 8), :])

    def params(k):
        return par[c, k, pl.ds(pl.multiple_of(r * 16, 16), 16), :]

    def park():
        put(V_STEP, (params(0), params(1)))
        put(V_START, (params(0) * 128.0, params(1) * 128.0))

    def setup_lo(h):
        def fn():
            z = _cexp(*get(V_STEP, h))
            put(V_STEP, z, h)
            z = _csq(z)
            put(V_STEP + 32, z, h)
            put(V_STEP + 64, _csq(z), h)
        return fn

    def setup_y(h):
        def fn():
            z1, z2, z4 = get(V_STEP, h), get(V_STEP + 32, h), get(V_STEP + 64, h)
            s = lax.broadcasted_iota(jnp.int32, (8, 128), 0)
            fs = [(jnp.where((s >> k) & 1 == 1, z[0], 1.0), jnp.where((s >> k) & 1 == 1, z[1], 0.0))
                  for k, z in enumerate((z1, z2, z4))]
            y = _cmul(_cmul(fs[0], fs[1]), fs[2])
            for k in range(8):
                put(V_YTAB + 32 * k, y, h)
                if k < 7:
                    y = _cmul(y, z1)
                    y = (jnp.where(s == 7 - k, 1.0, y[0]), jnp.where(s == 7 - k, 0.0, y[1]))
            z = z4
            for k in range(4):
                z = _csq(z)
                put(V_STEP + 32 * k, z, h)
        return fn

    def setup_hi(h):
        def fn():
            z = _cexp(*get(V_START, h))
            cf = (params(2)[8 * h:8 * h + 8], params(3)[8 * h:8 * h + 8])
            put(V_START, cf, h)
            for g in range(1, 5):
                put(V_START + 32 * g, _cmul(cf, z), h)
                if g < 4:
                    z = _csq(z)
        return fn

    def square(k0, k1):
        def fn():
            for k in range(k0, k1):
                put(V_YTAB + 32 * k, _csq(get(V_YTAB + 32 * k)))
        return fn

    def rows_of(g, i0, ni):
        n_i = 16 + (g == 4)

        def fn():
            x = st.pop('x') if i0 > 0 else get(V_START + 32 * g)
            step = get(V_STEP + 32 * max(g - 1, 0))
            xs = []
            for t in range(ni):
                xs.append(x)
                if i0 + t + 1 < n_i:
                    x = _cmul(x, step)
            if i0 + ni < n_i:
                st['x'] = x
            acc = [None] * ni
            for k in range(8):
                yr, yi = get(V_YTAB + 32 * k)
                for t in range(ni):
                    v = xs[t][0] * yr - xs[t][1] * yi
                    v = v[:8] + v[8:]
                    if k:
                        v = pltpu.roll(v, k, 0)
                    acc[t] = v if acc[t] is None else acc[t] + v
            for t in range(ni):
                row = 128 * g + 8 * (i0 + t)
                a = acc[t]
                if row == 640:
                    a = jnp.where(lax.broadcasted_iota(jnp.int32, (8, 128), 0) == 0, a, 0.0)
                taps[tslot, pl.ds(row, 8), :] = taps[tslot, pl.ds(row, 8), :] + a
        return fn

    pieces = [(4, park), (160, setup_lo(0)), (160, setup_lo(1)), (100, setup_y(0)), (100, setup_y(1)),
              (190, setup_hi(0)), (190, setup_hi(1))]
    for g in range(5):
        if g >= 2:
            pieces += [(40, square(0, 4)), (40, square(4, 8))]
        for i0 in range(0, 16 + (g == 4), KNI):
            ni = min(KNI, 16 + (g == 4) - i0)
            pieces.append((83 * ni, rows_of(g, i0, ni)))
    return pieces


def _conv_pieces(c, r, buf, fs_ref, us, taps, vb, yf):
    st = {}

    def fwd_u(b0, b1):
        def fn():
            lhs = fs_ref[r, pl.ds(0, 32), :]
            for b in range(b0, b1):
                w = pltpu.bitcast(us[c, pl.ds(b * 64, 64), :], bf16)
                res = jnp.dot(lhs, w, preferred_element_type=f32)
                row = V_UF + 32 * b
                if b == 0:
                    vb[pl.ds(row, 32), :] = res
                else:
                    p = st['prev']
                    vb[pl.ds(row, 8), :] = res[0:8] - p[16:24]
                    vb[pl.ds(row + 8, 8), :] = res[8:16] + p[24:32]
                    vb[pl.ds(row + 16, 8), :] = res[16:24] + p[0:8]
                    vb[pl.ds(row + 24, 8), :] = res[24:32] - p[8:16]
                st['prev'] = res
        return fn

    def fwd_k(jobs):
        def fn():
            for (wi, t0, nb) in jobs:
                w0, wn, b0, _ = WINDOWS[wi]
                lhs = fs_ref[r, pl.ds((b0 + t0) * 32, nb * 32), pl.ds(0, wn)]
                w = taps[c, pl.ds(w0, wn), :].astype(bf16)
                vb[pl.ds(V_KF + 32 * (b0 + t0), 32 * nb), :] = jnp.dot(lhs, w, preferred_element_type=f32)
        return fn

    def mac(q, i0, ni, j0, j1):
        def fn():
            ld = lambda base, b: (vb[pl.ds(base + 32 * b + 8 * q, 8), :], vb[pl.ds(base + 32 * b + 16 + 8 * q, 8), :])
            zr, zi = st.pop('z') if j0 > 0 else ({}, {})
            ucache = {}
            for j in range(j0, j1):
                kr, ki = ld(V_KF, j)
                for i in range(max(i0, j), i0 + ni):
                    if i - j not in ucache:
                        ucache[i - j] = ld(V_UF, i - j)
                    ur, ui = ucache[i - j]
                    if i not in zr:
                        zr[i] = kr * ur - ki * ui
                        zi[i] = kr * ui + ki * ur
                    else:
                        zr[i] = zr[i] + kr * ur - ki * ui
                        zi[i] = zi[i] + kr * ui + ki * ur
            if j1 < i0 + ni:
                st['z'] = (zr, zi)
            else:
                row = pl.multiple_of(r * 16 + q * 8, 8)
                for i in range(i0, i0 + ni):
                    yf[buf, i, pl.ds(row, 8), :] = pltpu.pack_elementwise([zr[i], zi[i]], packed_dtype=bf16)
        return (8 * sum(1 for j in range(j0, j1) for i in range(max(i0, j), i0 + ni)), fn)

    fwd = [fwd_u(0, 8), fwd_u(8, 16), fwd_k(((0, 0, 1), (1, 0, 1), (2, 0, 1), (3, 0, 1))),
           fwd_k(((4, 0, 2), (6, 0, 2), (6, 2, 2), (6, 4, 2))), fwd_k(((4, 2, 1), (5, 0, 1), (6, 6, 1), (7, 0, 1)))]
    macs = []
    for q in range(2):
        for i0 in range(0, NBLK, 2):
            for j0 in range(0, i0 + 2, MACJ):
                macs.append(mac(q, i0, 2, j0, min(j0 + MACJ, i0 + 2)))
    return fwd, macs


def _inv_piece(c, b, buf, g_ref, us, vec, yf, outb):
    rows = pl.ds(pl.multiple_of(b * 64, 64), 64)
    w = pltpu.bitcast(yf[buf, b], bf16)
    y = jnp.dot(g_ref[...], w, preferred_element_type=f32)
    u = pltpu.bitcast(us[c, rows, :], bf16).astype(f32)
    sk = (u * vec[1, pl.ds(c, 1), :]).astype(bf16).astype(f32)
    o = (y.astype(bf16).astype(f32) + sk).astype(bf16)
    outb[c, rows, :] = pltpu.bitcast(o, u32)


def _attn_fill():
    n = 2 * (SEG + M)
    r = lax.broadcasted_iota(jnp.int32, (n, n), 0)
    c = lax.broadcasted_iota(jnp.int32, (n, n), 1)
    head = lambda i: jnp.where(i < 2 * SEG, i // SEG, (i - 2 * SEG) // M)
    same = head(r) == head(c)
    allowed = same & ((r >= 2 * SEG) | (c >= 2 * SEG) | (r >= c))
    return jnp.where(allowed, 0.0, jnp.where(same, -1e9, -jnp.inf)).astype(f32)


def _kernel(x_hbm, mem0_ref, wq_hbm, wk_hbm, wv_hbm, wo_hbm,
            u_hbm, p0, p1, p2, p3, p4, p5, ldt_ref, dsk_ref, fs_hbm, g_hbm,
            out_hbm,
            wqkv, wo, xs, h_ref, outs, fill_ref,
            praw, par, us, taps, vb, yf, outb, vec, fs_ref, g_ref,
            sem_w, sem_o, sem_x, sem_p, sem_u, sem_out, *rings):
    ring = rings[:NP]
    oring = rings[NP:2 * NP]
    lo_ref = rings[2 * NP:3 * NP]
    scale = E ** -0.5

    whbm = [w.bitcast(u32) for w in (wq_hbm, wk_hbm, wv_hbm)]

    def wcp(j, m, p):
        return pltpu.make_async_copy(whbm[m].at[:, p, j, :], wqkv.at[m, p, j], sem_w.at[(j * 3 + m) * 2 + p])

    def start_w(j):
        for m in range(3):
            for p in range(2):
                wcp(j, m, p).start()

    xcp0 = pltpu.make_async_copy(x_hbm.at[pl.ds(0, T0)], xs.at[pl.ds(0, T0)], sem_x.at[0])
    xcp1 = pltpu.make_async_copy(x_hbm.at[pl.ds(T0, S - T0)], xs.at[pl.ds(T0, S - T0)], sem_x.at[1])
    pcs = [pltpu.make_async_copy(p, praw.at[k], sem_p.at[k]) for k, p in enumerate((p0, p1, p2, p3, p4, p5))]
    ccs = [pltpu.make_async_copy(fs_hbm, fs_ref, sem_p.at[6]), pltpu.make_async_copy(g_hbm, g_ref, sem_p.at[7])]
    wou = wo_hbm.bitcast(u32)
    ocs = [pltpu.make_async_copy(wou.at[:, pl.ds(c * 128, 128)], wo.at[c], sem_o.at[c]) for c in range(8)]
    uu = u_hbm.bitcast(u32)
    ucs = [pltpu.make_async_copy(uu.at[:, pl.ds(c * 128, 128)], us.at[c], sem_u.at[c]) for c in range(NT)]

    for cp in pcs:
        cp.start()
    xcp0.start()
    start_w(0)
    vec[0] = ldt_ref[...].astype(f32)
    vec[1] = dsk_ref[...].astype(f32)
    taps[...] = jnp.zeros(taps.shape, f32)
    yf[1] = jnp.zeros(yf.shape[1:], u32)
    fill_ref[...] = _attn_fill()
    h_ref[pl.ds(0, M), :] = mem0_ref[...]
    for cp in pcs:
        cp.wait()
    start_w(1)

    with jax.named_scope("prep"):
        def prep(c, carry):
            _prep_tile(c, praw, vec, par)
            return carry
        lax.fori_loop(0, NT, prep, 0)

        def kg(r, carry):
            for _, p in _kgen_pieces(0, r, par, vb, taps, 0):
                p()
            return carry
        lax.fori_loop(0, 8, kg, 0)
    xcp0.wait()

    later = [[] for _ in range(NP)]
    for c in range(8):
        later[2 + c].append(ocs[c])
        later[2 + c].append(ucs[c])
    later[10].append(xcp1)
    later[11].extend(ccs)
    with jax.named_scope("bulk"):
        for j in range(NP):
            if j + 2 < NP:
                start_w(j + 2)
            for cp in later[j]:
                cp.start()

            def bulk(m, carry, j=j):
                for p in range(2):
                    pltpu.make_async_copy(wqkv.at[m, p, j], wqkv.at[m, p, j], sem_w.at[(j * 3 + m) * 2 + p]).wait()
                a = wqkv[m, 0, j]
                b = wqkv[m, 1, j]
                lo = (a & u32(0xFFFF)) | (b << 16)
                hi = (a >> 16) | (b & u32(0xFFFF0000))
                wqkv[m, 0, j] = lo
                wqkv[m, 1, j] = hi
                xb = xs[pl.ds(0, T0), :]
                for p, w in enumerate((lo, hi)):
                    r = jnp.dot(xb, pltpu.bitcast(w, bf16), preferred_element_type=f32)
                    ring[j][m, p, pl.ds(QOFF, T0), :] = r.astype(bf16)
                return carry
            lax.fori_loop(0, 3, bulk, 0)
    for cp in ocs + ucs + ccs + [xcp1]:
        cp.wait()

    ou = out_hbm.bitcast(u32)

    def outa_cp(row, n):
        return pltpu.make_async_copy(outs.at[pl.ds(row, n)], out_hbm.at[pl.ds(row, n), pl.ds(0, DM)], sem_out.at[0])

    def outb_cp(c, row, n):
        return pltpu.make_async_copy(outb.at[c, pl.ds(row, n)], ou.at[pl.ds(row, n), pl.ds(DM + c * 128, 128)],
                                     sem_out.at[1])

    def step(s, carry):
        tok0 = pl.multiple_of(T0 + TOK * s, 8)
        h_ref[pl.ds(M, TOK), :] = xs[pl.ds(tok0, TOK), :]
        h = h_ref[...]
        ppos = pl.multiple_of(lax.rem(TOK * s, RING), 8)
        cpos = pl.multiple_of(lax.rem(QOFF + SEG * s, RING), 32)
        opos = pl.multiple_of(lax.rem(SEG * s, RING), 32)
        orow = pl.multiple_of(TOK * s, 8)
        mem_rows = {}
        probs = {}

        ct = s // 8
        r = s % 8
        buf = ct % 2
        cprev = (ct + NT - 1) % NT
        fwd, macs = _conv_pieces(ct, r, buf, fs_ref, us, taps, vb, yf)
        kgen = _kgen_pieces((ct + 1) % NT, r, par, vb, taps, ct + 1)
        vpu = kgen + macs
        total = float(sum(cst for cst, _ in vpu))
        frow = pl.multiple_of(lax.rem(s * (V_ROWS - 8), V_ROWS - 8), 8)
        sched = {'slot': 0, 'next': 0, 'done': 0.0}

        def fence(v):
            sched['slot'] += 1
            first = True
            while sched['next'] < len(vpu) and sched['done'] < total * sched['slot'] / NSLOT:
                if first:
                    vb[pl.ds(frow, 8), :] = v
                    first = False
                cst, fn = vpu[sched['next']]
                fn()
                sched['next'] += 1
                sched['done'] += cst

        def stage_a(j):
            for m in range(3):
                mm = []
                for p in range(2):
                    w = pltpu.bitcast(wqkv[m, p, j], bf16)
                    res = jnp.dot(h, w, preferred_element_type=f32)
                    ring[j][m, p, pl.ds(ppos, TOK), :] = res[M:].astype(bf16)
                    mm.append(res[:M])
                    fence(res[:M])
                mem_rows[m, j] = jnp.concatenate(mm, axis=0).astype(bf16)

        def gather(m, j):
            return jnp.concatenate([ring[j][m, 0, pl.ds(cpos, SEG), :], ring[j][m, 1, pl.ds(cpos, SEG), :],
                                    mem_rows[m, j]], axis=0)

        scores = {}

        def stage_qk(j):
            scores[j] = lax.dot_general(gather(0, j), gather(1, j), (((1,), (1,)), ((), ())),
                                        preferred_element_type=f32)

        def stage_b(j):
            sc = scores.pop(j)
            fl = fill_ref[...]
            sc = jnp.where(fl == 0.0, sc * scale, fl)
            mx = jnp.max(sc, axis=-1, keepdims=True)
            e = jnp.exp(sc - mx)
            den = jnp.sum(e, axis=-1, keepdims=True)
            r0 = pl.reciprocal(den, approx=True)
            r1 = r0 * (2.0 - den * r0)
            probs[j] = (e * r1).astype(bf16)

        def stage_c(j):
            o = jnp.dot(probs[j], gather(2, j), preferred_element_type=f32)
            for p in range(2):
                oring[j][p, pl.ds(opos, SEG), :] = o[p * SEG:(p + 1) * SEG].astype(bf16)
                lo_ref[j][p, pl.ds(0, M), :] = o[2 * SEG + p * M:2 * SEG + (p + 1) * M].astype(bf16)
                lo_ref[j][p, pl.ds(M, TOK), :] = oring[j][p, pl.ds(ppos, TOK), :]

        acc = [None] * 8

        def stage_d(h0, h1, last=False):
            lhs = jnp.concatenate([lo_ref[hh // 2][hh % 2] for hh in range(h0, h1)], axis=1)
            for c in range(8):
                w = pltpu.bitcast(wo[c, pl.ds(h0 * 64, (h1 - h0) * 64), :], bf16)
                res = jnp.dot(lhs, w, preferred_element_type=f32)
                acc[c] = res if acc[c] is None else acc[c] + res
                if not last:
                    fence(res[:M])
                if last:
                    rb = acc[c].astype(bf16)
                    h_ref[pl.ds(0, M), pl.ds(c * 128, 128)] = rb[:M]
                    outs[pl.ds(orow, TOK), pl.ds(c * 128, 128)] = rb[M:]

        for t in range(2):
            _inv_piece(cprev, 2 * r + t, 1 - buf, g_ref, us, vec, yf, outb)
        for p in fwd:
            p()
        def attn_group(jq, jc):
            for j in jq:
                stage_qk(j)
            for j in jc:
                stage_c(j)
            for j in jq:
                stage_b(j)

        for j in range(NP):
            stage_a(j)
            if j >= 2 and j % 2 == 0:
                attn_group((j - 2, j - 1), (j - 4, j - 3) if j >= 4 else ())
        stage_d(0, 8)
        attn_group((14, 15), (12, 13))
        stage_d(8, 20)
        attn_group((), (14, 15))
        stage_d(20, 28)
        assert sched['next'] == len(vpu)
        stage_d(28, 32, last=True)

        outa_cp(orow, TOK).start()

        @pl.when(s >= 8)
        def _():
            outb_cp(cprev, pl.multiple_of(r * 128, 128), 128).start()
        return carry

    with jax.named_scope("steps"):
        lax.fori_loop(0, NSEG, step, 0)

    with jax.named_scope("flush"):
        for b in range(NBLK):
            _inv_piece(NT - 1, b, (NT - 1) % 2, g_ref, us, vec, yf, outb)
        outb_cp(NT - 1, 0, L // 2).start()
        done = TOK * NSEG
        p0_ = done % RING
        n0 = RING - p0_
        for (rp, n, t) in ((p0_, n0, done), (0, S - done - n0, done + n0)):
            lhs = jnp.concatenate([oring[hh // 2][hh % 2, pl.ds(rp, n), :] for hh in range(H)], axis=1)
            for c in range(8):
                outs[pl.ds(t, n), pl.ds(c * 128, 128)] = jnp.dot(
                    lhs, pltpu.bitcast(wo[c], bf16), preferred_element_type=f32).astype(bf16)
            outa_cp(t, n).start()
    outa_cp(0, S).wait()
    pltpu.make_async_copy(outb, outb, sem_out.at[1]).wait()


@functools.partial(jax.jit, static_argnames=("A_seg_len",))
def pallas_concat_heads__memory_aug_recurrent_mem_tr__ssm_conv_s4__prompt_kernel(
    A_x, A_mem0, A_Wq, A_Wk, A_Wv, A_Wo, A_seg_len,
    B_u, B_A_re, B_A_im, B_B_re, B_B_im, B_C_re, B_C_im, B_log_dt, B_Dskip,
):
    assert A_seg_len == SEG and A_x.shape == (1, S, DM) and B_u.shape == (1, L, D)
    fs, g = _dft_consts()
    w4 = lambda w: w.reshape(DM // 2, 2, H, E)
    any_ = pl.BlockSpec(memory_space=pl.ANY)
    vm = pl.BlockSpec(memory_space=pltpu.VMEM)
    V = pltpu.VMEM
    out = pl.pallas_call(
        _kernel,
        out_shape=jax.ShapeDtypeStruct((S, DM + D), bf16),
        in_specs=[any_, vm, any_, any_, any_, any_] + [any_] * 7 + [vm, vm, any_, any_],
        out_specs=any_,
        scratch_shapes=[
            V((3, 2, NP, DM // 2, E), u32),
            V((8, H * E // 2, 128), u32),
            V((S, DM), bf16),
            V((M + TOK, DM), bf16),
            V((S, DM), bf16),
            V((2 * (SEG + M), 2 * (SEG + M)), f32),
            V((6, D, N), bf16),
            V((NT, 4, N, 128), f32),
            V((NT, L // 2, 128), u32),
            V((NT + 1, TAPROWS, 128), f32),
            V((V_ROWS, 128), f32),
            V((2, NBLK, 128, 128), u32),
            V((NT, L // 2, 128), u32),
            V((2, 8, 128), f32),
            V((8, NBLK * 32, 128), bf16),
            V((BLK, 256), bf16),
            pltpu.SemaphoreType.DMA((6 * NP,)),
            pltpu.SemaphoreType.DMA((8,)),
            pltpu.SemaphoreType.DMA((2,)),
            pltpu.SemaphoreType.DMA((8,)),
            pltpu.SemaphoreType.DMA((NT,)),
            pltpu.SemaphoreType.DMA((2,)),
        ] + [V((3, 2, RING, E), bf16)] * NP + [V((2, RING, E), bf16)] * NP + [V((2, M + TOK, E), bf16)] * NP,
        compiler_params=pltpu.CompilerParams(vmem_limit_bytes=110 * 1024 * 1024),
    )(A_x.reshape(S, DM), A_mem0.reshape(M, DM), w4(A_Wq), w4(A_Wk), w4(A_Wv), A_Wo.reshape(H * E, DM),
      B_u.reshape(L, D), B_A_re, B_A_im, B_B_re, B_B_im, B_C_re, B_C_im,
      B_log_dt.reshape(8, 128), B_Dskip.reshape(8, 128),
      jnp.asarray(fs, bf16), jnp.asarray(g, bf16))
    return out.reshape(1, S, DM + D)
```

```python
import functools

import numpy as np
import jax
import jax.numpy as jnp
from jax import lax
import jax.experimental.pallas as pl
import jax.experimental.pallas.tpu as pltpu

bf16, f32, u32 = jnp.bfloat16, jnp.float32, jnp.uint32

S, DM, H, E, M, SEG = 2048, 1024, 32, 128, 8, 32
NSEG = S // SEG
TOK = 24
T0 = S - TOK * NSEG
RING = 576
QOFF = 64
NP = H // 2
KNI = 1
RC = 64
MACJ = 6
NSLOT = 118
L, D, N = 2048, 1024, 128
BLK = 128
NBLK = L // BLK
NT = D // 128
TAPROWS = 656
WINDOWS = ((0, 128, 0, 1), (128, 128, 1, 1), (256, 128, 2, 1), (320, 80, 3, 1),
           (384, 128, 4, 3), (480, 48, 7, 1), (512, 128, 8, 7), (624, 32, 15, 1))

V_FENCE = 0
V_MASK = 8
V_YTAB = 24
V_START = V_YTAB + 256
V_STEP = V_START + 160
V_UF = V_STEP + 128
V_KF = V_UF + NBLK * 32
V_ROWS = V_KF + NBLK * 32


def _bf16_round_int(l):
    u = np.asarray(l, np.float32).view(np.uint32)
    r = (u + 0x7FFF + ((u >> 16) & 1)) & 0xFFFF0000
    return r.astype(np.uint32).view(np.float32).astype(np.int64)


def _tap_row(lp):
    return np.where(lp < 256, lp, np.where(lp < 512, 256 + (lp - 256) // 2,
                    np.where(lp < 1024, 384 + (lp - 512) // 4, 512 + (lp - 1024) // 8)))


@functools.lru_cache(maxsize=None)
def _dft_consts():
    t = np.arange(BLK)
    F = np.zeros((8, 32, BLK))
    G = np.zeros((BLK, 8, 32))
    for r in range(8):
        f = np.concatenate([16 * r + 2 * np.arange(8), 16 * r + 2 * np.arange(8) + 1])
        th = 2 * np.pi * (f + 0.5) / (2 * BLK)
        F[r, :16] = np.cos(th[:, None] * t[None])
        F[r, 16:] = -np.sin(th[:, None] * t[None])
        G[:, r, 0::2] = np.cos(th[None] * t[:, None]) / BLK
        G[:, r, 1::2] = -np.sin(th[None] * t[:, None]) / BLK
    FS = np.zeros((8, NBLK, 32, 128))
    for (w0, wn, b0, nb) in WINDOWS:
        for j in range(b0, b0 + nb):
            rows = _tap_row(_bf16_round_int(BLK * j + t)) - w0
            assert rows.min() >= 0 and rows.max() < wn
            sel = np.zeros((BLK, 128))
            sel[t, rows] = 1.0
            FS[:, j] = F @ sel
    return (FS.reshape(8, NBLK * 32, 128).astype(np.float32),
            G.reshape(BLK, 256).astype(np.float32))


def _cmul(a, b):
    return (a[0] * b[0] - a[1] * b[1], a[0] * b[1] + a[1] * b[0])


def _csq(a):
    return (a[0] * a[0] - a[1] * a[1], 2.0 * (a[0] * a[1]))


def _cexp(lr, li):
    m = jnp.exp(lr)
    return (m * jnp.cos(li), m * jnp.sin(li))


def _prep_tile(c, praw, vec, par):
    rows = pl.ds(c * 128, 128)
    tr = lambda k: praw[k, rows, :].astype(f32).T
    dt = jnp.exp(vec[0, pl.ds(c, 1), :]).astype(bf16).astype(f32)
    par[c, 0] = dt * tr(0)
    par[c, 1] = dt * tr(1)
    cc = _cmul((tr(4), tr(5)), (dt * tr(2), dt * tr(3)))
    par[c, 2] = cc[0]
    par[c, 3] = cc[1]


def _kgen_pieces(c, r, par, vb, taps, tslot, frow):
    st = {}

    def put(row, z, h=None):
        if h is None:
            vb[pl.ds(row, 16), :] = z[0]
            vb[pl.ds(row + 16, 16), :] = z[1]
        else:
            vb[pl.ds(row + 8 * h, 8), :] = z[0]
            vb[pl.ds(row + 16 + 8 * h, 8), :] = z[1]

    def get(row, h=None):
        if h is None:
            return (vb[pl.ds(row, 16), :], vb[pl.ds(row + 16, 16), :])
        return (vb[pl.ds(row + 8 * h, 8), :], vb[pl.ds(row + 16 + 8 * h, 8), :])

    def params(k):
        return par[c, k, pl.ds(r * 16 if isinstance(r, int) else pl.multiple_of(r * 16, 16), 16), :]

    def park():
        put(V_STEP, (params(0), params(1)))
        put(V_START, (params(0) * 128.0, params(1) * 128.0))

    def setup_lo(h):
        def fn():
            z = _cexp(*get(V_STEP, h))
            put(V_STEP, z, h)
            z = _csq(z)
            put(V_STEP + 32, z, h)
            put(V_STEP + 64, _csq(z), h)
        return fn

    def setup_y(h):
        def fn():
            z1, z2, z4 = get(V_STEP, h), get(V_STEP + 32, h), get(V_STEP + 64, h)
            s = lax.broadcasted_iota(jnp.int32, (8, 128), 0)
            fs = [(jnp.where((s >> k) & 1 == 1, z[0], 1.0), jnp.where((s >> k) & 1 == 1, z[1], 0.0))
                  for k, z in enumerate((z1, z2, z4))]
            y = _cmul(_cmul(fs[0], fs[1]), fs[2])
            for k in range(8):
                put(V_YTAB + 32 * k, y, h)
                if k < 7:
                    y = _cmul(y, z1)
                    y = (jnp.where(s == 7 - k, 1.0, y[0]), jnp.where(s == 7 - k, 0.0, y[1]))
            z = z4
            for k in range(4):
                z = _csq(z)
                put(V_STEP + 32 * k, z, h)
        return fn

    def setup_hi(h):
        def fn():
            z = _cexp(*get(V_START, h))
            cf = (params(2)[8 * h:8 * h + 8], params(3)[8 * h:8 * h + 8])
            put(V_START, cf, h)
            for g in range(1, 5):
                put(V_START + 32 * g, _cmul(cf, z), h)
                if g < 4:
                    z = _csq(z)
        return fn

    def square(k0, k1):
        def fn():
            for k in range(k0, k1):
                put(V_YTAB + 32 * k, _csq(get(V_YTAB + 32 * k)))
        return fn

    def rows_of(g, i0, ni):
        n_i = 16 + (g == 4)

        def fn():
            x = st.pop('x') if i0 > 0 else get(V_START + 32 * g)
            step = get(V_STEP + 32 * max(g - 1, 0))
            xs = []
            for t in range(ni):
                xs.append(x)
                if i0 + t + 1 < n_i:
                    x = _cmul(x, step)
            if i0 + ni < n_i:
                st['x'] = x
            acc = [None] * ni
            for k in range(8):
                yr, yi = get(V_YTAB + 32 * k)
                for t in range(ni):
                    v = xs[t][0] * yr - xs[t][1] * yi
                    v = v[:8] + v[8:]
                    if k:
                        v = pltpu.roll(v, k, 0)
                    acc[t] = v if acc[t] is None else acc[t] + v
            for t in range(ni):
                row = 128 * g + 8 * (i0 + t)
                a = acc[t]
                if row == 640:
                    a = jnp.where(lax.broadcasted_iota(jnp.int32, (8, 128), 0) == 0, a, 0.0)
                taps[tslot, pl.ds(row, 8), :] = taps[tslot, pl.ds(row, 8), :] + a
                vb[pl.ds(frow, 8), :] = a
        return fn

    pieces = [(4, park), (160, setup_lo(0)), (160, setup_lo(1)), (100, setup_y(0)), (100, setup_y(1)),
              (190, setup_hi(0)), (190, setup_hi(1))]
    for g in range(5):
        if g >= 2:
            pieces += [(40, square(0, 4)), (40, square(4, 8))]
        for i0 in range(0, 16 + (g == 4), KNI):
            ni = min(KNI, 16 + (g == 4) - i0)
            pieces.append((83 * ni, rows_of(g, i0, ni)))
    return pieces


def _conv_pieces(c, r, buf, fs_ref, us, taps, vb, yf, frow):
    st = {}

    def fwd_u(b0, b1):
        def fn():
            lhs = fs_ref[r, pl.ds(0, 32), :]
            for b in range(b0, b1):
                w = pltpu.bitcast(us[c, pl.ds(b * 64, 64), :], bf16)
                res = jnp.dot(lhs, w, preferred_element_type=f32)
                row = V_UF + 32 * b
                if b == 0:
                    vb[pl.ds(row, 32), :] = res
                else:
                    p = st['prev']
                    vb[pl.ds(row, 8), :] = res[0:8] - p[16:24]
                    vb[pl.ds(row + 8, 8), :] = res[8:16] + p[24:32]
                    vb[pl.ds(row + 16, 8), :] = res[16:24] + p[0:8]
                    vb[pl.ds(row + 24, 8), :] = res[24:32] - p[8:16]
                st['prev'] = res
        return fn

    def fwd_k(jobs):
        def fn():
            for (wi, t0, nb) in jobs:
                w0, wn, b0, _ = WINDOWS[wi]
                lhs = fs_ref[r, pl.ds((b0 + t0) * 32, nb * 32), pl.ds(0, wn)]
                w = taps[c, pl.ds(w0, wn), :].astype(bf16)
                vb[pl.ds(V_KF + 32 * (b0 + t0), 32 * nb), :] = jnp.dot(lhs, w, preferred_element_type=f32)
        return fn

    def mac(q, i0, ni, j0, j1):
        def fn():
            ld = lambda base, b: (vb[pl.ds(base + 32 * b + 8 * q, 8), :], vb[pl.ds(base + 32 * b + 16 + 8 * q, 8), :])
            zr, zi = st.pop('z') if j0 > 0 else ({}, {})
            ucache = {}
            for j in range(j0, j1):
                kr, ki = ld(V_KF, j)
                for i in range(max(i0, j), i0 + ni):
                    if i - j not in ucache:
                        ucache[i - j] = ld(V_UF, i - j)
                    ur, ui = ucache[i - j]
                    if i not in zr:
                        zr[i] = kr * ur - ki * ui
                        zi[i] = kr * ui + ki * ur
                    else:
                        zr[i] = zr[i] + kr * ur - ki * ui
                        zi[i] = zi[i] + kr * ui + ki * ur
            vb[pl.ds(frow, 8), :] = zr[i0 + ni - 1]
            if j1 < i0 + ni:
                st['z'] = (zr, zi)
            else:
                row = pl.multiple_of(r * 16 + q * 8, 8)
                for i in range(i0, i0 + ni):
                    yf[buf, i, pl.ds(row, 8), :] = pltpu.pack_elementwise([zr[i], zi[i]], packed_dtype=bf16)
        return (8 * sum(1 for j in range(j0, j1) for i in range(max(i0, j), i0 + ni)), fn)

    fwd = [fwd_u(0, 8), fwd_u(8, 16), fwd_k(((0, 0, 1), (1, 0, 1), (2, 0, 1), (3, 0, 1))),
           fwd_k(((4, 0, 2), (6, 0, 2), (6, 2, 2), (6, 4, 2))), fwd_k(((4, 2, 1), (5, 0, 1), (6, 6, 1), (7, 0, 1)))]
    macs = []
    for q in range(2):
        for i0 in range(0, NBLK, 2):
            for j0 in range(0, i0 + 2, MACJ):
                macs.append(mac(q, i0, 2, j0, min(j0 + MACJ, i0 + 2)))
    return fwd, macs


def _inv_piece(c, b, buf, g_ref, us, vec, yf, outb):
    rows = pl.ds(pl.multiple_of(b * 64, 64), 64)
    w = pltpu.bitcast(yf[buf, b], bf16)
    y = jnp.dot(g_ref[...], w, preferred_element_type=f32)
    u = pltpu.bitcast(us[c, rows, :], bf16).astype(f32)
    sk = (u * vec[1, pl.ds(c, 1), :]).astype(bf16).astype(f32)
    o = (y.astype(bf16).astype(f32) + sk).astype(bf16)
    outb[c, rows, :] = pltpu.bitcast(o, u32)


def _attn_fill():
    n = 2 * (SEG + M)
    r = lax.broadcasted_iota(jnp.int32, (n, n), 0)
    c = lax.broadcasted_iota(jnp.int32, (n, n), 1)
    head = lambda i: jnp.where(i < 2 * SEG, i // SEG, (i - 2 * SEG) // M)
    same = head(r) == head(c)
    allowed = same & ((r >= 2 * SEG) | (c >= 2 * SEG) | (r >= c))
    return jnp.where(allowed, 0.0, jnp.where(same, -1e9, -jnp.inf)).astype(f32)


def _kernel(zero_ref, x_hbm, mem0_ref, wq_hbm, wk_hbm, wv_hbm, wo_hbm,
            u_hbm, p0, p1, p2, p3, p4, p5, ldt_ref, dsk_ref, fs_hbm, g_hbm,
            out_hbm,
            wq, wk, wv, wo, xb, xs, h_ref, outs, fill_ref,
            praw, par, us, taps, vb, yf, outb, vec, fs_ref, g_ref,
            sem_w, sem_o, sem_xb, sem_x, sem_p, sem_u, sem_out, *rings):
    wqkv = (wq, wk, wv)
    ring = rings[:NP]
    oring = rings[NP:2 * NP]
    lo_ref = rings[2 * NP:3 * NP]
    scale = E ** -0.5

    whbm = [w.bitcast(u32) for w in (wq_hbm, wk_hbm, wv_hbm)]

    def wcp(j, m, p):
        return pltpu.make_async_copy(whbm[m].at[:, p, j, :], wqkv[m].at[p, j], sem_w.at[(j * 3 + m) * 2 + p])

    def start_w(j):
        for m in range(3):
            for p in range(2):
                wcp(j, m, p).start()

    xu = x_hbm.bitcast(u32)
    xcs = [pltpu.make_async_copy(xu.at[pl.ds(0, T0 // 2), pl.ds(c * 128, 128)], xb.at[c], sem_xb.at[c])
           for c in range(8)]
    xcp1 = pltpu.make_async_copy(x_hbm.at[pl.ds(T0, S - T0)], xs, sem_x.at[0])
    pcs = [pltpu.make_async_copy(p, praw.at[k], sem_p.at[k]) for k, p in enumerate((p0, p1, p2, p3, p4, p5))]
    ccs = [pltpu.make_async_copy(fs_hbm, fs_ref, sem_p.at[6]), pltpu.make_async_copy(g_hbm, g_ref, sem_p.at[7])]
    wou = wo_hbm.bitcast(u32)
    ocs = [pltpu.make_async_copy(wou.at[:, pl.ds(c * 128, 128)], wo.at[c], sem_o.at[c]) for c in range(8)]
    uu = u_hbm.bitcast(u32)
    ucs = [pltpu.make_async_copy(uu.at[:, pl.ds(c * 128, 128)], us.at[c], sem_u.at[c]) for c in range(NT)]

    frow = pl.multiple_of(zero_ref[0] * 8, 8)
    zrow = [pl.multiple_of(zero_ref[k] * 8, 8) for k in range(T0 // RC)]

    def make_fence(vpu, nslot):
        total = float(sum(cst for cst, _ in vpu))
        sched = {'slot': 0, 'next': 0, 'done': 0.0}

        def fence(v):
            sched['slot'] += 1
            first = True
            while sched['next'] < len(vpu) and sched['done'] < total * sched['slot'] / nslot:
                if first:
                    vb[pl.ds(frow, 8), :] = v
                    first = False
                cst, fn = vpu[sched['next']]
                fn()
                sched['next'] += 1
                sched['done'] += cst
        return fence, (lambda: sched['next'] == len(vpu))

    def unpair(j, m, r0, nr):
        def fn():
            rows = pl.ds(r0, nr)
            m_lo = jnp.tile(pltpu.bitcast(vb[pl.ds(V_MASK, 8), :], u32), (nr // 8, 1))
            m_hi = jnp.tile(pltpu.bitcast(vb[pl.ds(V_MASK + 8, 8), :], u32), (nr // 8, 1))
            a = wqkv[m][0, j, rows, :]
            b = wqkv[m][1, j, rows, :]
            wqkv[m][0, j, rows, :] = (a & m_lo) | ((b & m_lo) << 16)
            wqkv[m][1, j, rows, :] = ((a & m_hi) >> 16) | (b & m_hi)
        return (nr, fn)

    def unpair_pieces(items):
        return [unpair(j, m, r0, 128) for (j, m) in items for r0 in range(0, DM // 2, 128)]

    for cp in xcs:
        cp.start()
    for p in range(2):
        wcp(0, 0, p).start()
    vec[0] = ldt_ref[...].astype(f32)
    vec[1] = dsk_ref[...].astype(f32)
    vb[pl.ds(V_MASK, 8), :] = pltpu.bitcast(jnp.full((8, 128), 0x0000FFFF, u32), f32)
    vb[pl.ds(V_MASK + 8, 8), :] = pltpu.bitcast(jnp.full((8, 128), 0xFFFF0000, u32), f32)
    taps[...] = jnp.zeros(taps.shape, f32)
    yf[1] = jnp.zeros(yf.shape[1:], u32)
    fill_ref[...] = _attn_fill()
    h_ref[pl.ds(0, M), :] = mem0_ref[...]

    items = [(j, m) for j in range(NP) for m in range(3)]
    wcs = lambda lo, hi: [wcp(j, m, p) for (j, m) in items[lo:hi] for p in range(2)]
    plan = {
        0: ((1, 2), wcs(2, 4), []),
        1: ((2, 4), wcs(4, 7), []),
        3: ((4, 7), wcs(7, 12) + pcs, []),
        6: ((7, 12), wcs(12, 21), []),
        11: ((12, 21), wcs(21, 33), pcs),
        20: ((21, 33), wcs(33, 48) + ocs[:4], []),
        32: ((33, 48), ocs[4:] + ucs + [xcp1] + ccs, []),
    }
    with jax.named_scope("bulk"):
        for cp in wcs(1, 2):
            cp.start()
        with jax.named_scope("waitx"):
            for cp in xcs + wcs(0, 1):
                cp.wait()
        for _, fn in unpair_pieces(items[0:1]):
            fn()
        points = sorted(plan) + [len(items)]
        for g in range(len(points) - 1):
            lo, hi = points[g], points[g + 1]
            (w_lo, w_hi), starts, waits = plan[lo]
            for cp in starts:
                cp.start()
            with jax.named_scope("wait%d" % lo):
                for cp in wcs(w_lo, w_hi) + waits:
                    cp.wait()
            assert w_hi == min(hi + 1, len(items))
            extra = []
            if lo == 11:
                extra = [(300, functools.partial(_prep_tile, c, praw, vec, par)) for c in range(NT)]
            elif lo == 20:
                for r in range(3):
                    extra += _kgen_pieces(0, r, par, vb, taps, 0, zrow[1])
            elif lo == 32:
                for r in range(3, 8):
                    extra += _kgen_pieces(0, r, par, vb, taps, 0, zrow[1])
            n_chunk = 2 * (T0 // RC)
            fence_x, fin_x = make_fence(extra, (hi - lo) * n_chunk - 2)
            for it in range(lo, hi):
                j, m = items[it]
                fence_w, fin_w = make_fence(unpair_pieces(items[it + 1:it + 2]), n_chunk - 3)
                for p in range(2):
                    for rc in range(T0 // RC):
                        w = pltpu.bitcast(wqkv[m][p, j, pl.ds(zrow[rc], DM // 2), :], bf16)
                        lhs = jnp.concatenate(
                            [pltpu.bitcast(xb[c, pl.ds(rc * RC // 2, RC // 2), :], bf16) for c in range(8)], axis=1)
                        res = jnp.dot(lhs, w, preferred_element_type=f32)
                        ring[j][m, p, pl.ds(QOFF + rc * RC, RC), :] = res.astype(bf16)
                        fence_w(res[:8])
                        fence_x(res[:8])
                assert fin_w()
            assert fin_x()
    with jax.named_scope("waitrest"):
        for cp in ocs + ucs + ccs + [xcp1]:
            cp.wait()

    ou = out_hbm.bitcast(u32)

    def outa_cp(row, n):
        return pltpu.make_async_copy(outs.at[pl.ds(row, n)], out_hbm.at[pl.ds(row, n), pl.ds(0, DM)], sem_out.at[0])

    def outb_cp(c, row, n):
        return pltpu.make_async_copy(outb.at[c, pl.ds(row, n)], ou.at[pl.ds(row, n), pl.ds(DM + c * 128, 128)],
                                     sem_out.at[1])

    def step(s, carry):
        tok0 = pl.multiple_of(TOK * s, 8)
        h_ref[pl.ds(M, TOK), :] = xs[pl.ds(tok0, TOK), :]
        h = h_ref[...]
        ppos = pl.multiple_of(lax.rem(TOK * s, RING), 8)
        cpos = pl.multiple_of(lax.rem(QOFF + SEG * s, RING), 32)
        opos = pl.multiple_of(lax.rem(SEG * s, RING), 32)
        orow = pl.multiple_of(TOK * s, 8)
        mem_rows = {}
        probs = {}

        ct = s // 8
        r = s % 8
        buf = ct % 2
        cprev = (ct + NT - 1) % NT
        fwd, macs = _conv_pieces(ct, r, buf, fs_ref, us, taps, vb, yf, zrow[1])
        kgen = _kgen_pieces((ct + 1) % NT, r, par, vb, taps, ct + 1, zrow[1])
        fence, finished = make_fence(kgen + macs, NSLOT)

        def stage_a(j):
            for m in range(3):
                mm = []
                for p in range(2):
                    w = pltpu.bitcast(wqkv[m][p, j], bf16)
                    res = jnp.dot(h, w, preferred_element_type=f32)
                    ring[j][m, p, pl.ds(ppos, TOK), :] = res[M:].astype(bf16)
                    mm.append(res[:M])
                    fence(res[:M])
                mem_rows[m, j] = jnp.concatenate(mm, axis=0).astype(bf16)

        def gather(m, j):
            return jnp.concatenate([ring[j][m, 0, pl.ds(cpos, SEG), :], ring[j][m, 1, pl.ds(cpos, SEG), :],
                                    mem_rows[m, j]], axis=0)

        scores = {}

        def stage_qk(j):
            scores[j] = lax.dot_general(gather(0, j), gather(1, j), (((1,), (1,)), ((), ())),
                                        preferred_element_type=f32)

        def stage_b(j):
            sc = scores.pop(j)
            fl = fill_ref[...]
            sc = jnp.where(fl == 0.0, sc * scale, fl)
            mx = jnp.max(sc, axis=-1, keepdims=True)
            e = jnp.exp(sc - mx)
            den = jnp.sum(e, axis=-1, keepdims=True)
            r0 = pl.reciprocal(den, approx=True)
            r1 = r0 * (2.0 - den * r0)
            probs[j] = (e * r1).astype(bf16)

        def stage_c(j):
            o = jnp.dot(probs[j], gather(2, j), preferred_element_type=f32)
            for p in range(2):
                oring[j][p, pl.ds(opos, SEG), :] = o[p * SEG:(p + 1) * SEG].astype(bf16)
                lo_ref[j][p, pl.ds(0, M), :] = o[2 * SEG + p * M:2 * SEG + (p + 1) * M].astype(bf16)
                lo_ref[j][p, pl.ds(M, TOK), :] = oring[j][p, pl.ds(ppos, TOK), :]

        acc = [None] * 8

        def stage_d(h0, h1, last=False):
            lhs = jnp.concatenate([lo_ref[hh // 2][hh % 2] for hh in range(h0, h1)], axis=1)
            for c in range(8):
                w = pltpu.bitcast(wo[c, pl.ds(h0 * 64, (h1 - h0) * 64), :], bf16)
                res = jnp.dot(lhs, w, preferred_element_type=f32)
                acc[c] = res if acc[c] is None else acc[c] + res
                if not last:
                    fence(res[:M])
                if last:
                    rb = acc[c].astype(bf16)
                    h_ref[pl.ds(0, M), pl.ds(c * 128, 128)] = rb[:M]
                    outs[pl.ds(orow, TOK), pl.ds(c * 128, 128)] = rb[M:]

        for t in range(2):
            _inv_piece(cprev, 2 * r + t, 1 - buf, g_ref, us, vec, yf, outb)
        for p in fwd:
            p()
        def attn_group(jq, jc):
            for j in jq:
                stage_qk(j)
            for j in jc:
                stage_c(j)
            for j in jq:
                stage_b(j)

        for j in range(NP):
            stage_a(j)
            if j >= 2 and j % 2 == 0:
                attn_group((j - 2, j - 1), (j - 4, j - 3) if j >= 4 else ())
        stage_d(0, 8)
        attn_group((14, 15), (12, 13))
        stage_d(8, 20)
        attn_group((), (14, 15))
        stage_d(20, 28)
        assert finished()
        stage_d(28, 32, last=True)

        outa_cp(orow, TOK).start()

        @pl.when(s >= 8)
        def _():
            outb_cp(cprev, pl.multiple_of(r * 128, 128), 128).start()
        return carry

    with jax.named_scope("steps"):
        lax.fori_loop(0, NSEG, step, 0)

    with jax.named_scope("flush"):
        for b in range(NBLK):
            _inv_piece(NT - 1, b, (NT - 1) % 2, g_ref, us, vec, yf, outb)
        outb_cp(NT - 1, 0, L // 2).start()
        done = TOK * NSEG
        p0_ = done % RING
        n0 = RING - p0_
        for (rp, n, t) in ((p0_, n0, done), (0, S - done - n0, done + n0)):
            lhs = jnp.concatenate([oring[hh // 2][hh % 2, pl.ds(rp, n), :] for hh in range(H)], axis=1)
            for c in range(8):
                outs[pl.ds(t, n), pl.ds(c * 128, 128)] = jnp.dot(
                    lhs, pltpu.bitcast(wo[c], bf16), preferred_element_type=f32).astype(bf16)
            outa_cp(t, n).start()
    with jax.named_scope("waitout"):
        outa_cp(0, S).wait()
        pltpu.make_async_copy(outb, outb, sem_out.at[1]).wait()


@functools.partial(jax.jit, static_argnames=("A_seg_len",))
def pallas_concat_heads__memory_aug_recurrent_mem_tr__ssm_conv_s4__prompt_kernel(
    A_x, A_mem0, A_Wq, A_Wk, A_Wv, A_Wo, A_seg_len,
    B_u, B_A_re, B_A_im, B_B_re, B_B_im, B_C_re, B_C_im, B_log_dt, B_Dskip,
):
    assert A_seg_len == SEG and A_x.shape == (1, S, DM) and B_u.shape == (1, L, D)
    fs, g = _dft_consts()
    w4 = lambda w: w.reshape(DM // 2, 2, H, E)
    any_ = pl.BlockSpec(memory_space=pl.ANY)
    vm = pl.BlockSpec(memory_space=pltpu.VMEM)
    V = pltpu.VMEM
    out = pl.pallas_call(
        _kernel,
        out_shape=jax.ShapeDtypeStruct((S, DM + D), bf16),
        in_specs=[pl.BlockSpec(memory_space=pltpu.SMEM), any_, vm, any_, any_, any_, any_] + [any_] * 7 + [vm, vm, any_, any_],
        out_specs=any_,
        scratch_shapes=[
            V((2, NP, DM // 2, E), u32),
            V((2, NP, DM // 2, E), u32),
            V((2, NP, DM // 2, E), u32),
            V((8, H * E // 2, 128), u32),
            V((8, T0 // 2, 128), u32),
            V((S - T0, DM), bf16),
            V((M + TOK, DM), bf16),
            V((S, DM), bf16),
            V((2 * (SEG + M), 2 * (SEG + M)), f32),
            V((6, D, N), bf16),
            V((NT, 4, N, 128), f32),
            V((NT, L // 2, 128), u32),
            V((NT + 1, TAPROWS, 128), f32),
            V((V_ROWS, 128), f32),
            V((2, NBLK, 128, 128), u32),
            V((NT, L // 2, 128), u32),
            V((2, 8, 128), f32),
            V((8, NBLK * 32, 128), bf16),
            V((BLK, 256), bf16),
            pltpu.SemaphoreType.DMA((6 * NP,)),
            pltpu.SemaphoreType.DMA((8,)),
            pltpu.SemaphoreType.DMA((8,)),
            pltpu.SemaphoreType.DMA((1,)),
            pltpu.SemaphoreType.DMA((8,)),
            pltpu.SemaphoreType.DMA((NT,)),
            pltpu.SemaphoreType.DMA((2,)),
        ] + [V((3, 2, RING, E), bf16)] * NP + [V((2, RING, E), bf16)] * NP + [V((2, M + TOK, E), bf16)] * NP,
        compiler_params=pltpu.CompilerParams(vmem_limit_bytes=110 * 1024 * 1024),
    )(jnp.asarray(np.zeros((8,), np.int32)), A_x.reshape(S, DM), A_mem0.reshape(M, DM), w4(A_Wq), w4(A_Wk), w4(A_Wv), A_Wo.reshape(H * E, DM),
      B_u.reshape(L, D), B_A_re, B_A_im, B_B_re, B_B_im, B_C_re, B_C_im,
      B_log_dt.reshape(8, 128), B_Dskip.reshape(8, 128),
      jnp.asarray(fs, bf16), jnp.asarray(g, bf16))
    return out.reshape(1, S, DM + D)
```

```python
import functools

import numpy as np
import jax
import jax.numpy as jnp
from jax import lax
import jax.experimental.pallas as pl
import jax.experimental.pallas.tpu as pltpu

bf16, f32, u32 = jnp.bfloat16, jnp.float32, jnp.uint32

S, DM, H, E, M, SEG = 2048, 1024, 32, 128, 8, 32
NSEG = S // SEG
TOK = 24
T0 = S - TOK * NSEG
RING = 576
QOFF = 64
NP = H // 2
LOG2E = 1.4426950408889634
QUICK = False
KNI = 2
KSPLIT = 2
PLAN = (('k0', 0, 96), ('m0', 96, 122), ('k1', 124, 220), ('m1', 220, 260))
DONE_K = True
DONE_M = True
DW_ODD = 1.5
RC = 64
MACJ = 6
NSLOT = 118
L, D, N = 2048, 1024, 128
BLK = 128
NBLK = L // BLK
NT = D // 128
TAPROWS = 656
WINDOWS = ((0, 128, 0, 1), (128, 128, 1, 1), (256, 128, 2, 1), (320, 80, 3, 1),
           (384, 128, 4, 3), (480, 48, 7, 1), (512, 128, 8, 7), (624, 32, 15, 1))

V_FENCE = 0
V_MASK = 8
V_YTAB = 24
V_START = V_YTAB + 256
V_STEP = V_START + 160
V_ROWS = V_STEP + 128
V_UF = 8
V_KF = V_UF + NBLK * 32
VM_ROWS = V_KF + NBLK * 32


def _bf16_round_int(l):
    u = np.asarray(l, np.float32).view(np.uint32)
    r = (u + 0x7FFF + ((u >> 16) & 1)) & 0xFFFF0000
    return r.astype(np.uint32).view(np.float32).astype(np.int64)


def _tap_row(lp):
    return np.where(lp < 256, lp, np.where(lp < 512, 256 + (lp - 256) // 2,
                    np.where(lp < 1024, 384 + (lp - 512) // 4, 512 + (lp - 1024) // 8)))


@functools.lru_cache(maxsize=None)
def _dft_consts():
    t = np.arange(BLK)
    F = np.zeros((8, 32, BLK))
    G = np.zeros((BLK, 8, 32))
    for r in range(8):
        f = np.concatenate([16 * r + 2 * np.arange(8), 16 * r + 2 * np.arange(8) + 1])
        th = 2 * np.pi * (f + 0.5) / (2 * BLK)
        F[r, :16] = np.cos(th[:, None] * t[None])
        F[r, 16:] = -np.sin(th[:, None] * t[None])
        G[:, r, 0::2] = np.cos(th[None] * t[:, None]) / BLK
        G[:, r, 1::2] = -np.sin(th[None] * t[:, None]) / BLK
    FS = np.zeros((8, NBLK, 32, 128))
    for (w0, wn, b0, nb) in WINDOWS:
        for j in range(b0, b0 + nb):
            rows = _tap_row(_bf16_round_int(BLK * j + t)) - w0
            assert rows.min() >= 0 and rows.max() < wn
            sel = np.zeros((BLK, 128))
            sel[t, rows] = 1.0
            FS[:, j] = F @ sel
    return (FS.reshape(8, NBLK * 32, 128).astype(np.float32),
            G.reshape(BLK, 256).astype(np.float32))


def _cmul(a, b):
    return (a[0] * b[0] - a[1] * b[1], a[0] * b[1] + a[1] * b[0])


def _csq(a):
    return (a[0] * a[0] - a[1] * a[1], 2.0 * (a[0] * a[1]))


def _cexp(lr, li):
    k = jnp.floor(li * (2.0 / np.pi) + 0.5)
    r = ((li - k * 1.5703125) - k * 4.837512969970703125e-4) - k * 7.54978995489188216e-8
    r = jnp.clip(r, -0.8, 0.8)
    r2 = r * r
    s = r + r * r2 * (-1.6666654611e-1 + r2 * (8.3321608736e-3 + r2 * -1.9515295891e-4))
    c = (1.0 - 0.5 * r2) + (r2 * r2) * (4.166664568298827e-2
                                        + r2 * (-1.388731625493765e-3 + r2 * 2.443315711809948e-5))
    q = k.astype(jnp.int32)
    swap = (q & 1) == 1
    m = jnp.exp(lr)
    flip = lambda v, bit: pltpu.bitcast(pltpu.bitcast(v, jnp.int32) ^ (bit << 30), f32)
    return (flip(m * jnp.where(swap, s, c), (q + 1) & 2), flip(m * jnp.where(swap, c, s), q & 2))


def _par_row(c, k):
    return 8 + (c * 6 + k) * N


def _prep_pieces(praw, vec, par):
    def stage1(c):
        def fn():
            tr = lambda k: praw[k, pl.ds(c * 128, 128), :].astype(f32).T
            dt = jnp.exp(vec[0, pl.ds(c, 1), :]).astype(bf16).astype(f32)
            cc = _cmul((tr(4), tr(5)), (dt * tr(2), dt * tr(3)))
            for k, v in ((0, dt * tr(0)), (1, dt * tr(1)), (4, cc[0]), (5, cc[1])):
                par[pl.ds(_par_row(c, k), N), :] = v
        return fn

    def stage2(c, n0):
        def fn():
            lr = par[pl.ds(_par_row(c, 0) + n0, 16), :]
            li = par[pl.ds(_par_row(c, 1) + n0, 16), :]
            for k, v in enumerate(_cexp(lr, li) + _cexp(lr * 128.0, li * 128.0)):
                par[pl.ds(_par_row(c, k) + n0, 16), :] = v
        return fn

    return ([(260, stage1(c)) for c in range(NT)]
            + [(190, stage2(c, n0)) for c in range(NT) for n0 in range(0, N, 16)])


def _kgen_pieces(c, r, par, vb, taps, tslot, frow):
    st = {}

    def put(row, z, h=None):
        if h is None:
            vb[pl.ds(row, 16), :] = z[0]
            vb[pl.ds(row + 16, 16), :] = z[1]
        else:
            vb[pl.ds(row + 8 * h, 8), :] = z[0]
            vb[pl.ds(row + 16 + 8 * h, 8), :] = z[1]

    def get(row, h=None):
        if h is None:
            return (vb[pl.ds(row, 16), :], vb[pl.ds(row + 16, 16), :])
        return (vb[pl.ds(row + 8 * h, 8), :], vb[pl.ds(row + 16 + 8 * h, 8), :])

    def params(k):
        row = _par_row(c, k) + r * 16
        return par[pl.ds(row if isinstance(row, int) else pl.multiple_of(row, 8), 16), :]

    def park():
        put(V_STEP, (params(0), params(1)))
        put(V_START + 32, (params(2), params(3)))
        put(V_START, (params(4), params(5)))

    def setup_y(h):
        def fn():
            z1 = get(V_STEP, h)
            z2 = _csq(z1)
            z4 = _csq(z2)
            s = lax.broadcasted_iota(jnp.int32, (8, 128), 0)
            fs = [(jnp.where((s >> k) & 1 == 1, z[0], 1.0), jnp.where((s >> k) & 1 == 1, z[1], 0.0))
                  for k, z in enumerate((z1, z2, z4))]
            y = _cmul(_cmul(fs[0], fs[1]), fs[2])
            for k in range(8):
                put(V_YTAB + 32 * k, y, h)
                if k < 7:
                    y = _cmul(y, z1)
                    y = (jnp.where(s == 7 - k, 1.0, y[0]), jnp.where(s == 7 - k, 0.0, y[1]))
            z = z4
            for k in range(4):
                z = _csq(z)
                put(V_STEP + 32 * k, z, h)
        return fn

    def setup_hi():
        z = get(V_START + 32)
        cf = get(V_START)
        for g in range(1, 5):
            put(V_START + 32 * g, _cmul(cf, z))
            if g < 4:
                z = _csq(z)

    def square(k0, k1):
        def fn():
            for k in range(k0, k1):
                put(V_YTAB + 32 * k, _csq(get(V_YTAB + 32 * k)))
        return fn

    def rows_of(g, i0, ni):
        n_i = 16 + (g == 4)

        def fn():
            x = st.pop('x') if i0 > 0 else get(V_START + 32 * g)
            step = get(V_STEP + 32 * max(g - 1, 0))
            xs = []
            for t in range(ni):
                xs.append(x)
                if i0 + t + 1 < n_i:
                    x = _cmul(x, step)
            if i0 + ni < n_i:
                st['x'] = x
            acc = [None] * ni
            for k in range(8):
                yr, yi = get(V_YTAB + 32 * k)
                for t in range(ni):
                    v = xs[t][0] * yr - xs[t][1] * yi
                    v = v[:8] + v[8:]
                    if k:
                        v = pltpu.roll(v, k, 0)
                    acc[t] = v if acc[t] is None else acc[t] + v
                if frow is not None and k % KSPLIT == KSPLIT - 1 and k < 7:
                    vb[pl.ds(frow, 8), :] = acc[ni - 1]
            for t in range(ni):
                row = 128 * g + 8 * (i0 + t)
                a = acc[t]
                if row == 640:
                    a = jnp.where(lax.broadcasted_iota(jnp.int32, (8, 128), 0) == 0, a, 0.0)
                taps[tslot, pl.ds(row, 8), :] = taps[tslot, pl.ds(row, 8), :] + a
                if frow is not None and t == ni - 1:
                    vb[pl.ds(frow, 8), :] = a
        return fn

    pieces = [(30, park), (110, setup_y(0)), (110, setup_y(1)), (80, setup_hi)]
    for g in range(5):
        if g >= 2:
            pieces += [(40, square(0, 4)), (40, square(4, 8))]
        for i0 in range(0, 16 + (g == 4), KNI):
            ni = min(KNI, 16 + (g == 4) - i0)
            pieces.append((83 * ni, rows_of(g, i0, ni)))
    return pieces


def _conv_pieces(c, r, buf, fs_ref, us, taps, vb, yf, frow):
    st = {}

    def fwd_u(b0, b1):
        def fn():
            lhs = fs_ref[r, pl.ds(0, 32), :]
            for b in range(b0, b1):
                w = pltpu.bitcast(us[c, pl.ds(b * 64, 64), :], bf16)
                res = jnp.dot(lhs, w, preferred_element_type=f32)
                row = V_UF + 32 * b
                if b == 0:
                    vb[pl.ds(row, 32), :] = res
                else:
                    p = st['prev']
                    vb[pl.ds(row, 8), :] = res[0:8] - p[16:24]
                    vb[pl.ds(row + 8, 8), :] = res[8:16] + p[24:32]
                    vb[pl.ds(row + 16, 8), :] = res[16:24] + p[0:8]
                    vb[pl.ds(row + 24, 8), :] = res[24:32] - p[8:16]
                st['prev'] = res
        return fn

    def fwd_k(jobs):
        def fn():
            for (wi, t0, nb) in jobs:
                w0, wn, b0, _ = WINDOWS[wi]
                lhs = fs_ref[r, pl.ds((b0 + t0) * 32, nb * 32), pl.ds(0, wn)]
                w = taps[c, pl.ds(w0, wn), :].astype(bf16)
                vb[pl.ds(V_KF + 32 * (b0 + t0), 32 * nb), :] = jnp.dot(lhs, w, preferred_element_type=f32)
        return fn

    def mac(q, i0, ni, j0, j1):
        def fn():
            ld = lambda base, b: (vb[pl.ds(base + 32 * b + 8 * q, 8), :], vb[pl.ds(base + 32 * b + 16 + 8 * q, 8), :])
            zr, zi = st.pop('z') if j0 > 0 else ({}, {})
            ucache = {}
            for j in range(j0, j1):
                kr, ki = ld(V_KF, j)
                for i in range(max(i0, j), i0 + ni):
                    if i - j not in ucache:
                        ucache[i - j] = ld(V_UF, i - j)
                    ur, ui = ucache[i - j]
                    if i not in zr:
                        zr[i] = kr * ur - ki * ui
                        zi[i] = kr * ui + ki * ur
                    else:
                        zr[i] = zr[i] + kr * ur - ki * ui
                        zi[i] = zi[i] + kr * ui + ki * ur
            if frow is not None:
                vb[pl.ds(frow, 8), :] = zr[i0 + ni - 1]
            if j1 < i0 + ni:
                st['z'] = (zr, zi)
            else:
                row = pl.multiple_of(r * 16 + q * 8, 8)
                for i in range(i0, i0 + ni):
                    yf[buf, i, pl.ds(row, 8), :] = pltpu.pack_elementwise([zr[i], zi[i]], packed_dtype=bf16)
        return (8 * sum(1 for j in range(j0, j1) for i in range(max(i0, j), i0 + ni)), fn)

    fwd = [fwd_u(0, 8), fwd_u(8, 16), fwd_k(((0, 0, 1), (1, 0, 1), (2, 0, 1), (3, 0, 1))),
           fwd_k(((4, 0, 2), (6, 0, 2), (6, 2, 2), (6, 4, 2))), fwd_k(((4, 2, 1), (5, 0, 1), (6, 6, 1), (7, 0, 1)))]
    macs = []
    for q in range(2):
        for i0 in range(0, NBLK, 2):
            for j0 in range(0, i0 + 2, MACJ):
                macs.append(mac(q, i0, 2, j0, min(j0 + MACJ, i0 + 2)))
    return fwd, macs


def _inv_piece(c, b, buf, g_ref, us, vec, yf, outb):
    rows = pl.ds(pl.multiple_of(b * 64, 64), 64)
    w = pltpu.bitcast(yf[buf, b], bf16)
    y = jnp.dot(g_ref[...], w, preferred_element_type=f32)
    u = pltpu.bitcast(us[c, rows, :], bf16).astype(f32)
    sk = (u * vec[1, pl.ds(c, 1), :]).astype(bf16).astype(f32)
    o = (y.astype(bf16).astype(f32) + sk).astype(bf16)
    outb[c, rows, :] = pltpu.bitcast(o, u32)


def _attn_fill():
    n = 2 * (SEG + M)
    r = lax.broadcasted_iota(jnp.int32, (n, n), 0)
    c = lax.broadcasted_iota(jnp.int32, (n, n), 1)
    head = lambda i: jnp.where(i < 2 * SEG, i // SEG, (i - 2 * SEG) // M)
    same = head(r) == head(c)
    allowed = same & ((r >= 2 * SEG) | (c >= 2 * SEG) | (r >= c))
    return jnp.where(allowed, 0.0, jnp.where(same, -1e9 * LOG2E, -jnp.inf)).astype(f32)


def _kernel(zero_ref, x_hbm, mem0_ref, wq_hbm, wk_hbm, wv_hbm, wo_hbm,
            u_hbm, p0, p1, p2, p3, p4, p5, ldt_ref, dsk_ref, fs_hbm, g_hbm,
            out_hbm,
            wq, wk, wv, wo, xb, xs, h_ref, outs, fill_ref,
            praw, par, us, taps, vb, vm, yf, outb, vec, fs_ref, g_ref,
            sem_w, sem_o, sem_xb, sem_x, sem_p, sem_u, sem_out, *rings):
    wqkv = (wq, wk, wv)
    ring = rings[:NP]
    lo_ref = rings[NP:]
    scale = E ** -0.5

    whbm = [w.bitcast(u32) for w in (wq_hbm, wk_hbm, wv_hbm)]

    def wcp(j, m, p):
        return pltpu.make_async_copy(whbm[m].at[:, p, j, :], wqkv[m].at[p, j], sem_w.at[(j * 3 + m) * 2 + p])

    def start_w(j):
        for m in range(3):
            for p in range(2):
                wcp(j, m, p).start()

    xu = x_hbm.bitcast(u32)
    xcs = [pltpu.make_async_copy(xu.at[pl.ds(0, T0 // 2), pl.ds(c * 128, 128)], xb.at[c], sem_xb.at[c])
           for c in range(8)]
    xcp1 = pltpu.make_async_copy(x_hbm.at[pl.ds(T0, S - T0)], xs, sem_x.at[0])
    pcs = [pltpu.make_async_copy(p, praw.at[k], sem_p.at[k]) for k, p in enumerate((p0, p1, p2, p3, p4, p5))]
    ccs = [pltpu.make_async_copy(fs_hbm, fs_ref, sem_p.at[6]), pltpu.make_async_copy(g_hbm, g_ref, sem_p.at[7])]
    wou = wo_hbm.bitcast(u32)
    ocs = [pltpu.make_async_copy(wou.at[:, pl.ds(c * 128, 128)], wo.at[c], sem_o.at[c]) for c in range(8)]
    uu = u_hbm.bitcast(u32)
    ucs = [pltpu.make_async_copy(uu.at[:, pl.ds(c * 128, 128)], us.at[c], sem_u.at[c]) for c in range(NT)]

    frow = pl.multiple_of(zero_ref[0] * 8, 8)
    zrow = [pl.multiple_of(zero_ref[k] * 8, 8) for k in range(T0 // RC)]

    class Pacer:
        def __init__(self, segments):
            self.t = 0.0
            self.todo = []
            for (pieces, buf, t0, t1) in segments:
                total = float(sum(c for c, _ in pieces))
                done = 0.0
                for (cst, fn) in pieces:
                    self.todo.append((t0 + (t1 - t0) * done / total, fn, buf))
                    done += cst

        def __call__(self, v, dt=1.0):
            self.t += dt
            fenced = []
            while self.todo and self.todo[0][0] < self.t:
                _, fn, buf = self.todo.pop(0)
                if not any(b is buf for b in fenced):
                    buf[pl.ds(frow, 8), :] = v
                    fenced.append(buf)
                fn()

        def finished(self):
            return not self.todo

    def make_fence(vpu, nslot, buf=vb):
        pc = Pacer([(vpu, buf, 0.0, float(nslot))])
        return pc, pc.finished

    def unpair(j, m, r0, nr):
        def fn():
            rows = pl.ds(r0, nr)
            m_lo = jnp.tile(pltpu.bitcast(vb[pl.ds(V_MASK, 8), :], u32), (nr // 8, 1))
            m_hi = jnp.tile(pltpu.bitcast(vb[pl.ds(V_MASK + 8, 8), :], u32), (nr // 8, 1))
            a = wqkv[m][0, j, rows, :]
            b = wqkv[m][1, j, rows, :]
            wqkv[m][0, j, rows, :] = (a & m_lo) | ((b & m_lo) << 16)
            wqkv[m][1, j, rows, :] = ((a & m_hi) >> 16) | (b & m_hi)
        return (nr, fn)

    def unpair_pieces(items):
        return [unpair(j, m, r0, 128) for (j, m) in items for r0 in range(0, DM // 2, 128)]

    for cp in xcs:
        cp.start()
    for p in range(2):
        wcp(0, 0, p).start()
    vec[0] = ldt_ref[...].astype(f32)
    vec[1] = dsk_ref[...].astype(f32)
    vb[pl.ds(V_MASK, 8), :] = pltpu.bitcast(jnp.full((8, 128), 0x0000FFFF, u32), f32)
    vb[pl.ds(V_MASK + 8, 8), :] = pltpu.bitcast(jnp.full((8, 128), 0xFFFF0000, u32), f32)
    taps[...] = jnp.zeros(taps.shape, f32)
    yf[1] = jnp.zeros(yf.shape[1:], u32)
    fill_ref[...] = _attn_fill()
    h_ref[pl.ds(0, M), :] = mem0_ref[...]

    items = [(j, m) for j in range(NP) for m in range(3)]
    wcs = lambda lo, hi: [wcp(j, m, p) for (j, m) in items[lo:hi] for p in range(2)]
    plan = {
        0: ((1, 2), wcs(2, 4), []),
        1: ((2, 4), wcs(4, 7), []),
        3: ((4, 7), wcs(7, 12) + pcs, []),
        6: ((7, 12), wcs(12, 21), []),
        11: ((12, 21), wcs(21, 33), pcs),
        20: ((21, 33), wcs(33, 48) + ocs[:4], []),
        32: ((33, 48), ocs[4:] + ucs + [xcp1] + ccs, []),
    }
    with jax.named_scope("bulk"):
        for cp in wcs(1, 2):
            cp.start()
        with jax.named_scope("waitx"):
            for cp in xcs + wcs(0, 1):
                cp.wait()
        for _, fn in unpair_pieces(items[0:1]):
            fn()
        points = sorted(plan) + [len(items)]
        if QUICK:
            for cp in wcs(2, 48) + pcs + ocs + ucs + [xcp1] + ccs:
                cp.start()
            for cp in wcs(1, 48) + pcs:
                cp.wait()
            for _, fn in unpair_pieces(items[1:]):
                fn()
            for _, fn in _prep_pieces(praw, vec, par):
                fn()

            def kg(r, carry):
                for _, fn in _kgen_pieces(0, r, par, vb, taps, 0, zrow[1]):
                    fn()
                return carry
            lax.fori_loop(0, 8, kg, 0)
            for (j, m) in items:
                def chunk(rc, carry, j=j, m=m):
                    for p in range(2):
                        lhs = jnp.concatenate(
                            [pltpu.bitcast(xb[c, pl.ds(pl.multiple_of(rc * 32, 32), 32), :], bf16) for c in range(8)], axis=1)
                        ring[j][m, p, pl.ds(pl.multiple_of(QOFF + rc * 64, 64), 64), :] = jnp.dot(
                            lhs, pltpu.bitcast(wqkv[m][p, j], bf16), preferred_element_type=f32).astype(bf16)
                    return carry
                lax.fori_loop(0, 8, chunk, 0)
            points = []
        for g in range(len(points) - 1):
            lo, hi = points[g], points[g + 1]
            (w_lo, w_hi), starts, waits = plan[lo]
            for cp in starts:
                cp.start()
            with jax.named_scope("wait%d" % lo):
                for cp in wcs(w_lo, w_hi) + waits:
                    cp.wait()
            assert w_hi == min(hi + 1, len(items))
            extra = []
            xbuf = vb
            if lo == 11:
                extra = _prep_pieces(praw, vec, par)
                xbuf = par
            elif lo == 20:
                for r in range(3):
                    extra += _kgen_pieces(0, r, par, vb, taps, 0, zrow[1])
            elif lo == 32:
                for r in range(3, 8):
                    extra += _kgen_pieces(0, r, par, vb, taps, 0, zrow[1])
            n_chunk = 2 * (T0 // RC)
            fence_x, fin_x = make_fence(extra, (hi - lo) * n_chunk - 2, xbuf)
            for it in range(lo, hi):
                j, m = items[it]
                fence_w, fin_w = make_fence(unpair_pieces(items[it + 1:it + 2]), n_chunk - 3)
                for p in range(2):
                    for rc in range(T0 // RC):
                        w = pltpu.bitcast(wqkv[m][p, j, pl.ds(zrow[rc], DM // 2), :], bf16)
                        lhs = jnp.concatenate(
                            [pltpu.bitcast(xb[c, pl.ds(rc * RC // 2, RC // 2), :], bf16) for c in range(8)], axis=1)
                        res = jnp.dot(lhs, w, preferred_element_type=f32)
                        ring[j][m, p, pl.ds(QOFF + rc * RC, RC), :] = res.astype(bf16)
                        fence_w(res[:8])
                        fence_x(res[:8])
                assert fin_w()
            assert fin_x()
    with jax.named_scope("waitrest"):
        for cp in ocs + ucs + ccs + [xcp1]:
            cp.wait()

    ou = out_hbm.bitcast(u32)

    def outa_cp(row, n):
        return pltpu.make_async_copy(outs.at[pl.ds(row, n)], out_hbm.at[pl.ds(row, n), pl.ds(0, DM)], sem_out.at[0])

    def outb_cp(c, row, n, sem):
        col = DM + c * 128
        return pltpu.make_async_copy(
            outb.at[c, pl.ds(row, n)],
            ou.at[pl.ds(row, n), pl.ds(col if isinstance(col, int) else pl.multiple_of(col, 128), 128)],
            sem_out.at[sem])

    def one_step(i, odd, ppos, cpos, fwd, fence):
        s = 2 * i + odd
        lo_cur = lo_ref[odd]
        n_out = TOK if odd == 0 else 2 * SEG - TOK
        orow = pl.multiple_of(2 * SEG * i + odd * TOK, 8)
        h_ref[pl.ds(M, TOK), :] = xs[pl.ds(pl.multiple_of(TOK * s, 8), TOK), :]
        h = h_ref[...]
        mem_rows = {}
        scores = {}
        probs = {}

        ct = i >> 2
        r = s & 7
        buf = ct & 1
        cprev = (ct + NT - 1) & (NT - 1)

        def stage_a(j):
            for m in range(3):
                mm = []
                for p in range(2):
                    w = pltpu.bitcast(wqkv[m][p, j], bf16)
                    res = jnp.dot(h, w, preferred_element_type=f32)
                    ring[j][m, p, pl.ds(ppos, TOK), :] = res[M:].astype(bf16)
                    mm.append(res[:M])
                    fence(res[:M])
                mem_rows[m, j] = jnp.concatenate(mm, axis=0).astype(bf16)

        def gather(m, j):
            return jnp.concatenate([ring[j][m, 0, pl.ds(cpos, SEG), :], ring[j][m, 1, pl.ds(cpos, SEG), :],
                                    mem_rows[m, j]], axis=0)

        def stage_qk(j):
            scores[j] = lax.dot_general(gather(0, j), gather(1, j), (((1,), (1,)), ((), ())),
                                        preferred_element_type=f32)

        def stage_b(j):
            fl = fill_ref[...]
            sc = jnp.where(fl == 0.0, scores.pop(j) * (scale * LOG2E), fl)
            e = jnp.exp2(sc - jnp.max(sc, axis=-1, keepdims=True))
            den = jnp.sum(e, axis=-1, keepdims=True)
            probs[j] = (e * pl.reciprocal(den, approx=True)).astype(bf16)

        def stage_c(j):
            o = jnp.dot(probs[j], gather(2, j), preferred_element_type=f32)
            for p in range(2):
                hh = 2 * j + p
                ox = o[p * SEG:(p + 1) * SEG]
                lo_cur[hh, pl.ds(0, M), :] = o[2 * SEG + p * M:2 * SEG + (p + 1) * M].astype(bf16)
                if odd == 0:
                    lo_ref[0][hh, pl.ds(M, TOK), :] = ox[:TOK].astype(bf16)
                    lo_ref[1][hh, pl.ds(M, SEG - TOK), :] = ox[TOK:].astype(bf16)
                else:
                    lo_ref[1][hh, pl.ds(M + SEG - TOK, SEG), :] = ox.astype(bf16)

        acc = [None] * 8

        def stage_d(h0, h1, last=False):
            lhs = jnp.concatenate([lo_cur[hh] for hh in range(h0, h1)], axis=1)
            for c in range(8):
                w = pltpu.bitcast(wo[c, pl.ds(h0 * 64, (h1 - h0) * 64), :], bf16)
                res = jnp.dot(lhs, w, preferred_element_type=f32)
                acc[c] = res if acc[c] is None else acc[c] + res
                if not last:
                    fence(res[:M], (h1 - h0) / 8.0 * (DW_ODD if odd else 1.0))
                else:
                    rb = acc[c].astype(bf16)
                    h_ref[pl.ds(0, M), pl.ds(c * 128, 128)] = rb[:M]
                    outs[pl.ds(orow, n_out), pl.ds(c * 128, 128)] = rb[M:]

        def attn_group(jq, jc):
            for j in jq:
                stage_qk(j)
            for j in jc:
                stage_c(j)
            for j in jq:
                stage_b(j)

        for t in range(2):
            _inv_piece(cprev, 2 * r + t, 1 - buf, g_ref, us, vec, yf, outb)
        for p in fwd:
            p()
        for j in range(NP):
            stage_a(j)
            if j >= 2 and j % 2 == 0:
                attn_group((j - 2, j - 1), (j - 4, j - 3) if j >= 4 else ())
        stage_d(0, 8)
        attn_group((14, 15), (12, 13))
        stage_d(8, 20)
        attn_group((), (14, 15))
        stage_d(20, 28)
        stage_d(28, 32, last=True)

    def two_steps(i, carry):
        pp, cp = carry
        ct = i >> 2
        cprev = (ct + NT - 1) & (NT - 1)
        conv = [_conv_pieces(ct, (2 * i + odd) & 7, ct & 1, fs_ref, us, taps, vm, yf,
                             zrow[1] if DONE_M else None) for odd in range(2)]
        kgen = [_kgen_pieces((ct + 1) & (NT - 1), (2 * i + odd) & 7, par, vb, taps, ct + 1,
                             zrow[1] if DONE_K else None) for odd in range(2)]
        work = {'k0': (kgen[0], vb), 'k1': (kgen[1], vb), 'm0': (conv[0][1], vm), 'm1': (conv[1][1], vm)}
        fence = Pacer([work[k] + (t0, t1) for (k, t0, t1) in PLAN])
        for odd in range(2):
            one_step(i, odd, pl.multiple_of(pp + odd * TOK, 8), pl.multiple_of(cp + odd * SEG, 32),
                     conv[odd][0], fence)
        assert fence.finished()
        outa_cp(pl.multiple_of(2 * SEG * i, 2 * SEG), 2 * SEG).start()
        outb_cp(cprev, pl.multiple_of((i & 3) * 256, 256), 256, jnp.where(i < 4, 2, 1)).start()
        wrap = lambda v: jnp.where(v >= RING, v - RING, v)
        return wrap(pp + 2 * TOK), wrap(cp + 2 * SEG)

    with jax.named_scope("steps"):
        lax.fori_loop(0, NSEG // 2, two_steps, (jnp.int32(0), jnp.int32(QOFF)))

    with jax.named_scope("flush"):
        outb_cp(NT - 1, 0, L // 2, 2).wait()
        for b in range(NBLK):
            _inv_piece(NT - 1, b, (NT - 1) % 2, g_ref, us, vec, yf, outb)
            if b % 4 == 3:
                outb_cp(NT - 1, (b - 3) * 64, 256, 1).start()
    with jax.named_scope("waitout"):
        outa_cp(0, S).wait()
        pltpu.make_async_copy(outb, outb, sem_out.at[1]).wait()


@functools.partial(jax.jit, static_argnames=("A_seg_len",))
def pallas_concat_heads__memory_aug_recurrent_mem_tr__ssm_conv_s4__prompt_kernel(
    A_x, A_mem0, A_Wq, A_Wk, A_Wv, A_Wo, A_seg_len,
    B_u, B_A_re, B_A_im, B_B_re, B_B_im, B_C_re, B_C_im, B_log_dt, B_Dskip,
):
    assert A_seg_len == SEG and A_x.shape == (1, S, DM) and B_u.shape == (1, L, D)
    fs, g = _dft_consts()
    w4 = lambda w: w.reshape(DM // 2, 2, H, E)
    any_ = pl.BlockSpec(memory_space=pl.ANY)
    vmem = pl.BlockSpec(memory_space=pltpu.VMEM)
    V = pltpu.VMEM
    out = pl.pallas_call(
        _kernel,
        out_shape=jax.ShapeDtypeStruct((S, DM + D), bf16),
        in_specs=[pl.BlockSpec(memory_space=pltpu.SMEM), any_, vmem, any_, any_, any_, any_]
        + [any_] * 7 + [vmem, vmem, any_, any_],
        out_specs=any_,
        scratch_shapes=[
            V((2, NP, DM // 2, E), u32),
            V((2, NP, DM // 2, E), u32),
            V((2, NP, DM // 2, E), u32),
            V((8, H * E // 2, 128), u32),
            V((8, T0 // 2, 128), u32),
            V((S - T0, DM), bf16),
            V((M + TOK, DM), bf16),
            V((S, DM), bf16),
            V((2 * (SEG + M), 2 * (SEG + M)), f32),
            V((6, D, N), bf16),
            V((8 + NT * 6 * N, 128), f32),
            V((NT, L // 2, 128), u32),
            V((NT + 1, TAPROWS, 128), f32),
            V((V_ROWS, 128), f32),
            V((VM_ROWS, 128), f32),
            V((2, NBLK, 128, 128), u32),
            V((NT, L // 2, 128), u32),
            V((2, 8, 128), f32),
            V((8, NBLK * 32, 128), bf16),
            V((BLK, 256), bf16),
            pltpu.SemaphoreType.DMA((6 * NP,)),
            pltpu.SemaphoreType.DMA((8,)),
            pltpu.SemaphoreType.DMA((8,)),
            pltpu.SemaphoreType.DMA((1,)),
            pltpu.SemaphoreType.DMA((8,)),
            pltpu.SemaphoreType.DMA((NT,)),
            pltpu.SemaphoreType.DMA((3,)),
        ] + [V((3, 2, RING, E), bf16)] * NP + [V((H, M + TOK, E), bf16), V((H, M + 2 * SEG - TOK, E), bf16)],
        compiler_params=pltpu.CompilerParams(vmem_limit_bytes=110 * 1024 * 1024, disable_bounds_checks=True),
    )(jnp.asarray(np.zeros((8,), np.int32)), A_x.reshape(S, DM), A_mem0.reshape(M, DM), w4(A_Wq), w4(A_Wk), w4(A_Wv), A_Wo.reshape(H * E, DM),
      B_u.reshape(L, D), B_A_re, B_A_im, B_B_re, B_B_im, B_C_re, B_C_im,
      B_log_dt.reshape(8, 128), B_Dskip.reshape(8, 128),
      jnp.asarray(fs, bf16), jnp.asarray(g, bf16))
    return out.reshape(1, S, DM + D)
```

```python
import functools

import numpy as np
import jax
import jax.numpy as jnp
from jax import lax
import jax.experimental.pallas as pl
import jax.experimental.pallas.tpu as pltpu

bf16, f32, u32 = jnp.bfloat16, jnp.float32, jnp.uint32

S, DM, H, E, M, SEG = 2048, 1024, 32, 128, 8, 32
NSEG = S // SEG
TOK = 24
T0 = S - TOK * NSEG
RING = 576
QOFF = 64
NP = H // 2
LOG2E = 1.4426950408889634
QUICK = False
NOB = ''
BKNI = 1
UNP = 64
KHALF = True
UNP_FRAC = 0.7
BKSPLIT = 4
BPLAN = (6.0, 7.0, 41.5, 47.7)
BULK_FROM = 0
NITER = NSEG // 2
KNI = 2
KSPLIT = 2
PLAN = (('k0', 0, 96), ('m0', 96, 122), ('k1', 124, 220), ('m1', 220, 260))
DONE_K = True
DONE_M = True
DW_ODD = 1.5
RC = 64
MACJ = 6
NSLOT = 118
L, D, N = 2048, 1024, 128
BLK = 128
NBLK = L // BLK
NT = D // 128
TAPROWS = 656
WINDOWS = ((0, 128, 0, 1), (128, 128, 1, 1), (256, 128, 2, 1), (320, 80, 3, 1),
           (384, 128, 4, 3), (480, 48, 7, 1), (512, 128, 8, 7), (624, 32, 15, 1))

V_FENCE = 0
V_YTAB = 8
V_START = V_YTAB + 256
V_STEP = V_START + 160
V_ROWS = V_STEP + 128
V_UF = 8
V_KF = V_UF + NBLK * 32
VM_ROWS = V_KF + NBLK * 32


def _bf16_round_int(l):
    u = np.asarray(l, np.float32).view(np.uint32)
    r = (u + 0x7FFF + ((u >> 16) & 1)) & 0xFFFF0000
    return r.astype(np.uint32).view(np.float32).astype(np.int64)


def _tap_row(lp):
    return np.where(lp < 256, lp, np.where(lp < 512, 256 + (lp - 256) // 2,
                    np.where(lp < 1024, 384 + (lp - 512) // 4, 512 + (lp - 1024) // 8)))


@functools.lru_cache(maxsize=None)
def _dft_consts():
    t = np.arange(BLK)
    F = np.zeros((8, 32, BLK))
    G = np.zeros((BLK, 8, 32))
    for r in range(8):
        f = np.concatenate([16 * r + 2 * np.arange(8), 16 * r + 2 * np.arange(8) + 1])
        th = 2 * np.pi * (f + 0.5) / (2 * BLK)
        F[r, :16] = np.cos(th[:, None] * t[None])
        F[r, 16:] = -np.sin(th[:, None] * t[None])
        G[:, r, 0::2] = np.cos(th[None] * t[:, None]) / BLK
        G[:, r, 1::2] = -np.sin(th[None] * t[:, None]) / BLK
    FS = np.zeros((8, NBLK, 32, 128))
    for (w0, wn, b0, nb) in WINDOWS:
        for j in range(b0, b0 + nb):
            rows = _tap_row(_bf16_round_int(BLK * j + t)) - w0
            assert rows.min() >= 0 and rows.max() < wn
            sel = np.zeros((BLK, 128))
            sel[t, rows] = 1.0
            FS[:, j] = F @ sel
    return (FS.reshape(8, NBLK * 32, 128).astype(np.float32),
            G.reshape(BLK, 256).astype(np.float32))


def _cmul(a, b):
    return (a[0] * b[0] - a[1] * b[1], a[0] * b[1] + a[1] * b[0])


def _csq(a):
    return (a[0] * a[0] - a[1] * a[1], 2.0 * (a[0] * a[1]))


def _cexp(lr, li):
    k = jnp.floor(li * (2.0 / np.pi) + 0.5)
    r = ((li - k * 1.5703125) - k * 4.837512969970703125e-4) - k * 7.54978995489188216e-8
    r = jnp.clip(r, -0.8, 0.8)
    r2 = r * r
    s = r + r * r2 * (-1.6666654611e-1 + r2 * (8.3321608736e-3 + r2 * -1.9515295891e-4))
    c = (1.0 - 0.5 * r2) + (r2 * r2) * (4.166664568298827e-2
                                        + r2 * (-1.388731625493765e-3 + r2 * 2.443315711809948e-5))
    q = k.astype(jnp.int32)
    swap = (q & 1) == 1
    m = jnp.exp(lr)
    flip = lambda v, bit: pltpu.bitcast(pltpu.bitcast(v, jnp.int32) ^ (bit << 30), f32)
    return (flip(m * jnp.where(swap, s, c), (q + 1) & 2), flip(m * jnp.where(swap, c, s), q & 2))


def _par_row(c, k):
    return 8 + (c * 6 + k) * N


def _prep_pieces(praw, vec, par):
    def stage1(c):
        def fn():
            tr = lambda k: praw[k, pl.ds(c * 128, 128), :].astype(f32).T
            dt = jnp.exp(vec[0, pl.ds(c, 1), :]).astype(bf16).astype(f32)
            cc = _cmul((tr(4), tr(5)), (dt * tr(2), dt * tr(3)))
            for k, v in ((0, dt * tr(0)), (1, dt * tr(1)), (4, cc[0]), (5, cc[1])):
                par[pl.ds(_par_row(c, k), N), :] = v
        return fn

    def stage2(c, n0):
        def fn():
            lr = par[pl.ds(_par_row(c, 0) + n0, 16), :]
            li = par[pl.ds(_par_row(c, 1) + n0, 16), :]
            for k, v in enumerate(_cexp(lr, li) + _cexp(lr * 128.0, li * 128.0)):
                par[pl.ds(_par_row(c, k) + n0, 16), :] = v
        return fn

    tile = lambda c: [(260, stage1(c))] + [(190, stage2(c, n0)) for n0 in range(0, N, 16)]
    return tile(0), [pc for c in range(1, NT) for pc in tile(c)]


def _kgen_pieces(c, r, par, vb, taps, tslot, frow, kni, ksplit):
    st = {}

    def put(row, z, h=None):
        if h is None:
            vb[pl.ds(row, 16), :] = z[0]
            vb[pl.ds(row + 16, 16), :] = z[1]
        else:
            vb[pl.ds(row + 8 * h, 8), :] = z[0]
            vb[pl.ds(row + 16 + 8 * h, 8), :] = z[1]

    def get(row, h=None):
        if h is None:
            return (vb[pl.ds(row, 16), :], vb[pl.ds(row + 16, 16), :])
        return (vb[pl.ds(row + 8 * h, 8), :], vb[pl.ds(row + 16 + 8 * h, 8), :])

    def params(k):
        row = _par_row(c, k) + r * 16
        return par[pl.ds(row if isinstance(row, int) else pl.multiple_of(row, 8), 16), :]

    def park():
        put(V_STEP, (params(0), params(1)))
        put(V_START + 32, (params(2), params(3)))
        put(V_START, (params(4), params(5)))

    def setup_y(h):
        def fn():
            z1 = get(V_STEP, h)
            z2 = _csq(z1)
            z4 = _csq(z2)
            s = lax.broadcasted_iota(jnp.int32, (8, 128), 0)
            fs = [(jnp.where((s >> k) & 1 == 1, z[0], 1.0), jnp.where((s >> k) & 1 == 1, z[1], 0.0))
                  for k, z in enumerate((z1, z2, z4))]
            y = _cmul(_cmul(fs[0], fs[1]), fs[2])
            for k in range(8):
                put(V_YTAB + 32 * k, y, h)
                if k < 7:
                    y = _cmul(y, z1)
                    y = (jnp.where(s == 7 - k, 1.0, y[0]), jnp.where(s == 7 - k, 0.0, y[1]))
            z = z4
            for k in range(4):
                z = _csq(z)
                put(V_STEP + 32 * k, z, h)
        return fn

    def setup_hi():
        z = get(V_START + 32)
        cf = get(V_START)
        for g in range(1, 5):
            put(V_START + 32 * g, _cmul(cf, z))
            if g < 4:
                z = _csq(z)

    def square(k0, k1):
        def fn():
            for k in range(k0, k1):
                put(V_YTAB + 32 * k, _csq(get(V_YTAB + 32 * k)))
        return fn

    def rows_of(g, i0, ni):
        n_i = 16 + (g == 4)

        def fn():
            x = st.pop('x') if i0 > 0 else get(V_START + 32 * g)
            step = get(V_STEP + 32 * max(g - 1, 0))
            xs = []
            for t in range(ni):
                xs.append(x)
                if i0 + t + 1 < n_i:
                    x = _cmul(x, step)
            if i0 + ni < n_i:
                st['x'] = x
            acc = [None] * ni
            for k in range(8):
                yr, yi = get(V_YTAB + 32 * k)
                for t in range(ni):
                    v = xs[t][0] * yr - xs[t][1] * yi
                    v = v[:8] + v[8:]
                    if k:
                        v = pltpu.roll(v, k, 0)
                    acc[t] = v if acc[t] is None else acc[t] + v
                if frow is not None and k % ksplit == ksplit - 1 and k < 7:
                    vb[pl.ds(frow, 8), :] = acc[ni - 1]
            for t in range(ni):
                row = 128 * g + 8 * (i0 + t)
                a = acc[t]
                if row == 640:
                    a = jnp.where(lax.broadcasted_iota(jnp.int32, (8, 128), 0) == 0, a, 0.0)
                taps[tslot, pl.ds(row, 8), :] = taps[tslot, pl.ds(row, 8), :] + a
                if frow is not None and t == ni - 1:
                    vb[pl.ds(frow, 8), :] = a
        return fn

    pieces = [(30, park), (110, setup_y(0)), (110, setup_y(1)), (80, setup_hi)]
    for g in range(5):
        if g >= 2:
            pieces += [(40, square(0, 4)), (40, square(4, 8))]
        for i0 in range(0, 16 + (g == 4), kni):
            ni = min(kni, 16 + (g == 4) - i0)
            pieces.append((83 * ni, rows_of(g, i0, ni)))
    return pieces


def _conv_pieces(c, r, buf, fs_ref, us, taps, vb, yf, frow):
    st = {}

    def fwd_u(b0, b1):
        def fn():
            lhs = fs_ref[r, pl.ds(0, 32), :]
            for b in range(b0, b1):
                w = pltpu.bitcast(us[c, pl.ds(b * 64, 64), :], bf16)
                res = jnp.dot(lhs, w, preferred_element_type=f32)
                row = V_UF + 32 * b
                if b == 0:
                    vb[pl.ds(row, 32), :] = res
                else:
                    p = st['prev']
                    vb[pl.ds(row, 8), :] = res[0:8] - p[16:24]
                    vb[pl.ds(row + 8, 8), :] = res[8:16] + p[24:32]
                    vb[pl.ds(row + 16, 8), :] = res[16:24] + p[0:8]
                    vb[pl.ds(row + 24, 8), :] = res[24:32] - p[8:16]
                st['prev'] = res
        return fn

    def fwd_k(jobs):
        def fn():
            for (wi, t0, nb) in jobs:
                w0, wn, b0, _ = WINDOWS[wi]
                lhs = fs_ref[r, pl.ds((b0 + t0) * 32, nb * 32), pl.ds(0, wn)]
                w = taps[c, pl.ds(w0, wn), :].astype(bf16)
                vb[pl.ds(V_KF + 32 * (b0 + t0), 32 * nb), :] = jnp.dot(lhs, w, preferred_element_type=f32)
        return fn

    def mac(q, i0, ni, j0, j1):
        def fn():
            ld = lambda base, b: (vb[pl.ds(base + 32 * b + 8 * q, 8), :], vb[pl.ds(base + 32 * b + 16 + 8 * q, 8), :])
            zr, zi = st.pop('z') if j0 > 0 else ({}, {})
            ucache = {}
            for j in range(j0, j1):
                kr, ki = ld(V_KF, j)
                for i in range(max(i0, j), i0 + ni):
                    if i - j not in ucache:
                        ucache[i - j] = ld(V_UF, i - j)
                    ur, ui = ucache[i - j]
                    if i not in zr:
                        zr[i] = kr * ur - ki * ui
                        zi[i] = kr * ui + ki * ur
                    else:
                        zr[i] = zr[i] + kr * ur - ki * ui
                        zi[i] = zi[i] + kr * ui + ki * ur
            if frow is not None:
                vb[pl.ds(frow, 8), :] = zr[i0 + ni - 1]
            if j1 < i0 + ni:
                st['z'] = (zr, zi)
            else:
                row = pl.multiple_of(r * 16 + q * 8, 8)
                for i in range(i0, i0 + ni):
                    yf[buf, i, pl.ds(row, 8), :] = pltpu.pack_elementwise([zr[i], zi[i]], packed_dtype=bf16)
        return (8 * sum(1 for j in range(j0, j1) for i in range(max(i0, j), i0 + ni)), fn)

    fwd = [fwd_u(0, 8), fwd_u(8, 16), fwd_k(((0, 0, 1), (1, 0, 1), (2, 0, 1), (3, 0, 1))),
           fwd_k(((4, 0, 2), (6, 0, 2), (6, 2, 2), (6, 4, 2))), fwd_k(((4, 2, 1), (5, 0, 1), (6, 6, 1), (7, 0, 1)))]
    macs = []
    for q in range(2):
        for i0 in range(0, NBLK, 2):
            for j0 in range(0, i0 + 2, MACJ):
                macs.append(mac(q, i0, 2, j0, min(j0 + MACJ, i0 + 2)))
    return fwd, macs


def _inv_piece(c, b, buf, g_ref, us, vec, yf, outb):
    rows = pl.ds(pl.multiple_of(b * 64, 64), 64)
    w = pltpu.bitcast(yf[buf, b], bf16)
    y = jnp.dot(g_ref[...], w, preferred_element_type=f32)
    u = pltpu.bitcast(us[c, rows, :], bf16).astype(f32)
    sk = (u * vec[1, pl.ds(c, 1), :]).astype(bf16).astype(f32)
    o = (y.astype(bf16).astype(f32) + sk).astype(bf16)
    outb[c, rows, :] = pltpu.bitcast(o, u32)


def _attn_fill():
    n = 2 * (SEG + M)
    r = lax.broadcasted_iota(jnp.int32, (n, n), 0)
    c = lax.broadcasted_iota(jnp.int32, (n, n), 1)
    head = lambda i: jnp.where(i < 2 * SEG, i // SEG, (i - 2 * SEG) // M)
    same = head(r) == head(c)
    allowed = same & ((r >= 2 * SEG) | (c >= 2 * SEG) | (r >= c))
    return jnp.where(allowed, 0.0, jnp.where(same, -1e9 * LOG2E, -jnp.inf)).astype(f32)


def _kernel(zero_hbm, x_hbm, mem0_hbm, wq_hbm, wk_hbm, wv_hbm, wo_hbm,
            u_hbm, p0, p1, p2, p3, p4, p5, ldt_hbm, dsk_hbm, fs_hbm, g_hbm,
            out_hbm,
            wq, wk, wv, wo, xb, xs, h_ref, outs, fill_ref,
            praw, par, us, taps, vb, vm, vu, pacc, yf, outb, vec, vraw, fs_ref, g_ref, zero_ref,
            sem_s, sem_w, sem_o, sem_xb, sem_x, sem_p, sem_u, sem_out, *rings):
    wqkv = (wq, wk, wv)
    ring = rings[:NP]
    lo_ref = rings[NP:]
    scale = E ** -0.5

    whbm = [w.bitcast(u32) for w in (wq_hbm, wk_hbm, wv_hbm)]

    def wcp(j, m, p):
        return pltpu.make_async_copy(whbm[m].at[:, p, j, :], wqkv[m].at[p, j], sem_w.at[(j * 3 + m) * 2 + p])

    def start_w(j):
        for m in range(3):
            for p in range(2):
                wcp(j, m, p).start()

    xu = x_hbm.bitcast(u32)
    xcs = [pltpu.make_async_copy(xu.at[pl.ds(0, T0 // 2), pl.ds(c * 128, 128)], xb.at[c], sem_xb.at[c])
           for c in range(8)]
    xcp1 = pltpu.make_async_copy(x_hbm.at[pl.ds(T0, S - T0)], xs, sem_x.at[0])
    pcs = [pltpu.make_async_copy(p, praw.at[k], sem_p.at[k]) for k, p in enumerate((p0, p1, p2, p3, p4, p5))]
    ccs = [pltpu.make_async_copy(fs_hbm, fs_ref, sem_p.at[6]), pltpu.make_async_copy(g_hbm, g_ref, sem_p.at[7])]
    wou = wo_hbm.bitcast(u32)
    ocs = [pltpu.make_async_copy(wou.at[:, pl.ds(c * 128, 128)], wo.at[c], sem_o.at[c]) for c in range(8)]
    uu = u_hbm.bitcast(u32)
    ucs = [pltpu.make_async_copy(uu.at[:, pl.ds(c * 128, 128)], us.at[c], sem_u.at[c]) for c in range(NT)]

    zcp = pltpu.make_async_copy(zero_hbm, zero_ref, sem_s.at[0])
    scs = [pltpu.make_async_copy(mem0_hbm, h_ref.at[pl.ds(0, M)], sem_s.at[1]),
           pltpu.make_async_copy(ldt_hbm, vraw.at[0], sem_s.at[2]),
           pltpu.make_async_copy(dsk_hbm, vraw.at[1], sem_s.at[3])]
    for cp in [zcp] + xcs + [wcp(0, 0, 0), wcp(0, 0, 1)]:
        cp.start()
    vu[pl.ds(8, 8), :] = pltpu.bitcast(jnp.full((8, 128), 0x0000FFFF, u32), f32)
    vu[pl.ds(16, 8), :] = pltpu.bitcast(jnp.full((8, 128), 0xFFFF0000, u32), f32)
    taps[...] = jnp.zeros(taps.shape, f32)
    yf[1] = jnp.zeros(yf.shape[1:], u32)
    fill_ref[...] = _attn_fill()
    for cp in [wcp(0, 1, 0), wcp(0, 1, 1)] + scs:
        cp.start()
    zcp.wait()

    frow = pl.multiple_of(zero_ref[0] * 8, 8)
    zrow = [pl.multiple_of(zero_ref[k] * 8, 8) for k in range(T0 // RC)]

    class Pacer:
        def __init__(self, segments):
            self.t = 0.0
            self.todo = []
            for (pieces, buf, t0, t1) in segments:
                total = float(sum(c for c, _ in pieces))
                done = 0.0
                for (cst, fn) in pieces:
                    self.todo.append((t0 + (t1 - t0) * done / total, fn, buf))
                    done += cst

        def __call__(self, v, dt=1.0):
            self.t += dt
            fenced = []
            while self.todo and self.todo[0][0] < self.t:
                _, fn, buf = self.todo.pop(0)
                if not any(b is buf for b in fenced):
                    buf[pl.ds(frow, 8), :] = v
                    fenced.append(buf)
                fn()

        def finished(self):
            return not self.todo

    def make_fence(vpu, nslot, buf=vb):
        pc = Pacer([(vpu, buf, 0.0, float(nslot))])
        return pc, pc.finished

    def unpair(j, m, r0, nr):
        def fn():
            rows = pl.ds(r0, nr)
            m_lo = jnp.tile(pltpu.bitcast(vu[pl.ds(8, 8), :], u32), (nr // 8, 1))
            m_hi = jnp.tile(pltpu.bitcast(vu[pl.ds(16, 8), :], u32), (nr // 8, 1))
            a = wqkv[m][0, j, rows, :]
            b = wqkv[m][1, j, rows, :]
            wqkv[m][0, j, rows, :] = (a & m_lo) | ((b & m_lo) << 16)
            wqkv[m][1, j, rows, :] = ((a & m_hi) >> 16) | (b & m_hi)
        return (nr, fn)

    def unpair_pieces(items):
        return [unpair(j, m, r0, UNP) for (j, m) in items for r0 in range(0, DM // 2, UNP)]

    items = [(j, m) for j in range(NP) for m in range(3)]
    wcs = lambda lo, hi: [wcp(j, m, p) for (j, m) in items[lo:hi] for p in range(2)]
    plan = {
        0: ((1, 2), wcs(2, 4), []),
        1: ((2, 4), wcs(4, 7), []),
        3: ((4, 7), pcs + wcs(7, 12), []),
        6: ((7, 12), wcs(12, 21), pcs + scs),
        11: ((12, 21), wcs(21, 33), []),
        20: ((21, 33), wcs(33, 48) + ocs[:4], []),
        32: ((33, 48), ocs[4:] + ucs + [xcp1] + ccs, []),
    }
    with jax.named_scope("bulk"):
        with jax.named_scope("waitx"):
            for cp in xcs + wcs(0, 1):
                cp.wait()
        for _, fn in unpair_pieces(items[0:1]):
            fn()
        points = sorted(plan) + [len(items)]
        if QUICK in (1, 2):
            for cp in wcs(2, 48) + pcs + ocs + ucs + [xcp1] + ccs:
                cp.start()
            for cp in wcs(1, 48) + pcs + scs:
                cp.wait()
            vec[...] = vraw[...].astype(f32)
            for _, fn in (unpair_pieces(items[1:]) + sum(_prep_pieces(praw, vec, par), [])) if QUICK != 2 else []:
                fn()

            def kg(r, carry):
                for _, fn in _kgen_pieces(0, r, par, vb, taps, 0, zrow[1], BKNI, BKSPLIT):
                    fn()
                return carry
            lax.fori_loop(0, 8, kg, 0)
            for (j, m) in (items if QUICK != 2 else []):
                def chunk(rc, carry, j=j, m=m):
                    for p in range(2):
                        lhs = jnp.concatenate(
                            [pltpu.bitcast(xb[c, pl.ds(pl.multiple_of(rc * 32, 32), 32), :], bf16) for c in range(8)], axis=1)
                        ring[j][m, p, pl.ds(pl.multiple_of(QOFF + rc * 64, 64), 64), :] = jnp.dot(
                            lhs, pltpu.bitcast(wqkv[m][p, j], bf16), preferred_element_type=f32).astype(bf16)
                    return carry
                lax.fori_loop(0, 8, chunk, 0)
            points = []
        n_chunk = 2 * (T0 // RC)
        prep = _prep_pieces(praw, vec, par)
        kg0 = [pc for r in range(8) for pc in _kgen_pieces(0, r, par, vb, taps, 0, zrow[1], BKNI, BKSPLIT)]
        t_a, t_b, t_c, t_d = [v * n_chunk for v in BPLAN]
        fence_x = Pacer([(prep[0], par, t_a, t_b), (kg0, vb, t_b, t_c), (prep[1], par, t_c, t_d)])
        fence_x.t = float(BULK_FROM * n_chunk)
        for g in range(len(points) - 1):
            lo, hi = points[g], points[g + 1]
            (w_lo, w_hi), starts, waits = plan[lo]
            for cp in starts:
                cp.start()
            with jax.named_scope("wait%d" % lo):
                for cp in wcs(w_lo, w_hi) + waits:
                    cp.wait()
            assert w_hi == min(hi + 1, len(items))
            if lo == 6:
                vec[...] = vraw[...].astype(f32)
            if lo < BULK_FROM:
                continue
            for it in range(lo, hi):
                j, m = items[it]
                fence_w, fin_w = make_fence(unpair_pieces(items[it + 1:it + 2]), n_chunk * UNP_FRAC, vu)
                for p in range(2):
                    if KHALF:
                        for half in range(2):
                            w = pltpu.bitcast(wqkv[m][p, j, pl.ds(half * (DM // 4), DM // 4), :], bf16)
                            lhs = jnp.concatenate(
                                [pltpu.bitcast(xb[c], bf16) for c in range(4 * half, 4 * half + 4)], axis=1)
                            res = jnp.dot(lhs, w, preferred_element_type=f32)
                            for rc in range(T0 // RC):
                                v = res[rc * RC:(rc + 1) * RC]
                                if half == 0:
                                    pacc[pl.ds(rc * RC, RC), :] = v
                                else:
                                    v = v + pacc[pl.ds(rc * RC, RC), :]
                                    ring[j][m, p, pl.ds(QOFF + rc * RC, RC), :] = v.astype(bf16)
                                fence_w(v[:8], 0.5)
                                fence_x(v[:8], 0.5)
                        continue
                    for rc in range(T0 // RC):
                        w = pltpu.bitcast(wqkv[m][p, j, pl.ds(zrow[rc], DM // 2), :], bf16)
                        lhs = jnp.concatenate(
                            [pltpu.bitcast(xb[c, pl.ds(rc * RC // 2, RC // 2), :], bf16) for c in range(8)], axis=1)
                        res = jnp.dot(lhs, w, preferred_element_type=f32)
                        ring[j][m, p, pl.ds(QOFF + rc * RC, RC), :] = res.astype(bf16)
                        fence_w(res[:8])
                        fence_x(res[:8])
                assert fin_w()
        assert QUICK or BULK_FROM or fence_x.finished()
    with jax.named_scope("waitrest"):
        for cp in ocs + ucs + ccs + [xcp1]:
            cp.wait()

    ou = out_hbm.bitcast(u32)

    def outa_cp(row, n):
        return pltpu.make_async_copy(outs.at[pl.ds(row, n)], out_hbm.at[pl.ds(row, n), pl.ds(0, DM)], sem_out.at[0])

    def outb_cp(c, row, n, sem):
        col = DM + c * 128
        return pltpu.make_async_copy(
            outb.at[c, pl.ds(row, n)],
            ou.at[pl.ds(row, n), pl.ds(col if isinstance(col, int) else pl.multiple_of(col, 128), 128)],
            sem_out.at[sem])

    def one_step(i, odd, ppos, cpos, fwd, fence):
        s = 2 * i + odd
        lo_cur = lo_ref[odd]
        n_out = TOK if odd == 0 else 2 * SEG - TOK
        orow = pl.multiple_of(2 * SEG * i + odd * TOK, 8)
        h_ref[pl.ds(M, TOK), :] = xs[pl.ds(pl.multiple_of(TOK * s, 8), TOK), :]
        h = h_ref[...]
        mem_rows = {}
        scores = {}
        probs = {}

        ct = i >> 2
        r = s & 7
        buf = ct & 1
        cprev = (ct + NT - 1) & (NT - 1)

        def stage_a(j):
            for m in range(3):
                mm = []
                for p in range(2):
                    w = pltpu.bitcast(wqkv[m][p, j], bf16)
                    res = jnp.dot(h, w, preferred_element_type=f32)
                    ring[j][m, p, pl.ds(ppos, TOK), :] = res[M:].astype(bf16)
                    mm.append(res[:M])
                    fence(res[:M])
                mem_rows[m, j] = jnp.concatenate(mm, axis=0).astype(bf16)

        def gather(m, j):
            return jnp.concatenate([ring[j][m, 0, pl.ds(cpos, SEG), :], ring[j][m, 1, pl.ds(cpos, SEG), :],
                                    mem_rows[m, j]], axis=0)

        def stage_qk(j):
            scores[j] = lax.dot_general(gather(0, j), gather(1, j), (((1,), (1,)), ((), ())),
                                        preferred_element_type=f32)

        def stage_b(j):
            fl = fill_ref[...]
            sc = jnp.where(fl == 0.0, scores.pop(j) * (scale * LOG2E), fl)
            e = jnp.exp2(sc - jnp.max(sc, axis=-1, keepdims=True))
            den = jnp.sum(e, axis=-1, keepdims=True)
            probs[j] = (e * pl.reciprocal(den, approx=True)).astype(bf16)

        def stage_c(j):
            o = jnp.dot(probs[j], gather(2, j), preferred_element_type=f32)
            for p in range(2):
                hh = 2 * j + p
                ox = o[p * SEG:(p + 1) * SEG]
                lo_cur[hh, pl.ds(0, M), :] = o[2 * SEG + p * M:2 * SEG + (p + 1) * M].astype(bf16)
                if odd == 0:
                    lo_ref[0][hh, pl.ds(M, TOK), :] = ox[:TOK].astype(bf16)
                    lo_ref[1][hh, pl.ds(M, SEG - TOK), :] = ox[TOK:].astype(bf16)
                else:
                    lo_ref[1][hh, pl.ds(M + SEG - TOK, SEG), :] = ox.astype(bf16)

        acc = [None] * 8

        def stage_d(h0, h1, last=False):
            lhs = jnp.concatenate([lo_cur[hh] for hh in range(h0, h1)], axis=1)
            for c in range(8):
                w = pltpu.bitcast(wo[c, pl.ds(h0 * 64, (h1 - h0) * 64), :], bf16)
                res = jnp.dot(lhs, w, preferred_element_type=f32)
                acc[c] = res if acc[c] is None else acc[c] + res
                if not last:
                    fence(res[:M], (h1 - h0) / 8.0 * (DW_ODD if odd else 1.0))
                else:
                    rb = acc[c].astype(bf16)
                    h_ref[pl.ds(0, M), pl.ds(c * 128, 128)] = rb[:M]
                    outs[pl.ds(orow, n_out), pl.ds(c * 128, 128)] = rb[M:]

        def attn_group(jq, jc):
            for j in jq:
                stage_qk(j)
            for j in jc:
                stage_c(j)
            for j in jq:
                stage_b(j)

        for t in range(2):
            _inv_piece(cprev, 2 * r + t, 1 - buf, g_ref, us, vec, yf, outb)
        for p in fwd:
            p()
        for j in range(NP):
            stage_a(j)
            if j >= 2 and j % 2 == 0:
                attn_group((j - 2, j - 1), (j - 4, j - 3) if j >= 4 else ())
        stage_d(0, 8)
        attn_group((14, 15), (12, 13))
        stage_d(8, 20)
        attn_group((), (14, 15))
        stage_d(20, 28)
        stage_d(28, 32, last=True)

    def two_steps(i, carry):
        pp, cp = carry
        ct = i >> 2
        cprev = (ct + NT - 1) & (NT - 1)
        conv = [_conv_pieces(ct, (2 * i + odd) & 7, ct & 1, fs_ref, us, taps, vm, yf,
                             zrow[1] if DONE_M else None) for odd in range(2)]
        kgen = [_kgen_pieces((ct + 1) & (NT - 1), (2 * i + odd) & 7, par, vb, taps, ct + 1,
                             zrow[1] if DONE_K else None, KNI, KSPLIT) for odd in range(2)]
        work = {'k0': (kgen[0], vb), 'k1': (kgen[1], vb), 'm0': (conv[0][1], vm), 'm1': (conv[1][1], vm)}
        fence = Pacer([work[k] + (t0, t1) for (k, t0, t1) in PLAN if k[0] not in NOB])
        for odd in range(2):
            one_step(i, odd, pl.multiple_of(pp + odd * TOK, 8), pl.multiple_of(cp + odd * SEG, 32),
                     conv[odd][0], fence)
        assert fence.finished() or NOB
        outa_cp(pl.multiple_of(2 * SEG * i, 2 * SEG), 2 * SEG).start()
        outb_cp(cprev, pl.multiple_of((i & 3) * 256, 256), 256, jnp.where(i < 4, 2, 1)).start()
        wrap = lambda v: jnp.where(v >= RING, v - RING, v)
        return wrap(pp + 2 * TOK), wrap(cp + 2 * SEG)

    with jax.named_scope("steps"):
        if NITER:
            lax.fori_loop(0, NITER, two_steps, (jnp.int32(0), jnp.int32(QOFF)))

    with jax.named_scope("flush"):
        outb_cp(NT - 1, 0, L // 2, 2).wait()
        for b in range(NBLK):
            _inv_piece(NT - 1, b, (NT - 1) % 2, g_ref, us, vec, yf, outb)
            if b % 4 == 3:
                outb_cp(NT - 1, (b - 3) * 64, 256, 1).start()
    with jax.named_scope("waitout"):
        outa_cp(0, S).wait()
        pltpu.make_async_copy(outb, outb, sem_out.at[1]).wait()


@functools.partial(jax.jit, static_argnames=("A_seg_len",))
def pallas_concat_heads__memory_aug_recurrent_mem_tr__ssm_conv_s4__prompt_kernel(
    A_x, A_mem0, A_Wq, A_Wk, A_Wv, A_Wo, A_seg_len,
    B_u, B_A_re, B_A_im, B_B_re, B_B_im, B_C_re, B_C_im, B_log_dt, B_Dskip,
):
    assert A_seg_len == SEG and A_x.shape == (1, S, DM) and B_u.shape == (1, L, D)
    fs, g = _dft_consts()
    w4 = lambda w: w.reshape(DM // 2, 2, H, E)
    any_ = pl.BlockSpec(memory_space=pl.ANY)
    V = pltpu.VMEM
    out = pl.pallas_call(
        _kernel,
        out_shape=jax.ShapeDtypeStruct((S, DM + D), bf16),
        in_specs=[any_] * 18,
        out_specs=any_,
        scratch_shapes=[
            V((2, NP, DM // 2, E), u32),
            V((2, NP, DM // 2, E), u32),
            V((2, NP, DM // 2, E), u32),
            V((8, H * E // 2, 128), u32),
            V((8, T0 // 2, 128), u32),
            V((S - T0, DM), bf16),
            V((M + TOK, DM), bf16),
            V((S, DM), bf16),
            V((2 * (SEG + M), 2 * (SEG + M)), f32),
            V((6, D, N), bf16),
            V((8 + NT * 6 * N, 128), f32),
            V((NT, L // 2, 128), u32),
            V((NT + 1, TAPROWS, 128), f32),
            V((V_ROWS, 128), f32),
            V((VM_ROWS, 128), f32),
            V((24, 128), f32),
            V((T0, 128), f32),
            V((2, NBLK, 128, 128), u32),
            V((NT, L // 2, 128), u32),
            V((2, 8, 128), f32),
            V((2, 8, 128), bf16),
            V((8, NBLK * 32, 128), bf16),
            V((BLK, 256), bf16),
            pltpu.SMEM((8,), jnp.int32),
            pltpu.SemaphoreType.DMA((4,)),
            pltpu.SemaphoreType.DMA((6 * NP,)),
            pltpu.SemaphoreType.DMA((8,)),
            pltpu.SemaphoreType.DMA((8,)),
            pltpu.SemaphoreType.DMA((1,)),
            pltpu.SemaphoreType.DMA((8,)),
            pltpu.SemaphoreType.DMA((NT,)),
            pltpu.SemaphoreType.DMA((3,)),
        ] + [V((3, 2, RING, E), bf16)] * NP + [V((H, M + TOK, E), bf16), V((H, M + 2 * SEG - TOK, E), bf16)],
        compiler_params=pltpu.CompilerParams(vmem_limit_bytes=110 * 1024 * 1024, disable_bounds_checks=True),
    )(jnp.asarray(np.zeros((8,), np.int32)), A_x.reshape(S, DM), A_mem0.reshape(M, DM), w4(A_Wq), w4(A_Wk), w4(A_Wv), A_Wo.reshape(H * E, DM),
      B_u.reshape(L, D), B_A_re, B_A_im, B_B_re, B_B_im, B_C_re, B_C_im,
      B_log_dt.reshape(8, 128), B_Dskip.reshape(8, 128),
      jnp.asarray(fs, bf16), jnp.asarray(g, bf16))
    return out.reshape(1, S, DM + D)
```

```python
import functools

import numpy as np
import jax
import jax.numpy as jnp
from jax import lax
import jax.experimental.pallas as pl
import jax.experimental.pallas.tpu as pltpu

bf16, f32, u32 = jnp.bfloat16, jnp.float32, jnp.uint32

S, DM, H, E, M, SEG = 2048, 1024, 32, 128, 8, 32
NSEG = S // SEG
TOK = 24
T0 = S - TOK * NSEG
RING = 576
QOFF = 64
NP = H // 2
LOG2E = 1.4426950408889634
QUICK = False
NOB = ''
BKNI = 1
UNP = 64
KHALF = True
UNP_FRAC = 0.7
BKSPLIT = 4
BPLAN = (6.0, 7.0, 41.5, 47.7)
BULK_FROM = 0
NITER = NSEG // 2
KNI = 2
KSPLIT = 2
PLAN = (('k0', 0, 96), ('m0', 96, 122), ('k1', 124, 220), ('m1', 220, 260))
DONE_K = True
DONE_M = True
DW_ODD = 1.5
RC = 64
MACJ = 6
NSLOT = 118
L, D, N = 2048, 1024, 128
BLK = 128
NBLK = L // BLK
NT = D // 128
TAPROWS = 672
WINDOWS = ((0, 128, 0, 1), (128, 128, 1, 1), (256, 128, 2, 1), (320, 80, 3, 1),
           (384, 128, 4, 3), (480, 48, 7, 1), (512, 128, 8, 7), (624, 32, 15, 1))

V_FENCE = 0
V_YTAB = 8
V_START = V_YTAB + 256
V_STEP = V_START + 160
V_ROWS = V_STEP + 128
V_UF = 8
V_KF = V_UF + NBLK * 32
VM_ROWS = V_KF + NBLK * 32


def _bf16_round_int(l):
    u = np.asarray(l, np.float32).view(np.uint32)
    r = (u + 0x7FFF + ((u >> 16) & 1)) & 0xFFFF0000
    return r.astype(np.uint32).view(np.float32).astype(np.int64)


def _tap_row(lp):
    return np.where(lp < 256, lp, np.where(lp < 512, 256 + (lp - 256) // 2,
                    np.where(lp < 1024, 384 + (lp - 512) // 4, 512 + (lp - 1024) // 8)))


@functools.lru_cache(maxsize=None)
def _dft_consts():
    t = np.arange(BLK)
    F = np.zeros((8, 32, BLK))
    G = np.zeros((BLK, 8, 32))
    for r in range(8):
        f = np.concatenate([16 * r + 2 * np.arange(8), 16 * r + 2 * np.arange(8) + 1])
        th = 2 * np.pi * (f + 0.5) / (2 * BLK)
        F[r, :16] = np.cos(th[:, None] * t[None])
        F[r, 16:] = -np.sin(th[:, None] * t[None])
        G[:, r, 0::2] = np.cos(th[None] * t[:, None]) / BLK
        G[:, r, 1::2] = -np.sin(th[None] * t[:, None]) / BLK
    FS = np.zeros((8, NBLK, 32, 128))
    for (w0, wn, b0, nb) in WINDOWS:
        for j in range(b0, b0 + nb):
            rows = _tap_row(_bf16_round_int(BLK * j + t)) - w0
            assert rows.min() >= 0 and rows.max() < wn
            sel = np.zeros((BLK, 128))
            sel[t, rows] = 1.0
            FS[:, j] = F @ sel
    return (FS.reshape(8, NBLK * 32, 128).astype(np.float32),
            G.reshape(BLK, 256).astype(np.float32))


def _cmul(a, b):
    return (a[0] * b[0] - a[1] * b[1], a[0] * b[1] + a[1] * b[0])


def _csq(a):
    return (a[0] * a[0] - a[1] * a[1], 2.0 * (a[0] * a[1]))


def _cexp(lr, li):
    k = jnp.floor(li * (2.0 / np.pi) + 0.5)
    r = ((li - k * 1.5703125) - k * 4.837512969970703125e-4) - k * 7.54978995489188216e-8
    r = jnp.clip(r, -0.8, 0.8)
    r2 = r * r
    s = r + r * r2 * (-1.6666654611e-1 + r2 * (8.3321608736e-3 + r2 * -1.9515295891e-4))
    c = (1.0 - 0.5 * r2) + (r2 * r2) * (4.166664568298827e-2
                                        + r2 * (-1.388731625493765e-3 + r2 * 2.443315711809948e-5))
    q = k.astype(jnp.int32)
    swap = (q & 1) == 1
    m = jnp.exp(lr)
    flip = lambda v, bit: pltpu.bitcast(pltpu.bitcast(v, jnp.int32) ^ (bit << 30), f32)
    return (flip(m * jnp.where(swap, s, c), (q + 1) & 2), flip(m * jnp.where(swap, c, s), q & 2))


def _par_row(c, k):
    return 8 + (c * 6 + k) * N


def _prep_pieces(praw, vec, par):
    def stage1(c):
        def fn():
            tr = lambda k: praw[k, pl.ds(c * 128, 128), :].astype(f32).T
            dt = jnp.exp(vec[0, pl.ds(c, 1), :]).astype(bf16).astype(f32)
            cc = _cmul((tr(4), tr(5)), (dt * tr(2), dt * tr(3)))
            for k, v in ((0, dt * tr(0)), (1, dt * tr(1)), (4, cc[0]), (5, cc[1])):
                par[pl.ds(_par_row(c, k), N), :] = v
        return fn

    def stage2(c, n0):
        def fn():
            lr = par[pl.ds(_par_row(c, 0) + n0, 16), :]
            li = par[pl.ds(_par_row(c, 1) + n0, 16), :]
            for k, v in enumerate(_cexp(lr, li) + _cexp(lr * 128.0, li * 128.0)):
                par[pl.ds(_par_row(c, k) + n0, 16), :] = v
        return fn

    tile = lambda c: [(260, stage1(c))] + [(190, stage2(c, n0)) for n0 in range(0, N, 16)]
    return tile(0), [pc for c in range(1, NT) for pc in tile(c)]


def _kgen_pieces(c, r, par, vb, taps, tslot, frow, kni, ksplit):
    st = {}

    def put(row, z, h=None):
        if h is None:
            vb[pl.ds(row, 16), :] = z[0]
            vb[pl.ds(row + 16, 16), :] = z[1]
        else:
            vb[pl.ds(row + 8 * h, 8), :] = z[0]
            vb[pl.ds(row + 16 + 8 * h, 8), :] = z[1]

    def get(row, h=None):
        if h is None:
            return (vb[pl.ds(row, 16), :], vb[pl.ds(row + 16, 16), :])
        return (vb[pl.ds(row + 8 * h, 8), :], vb[pl.ds(row + 16 + 8 * h, 8), :])

    def params(k):
        if isinstance(r, int):
            return par[pl.ds(_par_row(c, k) + r * 16, 16), :]
        return par[pl.ds(pl.multiple_of(c * (6 * N) + r[0] * 32, 32) + (_par_row(0, k) + r[1] * 16), 16), :]

    def park():
        put(V_STEP, (params(0), params(1)))
        put(V_START + 32, (params(2), params(3)))
        put(V_START, (params(4), params(5)))

    def setup_y(h):
        def fn():
            z1 = get(V_STEP, h)
            z2 = _csq(z1)
            z4 = _csq(z2)
            s = lax.broadcasted_iota(jnp.int32, (8, 128), 0)
            fs = [(jnp.where((s >> k) & 1 == 1, z[0], 1.0), jnp.where((s >> k) & 1 == 1, z[1], 0.0))
                  for k, z in enumerate((z1, z2, z4))]
            y = _cmul(_cmul(fs[0], fs[1]), fs[2])
            for k in range(8):
                put(V_YTAB + 32 * k, y, h)
                if k < 7:
                    y = _cmul(y, z1)
                    y = (jnp.where(s == 7 - k, 1.0, y[0]), jnp.where(s == 7 - k, 0.0, y[1]))
            z = z4
            for k in range(4):
                z = _csq(z)
                put(V_STEP + 32 * k, z, h)
        return fn

    def setup_hi():
        z = get(V_START + 32)
        cf = get(V_START)
        for g in range(1, 5):
            put(V_START + 32 * g, _cmul(cf, z))
            if g < 4:
                z = _csq(z)

    def square(k0, k1):
        def fn():
            for k in range(k0, k1):
                put(V_YTAB + 32 * k, _csq(get(V_YTAB + 32 * k)))
        return fn

    def rows_of(g, i0, ni):
        n_i = 16 + (g == 4)

        def fn():
            x = st.pop('x') if i0 > 0 else get(V_START + 32 * g)
            step = get(V_STEP + 32 * max(g - 1, 0))
            xs = []
            for t in range(ni):
                xs.append(x)
                if i0 + t + 1 < n_i:
                    x = _cmul(x, step)
            if i0 + ni < n_i:
                st['x'] = x
            acc = [None] * ni
            for k in range(8):
                yr, yi = get(V_YTAB + 32 * k)
                for t in range(ni):
                    v = xs[t][0] * yr - xs[t][1] * yi
                    v = v[:8] + v[8:]
                    if k:
                        v = pltpu.roll(v, k, 0)
                    acc[t] = v if acc[t] is None else acc[t] + v
                if frow is not None and k % ksplit == ksplit - 1 and k < 7:
                    vb[pl.ds(frow, 8), :] = acc[ni - 1]
            for t in range(ni):
                row = 128 * g + 8 * (i0 + t)
                a = acc[t]
                if row == 640:
                    a = jnp.where(lax.broadcasted_iota(jnp.int32, (8, 128), 0) == 0, a, 0.0)
                taps[tslot, pl.ds(row, 8), :] = taps[tslot, pl.ds(row, 8), :] + a
                if frow is not None and t == ni - 1:
                    vb[pl.ds(frow, 8), :] = a
        return fn

    pieces = [(30, park), (110, setup_y(0)), (110, setup_y(1)), (80, setup_hi)]
    for g in range(5):
        if g >= 2:
            pieces += [(40, square(0, 4)), (40, square(4, 8))]
        for i0 in range(0, 16 + (g == 4), kni):
            ni = min(kni, 16 + (g == 4) - i0)
            pieces.append((83 * ni, rows_of(g, i0, ni)))
    return pieces


def _conv_pieces(c, r, buf, fs_ref, us, taps, vb, yf, frow):
    st = {}

    def fwd_u(b0, b1):
        def fn():
            lhs = fs_ref[2 * r[0] + r[1], pl.ds(0, 32), :]
            for b in range(b0, b1):
                w = pltpu.bitcast(us[c, pl.ds(b * 64, 64), :], bf16)
                res = jnp.dot(lhs, w, preferred_element_type=f32)
                row = V_UF + 32 * b
                if b == 0:
                    vb[pl.ds(row, 32), :] = res
                else:
                    p = st['prev']
                    vb[pl.ds(row, 8), :] = res[0:8] - p[16:24]
                    vb[pl.ds(row + 8, 8), :] = res[8:16] + p[24:32]
                    vb[pl.ds(row + 16, 8), :] = res[16:24] + p[0:8]
                    vb[pl.ds(row + 24, 8), :] = res[24:32] - p[8:16]
                st['prev'] = res
        return fn

    def fwd_k(jobs):
        def fn():
            for (wi, t0, nb) in jobs:
                w0, wn, b0, _ = WINDOWS[wi]
                lhs = fs_ref[2 * r[0] + r[1], pl.ds((b0 + t0) * 32, nb * 32), pl.ds(0, wn)]
                w = taps[c, pl.ds(w0, wn), :].astype(bf16)
                vb[pl.ds(V_KF + 32 * (b0 + t0), 32 * nb), :] = jnp.dot(lhs, w, preferred_element_type=f32)
        return fn

    def mac(q, i0, ni, j0, j1):
        def fn():
            ld = lambda base, b: (vb[pl.ds(base + 32 * b + 8 * q, 8), :], vb[pl.ds(base + 32 * b + 16 + 8 * q, 8), :])
            zr, zi = st.pop('z') if j0 > 0 else ({}, {})
            ucache = {}
            for j in range(j0, j1):
                kr, ki = ld(V_KF, j)
                for i in range(max(i0, j), i0 + ni):
                    if i - j not in ucache:
                        ucache[i - j] = ld(V_UF, i - j)
                    ur, ui = ucache[i - j]
                    if i not in zr:
                        zr[i] = kr * ur - ki * ui
                        zi[i] = kr * ui + ki * ur
                    else:
                        zr[i] = zr[i] + kr * ur - ki * ui
                        zi[i] = zi[i] + kr * ui + ki * ur
            if frow is not None:
                vb[pl.ds(frow, 8), :] = zr[i0 + ni - 1]
            if j1 < i0 + ni:
                st['z'] = (zr, zi)
            else:
                row = pl.multiple_of(r[0] * 32, 32) + (r[1] * 16 + q * 8)
                for i in range(i0, i0 + ni):
                    yf[buf, i, pl.ds(row, 8), :] = pltpu.pack_elementwise([zr[i], zi[i]], packed_dtype=bf16)
        return (8 * sum(1 for j in range(j0, j1) for i in range(max(i0, j), i0 + ni)), fn)

    fwd = [fwd_u(0, 8), fwd_u(8, 16), fwd_k(((0, 0, 1), (1, 0, 1), (2, 0, 1), (3, 0, 1))),
           fwd_k(((4, 0, 2), (6, 0, 2), (6, 2, 2), (6, 4, 2))), fwd_k(((4, 2, 1), (5, 0, 1), (6, 6, 1), (7, 0, 1)))]
    macs = []
    for q in range(2):
        for i0 in range(0, NBLK, 2):
            for j0 in range(0, i0 + 2, MACJ):
                macs.append(mac(q, i0, 2, j0, min(j0 + MACJ, i0 + 2)))
    return fwd, macs


def _inv_piece(c, b, buf, g_ref, us, vec, yf, outb):
    rows = pl.ds(pl.multiple_of(b * 64, 64), 64)
    w = pltpu.bitcast(yf[buf, b], bf16)
    y = jnp.dot(g_ref[...], w, preferred_element_type=f32)
    u = pltpu.bitcast(us[c, rows, :], bf16).astype(f32)
    sk = (u * vec[1, pl.ds(c, 1), :]).astype(bf16).astype(f32)
    o = (y.astype(bf16).astype(f32) + sk).astype(bf16)
    outb[c, rows, :] = pltpu.bitcast(o, u32)


def _attn_fill():
    n = 2 * (SEG + M)
    r = lax.broadcasted_iota(jnp.int32, (n, n), 0)
    c = lax.broadcasted_iota(jnp.int32, (n, n), 1)
    head = lambda i: jnp.where(i < 2 * SEG, i // SEG, (i - 2 * SEG) // M)
    same = head(r) == head(c)
    allowed = same & ((r >= 2 * SEG) | (c >= 2 * SEG) | (r >= c))
    return jnp.where(allowed, 0.0, jnp.where(same, -1e9 * LOG2E, -jnp.inf)).astype(f32)


def _kernel(zero_hbm, x_hbm, mem0_hbm, wq_hbm, wk_hbm, wv_hbm, wo_hbm,
            u_hbm, p0, p1, p2, p3, p4, p5, ldt_hbm, dsk_hbm, fs_hbm, g_hbm,
            out_hbm,
            wq, wk, wv, wo, xb, xs, h_ref, outs, fill_ref,
            praw, par, us, taps, vb, vm, vu, pacc, yf, outb, vec, vraw, fs_ref, g_ref, zero_ref,
            sem_s, sem_w, sem_o, sem_xb, sem_x, sem_p, sem_u, sem_out, *rings):
    wqkv = (wq, wk, wv)
    ring = rings[:NP]
    lo_ref = rings[NP:]
    scale = E ** -0.5

    whbm = [w.bitcast(u32) for w in (wq_hbm, wk_hbm, wv_hbm)]

    def wcp(j, m, p):
        return pltpu.make_async_copy(whbm[m].at[:, p, j, :], wqkv[m].at[p, j], sem_w.at[(j * 3 + m) * 2 + p])

    def start_w(j):
        for m in range(3):
            for p in range(2):
                wcp(j, m, p).start()

    xu = x_hbm.bitcast(u32)
    xcs = [pltpu.make_async_copy(xu.at[pl.ds(0, T0 // 2), pl.ds(c * 128, 128)], xb.at[c], sem_xb.at[c])
           for c in range(8)]
    xcp1 = pltpu.make_async_copy(x_hbm.at[pl.ds(T0, S - T0)], xs, sem_x.at[0])
    pcs = [pltpu.make_async_copy(p, praw.at[k], sem_p.at[k]) for k, p in enumerate((p0, p1, p2, p3, p4, p5))]
    ccs = [pltpu.make_async_copy(fs_hbm, fs_ref, sem_p.at[6]), pltpu.make_async_copy(g_hbm, g_ref, sem_p.at[7])]
    wou = wo_hbm.bitcast(u32)
    ocs = [pltpu.make_async_copy(wou.at[:, pl.ds(c * 128, 128)], wo.at[c], sem_o.at[c]) for c in range(8)]
    uu = u_hbm.bitcast(u32)
    ucs = [pltpu.make_async_copy(uu.at[:, pl.ds(c * 128, 128)], us.at[c], sem_u.at[c]) for c in range(NT)]

    zcp = pltpu.make_async_copy(zero_hbm, zero_ref, sem_s.at[0])
    scs = [pltpu.make_async_copy(mem0_hbm, h_ref.at[pl.ds(0, M)], sem_s.at[1]),
           pltpu.make_async_copy(ldt_hbm, vraw.at[0], sem_s.at[2]),
           pltpu.make_async_copy(dsk_hbm, vraw.at[1], sem_s.at[3])]
    for cp in [zcp] + xcs + [wcp(0, 0, 0), wcp(0, 0, 1)]:
        cp.start()
    vu[pl.ds(8, 8), :] = pltpu.bitcast(jnp.full((8, 128), 0x0000FFFF, u32), f32)
    vu[pl.ds(16, 8), :] = pltpu.bitcast(jnp.full((8, 128), 0xFFFF0000, u32), f32)
    taps[...] = jnp.zeros(taps.shape, f32)
    yf[1] = jnp.zeros(yf.shape[1:], u32)
    fill_ref[...] = _attn_fill()
    for cp in [wcp(0, 1, 0), wcp(0, 1, 1)] + scs:
        cp.start()
    zcp.wait()

    frow = pl.multiple_of(zero_ref[0] * 8, 8)
    zrow = [pl.multiple_of(zero_ref[k] * 8, 8) for k in range(T0 // RC)]

    class Pacer:
        def __init__(self, segments):
            self.t = 0.0
            self.todo = []
            for (pieces, buf, t0, t1) in segments:
                total = float(sum(c for c, _ in pieces))
                done = 0.0
                for (cst, fn) in pieces:
                    self.todo.append((t0 + (t1 - t0) * done / total, fn, buf))
                    done += cst

        def __call__(self, v, dt=1.0):
            self.t += dt
            fenced = []
            while self.todo and self.todo[0][0] < self.t:
                _, fn, buf = self.todo.pop(0)
                if not any(b is buf for b in fenced):
                    buf[pl.ds(frow, 8), :] = v
                    fenced.append(buf)
                fn()

        def finished(self):
            return not self.todo

    def make_fence(vpu, nslot, buf=vb):
        pc = Pacer([(vpu, buf, 0.0, float(nslot))])
        return pc, pc.finished

    def unpair(j, m, r0, nr):
        def fn():
            rows = pl.ds(r0, nr)
            m_lo = jnp.tile(pltpu.bitcast(vu[pl.ds(8, 8), :], u32), (nr // 8, 1))
            m_hi = jnp.tile(pltpu.bitcast(vu[pl.ds(16, 8), :], u32), (nr // 8, 1))
            a = wqkv[m][0, j, rows, :]
            b = wqkv[m][1, j, rows, :]
            wqkv[m][0, j, rows, :] = (a & m_lo) | ((b & m_lo) << 16)
            wqkv[m][1, j, rows, :] = ((a & m_hi) >> 16) | (b & m_hi)
        return (nr, fn)

    def unpair_pieces(items):
        return [unpair(j, m, r0, UNP) for (j, m) in items for r0 in range(0, DM // 2, UNP)]

    items = [(j, m) for j in range(NP) for m in range(3)]
    wcs = lambda lo, hi: [wcp(j, m, p) for (j, m) in items[lo:hi] for p in range(2)]
    plan = {
        0: ((1, 2), wcs(2, 4), []),
        1: ((2, 4), wcs(4, 7), []),
        3: ((4, 7), pcs + wcs(7, 12), []),
        6: ((7, 12), wcs(12, 21), pcs + scs),
        11: ((12, 21), wcs(21, 33), []),
        20: ((21, 33), wcs(33, 48) + ocs[:4], []),
        32: ((33, 48), ocs[4:] + ucs + [xcp1] + ccs, []),
    }
    with jax.named_scope("bulk"):
        with jax.named_scope("waitx"):
            for cp in xcs + wcs(0, 1):
                cp.wait()
        for _, fn in unpair_pieces(items[0:1]):
            fn()
        points = sorted(plan) + [len(items)]
        if QUICK in (1, 2):
            for cp in wcs(2, 48) + pcs + ocs + ucs + [xcp1] + ccs:
                cp.start()
            for cp in wcs(1, 48) + pcs + scs:
                cp.wait()
            vec[...] = vraw[...].astype(f32)
            for _, fn in (unpair_pieces(items[1:]) + sum(_prep_pieces(praw, vec, par), [])) if QUICK != 2 else []:
                fn()

            def kg(r, carry):
                for odd in range(2):
                    for _, fn in _kgen_pieces(0, (r, odd), par, vb, taps, 0, zrow[1], BKNI, BKSPLIT):
                        fn()
                return carry
            lax.fori_loop(0, 4, kg, 0)
            for (j, m) in (items if QUICK != 2 else []):
                def chunk(rc, carry, j=j, m=m):
                    for p in range(2):
                        lhs = jnp.concatenate(
                            [pltpu.bitcast(xb[c, pl.ds(pl.multiple_of(rc * 32, 32), 32), :], bf16) for c in range(8)], axis=1)
                        ring[j][m, p, pl.ds(pl.multiple_of(QOFF + rc * 64, 64), 64), :] = jnp.dot(
                            lhs, pltpu.bitcast(wqkv[m][p, j], bf16), preferred_element_type=f32).astype(bf16)
                    return carry
                lax.fori_loop(0, 8, chunk, 0)
            points = []
        n_chunk = 2 * (T0 // RC)
        prep = _prep_pieces(praw, vec, par)
        kg0 = [pc for r in range(8) for pc in _kgen_pieces(0, r, par, vb, taps, 0, zrow[1], BKNI, BKSPLIT)]
        t_a, t_b, t_c, t_d = [v * n_chunk for v in BPLAN]
        fence_x = Pacer([(prep[0], par, t_a, t_b), (kg0, vb, t_b, t_c), (prep[1], par, t_c, t_d)])
        fence_x.t = float(BULK_FROM * n_chunk)
        for g in range(len(points) - 1):
            lo, hi = points[g], points[g + 1]
            (w_lo, w_hi), starts, waits = plan[lo]
            for cp in starts:
                cp.start()
            with jax.named_scope("wait%d" % lo):
                for cp in wcs(w_lo, w_hi) + waits:
                    cp.wait()
            assert w_hi == min(hi + 1, len(items))
            if lo == 6:
                vec[...] = vraw[...].astype(f32)
            if lo < BULK_FROM:
                continue
            for it in range(lo, hi):
                j, m = items[it]
                fence_w, fin_w = make_fence(unpair_pieces(items[it + 1:it + 2]), n_chunk * UNP_FRAC, vu)
                for p in range(2):
                    if KHALF:
                        for half in range(2):
                            w = pltpu.bitcast(wqkv[m][p, j, pl.ds(half * (DM // 4), DM // 4), :], bf16)
                            lhs = jnp.concatenate(
                                [pltpu.bitcast(xb[c], bf16) for c in range(4 * half, 4 * half + 4)], axis=1)
                            res = jnp.dot(lhs, w, preferred_element_type=f32)
                            for rc in range(T0 // RC):
                                v = res[rc * RC:(rc + 1) * RC]
                                if half == 0:
                                    pacc[pl.ds(rc * RC, RC), :] = v
                                else:
                                    v = v + pacc[pl.ds(rc * RC, RC), :]
                                    ring[j][m, p, pl.ds(QOFF + rc * RC, RC), :] = v.astype(bf16)
                                fence_w(v[:8], 0.5)
                                fence_x(v[:8], 0.5)
                        continue
                    for rc in range(T0 // RC):
                        w = pltpu.bitcast(wqkv[m][p, j, pl.ds(zrow[rc], DM // 2), :], bf16)
                        lhs = jnp.concatenate(
                            [pltpu.bitcast(xb[c, pl.ds(rc * RC // 2, RC // 2), :], bf16) for c in range(8)], axis=1)
                        res = jnp.dot(lhs, w, preferred_element_type=f32)
                        ring[j][m, p, pl.ds(QOFF + rc * RC, RC), :] = res.astype(bf16)
                        fence_w(res[:8])
                        fence_x(res[:8])
                assert fin_w()
        assert QUICK or BULK_FROM or fence_x.finished()
    with jax.named_scope("waitrest"):
        for cp in ocs + ucs + ccs + [xcp1]:
            cp.wait()

    ou = out_hbm.bitcast(u32)

    def outa_cp(row, n):
        return pltpu.make_async_copy(outs.at[pl.ds(row, n)], out_hbm.at[pl.ds(row, n), pl.ds(0, DM)], sem_out.at[0])

    def outb_cp(c, row, n, sem):
        col = DM + c * 128
        return pltpu.make_async_copy(
            outb.at[c, pl.ds(row, n)],
            ou.at[pl.ds(row, n), pl.ds(col if isinstance(col, int) else pl.multiple_of(col, 128), 128)],
            sem_out.at[sem])

    def one_step(i, odd, ppos, cpos, fwd, fence):
        s = 2 * i + odd
        lo_cur = lo_ref[odd]
        n_out = TOK if odd == 0 else 2 * SEG - TOK
        orow = pl.multiple_of(2 * SEG * i + odd * TOK, 8)
        h_ref[pl.ds(M, TOK), :] = xs[pl.ds(pl.multiple_of(TOK * s, 8), TOK), :]
        h = h_ref[...]
        mem_rows = {}
        scores = {}
        probs = {}

        ct = i >> 2
        r = s & 7
        buf = ct & 1
        cprev = (ct + NT - 1) & (NT - 1)

        def stage_a(j):
            for m in range(3):
                mm = []
                for p in range(2):
                    w = pltpu.bitcast(wqkv[m][p, j], bf16)
                    res = jnp.dot(h, w, preferred_element_type=f32)
                    ring[j][m, p, pl.ds(ppos, TOK), :] = res[M:].astype(bf16)
                    mm.append(res[:M])
                    fence(res[:M])
                mem_rows[m, j] = jnp.concatenate(mm, axis=0).astype(bf16)

        def gather(m, j):
            return jnp.concatenate([ring[j][m, 0, pl.ds(cpos, SEG), :], ring[j][m, 1, pl.ds(cpos, SEG), :],
                                    mem_rows[m, j]], axis=0)

        def stage_qk(j):
            scores[j] = lax.dot_general(gather(0, j), gather(1, j), (((1,), (1,)), ((), ())),
                                        preferred_element_type=f32)

        def stage_b(j):
            fl = fill_ref[...]
            sc = jnp.where(fl == 0.0, scores.pop(j) * (scale * LOG2E), fl)
            e = jnp.exp2(sc - jnp.max(sc, axis=-1, keepdims=True))
            den = jnp.sum(e, axis=-1, keepdims=True)
            probs[j] = (e * pl.reciprocal(den, approx=True)).astype(bf16)

        def stage_c(j):
            o = jnp.dot(probs[j], gather(2, j), preferred_element_type=f32)
            for p in range(2):
                hh = 2 * j + p
                ox = o[p * SEG:(p + 1) * SEG]
                lo_cur[hh, pl.ds(0, M), :] = o[2 * SEG + p * M:2 * SEG + (p + 1) * M].astype(bf16)
                if odd == 0:
                    lo_ref[0][hh, pl.ds(M, TOK), :] = ox[:TOK].astype(bf16)
                    lo_ref[1][hh, pl.ds(M, SEG - TOK), :] = ox[TOK:].astype(bf16)
                else:
                    lo_ref[1][hh, pl.ds(M + SEG - TOK, SEG), :] = ox.astype(bf16)

        acc = [None] * 8

        def stage_d(h0, h1, last=False):
            lhs = jnp.concatenate([lo_cur[hh] for hh in range(h0, h1)], axis=1)
            for c in range(8):
                w = pltpu.bitcast(wo[c, pl.ds(h0 * 64, (h1 - h0) * 64), :], bf16)
                res = jnp.dot(lhs, w, preferred_element_type=f32)
                acc[c] = res if acc[c] is None else acc[c] + res
                if not last:
                    fence(res[:M], (h1 - h0) / 8.0 * (DW_ODD if odd else 1.0))
                else:
                    rb = acc[c].astype(bf16)
                    h_ref[pl.ds(0, M), pl.ds(c * 128, 128)] = rb[:M]
                    outs[pl.ds(orow, n_out), pl.ds(c * 128, 128)] = rb[M:]

        def attn_group(jq, jc):
            for j in jq:
                stage_qk(j)
            for j in jc:
                stage_c(j)
            for j in jq:
                stage_b(j)

        for t in range(2):
            _inv_piece(cprev, 2 * r + t, 1 - buf, g_ref, us, vec, yf, outb)
        for p in fwd:
            p()
        for j in range(NP):
            stage_a(j)
            if j >= 2 and j % 2 == 0:
                attn_group((j - 2, j - 1), (j - 4, j - 3) if j >= 4 else ())
        stage_d(0, 8)
        attn_group((14, 15), (12, 13))
        stage_d(8, 20)
        attn_group((), (14, 15))
        stage_d(20, 28)
        stage_d(28, 32, last=True)

    def two_steps(i, carry):
        pp, cp = carry
        ct = i >> 2
        cprev = (ct + NT - 1) & (NT - 1)
        conv = [_conv_pieces(ct, (i & 3, odd), ct & 1, fs_ref, us, taps, vm, yf,
                             zrow[1] if DONE_M else None) for odd in range(2)]
        kgen = [_kgen_pieces((ct + 1) & (NT - 1), (i & 3, odd), par, vb, taps, ct + 1,
                             zrow[1] if DONE_K else None, KNI, KSPLIT) for odd in range(2)]
        work = {'k0': (kgen[0], vb), 'k1': (kgen[1], vb), 'm0': (conv[0][1], vm), 'm1': (conv[1][1], vm)}
        fence = Pacer([work[k] + (t0, t1) for (k, t0, t1) in PLAN if k[0] not in NOB])
        for odd in range(2):
            one_step(i, odd, pl.multiple_of(pp, 16) + odd * TOK, pl.multiple_of(cp, 64) + odd * SEG,
                     conv[odd][0], fence)
        assert fence.finished() or NOB
        outa_cp(pl.multiple_of(2 * SEG * i, 2 * SEG), 2 * SEG).start()
        outb_cp(cprev, pl.multiple_of((i & 3) * 256, 256), 256, jnp.where(i < 4, 2, 1)).start()
        wrap = lambda v: jnp.where(v >= RING, v - RING, v)
        return wrap(pp + 2 * TOK), wrap(cp + 2 * SEG)

    with jax.named_scope("steps"):
        if NITER:
            lax.fori_loop(0, NITER, two_steps, (jnp.int32(0), jnp.int32(QOFF)))

    with jax.named_scope("flush"):
        outb_cp(NT - 1, 0, L // 2, 2).wait()
        for b in range(NBLK):
            _inv_piece(NT - 1, b, (NT - 1) % 2, g_ref, us, vec, yf, outb)
            if b % 4 == 3:
                outb_cp(NT - 1, (b - 3) * 64, 256, 1).start()
    with jax.named_scope("waitout"):
        outa_cp(0, S).wait()
        pltpu.make_async_copy(outb, outb, sem_out.at[1]).wait()


@functools.partial(jax.jit, static_argnames=("A_seg_len",))
def pallas_concat_heads__memory_aug_recurrent_mem_tr__ssm_conv_s4__prompt_kernel(
    A_x, A_mem0, A_Wq, A_Wk, A_Wv, A_Wo, A_seg_len,
    B_u, B_A_re, B_A_im, B_B_re, B_B_im, B_C_re, B_C_im, B_log_dt, B_Dskip,
):
    assert A_seg_len == SEG and A_x.shape == (1, S, DM) and B_u.shape == (1, L, D)
    fs, g = _dft_consts()
    w4 = lambda w: w.reshape(DM // 2, 2, H, E)
    any_ = pl.BlockSpec(memory_space=pl.ANY)
    V = pltpu.VMEM
    out = pl.pallas_call(
        _kernel,
        out_shape=jax.ShapeDtypeStruct((S, DM + D), bf16),
        in_specs=[any_] * 18,
        out_specs=any_,
        scratch_shapes=[
            V((2, NP, DM // 2, E), u32),
            V((2, NP, DM // 2, E), u32),
            V((2, NP, DM // 2, E), u32),
            V((8, H * E // 2, 128), u32),
            V((8, T0 // 2, 128), u32),
            V((S - T0, DM), bf16),
            V((M + TOK, DM), bf16),
            V((S, DM), bf16),
            V((2 * (SEG + M), 2 * (SEG + M)), f32),
            V((6, D, N), bf16),
            V((8 + NT * 6 * N, 128), f32),
            V((NT, L // 2, 128), u32),
            V((NT + 1, TAPROWS, 128), f32),
            V((V_ROWS, 128), f32),
            V((VM_ROWS, 128), f32),
            V((24, 128), f32),
            V((T0, 128), f32),
            V((2, NBLK, 128, 128), u32),
            V((NT, L // 2, 128), u32),
            V((2, 8, 128), f32),
            V((2, 8, 128), bf16),
            V((8, NBLK * 32, 128), bf16),
            V((BLK, 256), bf16),
            pltpu.SMEM((8,), jnp.int32),
            pltpu.SemaphoreType.DMA((4,)),
            pltpu.SemaphoreType.DMA((6 * NP,)),
            pltpu.SemaphoreType.DMA((8,)),
            pltpu.SemaphoreType.DMA((8,)),
            pltpu.SemaphoreType.DMA((1,)),
            pltpu.SemaphoreType.DMA((8,)),
            pltpu.SemaphoreType.DMA((NT,)),
            pltpu.SemaphoreType.DMA((3,)),
        ] + [V((3, 2, RING, E), bf16)] * NP + [V((H, M + TOK, E), bf16), V((H, M + 2 * SEG - TOK, E), bf16)],
        compiler_params=pltpu.CompilerParams(vmem_limit_bytes=110 * 1024 * 1024, disable_bounds_checks=True),
    )(jnp.asarray(np.zeros((8,), np.int32)), A_x.reshape(S, DM), A_mem0.reshape(M, DM), w4(A_Wq), w4(A_Wk), w4(A_Wv), A_Wo.reshape(H * E, DM),
      B_u.reshape(L, D), B_A_re, B_A_im, B_B_re, B_B_im, B_C_re, B_C_im,
      B_log_dt.reshape(8, 128), B_Dskip.reshape(8, 128),
      jnp.asarray(fs, bf16), jnp.asarray(g, bf16))
    return out.reshape(1, S, DM + D)
```

```python
import functools

import numpy as np
import jax
import jax.numpy as jnp
from jax import lax
import jax.experimental.pallas as pl
import jax.experimental.pallas.tpu as pltpu

bf16, f32, u32 = jnp.bfloat16, jnp.float32, jnp.uint32

S, DM, H, E, M, SEG = 2048, 1024, 32, 128, 8, 32
NSEG = S // SEG
TOK = 24
PRE = SEG - TOK
T0 = PRE * NSEG
NP = H // 2
LOG2E = 1.4426950408889634
QUICK = False
NOB = ''
BKNI = 1
UNP = 64
UNP_FRAC = 0.7
BKSPLIT = 4
BPLAN = (6.0, 7.0, 41.5, 47.7)
BULK_FROM = 0
NITER = NSEG // 2
KNI = 2
KSPLIT = 2
PLAN = (('k0', 0, 96), ('m0', 96, 122), ('k1', 124, 220), ('m1', 220, 260))
DONE_K = True
DONE_M = True
DW_ODD = 1.5
RC = 64
MACJ = 6
NSLOT = 118
L, D, N = 2048, 1024, 128
BLK = 128
NBLK = L // BLK
NT = D // 128
TAPROWS = 672
WINDOWS = ((0, 128, 0, 1), (128, 128, 1, 1), (256, 128, 2, 1), (320, 80, 3, 1),
           (384, 128, 4, 3), (480, 48, 7, 1), (512, 128, 8, 7), (624, 32, 15, 1))

V_FENCE = 0
V_YTAB = 8
V_START = V_YTAB + 256
V_STEP = V_START + 160
V_ROWS = V_STEP + 128
V_UF = 8
V_KF = V_UF + NBLK * 32
VM_ROWS = V_KF + NBLK * 32


def _bf16_round_int(l):
    u = np.asarray(l, np.float32).view(np.uint32)
    r = (u + 0x7FFF + ((u >> 16) & 1)) & 0xFFFF0000
    return r.astype(np.uint32).view(np.float32).astype(np.int64)


def _tap_row(lp):
    return np.where(lp < 256, lp, np.where(lp < 512, 256 + (lp - 256) // 2,
                    np.where(lp < 1024, 384 + (lp - 512) // 4, 512 + (lp - 1024) // 8)))


@functools.lru_cache(maxsize=None)
def _dft_consts():
    t = np.arange(BLK)
    F = np.zeros((8, 32, BLK))
    G = np.zeros((BLK, 8, 32))
    for r in range(8):
        f = np.concatenate([16 * r + 2 * np.arange(8), 16 * r + 2 * np.arange(8) + 1])
        th = 2 * np.pi * (f + 0.5) / (2 * BLK)
        F[r, :16] = np.cos(th[:, None] * t[None])
        F[r, 16:] = -np.sin(th[:, None] * t[None])
        G[:, r, 0::2] = np.cos(th[None] * t[:, None]) / BLK
        G[:, r, 1::2] = -np.sin(th[None] * t[:, None]) / BLK
    FS = np.zeros((8, NBLK, 32, 128))
    for (w0, wn, b0, nb) in WINDOWS:
        for j in range(b0, b0 + nb):
            rows = _tap_row(_bf16_round_int(BLK * j + t)) - w0
            assert rows.min() >= 0 and rows.max() < wn
            sel = np.zeros((BLK, 128))
            sel[t, rows] = 1.0
            FS[:, j] = F @ sel
    return (FS.reshape(8, NBLK * 32, 128).astype(np.float32),
            G.reshape(BLK, 256).astype(np.float32))


def _cmul(a, b):
    return (a[0] * b[0] - a[1] * b[1], a[0] * b[1] + a[1] * b[0])


def _csq(a):
    return (a[0] * a[0] - a[1] * a[1], 2.0 * (a[0] * a[1]))


def _cexp(lr, li):
    k = jnp.floor(li * (2.0 / np.pi) + 0.5)
    r = ((li - k * 1.5703125) - k * 4.837512969970703125e-4) - k * 7.54978995489188216e-8
    r = jnp.clip(r, -0.8, 0.8)
    r2 = r * r
    s = r + r * r2 * (-1.6666654611e-1 + r2 * (8.3321608736e-3 + r2 * -1.9515295891e-4))
    c = (1.0 - 0.5 * r2) + (r2 * r2) * (4.166664568298827e-2
                                        + r2 * (-1.388731625493765e-3 + r2 * 2.443315711809948e-5))
    q = k.astype(jnp.int32)
    swap = (q & 1) == 1
    m = jnp.exp(lr)
    flip = lambda v, bit: pltpu.bitcast(pltpu.bitcast(v, jnp.int32) ^ (bit << 30), f32)
    return (flip(m * jnp.where(swap, s, c), (q + 1) & 2), flip(m * jnp.where(swap, c, s), q & 2))


def _par_row(c, k):
    return 8 + (c * 6 + k) * N


def _prep_pieces(praw, vec, par):
    def stage1(c):
        def fn():
            tr = lambda k: praw[k, pl.ds(c * 128, 128), :].astype(f32).T
            dt = jnp.exp(vec[0, pl.ds(c, 1), :]).astype(bf16).astype(f32)
            cc = _cmul((tr(4), tr(5)), (dt * tr(2), dt * tr(3)))
            for k, v in ((0, dt * tr(0)), (1, dt * tr(1)), (4, cc[0]), (5, cc[1])):
                par[pl.ds(_par_row(c, k), N), :] = v
        return fn

    def stage2(c, n0):
        def fn():
            lr = par[pl.ds(_par_row(c, 0) + n0, 16), :]
            li = par[pl.ds(_par_row(c, 1) + n0, 16), :]
            for k, v in enumerate(_cexp(lr, li) + _cexp(lr * 128.0, li * 128.0)):
                par[pl.ds(_par_row(c, k) + n0, 16), :] = v
        return fn

    tile = lambda c: [(260, stage1(c))] + [(190, stage2(c, n0)) for n0 in range(0, N, 16)]
    return tile(0), [pc for c in range(1, NT) for pc in tile(c)]


def _kgen_pieces(c, r, par, vb, taps, tslot, frow, kni, ksplit):
    st = {}

    def put(row, z, h=None):
        if h is None:
            vb[pl.ds(row, 16), :] = z[0]
            vb[pl.ds(row + 16, 16), :] = z[1]
        else:
            vb[pl.ds(row + 8 * h, 8), :] = z[0]
            vb[pl.ds(row + 16 + 8 * h, 8), :] = z[1]

    def get(row, h=None):
        if h is None:
            return (vb[pl.ds(row, 16), :], vb[pl.ds(row + 16, 16), :])
        return (vb[pl.ds(row + 8 * h, 8), :], vb[pl.ds(row + 16 + 8 * h, 8), :])

    def params(k):
        if isinstance(r, int):
            return par[pl.ds(_par_row(c, k) + r * 16, 16), :]
        return par[pl.ds(pl.multiple_of(c * (6 * N) + r[0] * 32, 32) + (_par_row(0, k) + r[1] * 16), 16), :]

    def park():
        put(V_STEP, (params(0), params(1)))
        put(V_START + 32, (params(2), params(3)))
        put(V_START, (params(4), params(5)))

    def setup_y(h):
        def fn():
            z1 = get(V_STEP, h)
            z2 = _csq(z1)
            z4 = _csq(z2)
            s = lax.broadcasted_iota(jnp.int32, (8, 128), 0)
            fs = [(jnp.where((s >> k) & 1 == 1, z[0], 1.0), jnp.where((s >> k) & 1 == 1, z[1], 0.0))
                  for k, z in enumerate((z1, z2, z4))]
            y = _cmul(_cmul(fs[0], fs[1]), fs[2])
            for k in range(8):
                put(V_YTAB + 32 * k, y, h)
                if k < 7:
                    y = _cmul(y, z1)
                    y = (jnp.where(s == 7 - k, 1.0, y[0]), jnp.where(s == 7 - k, 0.0, y[1]))
            z = z4
            for k in range(4):
                z = _csq(z)
                put(V_STEP + 32 * k, z, h)
        return fn

    def setup_hi():
        z = get(V_START + 32)
        cf = get(V_START)
        for g in range(1, 5):
            put(V_START + 32 * g, _cmul(cf, z))
            if g < 4:
                z = _csq(z)

    def square(k0, k1):
        def fn():
            for k in range(k0, k1):
                put(V_YTAB + 32 * k, _csq(get(V_YTAB + 32 * k)))
        return fn

    def rows_of(g, i0, ni):
        n_i = 16 + (g == 4)

        def fn():
            x = st.pop('x') if i0 > 0 else get(V_START + 32 * g)
            step = get(V_STEP + 32 * max(g - 1, 0))
            xs = []
            for t in range(ni):
                xs.append(x)
                if i0 + t + 1 < n_i:
                    x = _cmul(x, step)
            if i0 + ni < n_i:
                st['x'] = x
            acc = [None] * ni
            for k in range(8):
                yr, yi = get(V_YTAB + 32 * k)
                for t in range(ni):
                    v = xs[t][0] * yr - xs[t][1] * yi
                    v = v[:8] + v[8:]
                    if k:
                        v = pltpu.roll(v, k, 0)
                    acc[t] = v if acc[t] is None else acc[t] + v
                if frow is not None and k % ksplit == ksplit - 1 and k < 7:
                    vb[pl.ds(frow, 8), :] = acc[ni - 1]
            for t in range(ni):
                row = 128 * g + 8 * (i0 + t)
                a = acc[t]
                if row == 640:
                    a = jnp.where(lax.broadcasted_iota(jnp.int32, (8, 128), 0) == 0, a, 0.0)
                taps[tslot, pl.ds(row, 8), :] = taps[tslot, pl.ds(row, 8), :] + a
                if frow is not None and t == ni - 1:
                    vb[pl.ds(frow, 8), :] = a
        return fn

    pieces = [(30, park), (110, setup_y(0)), (110, setup_y(1)), (80, setup_hi)]
    for g in range(5):
        if g >= 2:
            pieces += [(40, square(0, 4)), (40, square(4, 8))]
        for i0 in range(0, 16 + (g == 4), kni):
            ni = min(kni, 16 + (g == 4) - i0)
            pieces.append((83 * ni, rows_of(g, i0, ni)))
    return pieces


def _conv_pieces(c, r, buf, fs_ref, us, taps, vb, yf, frow):
    st = {}

    def fwd_u(b0, b1):
        def fn():
            lhs = fs_ref[2 * r[0] + r[1], pl.ds(0, 32), :]
            for b in range(b0, b1):
                w = pltpu.bitcast(us[c, pl.ds(b * 64, 64), :], bf16)
                res = jnp.dot(lhs, w, preferred_element_type=f32)
                row = V_UF + 32 * b
                if b == 0:
                    vb[pl.ds(row, 32), :] = res
                else:
                    p = st['prev']
                    vb[pl.ds(row, 8), :] = res[0:8] - p[16:24]
                    vb[pl.ds(row + 8, 8), :] = res[8:16] + p[24:32]
                    vb[pl.ds(row + 16, 8), :] = res[16:24] + p[0:8]
                    vb[pl.ds(row + 24, 8), :] = res[24:32] - p[8:16]
                st['prev'] = res
        return fn

    def fwd_k(jobs):
        def fn():
            for (wi, t0, nb) in jobs:
                w0, wn, b0, _ = WINDOWS[wi]
                lhs = fs_ref[2 * r[0] + r[1], pl.ds((b0 + t0) * 32, nb * 32), pl.ds(0, wn)]
                w = taps[c, pl.ds(w0, wn), :].astype(bf16)
                vb[pl.ds(V_KF + 32 * (b0 + t0), 32 * nb), :] = jnp.dot(lhs, w, preferred_element_type=f32)
        return fn

    def mac(q, i0, ni, j0, j1):
        def fn():
            ld = lambda base, b: (vb[pl.ds(base + 32 * b + 8 * q, 8), :], vb[pl.ds(base + 32 * b + 16 + 8 * q, 8), :])
            zr, zi = st.pop('z') if j0 > 0 else ({}, {})
            ucache = {}
            for j in range(j0, j1):
                kr, ki = ld(V_KF, j)
                for i in range(max(i0, j), i0 + ni):
                    if i - j not in ucache:
                        ucache[i - j] = ld(V_UF, i - j)
                    ur, ui = ucache[i - j]
                    if i not in zr:
                        zr[i] = kr * ur - ki * ui
                        zi[i] = kr * ui + ki * ur
                    else:
                        zr[i] = zr[i] + kr * ur - ki * ui
                        zi[i] = zi[i] + kr * ui + ki * ur
            if frow is not None:
                vb[pl.ds(frow, 8), :] = zr[i0 + ni - 1]
            if j1 < i0 + ni:
                st['z'] = (zr, zi)
            else:
                row = pl.multiple_of(r[0] * 32, 32) + (r[1] * 16 + q * 8)
                for i in range(i0, i0 + ni):
                    yf[buf, i, pl.ds(row, 8), :] = pltpu.pack_elementwise([zr[i], zi[i]], packed_dtype=bf16)
        return (8 * sum(1 for j in range(j0, j1) for i in range(max(i0, j), i0 + ni)), fn)

    fwd = [fwd_u(0, 8), fwd_u(8, 16), fwd_k(((0, 0, 1), (1, 0, 1), (2, 0, 1), (3, 0, 1))),
           fwd_k(((4, 0, 2), (6, 0, 2), (6, 2, 2), (6, 4, 2))), fwd_k(((4, 2, 1), (5, 0, 1), (6, 6, 1), (7, 0, 1)))]
    macs = []
    for q in range(2):
        for i0 in range(0, NBLK, 2):
            for j0 in range(0, i0 + 2, MACJ):
                macs.append(mac(q, i0, 2, j0, min(j0 + MACJ, i0 + 2)))
    return fwd, macs


def _inv_piece(c, b, buf, g_ref, us, vec, yf, outb):
    rows = pl.ds(pl.multiple_of(b * 64, 64), 64)
    w = pltpu.bitcast(yf[buf, b], bf16)
    y = jnp.dot(g_ref[...], w, preferred_element_type=f32)
    u = pltpu.bitcast(us[c, rows, :], bf16).astype(f32)
    sk = (u * vec[1, pl.ds(c, 1), :]).astype(bf16).astype(f32)
    o = (y.astype(bf16).astype(f32) + sk).astype(bf16)
    outb[c, rows, :] = pltpu.bitcast(o, u32)


def _attn_fill():
    n = 2 * (SEG + M)
    r = lax.broadcasted_iota(jnp.int32, (n, n), 0)
    c = lax.broadcasted_iota(jnp.int32, (n, n), 1)
    head = lambda i: jnp.where(i < 2 * SEG, i // SEG, (i - 2 * SEG) // PRE)
    pos = lambda i: jnp.where(i < 2 * SEG, i % SEG, i % PRE)
    is_mem = lambda i: (i < 2 * SEG) & (i % SEG < M)
    same = head(r) == head(c)
    allowed = same & (is_mem(r) | is_mem(c) | (pos(r) >= pos(c)))
    return jnp.where(allowed, 0.0, jnp.where(same, -1e9 * LOG2E, -jnp.inf)).astype(f32)


def _kernel(zero_hbm, x_hbm, mem0_hbm, wq_hbm, wk_hbm, wv_hbm, wo_hbm,
            u_hbm, p0, p1, p2, p3, p4, p5, ldt_hbm, dsk_hbm, fs_hbm, g_hbm,
            out_hbm,
            wq, wk, wv, wo, xb, xs, h_ref, outs, fill_ref,
            praw, par, us, taps, vb, vm, vu, pacc, yf, outb, vec, vraw, fs_ref, g_ref, zero_ref,
            sem_s, sem_w, sem_o, sem_xb, sem_x, sem_p, sem_u, sem_out, pre, own, lo0, lo1):
    wqkv = (wq, wk, wv)
    scale = E ** -0.5

    whbm = [w.bitcast(u32) for w in (wq_hbm, wk_hbm, wv_hbm)]

    def wcp(j, m, p):
        return pltpu.make_async_copy(whbm[m].at[:, p, j, :], wqkv[m].at[p, j], sem_w.at[(j * 3 + m) * 2 + p])

    xu = x_hbm.bitcast(u32)
    xcs = [pltpu.make_async_copy(xu.at[:, t, pl.ds(0, PRE // 2), pl.ds(c * 128, 128)],
                                 xb.at[c, :, pl.ds(t * (PRE // 2), PRE // 2), :], sem_xb.at[2 * c + t])
           for c in range(8) for t in range(2)]
    xcp1 = pltpu.make_async_copy(x_hbm.at[:, :, pl.ds(PRE, TOK), :], xs, sem_x.at[0])
    pcs = [pltpu.make_async_copy(p, praw.at[k], sem_p.at[k]) for k, p in enumerate((p0, p1, p2, p3, p4, p5))]
    ccs = [pltpu.make_async_copy(fs_hbm, fs_ref, sem_p.at[6]), pltpu.make_async_copy(g_hbm, g_ref, sem_p.at[7])]
    wou = wo_hbm.bitcast(u32)
    ocs = [pltpu.make_async_copy(wou.at[:, pl.ds(c * 128, 128)], wo.at[c], sem_o.at[c]) for c in range(8)]
    uu = u_hbm.bitcast(u32)
    ucs = [pltpu.make_async_copy(uu.at[:, pl.ds(c * 128, 128)], us.at[c], sem_u.at[c]) for c in range(NT)]

    zcp = pltpu.make_async_copy(zero_hbm, zero_ref, sem_s.at[0])
    scs = [pltpu.make_async_copy(mem0_hbm, h_ref.at[pl.ds(0, M)], sem_s.at[1]),
           pltpu.make_async_copy(ldt_hbm, vraw.at[0], sem_s.at[2]),
           pltpu.make_async_copy(dsk_hbm, vraw.at[1], sem_s.at[3])]
    for cp in [zcp] + xcs + [wcp(0, 0, 0), wcp(0, 0, 1)]:
        cp.start()
    vu[pl.ds(8, 8), :] = pltpu.bitcast(jnp.full((8, 128), 0x0000FFFF, u32), f32)
    vu[pl.ds(16, 8), :] = pltpu.bitcast(jnp.full((8, 128), 0xFFFF0000, u32), f32)
    taps[...] = jnp.zeros(taps.shape, f32)
    yf[1] = jnp.zeros(yf.shape[1:], u32)
    fill_ref[...] = _attn_fill()
    for cp in [wcp(0, 1, 0), wcp(0, 1, 1)] + scs:
        cp.start()
    zcp.wait()

    frow = pl.multiple_of(zero_ref[0] * 8, 8)
    zrow = [pl.multiple_of(zero_ref[k] * 8, 8) for k in range(T0 // RC)]

    class Pacer:
        def __init__(self, segments):
            self.t = 0.0
            self.todo = []
            for (pieces, buf, t0, t1) in segments:
                total = float(sum(c for c, _ in pieces))
                done = 0.0
                for (cst, fn) in pieces:
                    self.todo.append((t0 + (t1 - t0) * done / total, fn, buf))
                    done += cst

        def __call__(self, v, dt=1.0):
            self.t += dt
            fenced = []
            while self.todo and self.todo[0][0] < self.t:
                _, fn, buf = self.todo.pop(0)
                if not any(b is buf for b in fenced):
                    buf[pl.ds(frow, 8), :] = v
                    fenced.append(buf)
                fn()

        def finished(self):
            return not self.todo

    def make_fence(vpu, nslot, buf=vb):
        pc = Pacer([(vpu, buf, 0.0, float(nslot))])
        return pc, pc.finished

    def unpair(j, m, r0, nr):
        def fn():
            rows = pl.ds(r0, nr)
            m_lo = jnp.tile(pltpu.bitcast(vu[pl.ds(8, 8), :], u32), (nr // 8, 1))
            m_hi = jnp.tile(pltpu.bitcast(vu[pl.ds(16, 8), :], u32), (nr // 8, 1))
            a = wqkv[m][0, j, rows, :]
            b = wqkv[m][1, j, rows, :]
            wqkv[m][0, j, rows, :] = (a & m_lo) | ((b & m_lo) << 16)
            wqkv[m][1, j, rows, :] = ((a & m_hi) >> 16) | (b & m_hi)
        return (nr, fn)

    def unpair_pieces(items):
        return [unpair(j, m, r0, UNP) for (j, m) in items for r0 in range(0, DM // 2, UNP)]

    items = [(j, m) for j in range(NP) for m in range(3)]
    wcs = lambda lo, hi: [wcp(j, m, p) for (j, m) in items[lo:hi] for p in range(2)]
    plan = {
        0: ((1, 2), wcs(2, 4), []),
        1: ((2, 4), wcs(4, 7), []),
        3: ((4, 7), pcs + wcs(7, 12), []),
        6: ((7, 12), wcs(12, 21), pcs + scs),
        11: ((12, 21), wcs(21, 33), []),
        20: ((21, 33), wcs(33, 48) + ocs[:4], []),
        32: ((33, 48), ocs[4:] + ucs + [xcp1] + ccs, []),
    }
    with jax.named_scope("bulk"):
        with jax.named_scope("waitx"):
            for cp in xcs + wcs(0, 1):
                cp.wait()
        for _, fn in unpair_pieces(items[0:1]):
            fn()
        points = sorted(plan) + [len(items)]
        if QUICK in (1, 2):
            for cp in wcs(2, 48) + pcs + ocs + ucs + [xcp1] + ccs:
                cp.start()
            for cp in wcs(1, 48) + pcs + scs:
                cp.wait()
            vec[...] = vraw[...].astype(f32)
            for _, fn in (unpair_pieces(items[1:]) + sum(_prep_pieces(praw, vec, par), [])) if QUICK != 2 else []:
                fn()

            def kg(r, carry):
                for odd in range(2):
                    for _, fn in _kgen_pieces(0, (r, odd), par, vb, taps, 0, zrow[1], BKNI, BKSPLIT):
                        fn()
                return carry
            lax.fori_loop(0, 4, kg, 0)
            for (j, m) in (items if QUICK != 2 else []):
                def chunk(rc, carry, j=j, m=m):
                    lhs = jnp.concatenate(
                        [pltpu.bitcast(xb[c, pl.ds(rc * 4, 4)].reshape(32, 128), bf16) for c in range(8)], axis=1)
                    res = [jnp.dot(lhs, pltpu.bitcast(wqkv[m][p, j], bf16), preferred_element_type=f32)
                           for p in range(2)]
                    for t in range(8):
                        v = jnp.concatenate([res[0][8 * t:8 * t + 8], res[1][8 * t:8 * t + 8]], axis=0)
                        pre[rc * 8 + t, m * NP + j] = pltpu.bitcast(v.astype(bf16), u32)
                    return carry
                lax.fori_loop(0, 8, chunk, 0)
            points = []
        n_chunk = 2 * (T0 // RC)
        prep = _prep_pieces(praw, vec, par)
        kg0 = [pc for r in range(8) for pc in _kgen_pieces(0, r, par, vb, taps, 0, zrow[1], BKNI, BKSPLIT)]
        t_a, t_b, t_c, t_d = [v * n_chunk for v in BPLAN]
        fence_x = Pacer([(prep[0], par, t_a, t_b), (kg0, vb, t_b, t_c), (prep[1], par, t_c, t_d)])
        fence_x.t = float(BULK_FROM * n_chunk)
        for g in range(len(points) - 1):
            lo, hi = points[g], points[g + 1]
            (w_lo, w_hi), starts, waits = plan[lo]
            for cp in starts:
                cp.start()
            with jax.named_scope("wait%d" % lo):
                for cp in wcs(w_lo, w_hi) + waits:
                    cp.wait()
            assert w_hi == min(hi + 1, len(items))
            if lo == 6:
                vec[...] = vraw[...].astype(f32)
            if lo < BULK_FROM:
                continue
            for it in range(lo, hi):
                j, m = items[it]
                fence_w, fin_w = make_fence(unpair_pieces(items[it + 1:it + 2]), n_chunk * UNP_FRAC, vu)
                for p in range(2):
                    for half in range(2):
                        w = pltpu.bitcast(wqkv[m][p, j, pl.ds(half * (DM // 4), DM // 4), :], bf16)
                        lhs = jnp.concatenate([pltpu.bitcast(xb[c].reshape(T0 // 2, 128), bf16)
                                               for c in range(4 * half, 4 * half + 4)], axis=1)
                        res = jnp.dot(lhs, w, preferred_element_type=f32)
                        for rc in range(T0 // RC):
                            rows = pl.ds(rc * RC, RC)
                            v = res[rc * RC:(rc + 1) * RC]
                            if half == 1:
                                v = v + pacc[p, rows, :]
                            if p == 0 or half == 0:
                                pacc[p, rows, :] = v
                            else:
                                v0 = pacc[0, rows, :]
                                for t in range(RC // PRE):
                                    pr = jnp.concatenate([v0[PRE * t:PRE * (t + 1)], v[PRE * t:PRE * (t + 1)]], axis=0)
                                    pre[rc * (RC // PRE) + t, m * NP + j] = pltpu.bitcast(pr.astype(bf16), u32)
                            fence_w(v[:8], 0.5)
                            fence_x(v[:8], 0.5)
                assert fin_w()
        assert QUICK or BULK_FROM or fence_x.finished()
    with jax.named_scope("waitrest"):
        for cp in ocs + ucs + ccs + [xcp1]:
            cp.wait()

    ou = out_hbm.bitcast(u32)

    def outa_cp(row, n):
        return pltpu.make_async_copy(outs.at[pl.ds(row, n)], out_hbm.at[pl.ds(row, n), pl.ds(0, DM)], sem_out.at[0])

    def outb_cp(c, row, n, sem):
        col = DM + c * 128
        return pltpu.make_async_copy(
            outb.at[c, pl.ds(row, n)],
            ou.at[pl.ds(row, n), pl.ds(col if isinstance(col, int) else pl.multiple_of(col, 128), 128)],
            sem_out.at[sem])

    def one_step(i, odd, fwd, fence):
        s = 2 * i + odd
        lo_cur = (lo0, lo1)[odd]
        base = pl.multiple_of(2 * SEG * i, 2 * SEG)
        h_ref[pl.ds(M, TOK), :] = xs[i, odd]
        h = h_ref[...]
        scores = {}
        probs = {}

        ct = i >> 2
        r = s & 7
        buf = ct & 1
        cprev = (ct + NT - 1) & (NT - 1)

        def stage_a(j):
            for m in range(3):
                for p in range(2):
                    w = pltpu.bitcast(wqkv[m][p, j], bf16)
                    res = jnp.dot(h, w, preferred_element_type=f32)
                    own[m * NP + j, pl.ds(16 * p, 16), :] = pltpu.bitcast(res.astype(bf16), u32)
                    fence(res[:M])

        def gather(m, j):
            return pltpu.bitcast(jnp.concatenate([own[m * NP + j], pre[s, m * NP + j]], axis=0), bf16)

        def stage_qk(j):
            scores[j] = lax.dot_general(gather(0, j), gather(1, j), (((1,), (1,)), ((), ())),
                                        preferred_element_type=f32)

        def stage_b(j):
            fl = fill_ref[...]
            sc = jnp.where(fl == 0.0, scores.pop(j) * (scale * LOG2E), fl)
            e = jnp.exp2(sc - jnp.max(sc, axis=-1, keepdims=True))
            den = jnp.sum(e, axis=-1, keepdims=True)
            probs[j] = (e * pl.reciprocal(den, approx=True)).astype(bf16)

        def stage_c(j):
            o = jnp.dot(probs[j], gather(2, j), preferred_element_type=f32)
            for p in range(2):
                hh = 2 * j + p
                lo_cur[hh, pl.ds(0, 16), :] = pltpu.bitcast(o[p * SEG:(p + 1) * SEG].astype(bf16), u32)
                ob = o[2 * SEG + p * PRE:2 * SEG + (p + 1) * PRE]
                if odd == 0:
                    lo0[hh, pl.ds(16, 8), :] = pltpu.bitcast(ob, u32)
                else:
                    pr = jnp.concatenate([pltpu.bitcast(lo0[hh, pl.ds(16, 8), :], f32), ob], axis=0)
                    lo1[hh, pl.ds(16, 8), :] = pltpu.bitcast(pr.astype(bf16), u32)

        acc = [None] * 8

        def stage_d(h0, h1, last=False):
            lhs = jnp.concatenate([pltpu.bitcast(lo_cur[hh, pl.ds(0, 16 + 8 * odd), :], bf16)
                                   for hh in range(h0, h1)], axis=1)
            for c in range(8):
                w = pltpu.bitcast(wo[c, pl.ds(h0 * 64, (h1 - h0) * 64), :], bf16)
                res = jnp.dot(lhs, w, preferred_element_type=f32)
                acc[c] = res if acc[c] is None else acc[c] + res
                if not last:
                    fence(res[:M], (h1 - h0) / 8.0 * (DW_ODD if odd else 1.0))
                else:
                    rb = acc[c].astype(bf16)
                    cols = pl.ds(c * 128, 128)
                    h_ref[pl.ds(0, M), cols] = rb[:M]
                    outs[pl.ds(base + (odd * SEG + PRE), TOK), cols] = rb[M:SEG]
                    if odd:
                        outs[pl.ds(base, PRE), cols] = rb[SEG:SEG + PRE]
                        outs[pl.ds(base + SEG, PRE), cols] = rb[SEG + PRE:]

        def attn_group(jq, jc):
            for j in jq:
                stage_qk(j)
            for j in jc:
                stage_c(j)
            for j in jq:
                stage_b(j)

        for t in range(2):
            _inv_piece(cprev, 2 * r + t, 1 - buf, g_ref, us, vec, yf, outb)
        for p in fwd:
            p()
        for j in range(NP):
            stage_a(j)
            if j >= 2 and j % 2 == 0:
                attn_group((j - 2, j - 1), (j - 4, j - 3) if j >= 4 else ())
        stage_d(0, 8)
        attn_group((14, 15), (12, 13))
        stage_d(8, 20)
        attn_group((), (14, 15))
        stage_d(20, 28)
        stage_d(28, 32, last=True)

    def two_steps(i, carry):
        ct = i >> 2
        cprev = (ct + NT - 1) & (NT - 1)
        conv = [_conv_pieces(ct, (i & 3, odd), ct & 1, fs_ref, us, taps, vm, yf,
                             zrow[1] if DONE_M else None) for odd in range(2)]
        kgen = [_kgen_pieces((ct + 1) & (NT - 1), (i & 3, odd), par, vb, taps, ct + 1,
                             zrow[1] if DONE_K else None, KNI, KSPLIT) for odd in range(2)]
        work = {'k0': (kgen[0], vb), 'k1': (kgen[1], vb), 'm0': (conv[0][1], vm), 'm1': (conv[1][1], vm)}
        fence = Pacer([work[k] + (t0, t1) for (k, t0, t1) in PLAN if k[0] not in NOB])
        for odd in range(2):
            one_step(i, odd, conv[odd][0], fence)
        assert fence.finished() or NOB
        outa_cp(pl.multiple_of(2 * SEG * i, 2 * SEG), 2 * SEG).start()
        outb_cp(cprev, pl.multiple_of((i & 3) * 256, 256), 256, jnp.where(i < 4, 2, 1)).start()
        return carry

    with jax.named_scope("steps"):
        if NITER:
            lax.fori_loop(0, NITER, two_steps, 0)

    with jax.named_scope("flush"):
        outb_cp(NT - 1, 0, L // 2, 2).wait()
        for b in range(NBLK):
            _inv_piece(NT - 1, b, (NT - 1) % 2, g_ref, us, vec, yf, outb)
            if b % 4 == 3:
                outb_cp(NT - 1, (b - 3) * 64, 256, 1).start()
    with jax.named_scope("waitout"):
        outa_cp(0, S).wait()
        pltpu.make_async_copy(outb, outb, sem_out.at[1]).wait()


@functools.partial(jax.jit, static_argnames=("A_seg_len",))
def pallas_concat_heads__memory_aug_recurrent_mem_tr__ssm_conv_s4__prompt_kernel(
    A_x, A_mem0, A_Wq, A_Wk, A_Wv, A_Wo, A_seg_len,
    B_u, B_A_re, B_A_im, B_B_re, B_B_im, B_C_re, B_C_im, B_log_dt, B_Dskip,
):
    assert A_seg_len == SEG and A_x.shape == (1, S, DM) and B_u.shape == (1, L, D)
    fs, g = _dft_consts()
    w4 = lambda w: w.reshape(DM // 2, 2, H, E)
    any_ = pl.BlockSpec(memory_space=pl.ANY)
    V = pltpu.VMEM
    out = pl.pallas_call(
        _kernel,
        out_shape=jax.ShapeDtypeStruct((S, DM + D), bf16),
        in_specs=[any_] * 18,
        out_specs=any_,
        scratch_shapes=[
            V((2, NP, DM // 2, E), u32),
            V((2, NP, DM // 2, E), u32),
            V((2, NP, DM // 2, E), u32),
            V((8, H * E // 2, 128), u32),
            V((8, NSEG // 2, PRE, 128), u32),
            V((NSEG // 2, 2, TOK, DM), bf16),
            V((M + TOK, DM), bf16),
            V((S, DM), bf16),
            V((2 * (SEG + M), 2 * (SEG + M)), f32),
            V((6, D, N), bf16),
            V((8 + NT * 6 * N, 128), f32),
            V((NT, L // 2, 128), u32),
            V((NT + 1, TAPROWS, 128), f32),
            V((V_ROWS, 128), f32),
            V((VM_ROWS, 128), f32),
            V((24, 128), f32),
            V((2, T0, 128), f32),
            V((2, NBLK, 128, 128), u32),
            V((NT, L // 2, 128), u32),
            V((2, 8, 128), f32),
            V((2, 8, 128), bf16),
            V((8, NBLK * 32, 128), bf16),
            V((BLK, 256), bf16),
            pltpu.SMEM((8,), jnp.int32),
            pltpu.SemaphoreType.DMA((4,)),
            pltpu.SemaphoreType.DMA((6 * NP,)),
            pltpu.SemaphoreType.DMA((8,)),
            pltpu.SemaphoreType.DMA((16,)),
            pltpu.SemaphoreType.DMA((1,)),
            pltpu.SemaphoreType.DMA((8,)),
            pltpu.SemaphoreType.DMA((NT,)),
            pltpu.SemaphoreType.DMA((3,)),
            V((NSEG, 3 * NP, PRE, E), u32),
            V((3 * NP, SEG, E), u32),
            V((H, 24, E), u32),
            V((H, 24, E), u32),
        ],
        compiler_params=pltpu.CompilerParams(vmem_limit_bytes=110 * 1024 * 1024, disable_bounds_checks=True),
    )(jnp.asarray(np.zeros((8,), np.int32)), A_x.reshape(NSEG // 2, 2, SEG, DM), A_mem0.reshape(M, DM), w4(A_Wq), w4(A_Wk), w4(A_Wv), A_Wo.reshape(H * E, DM),
      B_u.reshape(L, D), B_A_re, B_A_im, B_B_re, B_B_im, B_C_re, B_C_im,
      B_log_dt.reshape(8, 128), B_Dskip.reshape(8, 128),
      jnp.asarray(fs, bf16), jnp.asarray(g, bf16))
    return out.reshape(1, S, DM + D)
```

```python
import functools

import numpy as np
import jax
import jax.numpy as jnp
from jax import lax
import jax.experimental.pallas as pl
import jax.experimental.pallas.tpu as pltpu

bf16, f32, u32 = jnp.bfloat16, jnp.float32, jnp.uint32

S, DM, H, E, M, SEG = 2048, 1024, 32, 128, 8, 32
NSEG = S // SEG
TOK = 24
PRE = SEG - TOK
T0 = PRE * NSEG
NP = H // 2
LOG2E = 1.4426950408889634
QUICK = False
NOB = ''
BKNI = 1
UNP = 64
UNP_FRAC = 0.7
BKSPLIT = 4
BPLAN = (6.0, 7.0, 41.5, 47.7)
BULK_FROM = 0
NITER = NSEG // 2
KNI = 2
KSPLIT = 2
PLAN = (('k0', 0, 96), ('m0', 96, 122), ('k1', 124, 220), ('m1', 220, 260))
DONE_K = True
DONE_M = True
DW_ODD = 1.5
RC = 64
MACJ = 3
NSLOT = 118
L, D, N = 2048, 1024, 128
BLK = 128
NBLK = L // BLK
NT = D // 128
TAPROWS = 672
WINDOWS = ((0, 128, 0, 1), (128, 128, 1, 1), (256, 128, 2, 1), (320, 80, 3, 1),
           (384, 128, 4, 3), (480, 48, 7, 1), (512, 128, 8, 7), (624, 32, 15, 1))

V_FENCE = 0
V_YTAB = 8
V_START = V_YTAB + 256
V_STEP = V_START + 160
V_ROWS = V_STEP + 128
V_UF = 8
V_KF = V_UF + NBLK * 32
VM_ROWS = V_KF + NBLK * 32


def _bf16_round_int(l):
    u = np.asarray(l, np.float32).view(np.uint32)
    r = (u + 0x7FFF + ((u >> 16) & 1)) & 0xFFFF0000
    return r.astype(np.uint32).view(np.float32).astype(np.int64)


def _tap_row(lp):
    return np.where(lp < 256, lp, np.where(lp < 512, 256 + (lp - 256) // 2,
                    np.where(lp < 1024, 384 + (lp - 512) // 4, 512 + (lp - 1024) // 8)))


@functools.lru_cache(maxsize=None)
def _dft_consts():
    t = np.arange(BLK)
    F = np.zeros((8, 32, BLK))
    G = np.zeros((BLK, 8, 32))
    for r in range(8):
        f = np.concatenate([16 * r + 2 * np.arange(8), 16 * r + 2 * np.arange(8) + 1])
        th = 2 * np.pi * (f + 0.5) / (2 * BLK)
        F[r, :16] = np.cos(th[:, None] * t[None])
        F[r, 16:] = -np.sin(th[:, None] * t[None])
        G[:, r, 0::2] = np.cos(th[None] * t[:, None]) / BLK
        G[:, r, 1::2] = -np.sin(th[None] * t[:, None]) / BLK
    FS = np.zeros((8, NBLK, 32, 128))
    for (w0, wn, b0, nb) in WINDOWS:
        for j in range(b0, b0 + nb):
            rows = _tap_row(_bf16_round_int(BLK * j + t)) - w0
            assert rows.min() >= 0 and rows.max() < wn
            sel = np.zeros((BLK, 128))
            sel[t, rows] = 1.0
            FS[:, j] = F @ sel
    return (FS.reshape(8, NBLK * 32, 128).astype(np.float32),
            G.reshape(BLK, 2, 128).transpose(1, 0, 2).astype(np.float32))


def _ld16(ref, *idx):
    return pltpu.bitcast(ref.bitcast(u32)[idx + (slice(None),)], bf16)


def _cmul(a, b):
    return (a[0] * b[0] - a[1] * b[1], a[0] * b[1] + a[1] * b[0])


def _csq(a):
    return (a[0] * a[0] - a[1] * a[1], 2.0 * (a[0] * a[1]))


def _cexp(lr, li):
    k = jnp.floor(li * (2.0 / np.pi) + 0.5)
    r = ((li - k * 1.5703125) - k * 4.837512969970703125e-4) - k * 7.54978995489188216e-8
    r = jnp.clip(r, -0.8, 0.8)
    r2 = r * r
    s = r + r * r2 * (-1.6666654611e-1 + r2 * (8.3321608736e-3 + r2 * -1.9515295891e-4))
    c = (1.0 - 0.5 * r2) + (r2 * r2) * (4.166664568298827e-2
                                        + r2 * (-1.388731625493765e-3 + r2 * 2.443315711809948e-5))
    q = k.astype(jnp.int32)
    swap = (q & 1) == 1
    m = jnp.exp(lr)
    flip = lambda v, bit: pltpu.bitcast(pltpu.bitcast(v, jnp.int32) ^ (bit << 30), f32)
    return (flip(m * jnp.where(swap, s, c), (q + 1) & 2), flip(m * jnp.where(swap, c, s), q & 2))


def _par_row(c, k):
    return 8 + (c * 6 + k) * N


def _prep_pieces(praw, vec, par):
    def stage1(c):
        def fn():
            tr = lambda k: praw[k, pl.ds(c * 128, 128), :].astype(f32).T
            dt = jnp.exp(vec[0, pl.ds(c, 1), :]).astype(bf16).astype(f32)
            cc = _cmul((tr(4), tr(5)), (dt * tr(2), dt * tr(3)))
            for k, v in ((0, dt * tr(0)), (1, dt * tr(1)), (4, cc[0]), (5, cc[1])):
                par[pl.ds(_par_row(c, k), N), :] = v
        return fn

    def stage2(c, n0):
        def fn():
            lr = par[pl.ds(_par_row(c, 0) + n0, 16), :]
            li = par[pl.ds(_par_row(c, 1) + n0, 16), :]
            for k, v in enumerate(_cexp(lr, li) + _cexp(lr * 128.0, li * 128.0)):
                par[pl.ds(_par_row(c, k) + n0, 16), :] = v
        return fn

    tile = lambda c: [(260, stage1(c))] + [(190, stage2(c, n0)) for n0 in range(0, N, 16)]
    return tile(0), [pc for c in range(1, NT) for pc in tile(c)]


def _kgen_pieces(c, r, par, vb, taps, tslot, frow, kni, ksplit):
    st = {}

    def put(row, z, h=None):
        if h is None:
            vb[pl.ds(row, 16), :] = z[0]
            vb[pl.ds(row + 16, 16), :] = z[1]
        else:
            vb[pl.ds(row + 8 * h, 8), :] = z[0]
            vb[pl.ds(row + 16 + 8 * h, 8), :] = z[1]

    def get(row, h=None):
        if h is None:
            return (vb[pl.ds(row, 16), :], vb[pl.ds(row + 16, 16), :])
        return (vb[pl.ds(row + 8 * h, 8), :], vb[pl.ds(row + 16 + 8 * h, 8), :])

    def params(k):
        if isinstance(r, int):
            return par[pl.ds(_par_row(c, k) + r * 16, 16), :]
        return par[pl.ds(pl.multiple_of(c * (6 * N) + r[0] * 32, 32) + (_par_row(0, k) + r[1] * 16), 16), :]

    def park():
        put(V_STEP, (params(0), params(1)))
        put(V_START + 32, (params(2), params(3)))
        put(V_START, (params(4), params(5)))

    def setup_y(h):
        def fn():
            z1 = get(V_STEP, h)
            z2 = _csq(z1)
            z4 = _csq(z2)
            s = lax.broadcasted_iota(jnp.int32, (8, 128), 0)
            fs = [(jnp.where((s >> k) & 1 == 1, z[0], 1.0), jnp.where((s >> k) & 1 == 1, z[1], 0.0))
                  for k, z in enumerate((z1, z2, z4))]
            y = _cmul(_cmul(fs[0], fs[1]), fs[2])
            for k in range(8):
                put(V_YTAB + 32 * k, y, h)
                if k < 7:
                    y = _cmul(y, z1)
                    y = (jnp.where(s == 7 - k, 1.0, y[0]), jnp.where(s == 7 - k, 0.0, y[1]))
            z = z4
            for k in range(4):
                z = _csq(z)
                put(V_STEP + 32 * k, z, h)
        return fn

    def setup_hi():
        z = get(V_START + 32)
        cf = get(V_START)
        for g in range(1, 5):
            put(V_START + 32 * g, _cmul(cf, z))
            if g < 4:
                z = _csq(z)

    def square(k0, k1):
        def fn():
            for k in range(k0, k1):
                put(V_YTAB + 32 * k, _csq(get(V_YTAB + 32 * k)))
        return fn

    def rows_of(g, i0, ni):
        n_i = 16 + (g == 4)

        def fn():
            x = st.pop('x') if i0 > 0 else get(V_START + 32 * g)
            step = get(V_STEP + 32 * max(g - 1, 0))
            xs = []
            for t in range(ni):
                xs.append(x)
                if i0 + t + 1 < n_i:
                    x = _cmul(x, step)
            if i0 + ni < n_i:
                st['x'] = x
            acc = [None] * ni
            for k in range(8):
                yr, yi = get(V_YTAB + 32 * k)
                for t in range(ni):
                    v = xs[t][0] * yr - xs[t][1] * yi
                    v = v[:8] + v[8:]
                    if k:
                        v = pltpu.roll(v, k, 0)
                    acc[t] = v if acc[t] is None else acc[t] + v
                if frow is not None and k % ksplit == ksplit - 1 and k < 7:
                    vb[pl.ds(frow, 8), :] = acc[ni - 1]
            for t in range(ni):
                row = 128 * g + 8 * (i0 + t)
                a = acc[t]
                if row == 640:
                    a = jnp.where(lax.broadcasted_iota(jnp.int32, (8, 128), 0) == 0, a, 0.0)
                taps[tslot, pl.ds(row, 8), :] = taps[tslot, pl.ds(row, 8), :] + a
                if frow is not None and t == ni - 1:
                    vb[pl.ds(frow, 8), :] = a
        return fn

    pieces = [(30, park), (110, setup_y(0)), (110, setup_y(1)), (80, setup_hi)]
    for g in range(5):
        if g >= 2:
            pieces += [(40, square(0, 4)), (40, square(4, 8))]
        for i0 in range(0, 16 + (g == 4), kni):
            ni = min(kni, 16 + (g == 4) - i0)
            pieces.append((83 * ni, rows_of(g, i0, ni)))
    return pieces


def _conv_pieces(c, r, buf, fs_ref, us, taps, vb, yf, frow):
    st = {}

    def fwd_u(b0, b1):
        def fn():
            lhs = _ld16(fs_ref, 2 * r[0] + r[1], pl.ds(0, 16))
            for b in range(b0, b1):
                w = pltpu.bitcast(us[c, pl.ds(b * 64, 64), :], bf16)
                res = jnp.dot(lhs, w, preferred_element_type=f32)
                row = V_UF + 32 * b
                if b == 0:
                    vb[pl.ds(row, 32), :] = res
                else:
                    p = st['prev']
                    vb[pl.ds(row, 8), :] = res[0:8] - p[16:24]
                    vb[pl.ds(row + 8, 8), :] = res[8:16] + p[24:32]
                    vb[pl.ds(row + 16, 8), :] = res[16:24] + p[0:8]
                    vb[pl.ds(row + 24, 8), :] = res[24:32] - p[8:16]
                st['prev'] = res
        return fn

    def fwd_k(jobs):
        def fn():
            for (wi, t0, nb) in jobs:
                w0, wn, b0, _ = WINDOWS[wi]
                lhs = _ld16(fs_ref, 2 * r[0] + r[1], pl.ds((b0 + t0) * 16, nb * 16))[:, :wn]
                w = taps[c, pl.ds(w0, wn), :].astype(bf16)
                vb[pl.ds(V_KF + 32 * (b0 + t0), 32 * nb), :] = jnp.dot(lhs, w, preferred_element_type=f32)
        return fn

    def mac(q, i0, ni, j0, j1):
        def fn():
            ld = lambda base, b: (vb[pl.ds(base + 32 * b + 8 * q, 8), :], vb[pl.ds(base + 32 * b + 16 + 8 * q, 8), :])
            zr, zi = st.pop('z') if j0 > 0 else ({}, {})
            ucache = {}
            for j in range(j0, j1):
                kr, ki = ld(V_KF, j)
                for i in range(max(i0, j), i0 + ni):
                    if i - j not in ucache:
                        ucache[i - j] = ld(V_UF, i - j)
                    ur, ui = ucache[i - j]
                    if i not in zr:
                        zr[i] = kr * ur - ki * ui
                        zi[i] = kr * ui + ki * ur
                    else:
                        zr[i] = zr[i] + kr * ur - ki * ui
                        zi[i] = zi[i] + kr * ui + ki * ur
            if frow is not None:
                vb[pl.ds(frow, 8), :] = zr[i0 + ni - 1]
            if j1 < i0 + ni:
                st['z'] = (zr, zi)
            else:
                row = pl.multiple_of(r[0] * 32, 32) + (r[1] * 16 + q * 8)
                for i in range(i0, i0 + ni):
                    yf[buf, i, pl.ds(row, 8), :] = pltpu.pack_elementwise([zr[i], zi[i]], packed_dtype=bf16)
        return (8 * sum(1 for j in range(j0, j1) for i in range(max(i0, j), i0 + ni)), fn)

    fwd = [fwd_u(0, 8), fwd_u(8, 16), fwd_k(((0, 0, 1), (1, 0, 1), (2, 0, 1), (3, 0, 1))),
           fwd_k(((4, 0, 2), (6, 0, 2), (6, 2, 2), (6, 4, 2))), fwd_k(((4, 2, 1), (5, 0, 1), (6, 6, 1), (7, 0, 1)))]
    macs = []
    for q in range(2):
        for i0 in range(0, NBLK, 2):
            for j0 in range(0, i0 + 2, MACJ):
                macs.append(mac(q, i0, 2, j0, min(j0 + MACJ, i0 + 2)))
    return fwd, macs


def _inv_piece(c, b, buf, g_ref, us, vec, yf, outb):
    rows = pl.ds(pl.multiple_of(b * 64, 64), 64)
    w = pltpu.bitcast(yf[buf, b], bf16)
    g = jnp.concatenate([_ld16(g_ref, k, slice(None)) for k in range(2)], axis=1)
    y = jnp.dot(g, w, preferred_element_type=f32)
    u = pltpu.bitcast(us[c, rows, :], bf16).astype(f32)
    sk = (u * vec[1, pl.ds(c, 1), :]).astype(bf16).astype(f32)
    o = (y.astype(bf16).astype(f32) + sk).astype(bf16)
    outb[c, pl.ds(pl.multiple_of(b * BLK, BLK) if not isinstance(b, int) else b * BLK, BLK), :] = o


def _attn_fill():
    n = 2 * (SEG + M)
    r = lax.broadcasted_iota(jnp.int32, (n, n), 0)
    c = lax.broadcasted_iota(jnp.int32, (n, n), 1)
    head = lambda i: jnp.where(i < 2 * SEG, i // SEG, (i - 2 * SEG) // PRE)
    pos = lambda i: jnp.where(i < 2 * SEG, i % SEG, i % PRE)
    is_mem = lambda i: (i < 2 * SEG) & (i % SEG < M)
    same = head(r) == head(c)
    allowed = same & (is_mem(r) | is_mem(c) | (pos(r) >= pos(c)))
    return jnp.where(allowed, 0.0, jnp.where(same, -1e9 * LOG2E, -jnp.inf)).astype(f32)


def _kernel(zero_hbm, x_hbm, mem0_hbm, wq_hbm, wk_hbm, wv_hbm, wo_hbm,
            u_hbm, p0, p1, p2, p3, p4, p5, ldt_hbm, dsk_hbm, fs_hbm, g_hbm,
            out_hbm,
            wq, wk, wv, wo, xb, xs, h_ref, outs, fill_ref,
            praw, par, us, taps, vb, vm, vu, pacc, yf, outb, vec, vraw, fs_ref, g_ref, zero_ref,
            sem_s, sem_w, sem_o, sem_xb, sem_x, sem_p, sem_u, sem_out, pre, own, lo0, lo1):
    wqkv = (wq, wk, wv)
    scale = E ** -0.5

    whbm = [w.bitcast(u32) for w in (wq_hbm, wk_hbm, wv_hbm)]

    def wcp(j, m, p):
        return pltpu.make_async_copy(whbm[m].at[:, p, j, :], wqkv[m].at[p, j], sem_w.at[(j * 3 + m) * 2 + p])

    xu = x_hbm.bitcast(u32)
    xcs = [pltpu.make_async_copy(xu.at[:, t, pl.ds(0, PRE // 2), pl.ds(c * 128, 128)],
                                 xb.at[c, :, pl.ds(t * (PRE // 2), PRE // 2), :], sem_xb.at[2 * c + t])
           for c in range(8) for t in range(2)]
    xcp1 = pltpu.make_async_copy(x_hbm.at[:, :, pl.ds(PRE, TOK), :], xs, sem_x.at[0])
    pcs = [pltpu.make_async_copy(p, praw.at[k], sem_p.at[k]) for k, p in enumerate((p0, p1, p2, p3, p4, p5))]
    ccs = [pltpu.make_async_copy(fs_hbm, fs_ref, sem_p.at[6]), pltpu.make_async_copy(g_hbm, g_ref, sem_p.at[7])]
    wou = wo_hbm.bitcast(u32)
    ocs = [pltpu.make_async_copy(wou.at[:, pl.ds(c * 128, 128)], wo.at[c], sem_o.at[c]) for c in range(8)]
    uu = u_hbm.bitcast(u32)
    ucs = [pltpu.make_async_copy(uu.at[:, pl.ds(c * 128, 128)], us.at[c], sem_u.at[c]) for c in range(NT)]

    zcp = pltpu.make_async_copy(zero_hbm, zero_ref, sem_s.at[0])
    scs = [pltpu.make_async_copy(mem0_hbm, h_ref.at[pl.ds(0, M)], sem_s.at[1]),
           pltpu.make_async_copy(ldt_hbm, vraw.at[0], sem_s.at[2]),
           pltpu.make_async_copy(dsk_hbm, vraw.at[1], sem_s.at[3])]
    for cp in [zcp] + xcs + [wcp(0, 0, 0), wcp(0, 0, 1)]:
        cp.start()
    vu[pl.ds(8, 8), :] = pltpu.bitcast(jnp.full((8, 128), 0x0000FFFF, u32), f32)
    vu[pl.ds(16, 8), :] = pltpu.bitcast(jnp.full((8, 128), 0xFFFF0000, u32), f32)
    taps[...] = jnp.zeros(taps.shape, f32)
    yf[1] = jnp.zeros(yf.shape[1:], u32)
    fill_ref[...] = _attn_fill()
    for cp in [wcp(0, 1, 0), wcp(0, 1, 1)] + scs:
        cp.start()
    zcp.wait()

    frow = pl.multiple_of(zero_ref[0] * 8, 8)
    zrow = [pl.multiple_of(zero_ref[k] * 8, 8) for k in range(T0 // RC)]

    class Pacer:
        def __init__(self, segments):
            self.t = 0.0
            self.todo = []
            for (pieces, buf, t0, t1) in segments:
                total = float(sum(c for c, _ in pieces))
                done = 0.0
                for (cst, fn) in pieces:
                    self.todo.append((t0 + (t1 - t0) * done / total, fn, buf))
                    done += cst

        def __call__(self, v, dt=1.0):
            self.t += dt
            fenced = []
            while self.todo and self.todo[0][0] < self.t:
                _, fn, buf = self.todo.pop(0)
                if not any(b is buf for b in fenced):
                    buf[pl.ds(frow, 8), :] = v
                    fenced.append(buf)
                fn()

        def finished(self):
            return not self.todo

    def make_fence(vpu, nslot, buf=vb):
        pc = Pacer([(vpu, buf, 0.0, float(nslot))])
        return pc, pc.finished

    def unpair(j, m, r0, nr):
        def fn():
            rows = pl.ds(r0, nr)
            m_lo = jnp.tile(pltpu.bitcast(vu[pl.ds(8, 8), :], u32), (nr // 8, 1))
            m_hi = jnp.tile(pltpu.bitcast(vu[pl.ds(16, 8), :], u32), (nr // 8, 1))
            a = wqkv[m][0, j, rows, :]
            b = wqkv[m][1, j, rows, :]
            wqkv[m][0, j, rows, :] = (a & m_lo) | ((b & m_lo) << 16)
            wqkv[m][1, j, rows, :] = ((a & m_hi) >> 16) | (b & m_hi)
        return (nr, fn)

    def unpair_pieces(items):
        return [unpair(j, m, r0, UNP) for (j, m) in items for r0 in range(0, DM // 2, UNP)]

    items = [(j, m) for j in range(NP) for m in range(3)]
    wcs = lambda lo, hi: [wcp(j, m, p) for (j, m) in items[lo:hi] for p in range(2)]
    plan = {
        0: ((1, 2), wcs(2, 4), []),
        1: ((2, 4), wcs(4, 7), []),
        3: ((4, 7), pcs + wcs(7, 12), []),
        6: ((7, 12), wcs(12, 21), pcs + scs),
        11: ((12, 21), wcs(21, 33), []),
        20: ((21, 33), wcs(33, 48) + ocs[:4], []),
        32: ((33, 48), ocs[4:] + ucs + [xcp1] + ccs, []),
    }
    with jax.named_scope("bulk"):
        with jax.named_scope("waitx"):
            for cp in xcs + wcs(0, 1):
                cp.wait()
        for _, fn in unpair_pieces(items[0:1]):
            fn()
        points = sorted(plan) + [len(items)]
        if QUICK in (1, 2):
            for cp in wcs(2, 48) + pcs + ocs + ucs + [xcp1] + ccs:
                cp.start()
            for cp in wcs(1, 48) + pcs + scs:
                cp.wait()
            vec[...] = vraw[...].astype(f32)
            for _, fn in (unpair_pieces(items[1:]) + sum(_prep_pieces(praw, vec, par), [])) if QUICK != 2 else []:
                fn()

            def kg(r, carry):
                for odd in range(2):
                    for _, fn in _kgen_pieces(0, (r, odd), par, vb, taps, 0, zrow[1], BKNI, BKSPLIT):
                        fn()
                return carry
            lax.fori_loop(0, 4, kg, 0)
            for (j, m) in (items if QUICK != 2 else []):
                def chunk(rc, carry, j=j, m=m):
                    lhs = jnp.concatenate(
                        [pltpu.bitcast(xb[c, pl.ds(rc * 4, 4)].reshape(32, 128), bf16) for c in range(8)], axis=1)
                    res = [jnp.dot(lhs, pltpu.bitcast(wqkv[m][p, j], bf16), preferred_element_type=f32)
                           for p in range(2)]
                    for t in range(8):
                        v = jnp.concatenate([res[0][8 * t:8 * t + 8], res[1][8 * t:8 * t + 8]], axis=0)
                        pre[rc * 8 + t, m * NP + j] = v.astype(bf16)
                    return carry
                lax.fori_loop(0, 8, chunk, 0)
            points = []
        n_chunk = 2 * (T0 // RC)
        prep = _prep_pieces(praw, vec, par)
        kg0 = [pc for r in range(8) for pc in _kgen_pieces(0, r, par, vb, taps, 0, zrow[1], BKNI, BKSPLIT)]
        t_a, t_b, t_c, t_d = [v * n_chunk for v in BPLAN]
        fence_x = Pacer([(prep[0], par, t_a, t_b), (kg0, vb, t_b, t_c), (prep[1], par, t_c, t_d)])
        fence_x.t = float(BULK_FROM * n_chunk)
        for g in range(len(points) - 1):
            lo, hi = points[g], points[g + 1]
            (w_lo, w_hi), starts, waits = plan[lo]
            for cp in starts:
                cp.start()
            with jax.named_scope("wait%d" % lo):
                for cp in wcs(w_lo, w_hi) + waits:
                    cp.wait()
            assert w_hi == min(hi + 1, len(items))
            if lo == 6:
                vec[...] = vraw[...].astype(f32)
            if lo < BULK_FROM:
                continue
            for it in range(lo, hi):
                j, m = items[it]
                fence_w, fin_w = make_fence(unpair_pieces(items[it + 1:it + 2]), n_chunk * UNP_FRAC, vu)
                for p in range(2):
                    for half in range(2):
                        w = pltpu.bitcast(wqkv[m][p, j, pl.ds(half * (DM // 4), DM // 4), :], bf16)
                        lhs = jnp.concatenate([pltpu.bitcast(xb[c].reshape(T0 // 2, 128), bf16)
                                               for c in range(4 * half, 4 * half + 4)], axis=1)
                        res = jnp.dot(lhs, w, preferred_element_type=f32)
                        for rc in range(T0 // RC):
                            rows = pl.ds(rc * RC, RC)
                            v = res[rc * RC:(rc + 1) * RC]
                            if half == 1:
                                v = v + pacc[p, rows, :]
                            if p == 0 or half == 0:
                                pacc[p, rows, :] = v
                            else:
                                v0 = pacc[0, rows, :]
                                for t in range(RC // PRE):
                                    pr = jnp.concatenate([v0[PRE * t:PRE * (t + 1)], v[PRE * t:PRE * (t + 1)]], axis=0)
                                    pre[rc * (RC // PRE) + t, m * NP + j] = pr.astype(bf16)
                            fence_w(v[:8], 0.5)
                            fence_x(v[:8], 0.5)
                assert fin_w()
        assert QUICK or BULK_FROM or fence_x.finished()
    with jax.named_scope("waitrest"):
        for cp in ocs + ucs + ccs + [xcp1]:
            cp.wait()

    def outa_cp(row, n):
        return pltpu.make_async_copy(outs.at[pl.ds(row, n)], out_hbm.at[pl.ds(row, n), pl.ds(0, DM)], sem_out.at[0])

    def outb_cp(c, row, n, sem):
        col = DM + c * 128
        return pltpu.make_async_copy(
            outb.at[c, pl.ds(row, n)],
            out_hbm.at[pl.ds(row, n), pl.ds(col if isinstance(col, int) else pl.multiple_of(col, 128), 128)],
            sem_out.at[sem])

    def one_step(i, odd, fwd, fence):
        s = 2 * i + odd
        lo_cur = (lo0, lo1)[odd]
        base = pl.multiple_of(2 * SEG * i, 2 * SEG)
        h_ref[pl.ds(M, TOK), :] = xs[i, odd]
        h = h_ref[...]
        scores = {}
        probs = {}
        zown = 0

        ct = i >> 2
        r = s & 7
        buf = ct & 1
        cprev = (ct + NT - 1) & (NT - 1)

        def stage_a(j):
            for m in range(3):
                for p in range(2):
                    w = pltpu.bitcast(wqkv[m][p, j], bf16)
                    res = jnp.dot(h, w, preferred_element_type=f32)
                    own[m * NP + j, pl.ds(SEG * p, SEG), :] = res.astype(bf16)
                    fence(res[:M])

        def gather(m, j):
            return pltpu.bitcast(jnp.concatenate([own.bitcast(u32)[m * NP + j + zown],
                                                  pre.bitcast(u32)[s, m * NP + j]], axis=0), bf16)

        def stage_qk(j):
            scores[j] = lax.dot_general(gather(0, j), gather(1, j), (((1,), (1,)), ((), ())),
                                        preferred_element_type=f32)

        def stage_b(j):
            fl = fill_ref[...]
            sc = jnp.where(fl == 0.0, scores.pop(j) * (scale * LOG2E), fl)
            e = jnp.exp2(sc - jnp.max(sc, axis=-1, keepdims=True))
            den = jnp.sum(e, axis=-1, keepdims=True)
            probs[j] = (e * pl.reciprocal(den, approx=True)).astype(bf16)

        def stage_c(j):
            o = jnp.dot(probs[j], gather(2, j), preferred_element_type=f32)
            for p in range(2):
                hh = 2 * j + p
                lo_cur[hh, pl.ds(0, SEG), :] = o[p * SEG:(p + 1) * SEG].astype(bf16)
                ob = o[2 * SEG + p * PRE:2 * SEG + (p + 1) * PRE]
                lo1[hh, pl.ds(SEG + odd * PRE, PRE), :] = ob.astype(bf16)

        acc = [None] * 8

        def stage_d(h0, h1, last=False):
            lhs = jnp.concatenate([_ld16(lo_cur, hh, slice(None)) for hh in range(h0, h1)], axis=1)
            for c in range(8):
                w = pltpu.bitcast(wo[c, pl.ds(h0 * 64, (h1 - h0) * 64), :], bf16)
                res = jnp.dot(lhs, w, preferred_element_type=f32)
                acc[c] = res if acc[c] is None else acc[c] + res
                if not last:
                    fence(res[:M], (h1 - h0) / 8.0 * (DW_ODD if odd else 1.0))
                else:
                    rb = acc[c].astype(bf16)
                    cols = pl.ds(c * 128, 128)
                    h_ref[pl.ds(0, M), cols] = rb[:M]
                    outs[pl.ds(base + (odd * SEG + PRE), TOK), cols] = rb[M:SEG]
                    if odd:
                        outs[pl.ds(base, PRE), cols] = rb[SEG:SEG + PRE]
                        outs[pl.ds(base + SEG, PRE), cols] = rb[SEG + PRE:]

        def attn_group(jq, jc):
            for j in jq:
                stage_qk(j)
            for j in jc:
                stage_c(j)
            for j in jq:
                stage_b(j)

        for t in range(2):
            _inv_piece(cprev, 2 * r + t, 1 - buf, g_ref, us, vec, yf, outb)
        for p in fwd:
            p()
        for j in range(NP):
            stage_a(j)
            if j >= 2 and j % 2 == 0:
                attn_group((j - 2, j - 1), (j - 4, j - 3) if j >= 4 else ())
        stage_d(0, 8)
        attn_group((14, 15), (12, 13))
        stage_d(8, 20)
        attn_group((), (14, 15))
        stage_d(20, 28)
        stage_d(28, 32, last=True)

    def two_steps(i, carry):
        ct = i >> 2
        cprev = (ct + NT - 1) & (NT - 1)
        conv = [_conv_pieces(ct, (i & 3, odd), ct & 1, fs_ref, us, taps, vm, yf,
                             zrow[1] if DONE_M else None) for odd in range(2)]
        kgen = [_kgen_pieces((ct + 1) & (NT - 1), (i & 3, odd), par, vb, taps, ct + 1,
                             zrow[1] if DONE_K else None, KNI, KSPLIT) for odd in range(2)]
        work = {'k0': (kgen[0], vb), 'k1': (kgen[1], vb), 'm0': (conv[0][1], vm), 'm1': (conv[1][1], vm)}
        fence = Pacer([work[k] + (t0, t1) for (k, t0, t1) in PLAN if k[0] not in NOB])
        for odd in range(2):
            one_step(i, odd, conv[odd][0], fence)
        assert fence.finished() or NOB
        outa_cp(pl.multiple_of(2 * SEG * i, 2 * SEG), 2 * SEG).start()
        outb_cp(cprev, pl.multiple_of((i & 3) * 512, 512), 512, jnp.where(i < 4, 2, 1)).start()
        return carry

    with jax.named_scope("steps"):
        if NITER:
            lax.fori_loop(0, NITER, two_steps, 0)

    with jax.named_scope("flush"):
        outb_cp(NT - 1, 0, L, 2).wait()
        for b in range(NBLK):
            _inv_piece(NT - 1, b, (NT - 1) % 2, g_ref, us, vec, yf, outb)
            if b % 4 == 3:
                outb_cp(NT - 1, (b - 3) * BLK, 4 * BLK, 1).start()
    with jax.named_scope("waitout"):
        outa_cp(0, S).wait()
        pltpu.make_async_copy(outb, outb, sem_out.at[1]).wait()


@functools.partial(jax.jit, static_argnames=("A_seg_len",))
def pallas_concat_heads__memory_aug_recurrent_mem_tr__ssm_conv_s4__prompt_kernel(
    A_x, A_mem0, A_Wq, A_Wk, A_Wv, A_Wo, A_seg_len,
    B_u, B_A_re, B_A_im, B_B_re, B_B_im, B_C_re, B_C_im, B_log_dt, B_Dskip,
):
    assert A_seg_len == SEG and A_x.shape == (1, S, DM) and B_u.shape == (1, L, D)
    fs, g = _dft_consts()
    w4 = lambda w: w.reshape(DM // 2, 2, H, E)
    any_ = pl.BlockSpec(memory_space=pl.ANY)
    V = pltpu.VMEM
    out = pl.pallas_call(
        _kernel,
        out_shape=jax.ShapeDtypeStruct((S, DM + D), bf16),
        in_specs=[any_] * 18,
        out_specs=any_,
        scratch_shapes=[
            V((2, NP, DM // 2, E), u32),
            V((2, NP, DM // 2, E), u32),
            V((2, NP, DM // 2, E), u32),
            V((8, H * E // 2, 128), u32),
            V((8, NSEG // 2, PRE, 128), u32),
            V((NSEG // 2, 2, TOK, DM), bf16),
            V((M + TOK, DM), bf16),
            V((S, DM), bf16),
            V((2 * (SEG + M), 2 * (SEG + M)), f32),
            V((6, D, N), bf16),
            V((8 + NT * 6 * N, 128), f32),
            V((NT, L // 2, 128), u32),
            V((NT + 1, TAPROWS, 128), f32),
            V((V_ROWS, 128), f32),
            V((VM_ROWS, 128), f32),
            V((24, 128), f32),
            V((2, T0, 128), f32),
            V((2, NBLK, 128, 128), u32),
            V((NT, L, 128), bf16),
            V((2, 8, 128), f32),
            V((2, 8, 128), bf16),
            V((8, NBLK * 32, 128), bf16),
            V((2, BLK, 128), bf16),
            pltpu.SMEM((8,), jnp.int32),
            pltpu.SemaphoreType.DMA((4,)),
            pltpu.SemaphoreType.DMA((6 * NP,)),
            pltpu.SemaphoreType.DMA((8,)),
            pltpu.SemaphoreType.DMA((16,)),
            pltpu.SemaphoreType.DMA((1,)),
            pltpu.SemaphoreType.DMA((8,)),
            pltpu.SemaphoreType.DMA((NT,)),
            pltpu.SemaphoreType.DMA((3,)),
            V((NSEG, 3 * NP, 2 * PRE, E), bf16),
            V((3 * NP, 2 * SEG, E), bf16),
            V((H, SEG, E), bf16),
            V((H, SEG + 2 * PRE, E), bf16),
        ],
        compiler_params=pltpu.CompilerParams(vmem_limit_bytes=110 * 1024 * 1024, disable_bounds_checks=True),
    )(jnp.asarray(np.zeros((8,), np.int32)), A_x.reshape(NSEG // 2, 2, SEG, DM), A_mem0.reshape(M, DM), w4(A_Wq), w4(A_Wk), w4(A_Wv), A_Wo.reshape(H * E, DM),
      B_u.reshape(L, D), B_A_re, B_A_im, B_B_re, B_B_im, B_C_re, B_C_im,
      B_log_dt.reshape(8, 128), B_Dskip.reshape(8, 128),
      jnp.asarray(fs, bf16), jnp.asarray(g, bf16))
    return out.reshape(1, S, DM + D)
```

```python
import functools

import numpy as np
import jax
import jax.numpy as jnp
from jax import lax
import jax.experimental.pallas as pl
import jax.experimental.pallas.tpu as pltpu

bf16, f32, u32 = jnp.bfloat16, jnp.float32, jnp.uint32

S, DM, H, E, M, SEG = 2048, 1024, 32, 128, 8, 32
NSEG = S // SEG
TOK = 24
PRE = SEG - TOK
T0 = PRE * NSEG
NP = H // 2
LOG2E = 1.4426950408889634
QUICK = False
NOB = ''
BKNI = 1
UNP = 64
UNP_FRAC = 0.7
BKSPLIT = 4
BPLAN = (10.0, 11.0, 42.5, 47.7)
WAITS = {1: 2, 2: 3, 3: 5, 4: 6, 5: 8, 7: 11, 10: 13, 12: 17, 16: 23, 22: 33, 32: 48}
PAR_WAIT = 10
STARTS = {0: (2, False, 0), 1: (3, False, 0), 2: (5, False, 0), 4: (6, False, 0), 6: (8, False, 0),
          8: (9, False, 0), 10: (11, False, 0), 14: (13, True, 0), 20: (17, False, 0), 24: (23, False, 0),
          32: (33, False, 0), 44: (48, False, 3), 64: (48, False, 19)}
NITER = NSEG // 2
KNI = 2
KSPLIT = 2
PLAN = (('k0', 0, 96), ('m0', 96, 122), ('k1', 124, 220), ('m1', 220, 260))
DONE_K = True
DONE_M = True
DW_ODD = 1.5
RC = 64
MACJ = 3
NSLOT = 118
L, D, N = 2048, 1024, 128
BLK = 128
NBLK = L // BLK
NT = D // 128
TAPROWS = 672
WINDOWS = ((0, 128, 0, 1), (128, 128, 1, 1), (256, 128, 2, 1), (320, 80, 3, 1),
           (384, 128, 4, 3), (480, 48, 7, 1), (512, 128, 8, 7), (624, 32, 15, 1))

V_FENCE = 0
V_YTAB = 8
V_START = V_YTAB + 256
V_STEP = V_START + 160
V_ROWS = V_STEP + 128
V_UF = 8
V_KF = V_UF + NBLK * 32
VM_ROWS = V_KF + NBLK * 32


def _bf16_round_int(l):
    u = np.asarray(l, np.float32).view(np.uint32)
    r = (u + 0x7FFF + ((u >> 16) & 1)) & 0xFFFF0000
    return r.astype(np.uint32).view(np.float32).astype(np.int64)


def _tap_row(lp):
    return np.where(lp < 256, lp, np.where(lp < 512, 256 + (lp - 256) // 2,
                    np.where(lp < 1024, 384 + (lp - 512) // 4, 512 + (lp - 1024) // 8)))


@functools.lru_cache(maxsize=None)
def _dft_consts():
    t = np.arange(BLK)
    F = np.zeros((8, 32, BLK))
    G = np.zeros((BLK, 8, 32))
    for r in range(8):
        f = np.concatenate([16 * r + 2 * np.arange(8), 16 * r + 2 * np.arange(8) + 1])
        th = 2 * np.pi * (f + 0.5) / (2 * BLK)
        F[r, :16] = np.cos(th[:, None] * t[None])
        F[r, 16:] = -np.sin(th[:, None] * t[None])
        G[:, r, 0::2] = np.cos(th[None] * t[:, None]) / BLK
        G[:, r, 1::2] = -np.sin(th[None] * t[:, None]) / BLK
    FS = np.zeros((8, NBLK, 32, 128))
    for (w0, wn, b0, nb) in WINDOWS:
        for j in range(b0, b0 + nb):
            rows = _tap_row(_bf16_round_int(BLK * j + t)) - w0
            assert rows.min() >= 0 and rows.max() < wn
            sel = np.zeros((BLK, 128))
            sel[t, rows] = 1.0
            FS[:, j] = F @ sel
    return (FS.reshape(8, NBLK * 32, 128).astype(np.float32),
            G.reshape(BLK, 2, 128).transpose(1, 0, 2).astype(np.float32))


def _ld16(ref, *idx):
    return pltpu.bitcast(ref.bitcast(u32)[idx + (slice(None),)], bf16)


def _cmul(a, b):
    return (a[0] * b[0] - a[1] * b[1], a[0] * b[1] + a[1] * b[0])


def _csq(a):
    return (a[0] * a[0] - a[1] * a[1], 2.0 * (a[0] * a[1]))


def _cexp(lr, li):
    k = jnp.floor(li * (2.0 / np.pi) + 0.5)
    r = ((li - k * 1.5703125) - k * 4.837512969970703125e-4) - k * 7.54978995489188216e-8
    r = jnp.clip(r, -0.8, 0.8)
    r2 = r * r
    s = r + r * r2 * (-1.6666654611e-1 + r2 * (8.3321608736e-3 + r2 * -1.9515295891e-4))
    c = (1.0 - 0.5 * r2) + (r2 * r2) * (4.166664568298827e-2
                                        + r2 * (-1.388731625493765e-3 + r2 * 2.443315711809948e-5))
    q = k.astype(jnp.int32)
    swap = (q & 1) == 1
    m = jnp.exp(lr)
    flip = lambda v, bit: pltpu.bitcast(pltpu.bitcast(v, jnp.int32) ^ (bit << 30), f32)
    return (flip(m * jnp.where(swap, s, c), (q + 1) & 2), flip(m * jnp.where(swap, c, s), q & 2))


def _par_row(c, k):
    return 8 + (c * 6 + k) * N


def _prep_pieces(praw, vec, par):
    def stage1(c):
        def fn():
            tr = lambda k: praw[k, pl.ds(c * 128, 128), :].astype(f32).T
            dt = jnp.exp(vec[0, pl.ds(c, 1), :]).astype(bf16).astype(f32)
            cc = _cmul((tr(4), tr(5)), (dt * tr(2), dt * tr(3)))
            for k, v in ((0, dt * tr(0)), (1, dt * tr(1)), (4, cc[0]), (5, cc[1])):
                par[pl.ds(_par_row(c, k), N), :] = v
        return fn

    def stage2(c, n0):
        def fn():
            lr = par[pl.ds(_par_row(c, 0) + n0, 16), :]
            li = par[pl.ds(_par_row(c, 1) + n0, 16), :]
            for k, v in enumerate(_cexp(lr, li) + _cexp(lr * 128.0, li * 128.0)):
                par[pl.ds(_par_row(c, k) + n0, 16), :] = v
        return fn

    tile = lambda c: [(260, stage1(c))] + [(190, stage2(c, n0)) for n0 in range(0, N, 16)]
    return tile(0), [pc for c in range(1, NT) for pc in tile(c)]


def _kgen_pieces(c, r, par, vb, taps, tslot, frow, kni, ksplit):
    st = {}

    def put(row, z, h=None):
        if h is None:
            vb[pl.ds(row, 16), :] = z[0]
            vb[pl.ds(row + 16, 16), :] = z[1]
        else:
            vb[pl.ds(row + 8 * h, 8), :] = z[0]
            vb[pl.ds(row + 16 + 8 * h, 8), :] = z[1]

    def get(row, h=None):
        if h is None:
            return (vb[pl.ds(row, 16), :], vb[pl.ds(row + 16, 16), :])
        return (vb[pl.ds(row + 8 * h, 8), :], vb[pl.ds(row + 16 + 8 * h, 8), :])

    def params(k):
        if isinstance(r, int):
            return par[pl.ds(_par_row(c, k) + r * 16, 16), :]
        return par[pl.ds(pl.multiple_of(c * (6 * N) + r[0] * 32, 32) + (_par_row(0, k) + r[1] * 16), 16), :]

    def park():
        put(V_STEP, (params(0), params(1)))
        put(V_START + 32, (params(2), params(3)))
        put(V_START, (params(4), params(5)))

    def setup_y(h):
        def fn():
            z1 = get(V_STEP, h)
            z2 = _csq(z1)
            z4 = _csq(z2)
            s = lax.broadcasted_iota(jnp.int32, (8, 128), 0)
            fs = [(jnp.where((s >> k) & 1 == 1, z[0], 1.0), jnp.where((s >> k) & 1 == 1, z[1], 0.0))
                  for k, z in enumerate((z1, z2, z4))]
            y = _cmul(_cmul(fs[0], fs[1]), fs[2])
            for k in range(8):
                put(V_YTAB + 32 * k, y, h)
                if k < 7:
                    y = _cmul(y, z1)
                    y = (jnp.where(s == 7 - k, 1.0, y[0]), jnp.where(s == 7 - k, 0.0, y[1]))
            z = z4
            for k in range(4):
                z = _csq(z)
                put(V_STEP + 32 * k, z, h)
        return fn

    def setup_hi():
        z = get(V_START + 32)
        cf = get(V_START)
        for g in range(1, 5):
            put(V_START + 32 * g, _cmul(cf, z))
            if g < 4:
                z = _csq(z)

    def square(k0, k1):
        def fn():
            for k in range(k0, k1):
                put(V_YTAB + 32 * k, _csq(get(V_YTAB + 32 * k)))
        return fn

    def rows_of(g, i0, ni):
        n_i = 16 + (g == 4)

        def fn():
            x = st.pop('x') if i0 > 0 else get(V_START + 32 * g)
            step = get(V_STEP + 32 * max(g - 1, 0))
            xs = []
            for t in range(ni):
                xs.append(x)
                if i0 + t + 1 < n_i:
                    x = _cmul(x, step)
            if i0 + ni < n_i:
                st['x'] = x
            acc = [None] * ni
            for k in range(8):
                yr, yi = get(V_YTAB + 32 * k)
                for t in range(ni):
                    v = xs[t][0] * yr - xs[t][1] * yi
                    v = v[:8] + v[8:]
                    if k:
                        v = pltpu.roll(v, k, 0)
                    acc[t] = v if acc[t] is None else acc[t] + v
                if frow is not None and k % ksplit == ksplit - 1 and k < 7:
                    vb[pl.ds(frow, 8), :] = acc[ni - 1]
            for t in range(ni):
                row = 128 * g + 8 * (i0 + t)
                a = acc[t]
                if row == 640:
                    a = jnp.where(lax.broadcasted_iota(jnp.int32, (8, 128), 0) == 0, a, 0.0)
                taps[tslot, pl.ds(row, 8), :] = taps[tslot, pl.ds(row, 8), :] + a
                if frow is not None and t == ni - 1:
                    vb[pl.ds(frow, 8), :] = a
        return fn

    pieces = [(30, park), (110, setup_y(0)), (110, setup_y(1)), (80, setup_hi)]
    for g in range(5):
        if g >= 2:
            pieces += [(40, square(0, 4)), (40, square(4, 8))]
        for i0 in range(0, 16 + (g == 4), kni):
            ni = min(kni, 16 + (g == 4) - i0)
            pieces.append((83 * ni, rows_of(g, i0, ni)))
    return pieces


def _conv_pieces(c, r, buf, fs_ref, us, taps, vb, yf, frow):
    st = {}

    def fwd_u(b0, b1):
        def fn():
            lhs = _ld16(fs_ref, 2 * r[0] + r[1], pl.ds(0, 16))
            for b in range(b0, b1):
                w = pltpu.bitcast(us[c, pl.ds(b * 64, 64), :], bf16)
                res = jnp.dot(lhs, w, preferred_element_type=f32)
                row = V_UF + 32 * b
                if b == 0:
                    vb[pl.ds(row, 32), :] = res
                else:
                    p = st['prev']
                    vb[pl.ds(row, 8), :] = res[0:8] - p[16:24]
                    vb[pl.ds(row + 8, 8), :] = res[8:16] + p[24:32]
                    vb[pl.ds(row + 16, 8), :] = res[16:24] + p[0:8]
                    vb[pl.ds(row + 24, 8), :] = res[24:32] - p[8:16]
                st['prev'] = res
        return fn

    def fwd_k(jobs):
        def fn():
            for (wi, t0, nb) in jobs:
                w0, wn, b0, _ = WINDOWS[wi]
                lhs = _ld16(fs_ref, 2 * r[0] + r[1], pl.ds((b0 + t0) * 16, nb * 16))[:, :wn]
                w = taps[c, pl.ds(w0, wn), :].astype(bf16)
                vb[pl.ds(V_KF + 32 * (b0 + t0), 32 * nb), :] = jnp.dot(lhs, w, preferred_element_type=f32)
        return fn

    def mac(q, i0, ni, j0, j1):
        def fn():
            ld = lambda base, b: (vb[pl.ds(base + 32 * b + 8 * q, 8), :], vb[pl.ds(base + 32 * b + 16 + 8 * q, 8), :])
            zr, zi = st.pop('z') if j0 > 0 else ({}, {})
            ucache = {}
            for j in range(j0, j1):
                kr, ki = ld(V_KF, j)
                for i in range(max(i0, j), i0 + ni):
                    if i - j not in ucache:
                        ucache[i - j] = ld(V_UF, i - j)
                    ur, ui = ucache[i - j]
                    if i not in zr:
                        zr[i] = kr * ur - ki * ui
                        zi[i] = kr * ui + ki * ur
                    else:
                        zr[i] = zr[i] + kr * ur - ki * ui
                        zi[i] = zi[i] + kr * ui + ki * ur
            if frow is not None:
                vb[pl.ds(frow, 8), :] = zr[i0 + ni - 1]
            if j1 < i0 + ni:
                st['z'] = (zr, zi)
            else:
                row = pl.multiple_of(r[0] * 32, 32) + (r[1] * 16 + q * 8)
                for i in range(i0, i0 + ni):
                    yf[buf, i, pl.ds(row, 8), :] = pltpu.pack_elementwise([zr[i], zi[i]], packed_dtype=bf16)
        return (8 * sum(1 for j in range(j0, j1) for i in range(max(i0, j), i0 + ni)), fn)

    fwd = [fwd_u(0, 8), fwd_u(8, 16), fwd_k(((0, 0, 1), (1, 0, 1), (2, 0, 1), (3, 0, 1))),
           fwd_k(((4, 0, 2), (6, 0, 2), (6, 2, 2), (6, 4, 2))), fwd_k(((4, 2, 1), (5, 0, 1), (6, 6, 1), (7, 0, 1)))]
    macs = []
    for q in range(2):
        for i0 in range(0, NBLK, 2):
            for j0 in range(0, i0 + 2, MACJ):
                macs.append(mac(q, i0, 2, j0, min(j0 + MACJ, i0 + 2)))
    return fwd, macs


def _inv_piece(c, b, buf, g_ref, us, vec, yf, outb):
    rows = pl.ds(pl.multiple_of(b * 64, 64), 64)
    w = pltpu.bitcast(yf[buf, b], bf16)
    g = jnp.concatenate([_ld16(g_ref, k, slice(None)) for k in range(2)], axis=1)
    y = jnp.dot(g, w, preferred_element_type=f32)
    u = pltpu.bitcast(us[c, rows, :], bf16).astype(f32)
    sk = (u * vec[1, pl.ds(c, 1), :]).astype(bf16).astype(f32)
    o = (y.astype(bf16).astype(f32) + sk).astype(bf16)
    outb[c, pl.ds(pl.multiple_of(b * BLK, BLK) if not isinstance(b, int) else b * BLK, BLK), :] = o


def _attn_fill():
    n = 2 * (SEG + M)
    r = lax.broadcasted_iota(jnp.int32, (n, n), 0)
    c = lax.broadcasted_iota(jnp.int32, (n, n), 1)
    head = lambda i: jnp.where(i < 2 * SEG, i // SEG, (i - 2 * SEG) // PRE)
    pos = lambda i: jnp.where(i < 2 * SEG, i % SEG, i % PRE)
    is_mem = lambda i: (i < 2 * SEG) & (i % SEG < M)
    same = head(r) == head(c)
    allowed = same & (is_mem(r) | is_mem(c) | (pos(r) >= pos(c)))
    return jnp.where(allowed, 0.0, jnp.where(same, -1e9 * LOG2E, -jnp.inf)).astype(f32)


def _kernel(zero_hbm, x_hbm, mem0_hbm, wq_hbm, wk_hbm, wv_hbm, wo_hbm,
            u_hbm, p0, p1, p2, p3, p4, p5, ldt_hbm, dsk_hbm, fs_hbm, g_hbm,
            out_hbm,
            wq, wk, wv, wo, xb, xs, h_ref, outs, fill_ref,
            praw, par, us, taps, vb, vm, vu, pacc, yf, outb, vec, vraw, fs_ref, g_ref, zero_ref,
            sem_s, sem_w, sem_o, sem_xb, sem_x, sem_p, sem_u, sem_out, pre, own, lo0, lo1):
    wqkv = (wq, wk, wv)
    scale = E ** -0.5

    whbm = [w.bitcast(u32) for w in (wq_hbm, wk_hbm, wv_hbm)]

    def wcp(j, m, p):
        return pltpu.make_async_copy(whbm[m].at[:, p, j, :], wqkv[m].at[p, j], sem_w.at[(j * 3 + m) * 2 + p])

    xu = x_hbm.bitcast(u32)
    xcs = [pltpu.make_async_copy(xu.at[:, t, pl.ds(0, PRE // 2), pl.ds(c * 128, 128)],
                                 xb.at[c, :, pl.ds(t * (PRE // 2), PRE // 2), :], sem_xb.at[2 * c + t])
           for c in range(8) for t in range(2)]
    xcp1 = pltpu.make_async_copy(x_hbm.at[:, :, pl.ds(PRE, TOK), :], xs, sem_x.at[0])
    pcs = [pltpu.make_async_copy(p, praw.at[k], sem_p.at[k]) for k, p in enumerate((p0, p1, p2, p3, p4, p5))]
    ccs = [pltpu.make_async_copy(fs_hbm, fs_ref, sem_p.at[6]), pltpu.make_async_copy(g_hbm, g_ref, sem_p.at[7])]
    wou = wo_hbm.bitcast(u32)
    ocs = [pltpu.make_async_copy(wou.at[:, pl.ds(c * 128, 128)], wo.at[c], sem_o.at[c]) for c in range(8)]
    uu = u_hbm.bitcast(u32)
    ucs = [pltpu.make_async_copy(uu.at[:, pl.ds(c * 128, 128)], us.at[c], sem_u.at[c]) for c in range(NT)]

    zcp = pltpu.make_async_copy(zero_hbm, zero_ref, sem_s.at[0])
    scs = [pltpu.make_async_copy(mem0_hbm, h_ref.at[pl.ds(0, M)], sem_s.at[1]),
           pltpu.make_async_copy(ldt_hbm, vraw.at[0], sem_s.at[2]),
           pltpu.make_async_copy(dsk_hbm, vraw.at[1], sem_s.at[3])]
    w0cs = [[pltpu.make_async_copy(whbm[0].at[pl.ds(half * (DM // 4), DM // 4), p, 0, :],
                                   wq.at[p, 0, pl.ds(half * (DM // 4), DM // 4)], sem_s.at[4 + 2 * half + p])
             for p in range(2)] for half in range(2)]
    for cp in [zcp] + w0cs[0] + xcs[:8]:
        cp.start()
    vu[pl.ds(8, 8), :] = pltpu.bitcast(jnp.full((8, 128), 0x0000FFFF, u32), f32)
    vu[pl.ds(16, 8), :] = pltpu.bitcast(jnp.full((8, 128), 0xFFFF0000, u32), f32)
    taps[...] = jnp.zeros(taps.shape, f32)
    yf[1] = jnp.zeros(yf.shape[1:], u32)
    fill_ref[...] = _attn_fill()
    for cp in w0cs[1] + xcs[8:] + scs:
        cp.start()
    zcp.wait()

    frow = pl.multiple_of(zero_ref[0] * 8, 8)
    zrow = [pl.multiple_of(zero_ref[k] * 8, 8) for k in range(T0 // RC)]

    class Pacer:
        def __init__(self, segments):
            self.t = 0.0
            self.todo = []
            for (pieces, buf, t0, t1) in segments:
                total = float(sum(c for c, _ in pieces)) or 1.0
                done = 0.0
                for (cst, fn) in pieces:
                    self.todo.append((t0 + (t1 - t0) * done / total, fn, buf))
                    done += cst

        def __call__(self, v, dt=1.0):
            self.t += dt
            fenced = []
            while self.todo and self.todo[0][0] < self.t:
                _, fn, buf = self.todo.pop(0)
                if not any(b is buf for b in fenced):
                    buf[pl.ds(frow, 8), :] = v
                    fenced.append(buf)
                fn()

        def finished(self):
            return not self.todo

    def unpair(j, m, r0, nr):
        def fn():
            rows = pl.ds(r0, nr)
            m_lo = jnp.tile(pltpu.bitcast(vu[pl.ds(8, 8), :], u32), (nr // 8, 1))
            m_hi = jnp.tile(pltpu.bitcast(vu[pl.ds(16, 8), :], u32), (nr // 8, 1))
            a = wqkv[m][0, j, rows, :]
            b = wqkv[m][1, j, rows, :]
            wqkv[m][0, j, rows, :] = (a & m_lo) | ((b & m_lo) << 16)
            wqkv[m][1, j, rows, :] = ((a & m_hi) >> 16) | (b & m_hi)
        return (nr, fn)

    def unpair_pieces(items, lo=0, hi=DM // 2):
        return [unpair(j, m, r0, UNP) for (j, m) in items for r0 in range(lo, hi, UNP)]

    items = [(j, m) for j in range(NP) for m in range(3)]
    wcs = lambda lo, hi: [wcp(j, m, p) for (j, m) in items[lo:hi] for p in range(2)]
    rest = ocs + ccs + ucs + [xcp1]
    starts = [[] for _ in range(2 * len(items))]
    n_w, n_r = 1, 0
    for unit in sorted(STARTS):
        w_hi, with_par, r_hi = STARTS[unit]
        starts[unit] = (pcs if with_par else []) + wcs(n_w, w_hi) + rest[n_r:r_hi]
        n_w, n_r = w_hi, r_hi
    assert n_w == len(items) and n_r == len(rest)
    with jax.named_scope("bulk"):
        if QUICK in (1, 2):
            for cp in wcs(1, 48) + pcs + ocs + ucs + [xcp1] + ccs:
                cp.start()
            for cp in wcs(1, 48) + pcs + scs + xcs + w0cs[0] + w0cs[1]:
                cp.wait()
            vec[...] = vraw[...].astype(f32)
            for _, fn in (unpair_pieces(items) + sum(_prep_pieces(praw, vec, par), [])) if QUICK != 2 else []:
                fn()

            def kg(r, carry):
                for odd in range(2):
                    for _, fn in _kgen_pieces(0, (r, odd), par, vb, taps, 0, zrow[1], BKNI, BKSPLIT):
                        fn()
                return carry
            lax.fori_loop(0, 4, kg, 0)
            for (j, m) in (items if QUICK != 2 else []):
                def chunk(rc, carry, j=j, m=m):
                    lhs = jnp.concatenate(
                        [pltpu.bitcast(xb[c, pl.ds(rc * 4, 4)].reshape(32, 128), bf16) for c in range(8)], axis=1)
                    res = [jnp.dot(lhs, pltpu.bitcast(wqkv[m][p, j], bf16), preferred_element_type=f32)
                           for p in range(2)]
                    for t in range(8):
                        v = jnp.concatenate([res[0][8 * t:8 * t + 8], res[1][8 * t:8 * t + 8]], axis=0)
                        pre[rc * 8 + t, m * NP + j] = v.astype(bf16)
                    return carry
                lax.fori_loop(0, 8, chunk, 0)
            items = []
        n_chunk = 2 * (T0 // RC)
        prep = _prep_pieces(praw, vec, par)
        kg0 = [pc for r in range(8) for pc in _kgen_pieces(0, r, par, vb, taps, 0, zrow[1], BKNI, BKSPLIT)]
        t_a, t_b, t_c, t_d = [v * n_chunk for v in BPLAN]
        fence_x = Pacer([(prep[0], par, t_a, t_b), (kg0, vb, t_b, t_c), (prep[1], par, t_c, t_d)])
        landed = 1
        for it, (j, m) in enumerate(items):
            fence_w = None
            for half in range(2):
                for cp in starts[2 * it + half]:
                    cp.start()
                if it == 0:
                    with jax.named_scope("waitx%d" % half):
                        for cp in w0cs[half] + xcs[8 * half:8 * half + 8]:
                            cp.wait()
                    for _, fn in unpair_pieces(items[:1], half * (DM // 4), (half + 1) * (DM // 4)):
                        fn()
                    fence_w = Pacer([])
                elif half == 0:
                    late = landed == it
                    if it in WAITS:
                        with jax.named_scope("wait%d" % it):
                            for cp in wcs(landed, WAITS[it]) + (pcs + scs if it == PAR_WAIT else []):
                                cp.wait()
                        landed = WAITS[it]
                        if it == PAR_WAIT:
                            vec[...] = vraw[...].astype(f32)
                    if late:
                        for _, fn in unpair_pieces(items[it:it + 1]):
                            fn()
                    fence_w = Pacer([(unpair_pieces(items[it + 1:min(it + 2, landed)]), vu, 0.0, n_chunk * UNP_FRAC)])
                for p in range(2):
                    w = pltpu.bitcast(wqkv[m][p, j, pl.ds(half * (DM // 4), DM // 4), :], bf16)
                    lhs = jnp.concatenate([pltpu.bitcast(xb[c].reshape(T0 // 2, 128), bf16)
                                           for c in range(4 * half, 4 * half + 4)], axis=1)
                    res = jnp.dot(lhs, w, preferred_element_type=f32)
                    for rc in range(T0 // RC):
                        rows = pl.ds(rc * RC, RC)
                        v = res[rc * RC:(rc + 1) * RC]
                        if half == 1:
                            v = v + pacc[p, rows, :]
                        if p == 0 or half == 0:
                            pacc[p, rows, :] = v
                        else:
                            v0 = pacc[0, rows, :]
                            for t in range(RC // PRE):
                                pr = jnp.concatenate([v0[PRE * t:PRE * (t + 1)], v[PRE * t:PRE * (t + 1)]], axis=0)
                                pre[rc * (RC // PRE) + t, m * NP + j] = pr.astype(bf16)
                        fence_w(v[:8], 0.5)
                        fence_x(v[:8], 0.5)
            assert fence_w.finished() and landed > it
        assert QUICK or fence_x.finished()
    with jax.named_scope("waitrest"):
        for cp in ocs + ucs + ccs + [xcp1]:
            cp.wait()

    def outa_cp(row, n):
        return pltpu.make_async_copy(outs.at[pl.ds(row, n)], out_hbm.at[pl.ds(row, n), pl.ds(0, DM)], sem_out.at[0])

    def outb_cp(c, row, n, sem):
        col = DM + c * 128
        return pltpu.make_async_copy(
            outb.at[c, pl.ds(row, n)],
            out_hbm.at[pl.ds(row, n), pl.ds(col if isinstance(col, int) else pl.multiple_of(col, 128), 128)],
            sem_out.at[sem])

    def one_step(i, odd, fwd, fence):
        s = 2 * i + odd
        lo_cur = (lo0, lo1)[odd]
        base = pl.multiple_of(2 * SEG * i, 2 * SEG)
        h_ref[pl.ds(M, TOK), :] = xs[i, odd]
        h = h_ref[...]
        scores = {}
        probs = {}
        zown = 0

        ct = i >> 2
        r = s & 7
        buf = ct & 1
        cprev = (ct + NT - 1) & (NT - 1)

        def stage_a(j):
            for m in range(3):
                for p in range(2):
                    w = pltpu.bitcast(wqkv[m][p, j], bf16)
                    res = jnp.dot(h, w, preferred_element_type=f32)
                    own[m * NP + j, pl.ds(SEG * p, SEG), :] = res.astype(bf16)
                    fence(res[:M])

        def gather(m, j):
            return pltpu.bitcast(jnp.concatenate([own.bitcast(u32)[m * NP + j + zown],
                                                  pre.bitcast(u32)[s, m * NP + j]], axis=0), bf16)

        def stage_qk(j):
            scores[j] = lax.dot_general(gather(0, j), gather(1, j), (((1,), (1,)), ((), ())),
                                        preferred_element_type=f32)

        def stage_b(j):
            fl = fill_ref[...]
            sc = jnp.where(fl == 0.0, scores.pop(j) * (scale * LOG2E), fl)
            e = jnp.exp2(sc - jnp.max(sc, axis=-1, keepdims=True))
            den = jnp.sum(e, axis=-1, keepdims=True)
            probs[j] = (e * pl.reciprocal(den, approx=True)).astype(bf16)

        def stage_c(j):
            o = jnp.dot(probs[j], gather(2, j), preferred_element_type=f32)
            for p in range(2):
                hh = 2 * j + p
                lo_cur[hh, pl.ds(0, SEG), :] = o[p * SEG:(p + 1) * SEG].astype(bf16)
                ob = o[2 * SEG + p * PRE:2 * SEG + (p + 1) * PRE]
                lo1[hh, pl.ds(SEG + odd * PRE, PRE), :] = ob.astype(bf16)

        acc = [None] * 8

        def stage_d(h0, h1, last=False):
            lhs = jnp.concatenate([_ld16(lo_cur, hh, slice(None)) for hh in range(h0, h1)], axis=1)
            for c in range(8):
                w = pltpu.bitcast(wo[c, pl.ds(h0 * 64, (h1 - h0) * 64), :], bf16)
                res = jnp.dot(lhs, w, preferred_element_type=f32)
                acc[c] = res if acc[c] is None else acc[c] + res
                if not last:
                    fence(res[:M], (h1 - h0) / 8.0 * (DW_ODD if odd else 1.0))
                else:
                    rb = acc[c].astype(bf16)
                    cols = pl.ds(c * 128, 128)
                    h_ref[pl.ds(0, M), cols] = rb[:M]
                    outs[pl.ds(base + (odd * SEG + PRE), TOK), cols] = rb[M:SEG]
                    if odd:
                        outs[pl.ds(base, PRE), cols] = rb[SEG:SEG + PRE]
                        outs[pl.ds(base + SEG, PRE), cols] = rb[SEG + PRE:]

        def attn_group(jq, jc):
            for j in jq:
                stage_qk(j)
            for j in jc:
                stage_c(j)
            for j in jq:
                stage_b(j)

        for t in range(2):
            _inv_piece(cprev, 2 * r + t, 1 - buf, g_ref, us, vec, yf, outb)
        for p in fwd:
            p()
        for j in range(NP):
            stage_a(j)
            if j >= 2 and j % 2 == 0:
                attn_group((j - 2, j - 1), (j - 4, j - 3) if j >= 4 else ())
        stage_d(0, 8)
        attn_group((14, 15), (12, 13))
        stage_d(8, 20)
        attn_group((), (14, 15))
        stage_d(20, 28)
        stage_d(28, 32, last=True)

    def two_steps(i, carry):
        ct = i >> 2
        cprev = (ct + NT - 1) & (NT - 1)
        conv = [_conv_pieces(ct, (i & 3, odd), ct & 1, fs_ref, us, taps, vm, yf,
                             zrow[1] if DONE_M else None) for odd in range(2)]
        kgen = [_kgen_pieces((ct + 1) & (NT - 1), (i & 3, odd), par, vb, taps, ct + 1,
                             zrow[1] if DONE_K else None, KNI, KSPLIT) for odd in range(2)]
        work = {'k0': (kgen[0], vb), 'k1': (kgen[1], vb), 'm0': (conv[0][1], vm), 'm1': (conv[1][1], vm)}
        fence = Pacer([work[k] + (t0, t1) for (k, t0, t1) in PLAN if k[0] not in NOB])
        for odd in range(2):
            one_step(i, odd, conv[odd][0], fence)
        assert fence.finished() or NOB
        outa_cp(pl.multiple_of(2 * SEG * i, 2 * SEG), 2 * SEG).start()
        outb_cp(cprev, pl.multiple_of((i & 3) * 512, 512), 512, jnp.where(i < 4, 2, 1)).start()
        return carry

    with jax.named_scope("steps"):
        if NITER:
            lax.fori_loop(0, NITER, two_steps, 0)

    with jax.named_scope("flush"):
        outb_cp(NT - 1, 0, L, 2).wait()
        for b in range(NBLK):
            _inv_piece(NT - 1, b, (NT - 1) % 2, g_ref, us, vec, yf, outb)
            if b % 4 == 3:
                outb_cp(NT - 1, (b - 3) * BLK, 4 * BLK, 1).start()
    with jax.named_scope("waitout"):
        outa_cp(0, S).wait()
        pltpu.make_async_copy(outb, outb, sem_out.at[1]).wait()


@functools.partial(jax.jit, static_argnames=("A_seg_len",))
def pallas_concat_heads__memory_aug_recurrent_mem_tr__ssm_conv_s4__prompt_kernel(
    A_x, A_mem0, A_Wq, A_Wk, A_Wv, A_Wo, A_seg_len,
    B_u, B_A_re, B_A_im, B_B_re, B_B_im, B_C_re, B_C_im, B_log_dt, B_Dskip,
):
    assert A_seg_len == SEG and A_x.shape == (1, S, DM) and B_u.shape == (1, L, D)
    fs, g = _dft_consts()
    w4 = lambda w: w.reshape(DM // 2, 2, H, E)
    any_ = pl.BlockSpec(memory_space=pl.ANY)
    V = pltpu.VMEM
    out = pl.pallas_call(
        _kernel,
        out_shape=jax.ShapeDtypeStruct((S, DM + D), bf16),
        in_specs=[any_] * 18,
        out_specs=any_,
        scratch_shapes=[
            V((2, NP, DM // 2, E), u32),
            V((2, NP, DM // 2, E), u32),
            V((2, NP, DM // 2, E), u32),
            V((8, H * E // 2, 128), u32),
            V((8, NSEG // 2, PRE, 128), u32),
            V((NSEG // 2, 2, TOK, DM), bf16),
            V((M + TOK, DM), bf16),
            V((S, DM), bf16),
            V((2 * (SEG + M), 2 * (SEG + M)), f32),
            V((6, D, N), bf16),
            V((8 + NT * 6 * N, 128), f32),
            V((NT, L // 2, 128), u32),
            V((NT + 1, TAPROWS, 128), f32),
            V((V_ROWS, 128), f32),
            V((VM_ROWS, 128), f32),
            V((24, 128), f32),
            V((2, T0, 128), f32),
            V((2, NBLK, 128, 128), u32),
            V((NT, L, 128), bf16),
            V((2, 8, 128), f32),
            V((2, 8, 128), bf16),
            V((8, NBLK * 32, 128), bf16),
            V((2, BLK, 128), bf16),
            pltpu.SMEM((8,), jnp.int32),
            pltpu.SemaphoreType.DMA((8,)),
            pltpu.SemaphoreType.DMA((6 * NP,)),
            pltpu.SemaphoreType.DMA((8,)),
            pltpu.SemaphoreType.DMA((16,)),
            pltpu.SemaphoreType.DMA((1,)),
            pltpu.SemaphoreType.DMA((8,)),
            pltpu.SemaphoreType.DMA((NT,)),
            pltpu.SemaphoreType.DMA((3,)),
            V((NSEG, 3 * NP, 2 * PRE, E), bf16),
            V((3 * NP, 2 * SEG, E), bf16),
            V((H, SEG, E), bf16),
            V((H, SEG + 2 * PRE, E), bf16),
        ],
        compiler_params=pltpu.CompilerParams(vmem_limit_bytes=110 * 1024 * 1024, disable_bounds_checks=True),
    )(jnp.asarray(np.zeros((8,), np.int32)), A_x.reshape(NSEG // 2, 2, SEG, DM), A_mem0.reshape(M, DM), w4(A_Wq), w4(A_Wk), w4(A_Wv), A_Wo.reshape(H * E, DM),
      B_u.reshape(L, D), B_A_re, B_A_im, B_B_re, B_B_im, B_C_re, B_C_im,
      B_log_dt.reshape(8, 128), B_Dskip.reshape(8, 128),
      jnp.asarray(fs, bf16), jnp.asarray(g, bf16))
    return out.reshape(1, S, DM + D)
```

```python
import functools

import numpy as np
import jax
import jax.numpy as jnp
from jax import lax
import jax.experimental.pallas as pl
import jax.experimental.pallas.tpu as pltpu

bf16, f32, u32 = jnp.bfloat16, jnp.float32, jnp.uint32

S, DM, H, E, M, SEG = 2048, 1024, 32, 128, 8, 32
NSEG = S // SEG
TOK = 24
PRE = SEG - TOK
T0 = PRE * NSEG
NP = H // 2
LOG2E = 1.4426950408889634
QUICK = False
NOB = ''
BKNI = 1
UNP = 64
UNP_FRAC = 0.7
BKSPLIT = 4
BPLAN = (10.0, 11.0, 42.5, 47.7)
WAITS = {1: 2, 2: 3, 3: 5, 4: 6, 5: 8, 7: 11, 10: 13, 12: 17, 16: 23, 22: 33, 32: 48}
PAR_WAIT = 10
STARTS = {0: (2, False, 0), 1: (3, False, 0), 2: (5, False, 0), 4: (6, False, 0), 6: (8, False, 0),
          8: (9, False, 0), 10: (11, False, 0), 14: (13, True, 0), 20: (17, False, 0), 24: (23, False, 0),
          32: (33, False, 0), 44: (48, False, 3), 64: (48, False, 19)}
NITER = NSEG // 2
KNI = 2
KSPLIT = 2
PLAN = (('k0', 0, 96), ('m0', 96, 122), ('k1', 124, 220), ('m1', 220, 260))
DW_ODD = 1.5
RC = 64
MACJ = 3
L, D, N = 2048, 1024, 128
BLK = 128
NBLK = L // BLK
NT = D // 128
TAPROWS = 672
WINDOWS = ((0, 128, 0, 1), (128, 128, 1, 1), (256, 128, 2, 1), (320, 80, 3, 1),
           (384, 128, 4, 3), (480, 48, 7, 1), (512, 128, 8, 7), (624, 32, 15, 1))

V_FENCE = 0
V_YTAB = 8
V_START = V_YTAB + 256
V_STEP = V_START + 160
V_ROWS = V_STEP + 128
V_UF = 8
V_KF = V_UF + NBLK * 32
VM_ROWS = V_KF + NBLK * 32


def _bf16_round_int(l):
    u = np.asarray(l, np.float32).view(np.uint32)
    r = (u + 0x7FFF + ((u >> 16) & 1)) & 0xFFFF0000
    return r.astype(np.uint32).view(np.float32).astype(np.int64)


def _tap_row(lp):
    return np.where(lp < 256, lp, np.where(lp < 512, 256 + (lp - 256) // 2,
                    np.where(lp < 1024, 384 + (lp - 512) // 4, 512 + (lp - 1024) // 8)))


@functools.lru_cache(maxsize=None)
def _dft_consts():
    t = np.arange(BLK)
    F = np.zeros((8, 32, BLK))
    G = np.zeros((BLK, 8, 32))
    for r in range(8):
        f = np.concatenate([16 * r + 2 * np.arange(8), 16 * r + 2 * np.arange(8) + 1])
        th = 2 * np.pi * (f + 0.5) / (2 * BLK)
        F[r, :16] = np.cos(th[:, None] * t[None])
        F[r, 16:] = -np.sin(th[:, None] * t[None])
        G[:, r, 0::2] = np.cos(th[None] * t[:, None]) / BLK
        G[:, r, 1::2] = -np.sin(th[None] * t[:, None]) / BLK
    FS = np.zeros((8, NBLK, 32, 128))
    for (w0, wn, b0, nb) in WINDOWS:
        for j in range(b0, b0 + nb):
            rows = _tap_row(_bf16_round_int(BLK * j + t)) - w0
            assert rows.min() >= 0 and rows.max() < wn
            sel = np.zeros((BLK, 128))
            sel[t, rows] = 1.0
            FS[:, j] = F @ sel
    return (FS.reshape(8, NBLK * 32, 128).astype(np.float32),
            G.reshape(BLK, 2, 128).transpose(1, 0, 2).astype(np.float32))


def _ld16(ref, *idx):
    return pltpu.bitcast(ref.bitcast(u32)[idx + (slice(None),)], bf16)


def _cmul(a, b):
    return (a[0] * b[0] - a[1] * b[1], a[0] * b[1] + a[1] * b[0])


def _csq(a):
    return (a[0] * a[0] - a[1] * a[1], 2.0 * (a[0] * a[1]))


def _cexp(lr, li):
    k = jnp.floor(li * (2.0 / np.pi) + 0.5)
    r = ((li - k * 1.5703125) - k * 4.837512969970703125e-4) - k * 7.54978995489188216e-8
    r = jnp.clip(r, -0.8, 0.8)
    r2 = r * r
    s = r + r * r2 * (-1.6666654611e-1 + r2 * (8.3321608736e-3 + r2 * -1.9515295891e-4))
    c = (1.0 - 0.5 * r2) + (r2 * r2) * (4.166664568298827e-2
                                        + r2 * (-1.388731625493765e-3 + r2 * 2.443315711809948e-5))
    q = k.astype(jnp.int32)
    swap = (q & 1) == 1
    m = jnp.exp(lr)
    flip = lambda v, bit: pltpu.bitcast(pltpu.bitcast(v, jnp.int32) ^ (bit << 30), f32)
    return (flip(m * jnp.where(swap, s, c), (q + 1) & 2), flip(m * jnp.where(swap, c, s), q & 2))


def _par_row(c, k):
    return 8 + (c * 6 + k) * N


def _prep_pieces(praw, vec, par):
    def stage1(c):
        def fn():
            tr = lambda k: praw[k, pl.ds(c * 128, 128), :].astype(f32).T
            dt = jnp.exp(vec[0, pl.ds(c, 1), :]).astype(bf16).astype(f32)
            cc = _cmul((tr(4), tr(5)), (dt * tr(2), dt * tr(3)))
            for k, v in ((0, dt * tr(0)), (1, dt * tr(1)), (4, cc[0]), (5, cc[1])):
                par[pl.ds(_par_row(c, k), N), :] = v
        return fn

    def stage2(c, n0):
        def fn():
            lr = par[pl.ds(_par_row(c, 0) + n0, 16), :]
            li = par[pl.ds(_par_row(c, 1) + n0, 16), :]
            for k, v in enumerate(_cexp(lr, li) + _cexp(lr * 128.0, li * 128.0)):
                par[pl.ds(_par_row(c, k) + n0, 16), :] = v
        return fn

    tile = lambda c: [(260, stage1(c))] + [(190, stage2(c, n0)) for n0 in range(0, N, 16)]
    return tile(0), [pc for c in range(1, NT) for pc in tile(c)]


def _kgen_pieces(c, r, par, vb, taps, tslot, frow, kni, ksplit):
    st = {}

    def put(row, z, h=None):
        if h is None:
            vb[pl.ds(row, 16), :] = z[0]
            vb[pl.ds(row + 16, 16), :] = z[1]
        else:
            vb[pl.ds(row + 8 * h, 8), :] = z[0]
            vb[pl.ds(row + 16 + 8 * h, 8), :] = z[1]

    def get(row, h=None):
        if h is None:
            return (vb[pl.ds(row, 16), :], vb[pl.ds(row + 16, 16), :])
        return (vb[pl.ds(row + 8 * h, 8), :], vb[pl.ds(row + 16 + 8 * h, 8), :])

    def params(k):
        if isinstance(r, int):
            return par[pl.ds(_par_row(c, k) + r * 16, 16), :]
        return par[pl.ds(pl.multiple_of(c * (6 * N) + r[0] * 32, 32) + (_par_row(0, k) + r[1] * 16), 16), :]

    def park():
        put(V_STEP, (params(0), params(1)))
        put(V_START + 32, (params(2), params(3)))
        put(V_START, (params(4), params(5)))

    def setup_y(h):
        def fn():
            z1 = get(V_STEP, h)
            z2 = _csq(z1)
            z4 = _csq(z2)
            s = lax.broadcasted_iota(jnp.int32, (8, 128), 0)
            fs = [(jnp.where((s >> k) & 1 == 1, z[0], 1.0), jnp.where((s >> k) & 1 == 1, z[1], 0.0))
                  for k, z in enumerate((z1, z2, z4))]
            y = _cmul(_cmul(fs[0], fs[1]), fs[2])
            for k in range(8):
                put(V_YTAB + 32 * k, y, h)
                if k < 7:
                    y = _cmul(y, z1)
                    y = (jnp.where(s == 7 - k, 1.0, y[0]), jnp.where(s == 7 - k, 0.0, y[1]))
            z = z4
            for k in range(4):
                z = _csq(z)
                put(V_STEP + 32 * k, z, h)
        return fn

    def setup_hi():
        z = get(V_START + 32)
        cf = get(V_START)
        for g in range(1, 5):
            put(V_START + 32 * g, _cmul(cf, z))
            if g < 4:
                z = _csq(z)

    def square(k0, k1):
        def fn():
            for k in range(k0, k1):
                put(V_YTAB + 32 * k, _csq(get(V_YTAB + 32 * k)))
        return fn

    def rows_of(g, i0, ni):
        n_i = 16 + (g == 4)

        def fn():
            x = st.pop('x') if i0 > 0 else get(V_START + 32 * g)
            step = get(V_STEP + 32 * max(g - 1, 0))
            xs = []
            for t in range(ni):
                xs.append(x)
                if i0 + t + 1 < n_i:
                    x = _cmul(x, step)
            if i0 + ni < n_i:
                st['x'] = x
            acc = [None] * ni
            for k in range(8):
                yr, yi = get(V_YTAB + 32 * k)
                for t in range(ni):
                    v = xs[t][0] * yr - xs[t][1] * yi
                    v = v[:8] + v[8:]
                    if k:
                        v = pltpu.roll(v, k, 0)
                    acc[t] = v if acc[t] is None else acc[t] + v
                if frow is not None and k % ksplit == ksplit - 1 and k < 7:
                    vb[pl.ds(frow, 8), :] = acc[ni - 1]
            for t in range(ni):
                row = 128 * g + 8 * (i0 + t)
                a = acc[t]
                if row == 640:
                    a = jnp.where(lax.broadcasted_iota(jnp.int32, (8, 128), 0) == 0, a, 0.0)
                taps[tslot, pl.ds(row, 8), :] = taps[tslot, pl.ds(row, 8), :] + a
                if frow is not None and t == ni - 1:
                    vb[pl.ds(frow, 8), :] = a
        return fn

    pieces = [(30, park), (110, setup_y(0)), (110, setup_y(1)), (80, setup_hi)]
    for g in range(5):
        if g >= 2:
            pieces += [(40, square(0, 4)), (40, square(4, 8))]
        for i0 in range(0, 16 + (g == 4), kni):
            ni = min(kni, 16 + (g == 4) - i0)
            pieces.append((83 * ni, rows_of(g, i0, ni)))
    return pieces


def _conv_pieces(c, r, buf, fs_ref, us, taps, vb, yf, frow):
    st = {}

    def fwd_u(b0, b1):
        def fn():
            lhs = _ld16(fs_ref, 2 * r[0] + r[1], pl.ds(0, 16))
            for b in range(b0, b1):
                w = pltpu.bitcast(us[c, pl.ds(b * 64, 64), :], bf16)
                res = jnp.dot(lhs, w, preferred_element_type=f32)
                row = V_UF + 32 * b
                if b == 0:
                    vb[pl.ds(row, 32), :] = res
                else:
                    p = st['prev']
                    vb[pl.ds(row, 8), :] = res[0:8] - p[16:24]
                    vb[pl.ds(row + 8, 8), :] = res[8:16] + p[24:32]
                    vb[pl.ds(row + 16, 8), :] = res[16:24] + p[0:8]
                    vb[pl.ds(row + 24, 8), :] = res[24:32] - p[8:16]
                st['prev'] = res
        return fn

    def fwd_k(jobs):
        def fn():
            for (wi, t0, nb) in jobs:
                w0, wn, b0, _ = WINDOWS[wi]
                lhs = _ld16(fs_ref, 2 * r[0] + r[1], pl.ds((b0 + t0) * 16, nb * 16))[:, :wn]
                w = taps[c, pl.ds(w0, wn), :].astype(bf16)
                vb[pl.ds(V_KF + 32 * (b0 + t0), 32 * nb), :] = jnp.dot(lhs, w, preferred_element_type=f32)
        return fn

    def mac(q, i0, ni, j0, j1):
        def fn():
            ld = lambda base, b: (vb[pl.ds(base + 32 * b + 8 * q, 8), :], vb[pl.ds(base + 32 * b + 16 + 8 * q, 8), :])
            zr, zi = st.pop('z') if j0 > 0 else ({}, {})
            ucache = {}
            for j in range(j0, j1):
                kr, ki = ld(V_KF, j)
                for i in range(max(i0, j), i0 + ni):
                    if i - j not in ucache:
                        ucache[i - j] = ld(V_UF, i - j)
                    ur, ui = ucache[i - j]
                    if i not in zr:
                        zr[i] = kr * ur - ki * ui
                        zi[i] = kr * ui + ki * ur
                    else:
                        zr[i] = zr[i] + kr * ur - ki * ui
                        zi[i] = zi[i] + kr * ui + ki * ur
            if frow is not None:
                vb[pl.ds(frow, 8), :] = zr[i0 + ni - 1]
            if j1 < i0 + ni:
                st['z'] = (zr, zi)
            else:
                row = pl.multiple_of(r[0] * 32, 32) + (r[1] * 16 + q * 8)
                for i in range(i0, i0 + ni):
                    yf[buf, i, pl.ds(row, 8), :] = pltpu.pack_elementwise([zr[i], zi[i]], packed_dtype=bf16)
        return (8 * sum(1 for j in range(j0, j1) for i in range(max(i0, j), i0 + ni)), fn)

    fwd = [fwd_u(0, 8), fwd_u(8, 16), fwd_k(((0, 0, 1), (1, 0, 1), (2, 0, 1), (3, 0, 1))),
           fwd_k(((4, 0, 2), (6, 0, 2), (6, 2, 2), (6, 4, 2))), fwd_k(((4, 2, 1), (5, 0, 1), (6, 6, 1), (7, 0, 1)))]
    macs = []
    for q in range(2):
        for i0 in range(0, NBLK, 2):
            for j0 in range(0, i0 + 2, MACJ):
                macs.append(mac(q, i0, 2, j0, min(j0 + MACJ, i0 + 2)))
    return fwd, macs


def _inv_piece(c, b, buf, g_ref, us, vec, yf, outb):
    rows = pl.ds(pl.multiple_of(b * 64, 64), 64)
    w = pltpu.bitcast(yf[buf, b], bf16)
    g = jnp.concatenate([_ld16(g_ref, k, slice(None)) for k in range(2)], axis=1)
    y = jnp.dot(g, w, preferred_element_type=f32)
    u = pltpu.bitcast(us[c, rows, :], bf16).astype(f32)
    sk = (u * vec[1, pl.ds(c, 1), :]).astype(bf16).astype(f32)
    o = (y.astype(bf16).astype(f32) + sk).astype(bf16)
    outb[c, pl.ds(pl.multiple_of(b * BLK, BLK) if not isinstance(b, int) else b * BLK, BLK), :] = o


def _attn_fill():
    n = 2 * (SEG + M)
    r = lax.broadcasted_iota(jnp.int32, (n, n), 0)
    c = lax.broadcasted_iota(jnp.int32, (n, n), 1)
    head = lambda i: jnp.where(i < 2 * SEG, i // SEG, (i - 2 * SEG) // PRE)
    pos = lambda i: jnp.where(i < 2 * SEG, i % SEG, i % PRE)
    is_mem = lambda i: (i < 2 * SEG) & (i % SEG < M)
    same = head(r) == head(c)
    allowed = same & (is_mem(r) | is_mem(c) | (pos(r) >= pos(c)))
    return jnp.where(allowed, 0.0, jnp.where(same, -1e9 * LOG2E, -jnp.inf)).astype(f32)


def _kernel(zero_hbm, x_hbm, mem0_hbm, wq_hbm, wk_hbm, wv_hbm, wo_hbm,
            u_hbm, p0, p1, p2, p3, p4, p5, ldt_hbm, dsk_hbm, fs_hbm, g_hbm,
            out_hbm,
            wq, wk, wv, wo, xb, xs, h_ref, outs, fill_ref,
            praw, par, us, taps, vb, vm, vu, pacc, yf, outb, vec, vraw, fs_ref, g_ref, zero_ref,
            sem_s, sem_w, sem_o, sem_xb, sem_x, sem_p, sem_u, sem_out, pre, own, lo0, lo1):
    wqkv = (wq, wk, wv)
    scale = E ** -0.5

    whbm = [w.bitcast(u32) for w in (wq_hbm, wk_hbm, wv_hbm)]

    def wcp(j, m, p):
        return pltpu.make_async_copy(whbm[m].at[:, p, j, :], wqkv[m].at[p, j], sem_w.at[(j * 3 + m) * 2 + p])

    xu = x_hbm.bitcast(u32)
    xcs = [pltpu.make_async_copy(xu.at[:, t, pl.ds(0, PRE // 2), pl.ds(c * 128, 128)],
                                 xb.at[c, :, pl.ds(t * (PRE // 2), PRE // 2), :], sem_xb.at[2 * c + t])
           for c in range(8) for t in range(2)]
    xcp1 = pltpu.make_async_copy(x_hbm.at[:, :, pl.ds(PRE, TOK), :], xs, sem_x.at[0])
    pcs = [pltpu.make_async_copy(p, praw.at[k], sem_p.at[k]) for k, p in enumerate((p0, p1, p2, p3, p4, p5))]
    ccs = [pltpu.make_async_copy(fs_hbm, fs_ref, sem_p.at[6]), pltpu.make_async_copy(g_hbm, g_ref, sem_p.at[7])]
    wou = wo_hbm.bitcast(u32)
    ocs = [pltpu.make_async_copy(wou.at[:, pl.ds(c * 128, 128)], wo.at[c], sem_o.at[c]) for c in range(8)]
    uu = u_hbm.bitcast(u32)
    ucs = [pltpu.make_async_copy(uu.at[:, pl.ds(c * 128, 128)], us.at[c], sem_u.at[c]) for c in range(NT)]

    zcp = pltpu.make_async_copy(zero_hbm, zero_ref, sem_s.at[0])
    scs = [pltpu.make_async_copy(mem0_hbm, h_ref.at[pl.ds(0, M)], sem_s.at[1]),
           pltpu.make_async_copy(ldt_hbm, vraw.at[0], sem_s.at[2]),
           pltpu.make_async_copy(dsk_hbm, vraw.at[1], sem_s.at[3])]
    w0cs = [[pltpu.make_async_copy(whbm[0].at[pl.ds(half * (DM // 4), DM // 4), p, 0, :],
                                   wq.at[p, 0, pl.ds(half * (DM // 4), DM // 4)], sem_s.at[4 + 2 * half + p])
             for p in range(2)] for half in range(2)]
    for cp in [zcp] + w0cs[0] + xcs[:8]:
        cp.start()
    vu[pl.ds(8, 8), :] = pltpu.bitcast(jnp.full((8, 128), 0x0000FFFF, u32), f32)
    vu[pl.ds(16, 8), :] = pltpu.bitcast(jnp.full((8, 128), 0xFFFF0000, u32), f32)
    taps[...] = jnp.zeros(taps.shape, f32)
    yf[1] = jnp.zeros(yf.shape[1:], u32)
    fill_ref[...] = _attn_fill()
    for cp in w0cs[1] + xcs[8:] + scs:
        cp.start()
    zcp.wait()

    def opaque_row(k, buf):
        return pl.multiple_of(jnp.clip(zero_ref[k] * 8, 0, buf.shape[0] - 8), 8)

    bufs = (vb, vm, vu, par)
    fence_rows = [opaque_row(0, b) for b in bufs]
    done_vb, done_vm = opaque_row(1, vb), opaque_row(1, vm)

    class Pacer:
        def __init__(self, segments):
            self.t = 0.0
            self.todo = []
            for (pieces, buf, t0, t1) in segments:
                total = float(sum(c for c, _ in pieces)) or 1.0
                done = 0.0
                for (cst, fn) in pieces:
                    self.todo.append((t0 + (t1 - t0) * done / total, fn, buf))
                    done += cst

        def __call__(self, v, dt=1.0):
            self.t += dt
            fenced = []
            while self.todo and self.todo[0][0] < self.t:
                _, fn, buf = self.todo.pop(0)
                if not any(b is buf for b in fenced):
                    buf[pl.ds([r for b, r in zip(bufs, fence_rows) if b is buf][0], 8), :] = v
                    fenced.append(buf)
                fn()

        def finished(self):
            return not self.todo

    def unpair(j, m, r0, nr):
        def fn():
            rows = pl.ds(r0, nr)
            m_lo = jnp.tile(pltpu.bitcast(vu[pl.ds(8, 8), :], u32), (nr // 8, 1))
            m_hi = jnp.tile(pltpu.bitcast(vu[pl.ds(16, 8), :], u32), (nr // 8, 1))
            a = wqkv[m][0, j, rows, :]
            b = wqkv[m][1, j, rows, :]
            wqkv[m][0, j, rows, :] = (a & m_lo) | ((b & m_lo) << 16)
            wqkv[m][1, j, rows, :] = ((a & m_hi) >> 16) | (b & m_hi)
        return (nr, fn)

    def unpair_pieces(items, lo=0, hi=DM // 2):
        return [unpair(j, m, r0, UNP) for (j, m) in items for r0 in range(lo, hi, UNP)]

    items = [(j, m) for j in range(NP) for m in range(3)]
    wcs = lambda lo, hi: [wcp(j, m, p) for (j, m) in items[lo:hi] for p in range(2)]
    rest = ocs + ccs + ucs + [xcp1]
    starts = [[] for _ in range(2 * len(items))]
    n_w, n_r = 1, 0
    for unit in sorted(STARTS):
        w_hi, with_par, r_hi = STARTS[unit]
        starts[unit] = (pcs if with_par else []) + wcs(n_w, w_hi) + rest[n_r:r_hi]
        n_w, n_r = w_hi, r_hi
    assert n_w == len(items) and n_r == len(rest)
    with jax.named_scope("bulk"):
        if QUICK in (1, 2):
            for cp in wcs(1, 48) + pcs + ocs + ucs + [xcp1] + ccs:
                cp.start()
            for cp in wcs(1, 48) + pcs + scs + xcs + w0cs[0] + w0cs[1]:
                cp.wait()
            vec[...] = vraw[...].astype(f32)
            for _, fn in (unpair_pieces(items) + sum(_prep_pieces(praw, vec, par), [])) if QUICK != 2 else []:
                fn()

            def kg(r, carry):
                for odd in range(2):
                    for _, fn in _kgen_pieces(0, (r, odd), par, vb, taps, 0, done_vb, BKNI, BKSPLIT):
                        fn()
                return carry
            lax.fori_loop(0, 4, kg, 0)
            for (j, m) in (items if QUICK != 2 else []):
                def chunk(rc, carry, j=j, m=m):
                    lhs = jnp.concatenate(
                        [pltpu.bitcast(xb[c, pl.ds(rc * 4, 4)].reshape(32, 128), bf16) for c in range(8)], axis=1)
                    res = [jnp.dot(lhs, pltpu.bitcast(wqkv[m][p, j], bf16), preferred_element_type=f32)
                           for p in range(2)]
                    for t in range(8):
                        v = jnp.concatenate([res[0][8 * t:8 * t + 8], res[1][8 * t:8 * t + 8]], axis=0)
                        pre[rc * 8 + t, m * NP + j] = v.astype(bf16)
                    return carry
                lax.fori_loop(0, 8, chunk, 0)
            items = []
        n_chunk = 2 * (T0 // RC)
        prep = _prep_pieces(praw, vec, par)
        kg0 = [pc for r in range(8) for pc in _kgen_pieces(0, r, par, vb, taps, 0, done_vb, BKNI, BKSPLIT)]
        t_a, t_b, t_c, t_d = [v * n_chunk for v in BPLAN]
        fence_x = Pacer([(prep[0], par, t_a, t_b), (kg0, vb, t_b, t_c), (prep[1], par, t_c, t_d)])
        landed = 1
        for it, (j, m) in enumerate(items):
            fence_w = None
            for half in range(2):
                for cp in starts[2 * it + half]:
                    cp.start()
                if it == 0:
                    with jax.named_scope("waitx%d" % half):
                        for cp in w0cs[half] + xcs[8 * half:8 * half + 8]:
                            cp.wait()
                    for _, fn in unpair_pieces(items[:1], half * (DM // 4), (half + 1) * (DM // 4)):
                        fn()
                    fence_w = Pacer([])
                elif half == 0:
                    late = landed == it
                    if it in WAITS:
                        with jax.named_scope("wait%d" % it):
                            for cp in wcs(landed, WAITS[it]) + (pcs + scs if it == PAR_WAIT else []):
                                cp.wait()
                        landed = WAITS[it]
                        if it == PAR_WAIT:
                            vec[...] = vraw[...].astype(f32)
                    if late:
                        for _, fn in unpair_pieces(items[it:it + 1]):
                            fn()
                    fence_w = Pacer([(unpair_pieces(items[it + 1:min(it + 2, landed)]), vu, 0.0, n_chunk * UNP_FRAC)])
                for p in range(2):
                    w = pltpu.bitcast(wqkv[m][p, j, pl.ds(half * (DM // 4), DM // 4), :], bf16)
                    lhs = jnp.concatenate([pltpu.bitcast(xb[c].reshape(T0 // 2, 128), bf16)
                                           for c in range(4 * half, 4 * half + 4)], axis=1)
                    res = jnp.dot(lhs, w, preferred_element_type=f32)
                    for rc in range(T0 // RC):
                        rows = pl.ds(rc * RC, RC)
                        v = res[rc * RC:(rc + 1) * RC]
                        if half == 1:
                            v = v + pacc[p, rows, :]
                        if p == 0 or half == 0:
                            pacc[p, rows, :] = v
                        else:
                            v0 = pacc[0, rows, :]
                            for t in range(RC // PRE):
                                pr = jnp.concatenate([v0[PRE * t:PRE * (t + 1)], v[PRE * t:PRE * (t + 1)]], axis=0)
                                pre[rc * (RC // PRE) + t, m * NP + j] = pr.astype(bf16)
                        fence_w(v[:8], 0.5)
                        fence_x(v[:8], 0.5)
            assert fence_w.finished() and landed > it
        assert QUICK or fence_x.finished()
    with jax.named_scope("waitrest"):
        for cp in ocs + ucs + ccs + [xcp1]:
            cp.wait()

    def outa_cp(row, n):
        return pltpu.make_async_copy(outs.at[pl.ds(row, n)], out_hbm.at[pl.ds(row, n), pl.ds(0, DM)], sem_out.at[0])

    def outb_cp(c, row, n, sem):
        col = DM + c * 128
        return pltpu.make_async_copy(
            outb.at[c, pl.ds(row, n)],
            out_hbm.at[pl.ds(row, n), pl.ds(col if isinstance(col, int) else pl.multiple_of(col, 128), 128)],
            sem_out.at[sem])

    def one_step(i, odd, fwd, fence):
        s = 2 * i + odd
        lo_cur = (lo0, lo1)[odd]
        base = pl.multiple_of(2 * SEG * i, 2 * SEG)
        h_ref[pl.ds(M, TOK), :] = xs[i, odd]
        h = h_ref[...]
        scores = {}
        probs = {}

        ct = i >> 2
        r = s & 7
        buf = ct & 1
        cprev = (ct + NT - 1) & (NT - 1)

        def stage_a(j):
            for m in range(3):
                for p in range(2):
                    w = pltpu.bitcast(wqkv[m][p, j], bf16)
                    res = jnp.dot(h, w, preferred_element_type=f32)
                    own[m * NP + j, pl.ds(SEG * p, SEG), :] = res.astype(bf16)
                    fence(res[:M])

        def gather(m, j):
            return pltpu.bitcast(jnp.concatenate([own.bitcast(u32)[m * NP + j],
                                                  pre.bitcast(u32)[s, m * NP + j]], axis=0), bf16)

        def stage_qk(j):
            scores[j] = lax.dot_general(gather(0, j), gather(1, j), (((1,), (1,)), ((), ())),
                                        preferred_element_type=f32)

        def stage_b(j):
            fl = fill_ref[...]
            sc = jnp.where(fl == 0.0, scores.pop(j) * (scale * LOG2E), fl)
            e = jnp.exp2(sc - jnp.max(sc, axis=-1, keepdims=True))
            den = jnp.sum(e, axis=-1, keepdims=True)
            probs[j] = (e * pl.reciprocal(den, approx=True)).astype(bf16)

        def stage_c(j):
            o = jnp.dot(probs[j], gather(2, j), preferred_element_type=f32)
            for p in range(2):
                hh = 2 * j + p
                lo_cur[hh, pl.ds(0, SEG), :] = o[p * SEG:(p + 1) * SEG].astype(bf16)
                ob = o[2 * SEG + p * PRE:2 * SEG + (p + 1) * PRE]
                lo1[hh, pl.ds(SEG + odd * PRE, PRE), :] = ob.astype(bf16)

        acc = [None] * 8

        def stage_d(h0, h1, last=False):
            lhs = jnp.concatenate([_ld16(lo_cur, hh, slice(None)) for hh in range(h0, h1)], axis=1)
            for c in range(8):
                w = pltpu.bitcast(wo[c, pl.ds(h0 * 64, (h1 - h0) * 64), :], bf16)
                res = jnp.dot(lhs, w, preferred_element_type=f32)
                acc[c] = res if acc[c] is None else acc[c] + res
                if not last:
                    fence(res[:M], (h1 - h0) / 8.0 * (DW_ODD if odd else 1.0))
                else:
                    rb = acc[c].astype(bf16)
                    cols = pl.ds(c * 128, 128)
                    h_ref[pl.ds(0, M), cols] = rb[:M]
                    outs[pl.ds(base + (odd * SEG + PRE), TOK), cols] = rb[M:SEG]
                    if odd:
                        outs[pl.ds(base, PRE), cols] = rb[SEG:SEG + PRE]
                        outs[pl.ds(base + SEG, PRE), cols] = rb[SEG + PRE:]

        def attn_group(jq, jc):
            for j in jq:
                stage_qk(j)
            for j in jc:
                stage_c(j)
            for j in jq:
                stage_b(j)

        for t in range(2):
            _inv_piece(cprev, 2 * r + t, 1 - buf, g_ref, us, vec, yf, outb)
        for p in fwd:
            p()
        for j in range(NP):
            stage_a(j)
            if j >= 2 and j % 2 == 0:
                attn_group((j - 2, j - 1), (j - 4, j - 3) if j >= 4 else ())
        stage_d(0, 8)
        attn_group((14, 15), (12, 13))
        stage_d(8, 20)
        attn_group((), (14, 15))
        stage_d(20, 28)
        stage_d(28, 32, last=True)

    def two_steps(i, carry):
        ct = i >> 2
        cprev = (ct + NT - 1) & (NT - 1)
        conv = [_conv_pieces(ct, (i & 3, odd), ct & 1, fs_ref, us, taps, vm, yf,
                             done_vm) for odd in range(2)]
        kgen = [_kgen_pieces((ct + 1) & (NT - 1), (i & 3, odd), par, vb, taps, ct + 1,
                             done_vb, KNI, KSPLIT) for odd in range(2)]
        work = {'k0': (kgen[0], vb), 'k1': (kgen[1], vb), 'm0': (conv[0][1], vm), 'm1': (conv[1][1], vm)}
        fence = Pacer([work[k] + (t0, t1) for (k, t0, t1) in PLAN if k[0] not in NOB])
        for odd in range(2):
            one_step(i, odd, conv[odd][0], fence)
        assert fence.finished() or NOB
        outa_cp(pl.multiple_of(2 * SEG * i, 2 * SEG), 2 * SEG).start()
        outb_cp(cprev, pl.multiple_of((i & 3) * 512, 512), 512, jnp.where(i < 4, 2, 1)).start()
        return carry

    with jax.named_scope("steps"):
        if NITER:
            lax.fori_loop(0, NITER, two_steps, 0)

    with jax.named_scope("flush"):
        outb_cp(NT - 1, 0, L, 2).wait()
        for b in range(NBLK):
            _inv_piece(NT - 1, b, (NT - 1) % 2, g_ref, us, vec, yf, outb)
            if b % 4 == 3:
                outb_cp(NT - 1, (b - 3) * BLK, 4 * BLK, 1).start()
    with jax.named_scope("waitout"):
        outa_cp(0, S).wait()
        pltpu.make_async_copy(outb, outb, sem_out.at[1]).wait()


@jax.jit
def pallas_concat_heads__memory_aug_recurrent_mem_tr__ssm_conv_s4__prompt_kernel(
    A_x, A_mem0, A_Wq, A_Wk, A_Wv, A_Wo, A_seg_len,
    B_u, B_A_re, B_A_im, B_B_re, B_B_im, B_C_re, B_C_im, B_log_dt, B_Dskip,
):
    del A_seg_len
    assert A_x.shape == (1, S, DM) and B_u.shape == (1, L, D)
    fs, g = _dft_consts()
    w4 = lambda w: w.reshape(DM // 2, 2, H, E)
    any_ = pl.BlockSpec(memory_space=pl.ANY)
    V = pltpu.VMEM
    out = pl.pallas_call(
        _kernel,
        out_shape=jax.ShapeDtypeStruct((S, DM + D), bf16),
        in_specs=[any_] * 18,
        out_specs=any_,
        scratch_shapes=[
            V((2, NP, DM // 2, E), u32),
            V((2, NP, DM // 2, E), u32),
            V((2, NP, DM // 2, E), u32),
            V((8, H * E // 2, 128), u32),
            V((8, NSEG // 2, PRE, 128), u32),
            V((NSEG // 2, 2, TOK, DM), bf16),
            V((M + TOK, DM), bf16),
            V((S, DM), bf16),
            V((2 * (SEG + M), 2 * (SEG + M)), f32),
            V((6, D, N), bf16),
            V((8 + NT * 6 * N, 128), f32),
            V((NT, L // 2, 128), u32),
            V((NT + 1, TAPROWS, 128), f32),
            V((V_ROWS, 128), f32),
            V((VM_ROWS, 128), f32),
            V((24, 128), f32),
            V((2, T0, 128), f32),
            V((2, NBLK, 128, 128), u32),
            V((NT, L, 128), bf16),
            V((2, 8, 128), f32),
            V((2, 8, 128), bf16),
            V((8, NBLK * 32, 128), bf16),
            V((2, BLK, 128), bf16),
            pltpu.SMEM((2,), jnp.int32),
            pltpu.SemaphoreType.DMA((8,)),
            pltpu.SemaphoreType.DMA((6 * NP,)),
            pltpu.SemaphoreType.DMA((8,)),
            pltpu.SemaphoreType.DMA((16,)),
            pltpu.SemaphoreType.DMA((1,)),
            pltpu.SemaphoreType.DMA((8,)),
            pltpu.SemaphoreType.DMA((NT,)),
            pltpu.SemaphoreType.DMA((3,)),
            V((NSEG, 3 * NP, 2 * PRE, E), bf16),
            V((3 * NP, 2 * SEG, E), bf16),
            V((H, SEG, E), bf16),
            V((H, SEG + 2 * PRE, E), bf16),
        ],
        compiler_params=pltpu.CompilerParams(vmem_limit_bytes=110 * 1024 * 1024, disable_bounds_checks=True),
    )(jnp.asarray(np.zeros((2,), np.int32)), A_x.reshape(NSEG // 2, 2, SEG, DM), A_mem0.reshape(M, DM), w4(A_Wq), w4(A_Wk), w4(A_Wv), A_Wo.reshape(H * E, DM),
      B_u.reshape(L, D), B_A_re, B_A_im, B_B_re, B_B_im, B_C_re, B_C_im,
      B_log_dt.reshape(8, 128), B_Dskip.reshape(8, 128),
      jnp.asarray(fs, bf16), jnp.asarray(g, bf16))
    return out.reshape(1, S, DM + D)
```

```python
import functools

import numpy as np
import jax
import jax.numpy as jnp
from jax import lax
import jax.experimental.pallas as pl
import jax.experimental.pallas.tpu as pltpu

bf16, f32, u32 = jnp.bfloat16, jnp.float32, jnp.uint32

S, DM, H, E, M, SEG = 2048, 1024, 32, 128, 8, 32
NSEG = S // SEG
TOK = 24
PRE = SEG - TOK
T0 = PRE * NSEG
NP = H // 2
LOG2E = 1.4426950408889634
QUICK = False
NOB = ''
BKNI = 1
UNP = 64
UNP_FRAC = 0.7
BKSPLIT = 4
BPLAN = (10.0, 11.0, 42.5, 47.7)
WAITS = {1: 2, 2: 3, 3: 5, 4: 6, 5: 8, 7: 11, 10: 13, 12: 17, 16: 23, 22: 33, 32: 48}
PAR_WAIT = 10
STARTS = {0: (2, False, 0), 1: (3, False, 0), 2: (5, False, 0), 4: (6, False, 0), 6: (8, False, 0),
          8: (9, False, 0), 10: (11, False, 0), 14: (13, True, 0), 20: (17, False, 0), 24: (23, False, 0),
          32: (33, False, 0), 44: (48, False, 3), 64: (48, False, 19)}
NITER = NSEG // 2
KNI = 2
KSPLIT = 2
PLAN = (('k0', 0, 96), ('m0', 96, 122), ('k1', 124, 220), ('m1', 220, 260))
DW_ODD = 1.5
RC = 64
MACJ = 3
L, D, N = 2048, 1024, 128
BLK = 128
NBLK = L // BLK
NT = D // 128
TAPROWS = 672
WINDOWS = ((0, 128, 0, 1), (128, 128, 1, 1), (256, 128, 2, 1), (320, 80, 3, 1),
           (384, 128, 4, 3), (480, 48, 7, 1), (512, 128, 8, 7), (624, 32, 15, 1))

V_FENCE = 0
V_YTAB = 8
V_START = V_YTAB + 256
V_STEP = V_START + 160
V_ROWS = V_STEP + 128
V_UF = 8
V_KF = V_UF + NBLK * 32
VM_ROWS = V_KF + NBLK * 32


def _bf16_round_int(l):
    u = np.asarray(l, np.float32).view(np.uint32)
    r = (u + 0x7FFF + ((u >> 16) & 1)) & 0xFFFF0000
    return r.astype(np.uint32).view(np.float32).astype(np.int64)


def _tap_row(lp):
    return np.where(lp < 256, lp, np.where(lp < 512, 256 + (lp - 256) // 2,
                    np.where(lp < 1024, 384 + (lp - 512) // 4, 512 + (lp - 1024) // 8)))


@functools.lru_cache(maxsize=None)
def _dft_consts():
    t = np.arange(BLK)
    F = np.zeros((8, 32, BLK))
    G = np.zeros((BLK, 8, 32))
    for r in range(8):
        f = np.concatenate([16 * r + 2 * np.arange(8), 16 * r + 2 * np.arange(8) + 1])
        th = 2 * np.pi * (f + 0.5) / (2 * BLK)
        F[r, :16] = np.cos(th[:, None] * t[None])
        F[r, 16:] = -np.sin(th[:, None] * t[None])
        G[:, r, 0::2] = np.cos(th[None] * t[:, None]) / BLK
        G[:, r, 1::2] = -np.sin(th[None] * t[:, None]) / BLK
    FS = np.zeros((8, NBLK, 32, 128))
    for (w0, wn, b0, nb) in WINDOWS:
        for j in range(b0, b0 + nb):
            rows = _tap_row(_bf16_round_int(BLK * j + t)) - w0
            assert rows.min() >= 0 and rows.max() < wn
            sel = np.zeros((BLK, 128))
            sel[t, rows] = 1.0
            FS[:, j] = F @ sel
    return (FS.reshape(8, NBLK * 32, 128).astype(np.float32),
            G.reshape(BLK, 2, 128).transpose(1, 0, 2).astype(np.float32))


def _ld16(ref, *idx):
    return pltpu.bitcast(ref.bitcast(u32)[idx + (slice(None),)], bf16)


def _cmul(a, b):
    return (a[0] * b[0] - a[1] * b[1], a[0] * b[1] + a[1] * b[0])


def _csq(a):
    return (a[0] * a[0] - a[1] * a[1], 2.0 * (a[0] * a[1]))


def _cexp(lr, li):
    k = jnp.floor(li * (2.0 / np.pi) + 0.5)
    r = ((li - k * 1.5703125) - k * 4.837512969970703125e-4) - k * 7.54978995489188216e-8
    r = jnp.clip(r, -0.8, 0.8)
    r2 = r * r
    s = r + r * r2 * (-1.6666654611e-1 + r2 * (8.3321608736e-3 + r2 * -1.9515295891e-4))
    c = (1.0 - 0.5 * r2) + (r2 * r2) * (4.166664568298827e-2
                                        + r2 * (-1.388731625493765e-3 + r2 * 2.443315711809948e-5))
    q = k.astype(jnp.int32)
    swap = (q & 1) == 1
    m = jnp.exp(lr)
    flip = lambda v, bit: pltpu.bitcast(pltpu.bitcast(v, jnp.int32) ^ (bit << 30), f32)
    return (flip(m * jnp.where(swap, s, c), (q + 1) & 2), flip(m * jnp.where(swap, c, s), q & 2))


def _par_row(c, k):
    return 8 + (c * 6 + k) * N


def _prep_pieces(praw, vec, par):
    def stage1(c):
        def fn():
            tr = lambda k: praw[k, pl.ds(c * 128, 128), :].astype(f32).T
            dt = jnp.exp(vec[0, pl.ds(c, 1), :]).astype(bf16).astype(f32)
            cc = _cmul((tr(4), tr(5)), (dt * tr(2), dt * tr(3)))
            for k, v in ((0, dt * tr(0)), (1, dt * tr(1)), (4, cc[0]), (5, cc[1])):
                par[pl.ds(_par_row(c, k), N), :] = v
        return fn

    def stage2(c, n0):
        def fn():
            lr = par[pl.ds(_par_row(c, 0) + n0, 16), :]
            li = par[pl.ds(_par_row(c, 1) + n0, 16), :]
            for k, v in enumerate(_cexp(lr, li) + _cexp(lr * 128.0, li * 128.0)):
                par[pl.ds(_par_row(c, k) + n0, 16), :] = v
        return fn

    tile = lambda c: [(260, stage1(c))] + [(190, stage2(c, n0)) for n0 in range(0, N, 16)]
    return tile(0), [pc for c in range(1, NT) for pc in tile(c)]


def _kgen_pieces(c, r, par, vb, taps, tslot, frow, kni, ksplit):
    st = {}

    def put(row, z, h=None):
        if h is None:
            vb[pl.ds(row, 16), :] = z[0]
            vb[pl.ds(row + 16, 16), :] = z[1]
        else:
            vb[pl.ds(row + 8 * h, 8), :] = z[0]
            vb[pl.ds(row + 16 + 8 * h, 8), :] = z[1]

    def get(row, h=None):
        if h is None:
            return (vb[pl.ds(row, 16), :], vb[pl.ds(row + 16, 16), :])
        return (vb[pl.ds(row + 8 * h, 8), :], vb[pl.ds(row + 16 + 8 * h, 8), :])

    def params(k):
        if isinstance(r, int):
            return par[pl.ds(_par_row(c, k) + r * 16, 16), :]
        return par[pl.ds(pl.multiple_of(c * (6 * N) + r[0] * 32, 32) + (_par_row(0, k) + r[1] * 16), 16), :]

    def park():
        put(V_STEP, (params(0), params(1)))
        put(V_START + 32, (params(2), params(3)))
        put(V_START, (params(4), params(5)))

    def setup_y(h):
        def fn():
            z1 = get(V_STEP, h)
            z2 = _csq(z1)
            z4 = _csq(z2)
            s = lax.broadcasted_iota(jnp.int32, (8, 128), 0)
            fs = [(jnp.where((s >> k) & 1 == 1, z[0], 1.0), jnp.where((s >> k) & 1 == 1, z[1], 0.0))
                  for k, z in enumerate((z1, z2, z4))]
            y = _cmul(_cmul(fs[0], fs[1]), fs[2])
            for k in range(8):
                put(V_YTAB + 32 * k, y, h)
                if k < 7:
                    y = _cmul(y, z1)
                    y = (jnp.where(s == 7 - k, 1.0, y[0]), jnp.where(s == 7 - k, 0.0, y[1]))
            z = z4
            for k in range(4):
                z = _csq(z)
                put(V_STEP + 32 * k, z, h)
        return fn

    def setup_hi():
        z = get(V_START + 32)
        cf = get(V_START)
        for g in range(1, 5):
            put(V_START + 32 * g, _cmul(cf, z))
            if g < 4:
                z = _csq(z)

    def square(k0, k1):
        def fn():
            rows = pl.ds(V_YTAB + 32 * k0, 32 * (k1 - k0))
            y = vb[rows, :].reshape(k1 - k0, 2, 16, 128)
            vb[rows, :] = jnp.stack(_csq((y[:, 0], y[:, 1])), axis=1).reshape(32 * (k1 - k0), 128)
        return fn

    def rows_of(g, i0, ni):
        n_i = 16 + (g == 4)

        def fn():
            x = st.pop('x') if i0 > 0 else get(V_START + 32 * g)
            step = get(V_STEP + 32 * max(g - 1, 0))
            xs = []
            for t in range(ni):
                xs.append(x)
                if i0 + t + 1 < n_i:
                    x = _cmul(x, step)
            if i0 + ni < n_i:
                st['x'] = x
            acc = [None] * ni
            for k0 in range(0, 8, ksplit):
                y = vb[pl.ds(V_YTAB + 32 * k0, 32 * ksplit), :].reshape(ksplit, 2, 16, 128)
                for t in range(ni):
                    v = xs[t][0][None] * y[:, 0] - xs[t][1][None] * y[:, 1]
                    v = v[:, :8] + v[:, 8:]
                    for k in range(ksplit):
                        vk = pltpu.roll(v[k], k0 + k, 0) if k0 + k else v[k]
                        acc[t] = vk if acc[t] is None else acc[t] + vk
                if k0 + ksplit < 8:
                    vb[pl.ds(frow, 8), :] = acc[ni - 1]
            for t in range(ni):
                row = 128 * g + 8 * (i0 + t)
                a = acc[t]
                if row == 640:
                    a = jnp.where(lax.broadcasted_iota(jnp.int32, (8, 128), 0) == 0, a, 0.0)
                taps[tslot, pl.ds(row, 8), :] = taps[tslot, pl.ds(row, 8), :] + a
                if t == ni - 1:
                    vb[pl.ds(frow, 8), :] = a
        return fn

    pieces = [(30, park), (110, setup_y(0)), (110, setup_y(1)), (80, setup_hi)]
    for g in range(5):
        if g >= 2:
            pieces += [(40, square(0, 4)), (40, square(4, 8))]
        for i0 in range(0, 16 + (g == 4), kni):
            ni = min(kni, 16 + (g == 4) - i0)
            pieces.append((83 * ni, rows_of(g, i0, ni)))
    return pieces


def _conv_pieces(c, r, buf, fs_ref, us, taps, vb, yf, frow):
    st = {}

    def fwd_u(b0, b1):
        def fn():
            lhs = _ld16(fs_ref, 2 * r[0] + r[1], pl.ds(0, 16))
            for b in range(b0, b1):
                w = pltpu.bitcast(us[c, pl.ds(b * 64, 64), :], bf16)
                res = jnp.dot(lhs, w, preferred_element_type=f32)
                row = V_UF + 32 * b
                if b == 0:
                    vb[pl.ds(row, 32), :] = res
                else:
                    p = st['prev']
                    vb[pl.ds(row, 8), :] = res[0:8] - p[16:24]
                    vb[pl.ds(row + 8, 8), :] = res[8:16] + p[24:32]
                    vb[pl.ds(row + 16, 8), :] = res[16:24] + p[0:8]
                    vb[pl.ds(row + 24, 8), :] = res[24:32] - p[8:16]
                st['prev'] = res
        return fn

    def fwd_k(jobs):
        def fn():
            for (wi, t0, nb) in jobs:
                w0, wn, b0, _ = WINDOWS[wi]
                lhs = _ld16(fs_ref, 2 * r[0] + r[1], pl.ds((b0 + t0) * 16, nb * 16))[:, :wn]
                w = taps[c, pl.ds(w0, wn), :].astype(bf16)
                vb[pl.ds(V_KF + 32 * (b0 + t0), 32 * nb), :] = jnp.dot(lhs, w, preferred_element_type=f32)
        return fn

    def mac(q, i0, ni, j0, j1):
        def fn():
            ld = lambda base, b: (vb[pl.ds(base + 32 * b + 8 * q, 8), :], vb[pl.ds(base + 32 * b + 16 + 8 * q, 8), :])
            zr, zi = st.pop('z') if j0 > 0 else ({}, {})
            ucache = {}
            for j in range(j0, j1):
                kr, ki = ld(V_KF, j)
                for i in range(max(i0, j), i0 + ni):
                    if i - j not in ucache:
                        ucache[i - j] = ld(V_UF, i - j)
                    ur, ui = ucache[i - j]
                    if i not in zr:
                        zr[i] = kr * ur - ki * ui
                        zi[i] = kr * ui + ki * ur
                    else:
                        zr[i] = zr[i] + kr * ur - ki * ui
                        zi[i] = zi[i] + kr * ui + ki * ur
            vb[pl.ds(frow, 8), :] = zr[i0 + ni - 1]
            if j1 < i0 + ni:
                st['z'] = (zr, zi)
            else:
                row = pl.multiple_of(r[0] * 32, 32) + (r[1] * 16 + q * 8)
                for i in range(i0, i0 + ni):
                    yf[buf, i, pl.ds(row, 8), :] = pltpu.pack_elementwise([zr[i], zi[i]], packed_dtype=bf16)
        return (8 * sum(1 for j in range(j0, j1) for i in range(max(i0, j), i0 + ni)), fn)

    fwd = [fwd_u(0, 8), fwd_u(8, 16), fwd_k(((0, 0, 1), (1, 0, 1), (2, 0, 1), (3, 0, 1))),
           fwd_k(((4, 0, 2), (6, 0, 2), (6, 2, 2), (6, 4, 2))), fwd_k(((4, 2, 1), (5, 0, 1), (6, 6, 1), (7, 0, 1)))]
    macs = []
    for q in range(2):
        for i0 in range(0, NBLK, 2):
            for j0 in range(0, i0 + 2, MACJ):
                macs.append(mac(q, i0, 2, j0, min(j0 + MACJ, i0 + 2)))
    return fwd, macs


def _inv_piece(c, b, buf, g_ref, us, vec, yf, outb):
    rows = pl.ds(pl.multiple_of(b * 64, 64), 64)
    w = pltpu.bitcast(yf[buf, b], bf16)
    g = jnp.concatenate([_ld16(g_ref, k, slice(None)) for k in range(2)], axis=1)
    y = jnp.dot(g, w, preferred_element_type=f32)
    u = pltpu.bitcast(us[c, rows, :], bf16).astype(f32)
    sk = (u * vec[1, pl.ds(c, 1), :]).astype(bf16).astype(f32)
    o = (y.astype(bf16).astype(f32) + sk).astype(bf16)
    outb[c, pl.ds(pl.multiple_of(b * BLK, BLK) if not isinstance(b, int) else b * BLK, BLK), :] = o


def _attn_fill():
    n = 2 * (SEG + M)
    r = lax.broadcasted_iota(jnp.int32, (n, n), 0)
    c = lax.broadcasted_iota(jnp.int32, (n, n), 1)
    head = lambda i: jnp.where(i < 2 * SEG, i // SEG, (i - 2 * SEG) // PRE)
    pos = lambda i: jnp.where(i < 2 * SEG, i % SEG, i % PRE)
    is_mem = lambda i: (i < 2 * SEG) & (i % SEG < M)
    same = head(r) == head(c)
    allowed = same & (is_mem(r) | is_mem(c) | (pos(r) >= pos(c)))
    return jnp.where(allowed, 0.0, jnp.where(same, -1e9 * LOG2E, -jnp.inf)).astype(f32)


def _kernel(zero_hbm, x_hbm, mem0_hbm, wq_hbm, wk_hbm, wv_hbm, wo_hbm,
            u_hbm, p0, p1, p2, p3, p4, p5, ldt_hbm, dsk_hbm, fs_hbm, g_hbm,
            out_hbm,
            wq, wk, wv, wo, xb, xs, h_ref, outs, fill_ref,
            praw, par, us, taps, vb, vm, vu, pacc, yf, outb, vec, vraw, fs_ref, g_ref, zero_ref,
            sem_s, sem_w, sem_o, sem_xb, sem_x, sem_p, sem_u, sem_out, pre, own, lo0, lo1):
    wqkv = (wq, wk, wv)
    scale = E ** -0.5

    whbm = [w.bitcast(u32) for w in (wq_hbm, wk_hbm, wv_hbm)]

    def wcp(j, m, p):
        return pltpu.make_async_copy(whbm[m].at[:, p, j, :], wqkv[m].at[p, j], sem_w.at[(j * 3 + m) * 2 + p])

    xu = x_hbm.bitcast(u32)
    xcs = [pltpu.make_async_copy(xu.at[:, t, pl.ds(0, PRE // 2), pl.ds(c * 128, 128)],
                                 xb.at[c, :, pl.ds(t * (PRE // 2), PRE // 2), :], sem_xb.at[2 * c + t])
           for c in range(8) for t in range(2)]
    xcp1 = pltpu.make_async_copy(x_hbm.at[:, :, pl.ds(PRE, TOK), :], xs, sem_x.at[0])
    pcs = [pltpu.make_async_copy(p, praw.at[k], sem_p.at[k]) for k, p in enumerate((p0, p1, p2, p3, p4, p5))]
    ccs = [pltpu.make_async_copy(fs_hbm, fs_ref, sem_p.at[6]), pltpu.make_async_copy(g_hbm, g_ref, sem_p.at[7])]
    wou = wo_hbm.bitcast(u32)
    ocs = [pltpu.make_async_copy(wou.at[:, pl.ds(c * 128, 128)], wo.at[c], sem_o.at[c]) for c in range(8)]
    uu = u_hbm.bitcast(u32)
    ucs = [pltpu.make_async_copy(uu.at[:, pl.ds(c * 128, 128)], us.at[c], sem_u.at[c]) for c in range(NT)]

    zcp = pltpu.make_async_copy(zero_hbm, zero_ref, sem_s.at[0])
    scs = [pltpu.make_async_copy(mem0_hbm, h_ref.at[pl.ds(0, M)], sem_s.at[1]),
           pltpu.make_async_copy(ldt_hbm, vraw.at[0], sem_s.at[2]),
           pltpu.make_async_copy(dsk_hbm, vraw.at[1], sem_s.at[3])]
    w0cs = [[pltpu.make_async_copy(whbm[0].at[pl.ds(half * (DM // 4), DM // 4), p, 0, :],
                                   wq.at[p, 0, pl.ds(half * (DM // 4), DM // 4)], sem_s.at[4 + 2 * half + p])
             for p in range(2)] for half in range(2)]
    for cp in [zcp] + w0cs[0] + xcs[:8]:
        cp.start()
    vu[pl.ds(8, 8), :] = pltpu.bitcast(jnp.full((8, 128), 0x0000FFFF, u32), f32)
    vu[pl.ds(16, 8), :] = pltpu.bitcast(jnp.full((8, 128), 0xFFFF0000, u32), f32)
    taps[...] = jnp.zeros(taps.shape, f32)
    yf[1] = jnp.zeros(yf.shape[1:], u32)
    fill_ref[...] = _attn_fill()
    for cp in w0cs[1] + xcs[8:] + scs:
        cp.start()
    zcp.wait()

    def opaque_row(k, buf):
        return pl.multiple_of(jnp.clip(zero_ref[k] * 8, 0, buf.shape[0] - 8), 8)

    bufs = (vb, vm, vu, par)
    fence_rows = [opaque_row(0, b) for b in bufs]
    done_vb, done_vm = opaque_row(1, vb), opaque_row(1, vm)

    class Pacer:
        def __init__(self, segments):
            self.t = 0.0
            self.todo = []
            for (pieces, buf, t0, t1) in segments:
                total = float(sum(c for c, _ in pieces)) or 1.0
                done = 0.0
                for (cst, fn) in pieces:
                    self.todo.append((t0 + (t1 - t0) * done / total, fn, buf))
                    done += cst

        def __call__(self, v, dt=1.0):
            self.t += dt
            fenced = []
            while self.todo and self.todo[0][0] < self.t:
                _, fn, buf = self.todo.pop(0)
                if not any(b is buf for b in fenced):
                    buf[pl.ds([r for b, r in zip(bufs, fence_rows) if b is buf][0], 8), :] = v
                    fenced.append(buf)
                fn()

        def finished(self):
            return not self.todo

    def unpair(j, m, r0, nr):
        def fn():
            rows = pl.ds(r0, nr)
            m_lo = pltpu.bitcast(vu[pl.ds(8, 8), :], u32)[None]
            m_hi = pltpu.bitcast(vu[pl.ds(16, 8), :], u32)[None]
            a = wqkv[m][0, j, rows, :].reshape(nr // 8, 8, E)
            b = wqkv[m][1, j, rows, :].reshape(nr // 8, 8, E)
            wqkv[m][0, j, rows, :] = ((a & m_lo) | ((b & m_lo) << 16)).reshape(nr, E)
            wqkv[m][1, j, rows, :] = (((a & m_hi) >> 16) | (b & m_hi)).reshape(nr, E)
        return (nr, fn)

    def unpair_pieces(items, lo=0, hi=DM // 2):
        return [unpair(j, m, r0, UNP) for (j, m) in items for r0 in range(lo, hi, UNP)]

    items = [(j, m) for j in range(NP) for m in range(3)]
    wcs = lambda lo, hi: [wcp(j, m, p) for (j, m) in items[lo:hi] for p in range(2)]
    rest = ocs + ccs + ucs + [xcp1]
    starts = [[] for _ in range(2 * len(items))]
    n_w, n_r = 1, 0
    for unit in sorted(STARTS):
        w_hi, with_par, r_hi = STARTS[unit]
        starts[unit] = (pcs if with_par else []) + wcs(n_w, w_hi) + rest[n_r:r_hi]
        n_w, n_r = w_hi, r_hi
    assert n_w == len(items) and n_r == len(rest)
    with jax.named_scope("bulk"):
        if QUICK in (1, 2):
            for cp in wcs(1, 48) + pcs + ocs + ucs + [xcp1] + ccs:
                cp.start()
            for cp in wcs(1, 48) + pcs + scs + xcs + w0cs[0] + w0cs[1]:
                cp.wait()
            vec[...] = vraw[...].astype(f32)
            for _, fn in (unpair_pieces(items) + sum(_prep_pieces(praw, vec, par), [])) if QUICK != 2 else []:
                fn()

            def kg(r, carry):
                for odd in range(2):
                    for _, fn in _kgen_pieces(0, (r, odd), par, vb, taps, 0, done_vb, BKNI, BKSPLIT):
                        fn()
                return carry
            lax.fori_loop(0, 4, kg, 0)
            for (j, m) in (items if QUICK != 2 else []):
                def chunk(rc, carry, j=j, m=m):
                    lhs = jnp.concatenate(
                        [pltpu.bitcast(xb[c, pl.ds(rc * 4, 4)].reshape(32, 128), bf16) for c in range(8)], axis=1)
                    res = [jnp.dot(lhs, pltpu.bitcast(wqkv[m][p, j], bf16), preferred_element_type=f32)
                           for p in range(2)]
                    for t in range(8):
                        v = jnp.concatenate([res[0][8 * t:8 * t + 8], res[1][8 * t:8 * t + 8]], axis=0)
                        pre[rc * 8 + t, m * NP + j] = v.astype(bf16)
                    return carry
                lax.fori_loop(0, 8, chunk, 0)
            items = []
        n_chunk = 2 * (T0 // RC)
        prep = _prep_pieces(praw, vec, par)
        kg0 = [pc for r in range(8) for pc in _kgen_pieces(0, r, par, vb, taps, 0, done_vb, BKNI, BKSPLIT)]
        t_a, t_b, t_c, t_d = [v * n_chunk for v in BPLAN]
        fence_x = Pacer([(prep[0], par, t_a, t_b), (kg0, vb, t_b, t_c), (prep[1], par, t_c, t_d)])
        landed = 1
        for it, (j, m) in enumerate(items):
            fence_w = None
            for half in range(2):
                for cp in starts[2 * it + half]:
                    cp.start()
                if it == 0:
                    with jax.named_scope("waitx%d" % half):
                        for cp in w0cs[half] + xcs[8 * half:8 * half + 8]:
                            cp.wait()
                    for _, fn in unpair_pieces(items[:1], half * (DM // 4), (half + 1) * (DM // 4)):
                        fn()
                    fence_w = Pacer([])
                elif half == 0:
                    late = landed == it
                    if it in WAITS:
                        with jax.named_scope("wait%d" % it):
                            for cp in wcs(landed, WAITS[it]) + (pcs + scs if it == PAR_WAIT else []):
                                cp.wait()
                        landed = WAITS[it]
                        if it == PAR_WAIT:
                            vec[...] = vraw[...].astype(f32)
                    if late:
                        for _, fn in unpair_pieces(items[it:it + 1]):
                            fn()
                    fence_w = Pacer([(unpair_pieces(items[it + 1:min(it + 2, landed)]), vu, 0.0, n_chunk * UNP_FRAC)])
                for p in range(2):
                    w = pltpu.bitcast(wqkv[m][p, j, pl.ds(half * (DM // 4), DM // 4), :], bf16)
                    lhs = jnp.concatenate([pltpu.bitcast(xb[c].reshape(T0 // 2, 128), bf16)
                                           for c in range(4 * half, 4 * half + 4)], axis=1)
                    res = jnp.dot(lhs, w, preferred_element_type=f32)
                    for rc in range(T0 // RC):
                        rows = pl.ds(rc * RC, RC)
                        v = res[rc * RC:(rc + 1) * RC]
                        if half == 1:
                            v = v + pacc[p, rows, :]
                        if p == 0 or half == 0:
                            pacc[p, rows, :] = v
                        else:
                            pr = jnp.concatenate([pacc[0, rows, :].reshape(RC // PRE, PRE, E),
                                                  v.reshape(RC // PRE, PRE, E)], axis=1)
                            pre[pl.ds(rc * (RC // PRE), RC // PRE), m * NP + j] = pr.astype(bf16)
                        fence_w(v[:8], 0.5)
                        fence_x(v[:8], 0.5)
            assert fence_w.finished() and landed > it
        assert QUICK or fence_x.finished()
    with jax.named_scope("waitrest"):
        for cp in ocs + ucs + ccs + [xcp1]:
            cp.wait()

    def outa_cp(row, n):
        return pltpu.make_async_copy(outs.at[pl.ds(row, n)], out_hbm.at[pl.ds(row, n), pl.ds(0, DM)], sem_out.at[0])

    def outb_cp(c, row, n, sem):
        col = DM + c * 128
        return pltpu.make_async_copy(
            outb.at[c, pl.ds(row, n)],
            out_hbm.at[pl.ds(row, n), pl.ds(col if isinstance(col, int) else pl.multiple_of(col, 128), 128)],
            sem_out.at[sem])

    def one_step(i, odd, fwd, fence):
        s = 2 * i + odd
        lo_cur = (lo0, lo1)[odd]
        base = pl.multiple_of(2 * SEG * i, 2 * SEG)
        h_ref[pl.ds(M, TOK), :] = xs[i, odd]
        h = h_ref[...]
        scores = {}
        probs = {}

        ct = i >> 2
        r = s & 7
        buf = ct & 1
        cprev = (ct + NT - 1) & (NT - 1)

        def stage_a(j):
            for m in range(3):
                for p in range(2):
                    w = pltpu.bitcast(wqkv[m][p, j], bf16)
                    res = jnp.dot(h, w, preferred_element_type=f32)
                    own[m * NP + j, pl.ds(SEG * p, SEG), :] = res.astype(bf16)
                    fence(res[:M])

        def gather(m, j):
            return pltpu.bitcast(jnp.concatenate([own.bitcast(u32)[m * NP + j],
                                                  pre.bitcast(u32)[s, m * NP + j]], axis=0), bf16)

        def stage_qk(j):
            scores[j] = lax.dot_general(gather(0, j), gather(1, j), (((1,), (1,)), ((), ())),
                                        preferred_element_type=f32)

        def stage_b(j):
            fl = fill_ref[...]
            sc = jnp.where(fl == 0.0, scores.pop(j) * (scale * LOG2E), fl)
            e = jnp.exp2(sc - jnp.max(sc, axis=-1, keepdims=True))
            den = jnp.sum(e, axis=-1, keepdims=True)
            probs[j] = (e * pl.reciprocal(den, approx=True)).astype(bf16)

        def stage_c(j):
            o = jnp.dot(probs[j], gather(2, j), preferred_element_type=f32)
            for p in range(2):
                hh = 2 * j + p
                lo_cur[hh, pl.ds(0, SEG), :] = o[p * SEG:(p + 1) * SEG].astype(bf16)
                ob = o[2 * SEG + p * PRE:2 * SEG + (p + 1) * PRE]
                lo1[hh, pl.ds(SEG + odd * PRE, PRE), :] = ob.astype(bf16)

        acc = [None] * 8

        def stage_d(h0, h1, last=False):
            lhs = jnp.concatenate([_ld16(lo_cur, hh, slice(None)) for hh in range(h0, h1)], axis=1)
            for c in range(8):
                w = pltpu.bitcast(wo[c, pl.ds(h0 * 64, (h1 - h0) * 64), :], bf16)
                res = jnp.dot(lhs, w, preferred_element_type=f32)
                acc[c] = res if acc[c] is None else acc[c] + res
                if not last:
                    fence(res[:M], (h1 - h0) / 8.0 * (DW_ODD if odd else 1.0))
                else:
                    rb = acc[c].astype(bf16)
                    cols = pl.ds(c * 128, 128)
                    h_ref[pl.ds(0, M), cols] = rb[:M]
                    outs[pl.ds(base + (odd * SEG + PRE), TOK), cols] = rb[M:SEG]
                    if odd:
                        outs[pl.ds(base, PRE), cols] = rb[SEG:SEG + PRE]
                        outs[pl.ds(base + SEG, PRE), cols] = rb[SEG + PRE:]

        def attn_group(jq, jc):
            for j in jq:
                stage_qk(j)
            for j in jc:
                stage_c(j)
            for j in jq:
                stage_b(j)

        for t in range(2):
            _inv_piece(cprev, 2 * r + t, 1 - buf, g_ref, us, vec, yf, outb)
        for p in fwd:
            p()
        for j in range(NP):
            stage_a(j)
            if j >= 2 and j % 2 == 0:
                attn_group((j - 2, j - 1), (j - 4, j - 3) if j >= 4 else ())
        stage_d(0, 8)
        attn_group((14, 15), (12, 13))
        stage_d(8, 20)
        attn_group((), (14, 15))
        stage_d(20, 28)
        stage_d(28, 32, last=True)

    def two_steps(i, carry):
        ct = i >> 2
        cprev = (ct + NT - 1) & (NT - 1)
        conv = [_conv_pieces(ct, (i & 3, odd), ct & 1, fs_ref, us, taps, vm, yf,
                             done_vm) for odd in range(2)]
        kgen = [_kgen_pieces((ct + 1) & (NT - 1), (i & 3, odd), par, vb, taps, ct + 1,
                             done_vb, KNI, KSPLIT) for odd in range(2)]
        work = {'k0': (kgen[0], vb), 'k1': (kgen[1], vb), 'm0': (conv[0][1], vm), 'm1': (conv[1][1], vm)}
        fence = Pacer([work[k] + (t0, t1) for (k, t0, t1) in PLAN if k[0] not in NOB])
        for odd in range(2):
            one_step(i, odd, conv[odd][0], fence)
        assert fence.finished() or NOB
        outa_cp(pl.multiple_of(2 * SEG * i, 2 * SEG), 2 * SEG).start()
        outb_cp(cprev, pl.multiple_of((i & 3) * 512, 512), 512, jnp.where(i < 4, 2, 1)).start()
        return carry

    with jax.named_scope("steps"):
        if NITER:
            lax.fori_loop(0, NITER, two_steps, 0)

    with jax.named_scope("flush"):
        outb_cp(NT - 1, 0, L, 2).wait()
        for b in range(NBLK):
            _inv_piece(NT - 1, b, (NT - 1) % 2, g_ref, us, vec, yf, outb)
            if b % 4 == 3:
                outb_cp(NT - 1, (b - 3) * BLK, 4 * BLK, 1).start()
    with jax.named_scope("waitout"):
        outa_cp(0, S).wait()
        pltpu.make_async_copy(outb, outb, sem_out.at[1]).wait()


@jax.jit
def pallas_concat_heads__memory_aug_recurrent_mem_tr__ssm_conv_s4__prompt_kernel(
    A_x, A_mem0, A_Wq, A_Wk, A_Wv, A_Wo, A_seg_len,
    B_u, B_A_re, B_A_im, B_B_re, B_B_im, B_C_re, B_C_im, B_log_dt, B_Dskip,
):
    del A_seg_len
    assert A_x.shape == (1, S, DM) and B_u.shape == (1, L, D)
    fs, g = _dft_consts()
    w4 = lambda w: w.reshape(DM // 2, 2, H, E)
    any_ = pl.BlockSpec(memory_space=pl.ANY)
    V = pltpu.VMEM
    out = pl.pallas_call(
        _kernel,
        out_shape=jax.ShapeDtypeStruct((S, DM + D), bf16),
        in_specs=[any_] * 18,
        out_specs=any_,
        scratch_shapes=[
            V((2, NP, DM // 2, E), u32),
            V((2, NP, DM // 2, E), u32),
            V((2, NP, DM // 2, E), u32),
            V((8, H * E // 2, 128), u32),
            V((8, NSEG // 2, PRE, 128), u32),
            V((NSEG // 2, 2, TOK, DM), bf16),
            V((M + TOK, DM), bf16),
            V((S, DM), bf16),
            V((2 * (SEG + M), 2 * (SEG + M)), f32),
            V((6, D, N), bf16),
            V((8 + NT * 6 * N, 128), f32),
            V((NT, L // 2, 128), u32),
            V((NT + 1, TAPROWS, 128), f32),
            V((V_ROWS, 128), f32),
            V((VM_ROWS, 128), f32),
            V((24, 128), f32),
            V((2, T0, 128), f32),
            V((2, NBLK, 128, 128), u32),
            V((NT, L, 128), bf16),
            V((2, 8, 128), f32),
            V((2, 8, 128), bf16),
            V((8, NBLK * 32, 128), bf16),
            V((2, BLK, 128), bf16),
            pltpu.SMEM((2,), jnp.int32),
            pltpu.SemaphoreType.DMA((8,)),
            pltpu.SemaphoreType.DMA((6 * NP,)),
            pltpu.SemaphoreType.DMA((8,)),
            pltpu.SemaphoreType.DMA((16,)),
            pltpu.SemaphoreType.DMA((1,)),
            pltpu.SemaphoreType.DMA((8,)),
            pltpu.SemaphoreType.DMA((NT,)),
            pltpu.SemaphoreType.DMA((3,)),
            V((NSEG, 3 * NP, 2 * PRE, E), bf16),
            V((3 * NP, 2 * SEG, E), bf16),
            V((H, SEG, E), bf16),
            V((H, SEG + 2 * PRE, E), bf16),
        ],
        compiler_params=pltpu.CompilerParams(vmem_limit_bytes=110 * 1024 * 1024, disable_bounds_checks=True),
    )(jnp.asarray(np.zeros((2,), np.int32)), A_x.reshape(NSEG // 2, 2, SEG, DM), A_mem0.reshape(M, DM), w4(A_Wq), w4(A_Wk), w4(A_Wv), A_Wo.reshape(H * E, DM),
      B_u.reshape(L, D), B_A_re, B_A_im, B_B_re, B_B_im, B_C_re, B_C_im,
      B_log_dt.reshape(8, 128), B_Dskip.reshape(8, 128),
      jnp.asarray(fs, bf16), jnp.asarray(g, bf16))
    return out.reshape(1, S, DM + D)
```

```python
import functools

import numpy as np
import jax
import jax.numpy as jnp
from jax import lax
import jax.experimental.pallas as pl
import jax.experimental.pallas.tpu as pltpu

bf16, f32, u32 = jnp.bfloat16, jnp.float32, jnp.uint32

S, DM, H, E, M, SEG = 2048, 1024, 32, 128, 8, 32
NSEG = S // SEG
TOK = 24
PRE = SEG - TOK
T0 = PRE * NSEG
NP = H // 2
LOG2E = 1.4426950408889634
QUICK = False
NOB = ''
BKNI = 1
UNP = 64
UNP_FRAC = 0.7
BKSPLIT = 4
BPLAN = (10.0, 11.0, 42.5, 47.7)
WAITS = {1: 2, 2: 3, 3: 5, 4: 6, 5: 8, 7: 11, 10: 13, 12: 17, 16: 23, 22: 33, 32: 48}
PAR_WAIT = 10
STARTS = {0: (2, False, 0), 1: (3, False, 0), 2: (5, False, 0), 4: (6, False, 0), 6: (8, False, 0),
          8: (9, False, 0), 10: (11, False, 0), 14: (13, True, 0), 20: (17, False, 0), 24: (23, False, 0),
          32: (33, False, 0), 44: (48, False, 3), 64: (48, False, 19)}
NITER = NSEG // 2
KNI = 2
KSPLIT = 2
PLAN = (('k0', 0, 96), ('m0', 96, 122), ('k1', 124, 220), ('m1', 220, 260))
DW_ODD = 1.5
RC = 64
MACJ = 3
L, D, N = 2048, 1024, 128
BLK = 128
NBLK = L // BLK
NT = D // 128
TAPROWS = 672
WINDOWS = ((0, 128, 0, 1), (128, 128, 1, 1), (256, 128, 2, 1), (320, 80, 3, 1),
           (384, 128, 4, 3), (480, 48, 7, 1), (512, 128, 8, 7), (624, 32, 15, 1))

V_FENCE = 0
V_YTAB = 8
V_START = V_YTAB + 256
V_STEP = V_START + 160
V_ROWS = V_STEP + 128
V_UF = 8
V_KF = V_UF + NBLK * 32
VM_ROWS = V_KF + NBLK * 32


def _bf16_round_int(l):
    u = np.asarray(l, np.float32).view(np.uint32)
    r = (u + 0x7FFF + ((u >> 16) & 1)) & 0xFFFF0000
    return r.astype(np.uint32).view(np.float32).astype(np.int64)


def _tap_row(lp):
    return np.where(lp < 256, lp, np.where(lp < 512, 256 + (lp - 256) // 2,
                    np.where(lp < 1024, 384 + (lp - 512) // 4, 512 + (lp - 1024) // 8)))


@functools.lru_cache(maxsize=None)
def _dft_consts():
    t = np.arange(BLK)
    F = np.zeros((8, 32, BLK))
    G = np.zeros((BLK, 8, 32))
    for r in range(8):
        f = np.concatenate([16 * r + 2 * np.arange(8), 16 * r + 2 * np.arange(8) + 1])
        th = 2 * np.pi * (f + 0.5) / (2 * BLK)
        F[r, :16] = np.cos(th[:, None] * t[None])
        F[r, 16:] = -np.sin(th[:, None] * t[None])
        G[:, r, 0::2] = np.cos(th[None] * t[:, None]) / BLK
        G[:, r, 1::2] = -np.sin(th[None] * t[:, None]) / BLK
    FS = np.zeros((8, NBLK, 32, 128))
    for (w0, wn, b0, nb) in WINDOWS:
        for j in range(b0, b0 + nb):
            rows = _tap_row(_bf16_round_int(BLK * j + t)) - w0
            assert rows.min() >= 0 and rows.max() < wn
            sel = np.zeros((BLK, 128))
            sel[t, rows] = 1.0
            FS[:, j] = F @ sel
    return (FS.reshape(8, NBLK * 32, 128).astype(np.float32),
            G.reshape(BLK, 2, 128).transpose(1, 0, 2).astype(np.float32))


def _ld16(ref, *idx):
    return pltpu.bitcast(ref.bitcast(u32)[idx + (slice(None),)], bf16)


def _cmul(a, b):
    return (a[0] * b[0] - a[1] * b[1], a[0] * b[1] + a[1] * b[0])


def _csq(a):
    return (a[0] * a[0] - a[1] * a[1], 2.0 * (a[0] * a[1]))


def _cexp(lr, li):
    k = jnp.floor(li * (2.0 / np.pi) + 0.5)
    r = ((li - k * 1.5703125) - k * 4.837512969970703125e-4) - k * 7.54978995489188216e-8
    r = jnp.clip(r, -0.8, 0.8)
    r2 = r * r
    s = r + r * r2 * (-1.6666654611e-1 + r2 * (8.3321608736e-3 + r2 * -1.9515295891e-4))
    c = (1.0 - 0.5 * r2) + (r2 * r2) * (4.166664568298827e-2
                                        + r2 * (-1.388731625493765e-3 + r2 * 2.443315711809948e-5))
    q = k.astype(jnp.int32)
    swap = (q & 1) == 1
    m = jnp.exp(lr)
    flip = lambda v, bit: pltpu.bitcast(pltpu.bitcast(v, jnp.int32) ^ (bit << 30), f32)
    return (flip(m * jnp.where(swap, s, c), (q + 1) & 2), flip(m * jnp.where(swap, c, s), q & 2))


def _par_row(c, k):
    return 8 + (c * 6 + k) * N


def _prep_pieces(praw, vec, par):
    def stage1(c):
        def fn():
            tr = lambda k: praw[k, pl.ds(c * 128, 128), :].astype(f32).T
            dt = jnp.exp(vec[0, pl.ds(c, 1), :]).astype(bf16).astype(f32)
            cc = _cmul((tr(4), tr(5)), (dt * tr(2), dt * tr(3)))
            for k, v in ((0, dt * tr(0)), (1, dt * tr(1)), (4, cc[0]), (5, cc[1])):
                par[pl.ds(_par_row(c, k), N), :] = v
        return fn

    def stage2(c, n0):
        def fn():
            lr = par[pl.ds(_par_row(c, 0) + n0, 16), :]
            li = par[pl.ds(_par_row(c, 1) + n0, 16), :]
            for k, v in enumerate(_cexp(lr, li) + _cexp(lr * 128.0, li * 128.0)):
                par[pl.ds(_par_row(c, k) + n0, 16), :] = v
        return fn

    tile = lambda c: [(260, stage1(c))] + [(190, stage2(c, n0)) for n0 in range(0, N, 16)]
    return tile(0), [pc for c in range(1, NT) for pc in tile(c)]


def _kgen_pieces(c, r, par, vb, taps, tslot, frow, kni, ksplit):
    st = {}

    def put(row, z, h=None):
        if h is None:
            vb[pl.ds(row, 16), :] = z[0]
            vb[pl.ds(row + 16, 16), :] = z[1]
        else:
            vb[pl.ds(row + 8 * h, 8), :] = z[0]
            vb[pl.ds(row + 16 + 8 * h, 8), :] = z[1]

    def get(row, h=None):
        if h is None:
            return (vb[pl.ds(row, 16), :], vb[pl.ds(row + 16, 16), :])
        return (vb[pl.ds(row + 8 * h, 8), :], vb[pl.ds(row + 16 + 8 * h, 8), :])

    def ytab(k0, k1):
        return [vb[pl.ds(V_YTAB + 128 * part + 16 * k0, 16 * (k1 - k0)), :].reshape(k1 - k0, 16, 128)
                for part in range(2)]

    def params(k):
        if isinstance(r, int):
            return par[pl.ds(_par_row(c, k) + r * 16, 16), :]
        return par[pl.ds(pl.multiple_of(c * (6 * N) + r[0] * 32, 32) + (_par_row(0, k) + r[1] * 16), 16), :]

    def park():
        put(V_STEP, (params(0), params(1)))
        put(V_START + 32, (params(2), params(3)))
        put(V_START, (params(4), params(5)))

    def setup_y(h):
        def fn():
            z1 = get(V_STEP, h)
            z2 = _csq(z1)
            z4 = _csq(z2)
            s = lax.broadcasted_iota(jnp.int32, (8, 128), 0)
            fs = [(jnp.where((s >> k) & 1 == 1, z[0], 1.0), jnp.where((s >> k) & 1 == 1, z[1], 0.0))
                  for k, z in enumerate((z1, z2, z4))]
            y = _cmul(_cmul(fs[0], fs[1]), fs[2])
            for k in range(8):
                vb[pl.ds(V_YTAB + 16 * k + 8 * h, 8), :] = y[0]
                vb[pl.ds(V_YTAB + 128 + 16 * k + 8 * h, 8), :] = y[1]
                if k < 7:
                    y = _cmul(y, z1)
                    y = (jnp.where(s == 7 - k, 1.0, y[0]), jnp.where(s == 7 - k, 0.0, y[1]))
            z = z4
            for k in range(4):
                z = _csq(z)
                put(V_STEP + 32 * k, z, h)
        return fn

    def setup_hi():
        z = get(V_START + 32)
        cf = get(V_START)
        for g in range(1, 5):
            put(V_START + 32 * g, _cmul(cf, z))
            if g < 4:
                z = _csq(z)

    def square(k0, k1):
        def fn():
            rows = [pl.ds(V_YTAB + 128 * part + 16 * k0, 16 * (k1 - k0)) for part in range(2)]
            y = _csq((vb[rows[0], :], vb[rows[1], :]))
            vb[rows[0], :] = y[0]
            vb[rows[1], :] = y[1]
        return fn

    def rows_of(g, i0, ni):
        n_i = 16 + (g == 4)

        def fn():
            x = st.pop('x') if i0 > 0 else get(V_START + 32 * g)
            step = get(V_STEP + 32 * max(g - 1, 0))
            xs = []
            for t in range(ni):
                xs.append(x)
                if i0 + t + 1 < n_i:
                    x = _cmul(x, step)
            if i0 + ni < n_i:
                st['x'] = x
            acc = [None] * ni
            for k0 in range(0, 8, ksplit):
                yr, yi = ytab(k0, k0 + ksplit)
                for t in range(ni):
                    v = xs[t][0] * yr - xs[t][1] * yi
                    v = lax.slice_in_dim(v, 0, 8, axis=1) + lax.slice_in_dim(v, 8, 16, axis=1)
                    v = jnp.sum(pltpu.roll(v, k0, 1, stride=1, stride_axis=0), axis=0)
                    acc[t] = v if acc[t] is None else acc[t] + v
                if k0 + ksplit < 8:
                    vb[pl.ds(frow, 8), :] = acc[ni - 1]
            for t in range(ni):
                row = 128 * g + 8 * (i0 + t)
                a = acc[t]
                if row == 640:
                    a = jnp.where(lax.broadcasted_iota(jnp.int32, (8, 128), 0) == 0, a, 0.0)
                taps[tslot, pl.ds(row, 8), :] = taps[tslot, pl.ds(row, 8), :] + a
                if t == ni - 1:
                    vb[pl.ds(frow, 8), :] = a
        return fn

    pieces = [(30, park), (110, setup_y(0)), (110, setup_y(1)), (80, setup_hi)]
    for g in range(5):
        if g >= 2:
            pieces += [(40, square(0, 4)), (40, square(4, 8))]
        for i0 in range(0, 16 + (g == 4), kni):
            ni = min(kni, 16 + (g == 4) - i0)
            pieces.append((83 * ni, rows_of(g, i0, ni)))
    return pieces


def _conv_pieces(c, r, buf, fs_ref, us, taps, vb, yf, frow):
    st = {}

    def fwd_u(b0, b1):
        def fn():
            lhs = _ld16(fs_ref, 2 * r[0] + r[1], pl.ds(0, 16))
            for b in range(b0, b1):
                w = pltpu.bitcast(us[c, pl.ds(b * 64, 64), :], bf16)
                res = jnp.dot(lhs, w, preferred_element_type=f32)
                row = V_UF + 32 * b
                if b == 0:
                    vb[pl.ds(row, 32), :] = res
                else:
                    p = st['prev']
                    vb[pl.ds(row, 8), :] = res[0:8] - p[16:24]
                    vb[pl.ds(row + 8, 8), :] = res[8:16] + p[24:32]
                    vb[pl.ds(row + 16, 8), :] = res[16:24] + p[0:8]
                    vb[pl.ds(row + 24, 8), :] = res[24:32] - p[8:16]
                st['prev'] = res
        return fn

    def fwd_k(jobs):
        def fn():
            for (wi, t0, nb) in jobs:
                w0, wn, b0, _ = WINDOWS[wi]
                lhs = _ld16(fs_ref, 2 * r[0] + r[1], pl.ds((b0 + t0) * 16, nb * 16))[:, :wn]
                w = taps[c, pl.ds(w0, wn), :].astype(bf16)
                vb[pl.ds(V_KF + 32 * (b0 + t0), 32 * nb), :] = jnp.dot(lhs, w, preferred_element_type=f32)
        return fn

    def mac(q, i0, ni, j0, j1):
        def fn():
            ld = lambda base, b: (vb[pl.ds(base + 32 * b + 8 * q, 8), :], vb[pl.ds(base + 32 * b + 16 + 8 * q, 8), :])
            zr, zi = st.pop('z') if j0 > 0 else ({}, {})
            ucache = {}
            for j in range(j0, j1):
                kr, ki = ld(V_KF, j)
                for i in range(max(i0, j), i0 + ni):
                    if i - j not in ucache:
                        ucache[i - j] = ld(V_UF, i - j)
                    ur, ui = ucache[i - j]
                    if i not in zr:
                        zr[i] = kr * ur - ki * ui
                        zi[i] = kr * ui + ki * ur
                    else:
                        zr[i] = zr[i] + kr * ur - ki * ui
                        zi[i] = zi[i] + kr * ui + ki * ur
            vb[pl.ds(frow, 8), :] = zr[i0 + ni - 1]
            if j1 < i0 + ni:
                st['z'] = (zr, zi)
            else:
                row = pl.multiple_of(r[0] * 32, 32) + (r[1] * 16 + q * 8)
                for i in range(i0, i0 + ni):
                    yf[buf, i, pl.ds(row, 8), :] = pltpu.pack_elementwise([zr[i], zi[i]], packed_dtype=bf16)
        return (8 * sum(1 for j in range(j0, j1) for i in range(max(i0, j), i0 + ni)), fn)

    fwd = [fwd_u(0, 8), fwd_u(8, 16), fwd_k(((0, 0, 1), (1, 0, 1), (2, 0, 1), (3, 0, 1))),
           fwd_k(((4, 0, 2), (6, 0, 2), (6, 2, 2), (6, 4, 2))), fwd_k(((4, 2, 1), (5, 0, 1), (6, 6, 1), (7, 0, 1)))]
    macs = []
    for q in range(2):
        for i0 in range(0, NBLK, 2):
            for j0 in range(0, i0 + 2, MACJ):
                macs.append(mac(q, i0, 2, j0, min(j0 + MACJ, i0 + 2)))
    return fwd, macs


def _inv_piece(c, b, buf, g_ref, us, vec, yf, outb):
    rows = pl.ds(pl.multiple_of(b * 64, 64), 64)
    w = pltpu.bitcast(yf[buf, b], bf16)
    g = jnp.concatenate([_ld16(g_ref, k, slice(None)) for k in range(2)], axis=1)
    y = jnp.dot(g, w, preferred_element_type=f32)
    u = pltpu.bitcast(us[c, rows, :], bf16).astype(f32)
    sk = (u * vec[1, pl.ds(c, 1), :]).astype(bf16).astype(f32)
    o = (y.astype(bf16).astype(f32) + sk).astype(bf16)
    outb[c, pl.ds(pl.multiple_of(b * BLK, BLK) if not isinstance(b, int) else b * BLK, BLK), :] = o


def _attn_fill():
    n = 2 * (SEG + M)
    r = lax.broadcasted_iota(jnp.int32, (n, n), 0)
    c = lax.broadcasted_iota(jnp.int32, (n, n), 1)
    head = lambda i: jnp.where(i < 2 * SEG, i // SEG, (i - 2 * SEG) // PRE)
    pos = lambda i: jnp.where(i < 2 * SEG, i % SEG, i % PRE)
    is_mem = lambda i: (i < 2 * SEG) & (i % SEG < M)
    same = head(r) == head(c)
    allowed = same & (is_mem(r) | is_mem(c) | (pos(r) >= pos(c)))
    return jnp.where(allowed, 0.0, jnp.where(same, -1e9 * LOG2E, -jnp.inf)).astype(f32)


def _kernel(zero_hbm, x_hbm, mem0_hbm, wq_hbm, wk_hbm, wv_hbm, wo_hbm,
            u_hbm, p0, p1, p2, p3, p4, p5, ldt_hbm, dsk_hbm, fs_hbm, g_hbm,
            out_hbm,
            wq, wk, wv, wo, xb, xs, h_ref, outs, fill_ref,
            praw, par, us, taps, vb, vm, vu, pacc, yf, outb, vec, vraw, fs_ref, g_ref, zero_ref,
            sem_s, sem_w, sem_o, sem_xb, sem_x, sem_p, sem_u, sem_out, pre, own, lo0, lo1):
    wqkv = (wq, wk, wv)
    scale = E ** -0.5

    whbm = [w.bitcast(u32) for w in (wq_hbm, wk_hbm, wv_hbm)]

    def wcp(j, m, p):
        return pltpu.make_async_copy(whbm[m].at[:, p, j, :], wqkv[m].at[p, j], sem_w.at[(j * 3 + m) * 2 + p])

    xu = x_hbm.bitcast(u32)
    xcs = [pltpu.make_async_copy(xu.at[:, t, pl.ds(0, PRE // 2), pl.ds(c * 128, 128)],
                                 xb.at[c, :, pl.ds(t * (PRE // 2), PRE // 2), :], sem_xb.at[2 * c + t])
           for c in range(8) for t in range(2)]
    xcp1 = pltpu.make_async_copy(x_hbm.at[:, :, pl.ds(PRE, TOK), :], xs, sem_x.at[0])
    pcs = [pltpu.make_async_copy(p, praw.at[k], sem_p.at[k]) for k, p in enumerate((p0, p1, p2, p3, p4, p5))]
    ccs = [pltpu.make_async_copy(fs_hbm, fs_ref, sem_p.at[6]), pltpu.make_async_copy(g_hbm, g_ref, sem_p.at[7])]
    wou = wo_hbm.bitcast(u32)
    ocs = [pltpu.make_async_copy(wou.at[:, pl.ds(c * 128, 128)], wo.at[c], sem_o.at[c]) for c in range(8)]
    uu = u_hbm.bitcast(u32)
    ucs = [pltpu.make_async_copy(uu.at[:, pl.ds(c * 128, 128)], us.at[c], sem_u.at[c]) for c in range(NT)]

    zcp = pltpu.make_async_copy(zero_hbm, zero_ref, sem_s.at[0])
    scs = [pltpu.make_async_copy(mem0_hbm, h_ref.at[pl.ds(0, M)], sem_s.at[1]),
           pltpu.make_async_copy(ldt_hbm, vraw.at[0], sem_s.at[2]),
           pltpu.make_async_copy(dsk_hbm, vraw.at[1], sem_s.at[3])]
    w0cs = [[pltpu.make_async_copy(whbm[0].at[pl.ds(half * (DM // 4), DM // 4), p, 0, :],
                                   wq.at[p, 0, pl.ds(half * (DM // 4), DM // 4)], sem_s.at[4 + 2 * half + p])
             for p in range(2)] for half in range(2)]
    for cp in [zcp] + w0cs[0] + xcs[:8]:
        cp.start()
    vu[pl.ds(8, 8), :] = pltpu.bitcast(jnp.full((8, 128), 0x0000FFFF, u32), f32)
    vu[pl.ds(16, 8), :] = pltpu.bitcast(jnp.full((8, 128), 0xFFFF0000, u32), f32)
    taps[...] = jnp.zeros(taps.shape, f32)
    yf[1] = jnp.zeros(yf.shape[1:], u32)
    fill_ref[...] = _attn_fill()
    for cp in w0cs[1] + xcs[8:] + scs:
        cp.start()
    zcp.wait()

    def opaque_row(k, buf):
        return pl.multiple_of(jnp.clip(zero_ref[k] * 8, 0, buf.shape[0] - 8), 8)

    bufs = (vb, vm, vu, par)
    fence_rows = [opaque_row(0, b) for b in bufs]
    done_vb, done_vm = opaque_row(1, vb), opaque_row(1, vm)

    class Pacer:
        def __init__(self, segments):
            self.t = 0.0
            self.todo = []
            for (pieces, buf, t0, t1) in segments:
                total = float(sum(c for c, _ in pieces)) or 1.0
                done = 0.0
                for (cst, fn) in pieces:
                    self.todo.append((t0 + (t1 - t0) * done / total, fn, buf))
                    done += cst

        def __call__(self, v, dt=1.0):
            self.t += dt
            fenced = []
            while self.todo and self.todo[0][0] < self.t:
                _, fn, buf = self.todo.pop(0)
                if not any(b is buf for b in fenced):
                    buf[pl.ds([r for b, r in zip(bufs, fence_rows) if b is buf][0], 8), :] = v
                    fenced.append(buf)
                fn()

        def finished(self):
            return not self.todo

    def unpair(j, m, r0, nr):
        def fn():
            rows = pl.ds(r0, nr)
            m_lo = pltpu.bitcast(vu[pl.ds(8, 8), :], u32)[None]
            m_hi = pltpu.bitcast(vu[pl.ds(16, 8), :], u32)[None]
            a = wqkv[m][0, j, rows, :].reshape(nr // 8, 8, E)
            b = wqkv[m][1, j, rows, :].reshape(nr // 8, 8, E)
            wqkv[m][0, j, rows, :] = ((a & m_lo) | ((b & m_lo) << 16)).reshape(nr, E)
            wqkv[m][1, j, rows, :] = (((a & m_hi) >> 16) | (b & m_hi)).reshape(nr, E)
        return (nr, fn)

    def unpair_pieces(items, lo=0, hi=DM // 2):
        return [unpair(j, m, r0, UNP) for (j, m) in items for r0 in range(lo, hi, UNP)]

    items = [(j, m) for j in range(NP) for m in range(3)]
    wcs = lambda lo, hi: [wcp(j, m, p) for (j, m) in items[lo:hi] for p in range(2)]
    rest = ocs + ccs + ucs + [xcp1]
    starts = [[] for _ in range(2 * len(items))]
    n_w, n_r = 1, 0
    for unit in sorted(STARTS):
        w_hi, with_par, r_hi = STARTS[unit]
        starts[unit] = (pcs if with_par else []) + wcs(n_w, w_hi) + rest[n_r:r_hi]
        n_w, n_r = w_hi, r_hi
    assert n_w == len(items) and n_r == len(rest)
    with jax.named_scope("bulk"):
        if QUICK in (1, 2):
            for cp in wcs(1, 48) + pcs + ocs + ucs + [xcp1] + ccs:
                cp.start()
            for cp in wcs(1, 48) + pcs + scs + xcs + w0cs[0] + w0cs[1]:
                cp.wait()
            vec[...] = vraw[...].astype(f32)
            for _, fn in (unpair_pieces(items) + sum(_prep_pieces(praw, vec, par), [])) if QUICK != 2 else []:
                fn()

            def kg(r, carry):
                for odd in range(2):
                    for _, fn in _kgen_pieces(0, (r, odd), par, vb, taps, 0, done_vb, BKNI, BKSPLIT):
                        fn()
                return carry
            lax.fori_loop(0, 4, kg, 0)
            for (j, m) in (items if QUICK != 2 else []):
                def chunk(rc, carry, j=j, m=m):
                    lhs = jnp.concatenate(
                        [pltpu.bitcast(xb[c, pl.ds(rc * 4, 4)].reshape(32, 128), bf16) for c in range(8)], axis=1)
                    res = [jnp.dot(lhs, pltpu.bitcast(wqkv[m][p, j], bf16), preferred_element_type=f32)
                           for p in range(2)]
                    for t in range(8):
                        v = jnp.concatenate([res[0][8 * t:8 * t + 8], res[1][8 * t:8 * t + 8]], axis=0)
                        pre[rc * 8 + t, m * NP + j] = v.astype(bf16)
                    return carry
                lax.fori_loop(0, 8, chunk, 0)
            items = []
        n_chunk = 2 * (T0 // RC)
        prep = _prep_pieces(praw, vec, par)
        kg0 = [pc for r in range(8) for pc in _kgen_pieces(0, r, par, vb, taps, 0, done_vb, BKNI, BKSPLIT)]
        t_a, t_b, t_c, t_d = [v * n_chunk for v in BPLAN]
        fence_x = Pacer([(prep[0], par, t_a, t_b), (kg0, vb, t_b, t_c), (prep[1], par, t_c, t_d)])
        landed = 1
        for it, (j, m) in enumerate(items):
            fence_w = None
            for half in range(2):
                for cp in starts[2 * it + half]:
                    cp.start()
                if it == 0:
                    with jax.named_scope("waitx%d" % half):
                        for cp in w0cs[half] + xcs[8 * half:8 * half + 8]:
                            cp.wait()
                    for _, fn in unpair_pieces(items[:1], half * (DM // 4), (half + 1) * (DM // 4)):
                        fn()
                    fence_w = Pacer([])
                elif half == 0:
                    late = landed == it
                    if it in WAITS:
                        with jax.named_scope("wait%d" % it):
                            for cp in wcs(landed, WAITS[it]) + (pcs + scs if it == PAR_WAIT else []):
                                cp.wait()
                        landed = WAITS[it]
                        if it == PAR_WAIT:
                            vec[...] = vraw[...].astype(f32)
                    if late:
                        for _, fn in unpair_pieces(items[it:it + 1]):
                            fn()
                    fence_w = Pacer([(unpair_pieces(items[it + 1:min(it + 2, landed)]), vu, 0.0, n_chunk * UNP_FRAC)])
                for p in range(2):
                    w = pltpu.bitcast(wqkv[m][p, j, pl.ds(half * (DM // 4), DM // 4), :], bf16)
                    lhs = jnp.concatenate([pltpu.bitcast(xb[c].reshape(T0 // 2, 128), bf16)
                                           for c in range(4 * half, 4 * half + 4)], axis=1)
                    res = jnp.dot(lhs, w, preferred_element_type=f32)
                    for rc in range(T0 // RC):
                        rows = pl.ds(rc * RC, RC)
                        v = res[rc * RC:(rc + 1) * RC]
                        if half == 1:
                            v = v + pacc[p, rows, :]
                        if p == 0 or half == 0:
                            pacc[p, rows, :] = v
                        else:
                            pr = jnp.concatenate([pacc[0, rows, :].reshape(RC // PRE, PRE, E),
                                                  v.reshape(RC // PRE, PRE, E)], axis=1)
                            pre[pl.ds(rc * (RC // PRE), RC // PRE), m * NP + j] = pr.astype(bf16)
                        fence_w(v[:8], 0.5)
                        fence_x(v[:8], 0.5)
            assert fence_w.finished() and landed > it
        assert QUICK or fence_x.finished()
    with jax.named_scope("waitrest"):
        for cp in ocs + ucs + ccs + [xcp1]:
            cp.wait()

    def outa_cp(row, n):
        return pltpu.make_async_copy(outs.at[pl.ds(row, n)], out_hbm.at[pl.ds(row, n), pl.ds(0, DM)], sem_out.at[0])

    def outb_cp(c, row, n, sem):
        col = DM + c * 128
        return pltpu.make_async_copy(
            outb.at[c, pl.ds(row, n)],
            out_hbm.at[pl.ds(row, n), pl.ds(col if isinstance(col, int) else pl.multiple_of(col, 128), 128)],
            sem_out.at[sem])

    def one_step(i, odd, fwd, fence):
        s = 2 * i + odd
        lo_cur = (lo0, lo1)[odd]
        base = pl.multiple_of(2 * SEG * i, 2 * SEG)
        h_ref[pl.ds(M, TOK), :] = xs[i, odd]
        h = h_ref[...]
        scores = {}
        probs = {}

        ct = i >> 2
        r = s & 7
        buf = ct & 1
        cprev = (ct + NT - 1) & (NT - 1)

        def stage_a(j):
            for m in range(3):
                for p in range(2):
                    w = pltpu.bitcast(wqkv[m][p, j], bf16)
                    res = jnp.dot(h, w, preferred_element_type=f32)
                    own[m * NP + j, pl.ds(SEG * p, SEG), :] = res.astype(bf16)
                    fence(res[:M])

        def gather(m, j):
            return pltpu.bitcast(jnp.concatenate([own.bitcast(u32)[m * NP + j],
                                                  pre.bitcast(u32)[s, m * NP + j]], axis=0), bf16)

        def stage_qk(j):
            scores[j] = lax.dot_general(gather(0, j), gather(1, j), (((1,), (1,)), ((), ())),
                                        preferred_element_type=f32)

        def stage_b(j):
            fl = fill_ref[...]
            sc = jnp.where(fl == 0.0, scores.pop(j) * (scale * LOG2E), fl)
            e = jnp.exp2(sc - jnp.max(sc, axis=-1, keepdims=True))
            den = jnp.sum(e, axis=-1, keepdims=True)
            probs[j] = (e * pl.reciprocal(den, approx=True)).astype(bf16)

        def stage_c(j):
            o = jnp.dot(probs[j], gather(2, j), preferred_element_type=f32)
            for p in range(2):
                hh = 2 * j + p
                lo_cur[hh, pl.ds(0, SEG), :] = o[p * SEG:(p + 1) * SEG].astype(bf16)
                ob = o[2 * SEG + p * PRE:2 * SEG + (p + 1) * PRE]
                lo1[hh, pl.ds(SEG + odd * PRE, PRE), :] = ob.astype(bf16)

        acc = [None] * 8

        def stage_d(h0, h1, last=False):
            lhs = jnp.concatenate([_ld16(lo_cur, hh, slice(None)) for hh in range(h0, h1)], axis=1)
            for c in range(8):
                w = pltpu.bitcast(wo[c, pl.ds(h0 * 64, (h1 - h0) * 64), :], bf16)
                res = jnp.dot(lhs, w, preferred_element_type=f32)
                acc[c] = res if acc[c] is None else acc[c] + res
                if not last:
                    fence(res[:M], (h1 - h0) / 8.0 * (DW_ODD if odd else 1.0))
                else:
                    rb = acc[c].astype(bf16)
                    cols = pl.ds(c * 128, 128)
                    h_ref[pl.ds(0, M), cols] = rb[:M]
                    outs[pl.ds(base + (odd * SEG + PRE), TOK), cols] = rb[M:SEG]
                    if odd:
                        outs[pl.ds(base, PRE), cols] = rb[SEG:SEG + PRE]
                        outs[pl.ds(base + SEG, PRE), cols] = rb[SEG + PRE:]

        def attn_group(jq, jc):
            for j in jq:
                stage_qk(j)
            for j in jc:
                stage_c(j)
            for j in jq:
                stage_b(j)

        for t in range(2):
            _inv_piece(cprev, 2 * r + t, 1 - buf, g_ref, us, vec, yf, outb)
        for p in fwd:
            p()
        for j in range(NP):
            stage_a(j)
            if j >= 2 and j % 2 == 0:
                attn_group((j - 2, j - 1), (j - 4, j - 3) if j >= 4 else ())
        stage_d(0, 8)
        attn_group((14, 15), (12, 13))
        stage_d(8, 20)
        attn_group((), (14, 15))
        stage_d(20, 28)
        stage_d(28, 32, last=True)

    def two_steps(i, carry):
        ct = i >> 2
        cprev = (ct + NT - 1) & (NT - 1)
        conv = [_conv_pieces(ct, (i & 3, odd), ct & 1, fs_ref, us, taps, vm, yf,
                             done_vm) for odd in range(2)]
        kgen = [_kgen_pieces((ct + 1) & (NT - 1), (i & 3, odd), par, vb, taps, ct + 1,
                             done_vb, KNI, KSPLIT) for odd in range(2)]
        work = {'k0': (kgen[0], vb), 'k1': (kgen[1], vb), 'm0': (conv[0][1], vm), 'm1': (conv[1][1], vm)}
        fence = Pacer([work[k] + (t0, t1) for (k, t0, t1) in PLAN if k[0] not in NOB])
        for odd in range(2):
            one_step(i, odd, conv[odd][0], fence)
        assert fence.finished() or NOB
        outa_cp(pl.multiple_of(2 * SEG * i, 2 * SEG), 2 * SEG).start()
        outb_cp(cprev, pl.multiple_of((i & 3) * 512, 512), 512, jnp.where(i < 4, 2, 1)).start()
        return carry

    with jax.named_scope("steps"):
        if NITER:
            lax.fori_loop(0, NITER, two_steps, 0)

    with jax.named_scope("flush"):
        outb_cp(NT - 1, 0, L, 2).wait()
        for b in range(NBLK):
            _inv_piece(NT - 1, b, (NT - 1) % 2, g_ref, us, vec, yf, outb)
            if b % 4 == 3:
                outb_cp(NT - 1, (b - 3) * BLK, 4 * BLK, 1).start()
    with jax.named_scope("waitout"):
        outa_cp(0, S).wait()
        pltpu.make_async_copy(outb, outb, sem_out.at[1]).wait()


@jax.jit
def pallas_concat_heads__memory_aug_recurrent_mem_tr__ssm_conv_s4__prompt_kernel(
    A_x, A_mem0, A_Wq, A_Wk, A_Wv, A_Wo, A_seg_len,
    B_u, B_A_re, B_A_im, B_B_re, B_B_im, B_C_re, B_C_im, B_log_dt, B_Dskip,
):
    del A_seg_len
    assert A_x.shape == (1, S, DM) and B_u.shape == (1, L, D)
    fs, g = _dft_consts()
    w4 = lambda w: w.reshape(DM // 2, 2, H, E)
    any_ = pl.BlockSpec(memory_space=pl.ANY)
    V = pltpu.VMEM
    out = pl.pallas_call(
        _kernel,
        out_shape=jax.ShapeDtypeStruct((S, DM + D), bf16),
        in_specs=[any_] * 18,
        out_specs=any_,
        scratch_shapes=[
            V((2, NP, DM // 2, E), u32),
            V((2, NP, DM // 2, E), u32),
            V((2, NP, DM // 2, E), u32),
            V((8, H * E // 2, 128), u32),
            V((8, NSEG // 2, PRE, 128), u32),
            V((NSEG // 2, 2, TOK, DM), bf16),
            V((M + TOK, DM), bf16),
            V((S, DM), bf16),
            V((2 * (SEG + M), 2 * (SEG + M)), f32),
            V((6, D, N), bf16),
            V((8 + NT * 6 * N, 128), f32),
            V((NT, L // 2, 128), u32),
            V((NT + 1, TAPROWS, 128), f32),
            V((V_ROWS, 128), f32),
            V((VM_ROWS, 128), f32),
            V((24, 128), f32),
            V((2, T0, 128), f32),
            V((2, NBLK, 128, 128), u32),
            V((NT, L, 128), bf16),
            V((2, 8, 128), f32),
            V((2, 8, 128), bf16),
            V((8, NBLK * 32, 128), bf16),
            V((2, BLK, 128), bf16),
            pltpu.SMEM((2,), jnp.int32),
            pltpu.SemaphoreType.DMA((8,)),
            pltpu.SemaphoreType.DMA((6 * NP,)),
            pltpu.SemaphoreType.DMA((8,)),
            pltpu.SemaphoreType.DMA((16,)),
            pltpu.SemaphoreType.DMA((1,)),
            pltpu.SemaphoreType.DMA((8,)),
            pltpu.SemaphoreType.DMA((NT,)),
            pltpu.SemaphoreType.DMA((3,)),
            V((NSEG, 3 * NP, 2 * PRE, E), bf16),
            V((3 * NP, 2 * SEG, E), bf16),
            V((H, SEG, E), bf16),
            V((H, SEG + 2 * PRE, E), bf16),
        ],
        compiler_params=pltpu.CompilerParams(vmem_limit_bytes=110 * 1024 * 1024, disable_bounds_checks=True),
    )(jnp.asarray(np.zeros((2,), np.int32)), A_x.reshape(NSEG // 2, 2, SEG, DM), A_mem0.reshape(M, DM), w4(A_Wq), w4(A_Wk), w4(A_Wv), A_Wo.reshape(H * E, DM),
      B_u.reshape(L, D), B_A_re, B_A_im, B_B_re, B_B_im, B_C_re, B_C_im,
      B_log_dt.reshape(8, 128), B_Dskip.reshape(8, 128),
      jnp.asarray(fs, bf16), jnp.asarray(g, bf16))
    return out.reshape(1, S, DM + D)
```

```python
import functools

import numpy as np
import jax
import jax.numpy as jnp
from jax import lax
import jax.experimental.pallas as pl
import jax.experimental.pallas.tpu as pltpu

bf16, f32, u32 = jnp.bfloat16, jnp.float32, jnp.uint32

S, DM, H, E, M, SEG = 2048, 1024, 32, 128, 8, 32
NSEG = S // SEG
TOK = 24
PRE = SEG - TOK
T0 = PRE * NSEG
NP = H // 2
LOG2E = 1.4426950408889634
QUICK = False
NOB = ''
BKNI = 1
UNP = 64
UNP_FRAC = 0.7
BKSPLIT = 4
BPLAN = (10.0, 11.0, 42.5, 47.7)
WAITS = {1: 2, 2: 3, 3: 5, 4: 6, 5: 8, 7: 11, 10: 13, 12: 17, 16: 23, 22: 33, 32: 48}
PAR_WAIT = 10
STARTS = {0: (2, False, 0), 1: (3, False, 0), 2: (5, False, 0), 4: (6, False, 0), 6: (8, False, 0),
          8: (9, False, 0), 10: (11, False, 0), 14: (13, True, 0), 20: (17, False, 0), 24: (23, False, 0),
          32: (33, False, 0), 44: (48, False, 3), 64: (48, False, 19)}
NITER = NSEG // 2
KNI = 2
KSPLIT = 2
PLAN = (('k0', 0, 96), ('m0', 96, 122), ('k1', 124, 220), ('m1', 220, 260))
DW_ODD = 1.5
RC = 64
MACJ = 3
L, D, N = 2048, 1024, 128
BLK = 128
NBLK = L // BLK
NT = D // 128
TAPROWS = 672
WINDOWS = ((0, 128, 0, 1), (128, 128, 1, 1), (256, 128, 2, 1), (320, 80, 3, 1),
           (384, 128, 4, 3), (480, 48, 7, 1), (512, 128, 8, 7), (624, 32, 15, 1))

V_FENCE = 0
V_YTAB = 8
V_START = V_YTAB + 256
V_STEP = V_START + 160
V_ROWS = V_STEP + 128
V_UF = 8
V_KF = V_UF + NBLK * 32
VM_ROWS = V_KF + NBLK * 32


def _bf16_round_int(l):
    u = np.asarray(l, np.float32).view(np.uint32)
    r = (u + 0x7FFF + ((u >> 16) & 1)) & 0xFFFF0000
    return r.astype(np.uint32).view(np.float32).astype(np.int64)


def _tap_row(lp):
    return np.where(lp < 256, lp, np.where(lp < 512, 256 + (lp - 256) // 2,
                    np.where(lp < 1024, 384 + (lp - 512) // 4, 512 + (lp - 1024) // 8)))


@functools.lru_cache(maxsize=None)
def _dft_consts():
    t = np.arange(BLK)
    F = np.zeros((8, 32, BLK))
    G = np.zeros((BLK, 8, 32))
    for r in range(8):
        f = np.concatenate([16 * r + 2 * np.arange(8), 16 * r + 2 * np.arange(8) + 1])
        th = 2 * np.pi * (f + 0.5) / (2 * BLK)
        F[r, :16] = np.cos(th[:, None] * t[None])
        F[r, 16:] = -np.sin(th[:, None] * t[None])
        for q in range(2):
            G[:, r, 16 * q:16 * q + 8] = np.cos(th[None, 8 * q:8 * q + 8] * t[:, None]) / BLK
            G[:, r, 16 * q + 8:16 * q + 16] = -np.sin(th[None, 8 * q:8 * q + 8] * t[:, None]) / BLK
    FS = np.zeros((8, NBLK, 32, 128))
    for (w0, wn, b0, nb) in WINDOWS:
        for j in range(b0, b0 + nb):
            rows = _tap_row(_bf16_round_int(BLK * j + t)) - w0
            assert rows.min() >= 0 and rows.max() < wn
            sel = np.zeros((BLK, 128))
            sel[t, rows] = 1.0
            FS[:, j] = F @ sel
    return (FS.reshape(8, NBLK * 32, 128).astype(np.float32),
            G.reshape(BLK, 2, 128).transpose(1, 0, 2).astype(np.float32))


def _ld16(ref, *idx):
    return pltpu.bitcast(ref.bitcast(u32)[idx + (slice(None),)], bf16)


def _cmul(a, b):
    return (a[0] * b[0] - a[1] * b[1], a[0] * b[1] + a[1] * b[0])


def _csq(a):
    return (a[0] * a[0] - a[1] * a[1], 2.0 * (a[0] * a[1]))


def _cexp(lr, li):
    k = jnp.floor(li * (2.0 / np.pi) + 0.5)
    r = ((li - k * 1.5703125) - k * 4.837512969970703125e-4) - k * 7.54978995489188216e-8
    r = jnp.clip(r, -0.8, 0.8)
    r2 = r * r
    s = r + r * r2 * (-1.6666654611e-1 + r2 * (8.3321608736e-3 + r2 * -1.9515295891e-4))
    c = (1.0 - 0.5 * r2) + (r2 * r2) * (4.166664568298827e-2
                                        + r2 * (-1.388731625493765e-3 + r2 * 2.443315711809948e-5))
    q = k.astype(jnp.int32)
    swap = (q & 1) == 1
    m = jnp.exp(lr)
    flip = lambda v, bit: pltpu.bitcast(pltpu.bitcast(v, jnp.int32) ^ (bit << 30), f32)
    return (flip(m * jnp.where(swap, s, c), (q + 1) & 2), flip(m * jnp.where(swap, c, s), q & 2))


def _par_row(c, k):
    return 8 + (c * 6 + k) * N


def _prep_pieces(praw, vec, par):
    def stage1(c):
        def fn():
            tr = lambda k: praw[k, pl.ds(c * 128, 128), :].astype(f32).T
            dt = jnp.exp(vec[0, pl.ds(c, 1), :]).astype(bf16).astype(f32)
            cc = _cmul((tr(4), tr(5)), (dt * tr(2), dt * tr(3)))
            for k, v in ((0, dt * tr(0)), (1, dt * tr(1)), (4, cc[0]), (5, cc[1])):
                par[pl.ds(_par_row(c, k), N), :] = v
        return fn

    def stage2(c, n0):
        def fn():
            lr = par[pl.ds(_par_row(c, 0) + n0, 16), :]
            li = par[pl.ds(_par_row(c, 1) + n0, 16), :]
            for k, v in enumerate(_cexp(lr, li) + _cexp(lr * 128.0, li * 128.0)):
                par[pl.ds(_par_row(c, k) + n0, 16), :] = v
        return fn

    tile = lambda c: [(260, stage1(c))] + [(190, stage2(c, n0)) for n0 in range(0, N, 16)]
    return tile(0), [pc for c in range(1, NT) for pc in tile(c)]


def _kgen_pieces(c, r, par, vb, taps, tslot, frow, kni, ksplit):
    st = {}

    def put(row, z, h=None):
        if h is None:
            vb[pl.ds(row, 16), :] = z[0]
            vb[pl.ds(row + 16, 16), :] = z[1]
        else:
            vb[pl.ds(row + 8 * h, 8), :] = z[0]
            vb[pl.ds(row + 16 + 8 * h, 8), :] = z[1]

    def get(row, h=None):
        if h is None:
            return (vb[pl.ds(row, 16), :], vb[pl.ds(row + 16, 16), :])
        return (vb[pl.ds(row + 8 * h, 8), :], vb[pl.ds(row + 16 + 8 * h, 8), :])

    def ytab(k0, k1):
        return [vb[pl.ds(V_YTAB + 128 * part + 16 * k0, 16 * (k1 - k0)), :].reshape(k1 - k0, 16, 128)
                for part in range(2)]

    def params(k):
        if isinstance(r, int):
            return par[pl.ds(_par_row(c, k) + r * 16, 16), :]
        return par[pl.ds(pl.multiple_of(c * (6 * N) + r[0] * 32, 32) + (_par_row(0, k) + r[1] * 16), 16), :]

    def park():
        put(V_STEP, (params(0), params(1)))
        put(V_START + 32, (params(2), params(3)))
        put(V_START, (params(4), params(5)))

    def setup_y(h):
        def fn():
            z1 = get(V_STEP, h)
            z2 = _csq(z1)
            z4 = _csq(z2)
            s = lax.broadcasted_iota(jnp.int32, (8, 128), 0)
            fs = [(jnp.where((s >> k) & 1 == 1, z[0], 1.0), jnp.where((s >> k) & 1 == 1, z[1], 0.0))
                  for k, z in enumerate((z1, z2, z4))]
            y = _cmul(_cmul(fs[0], fs[1]), fs[2])
            for k in range(8):
                vb[pl.ds(V_YTAB + 16 * k + 8 * h, 8), :] = y[0]
                vb[pl.ds(V_YTAB + 128 + 16 * k + 8 * h, 8), :] = y[1]
                if k < 7:
                    y = _cmul(y, z1)
                    y = (jnp.where(s == 7 - k, 1.0, y[0]), jnp.where(s == 7 - k, 0.0, y[1]))
            z = z4
            for k in range(4):
                z = _csq(z)
                put(V_STEP + 32 * k, z, h)
        return fn

    def setup_hi():
        z = get(V_START + 32)
        cf = get(V_START)
        for g in range(1, 5):
            put(V_START + 32 * g, _cmul(cf, z))
            if g < 4:
                z = _csq(z)

    def square(k0, k1):
        def fn():
            rows = [pl.ds(V_YTAB + 128 * part + 16 * k0, 16 * (k1 - k0)) for part in range(2)]
            y = _csq((vb[rows[0], :], vb[rows[1], :]))
            vb[rows[0], :] = y[0]
            vb[rows[1], :] = y[1]
        return fn

    def rows_of(g, i0, ni):
        n_i = 16 + (g == 4)

        def fn():
            x = st.pop('x') if i0 > 0 else get(V_START + 32 * g)
            step = get(V_STEP + 32 * max(g - 1, 0))
            xs = []
            for t in range(ni):
                xs.append(x)
                if i0 + t + 1 < n_i:
                    x = _cmul(x, step)
            if i0 + ni < n_i:
                st['x'] = x
            acc = [None] * ni
            for k0 in range(0, 8, ksplit):
                yr, yi = ytab(k0, k0 + ksplit)
                for t in range(ni):
                    v = xs[t][0] * yr - xs[t][1] * yi
                    v = lax.slice_in_dim(v, 0, 8, axis=1) + lax.slice_in_dim(v, 8, 16, axis=1)
                    v = jnp.sum(pltpu.roll(v, k0, 1, stride=1, stride_axis=0), axis=0)
                    acc[t] = v if acc[t] is None else acc[t] + v
                if k0 + ksplit < 8:
                    vb[pl.ds(frow, 8), :] = acc[ni - 1]
            for t in range(ni):
                row = 128 * g + 8 * (i0 + t)
                a = acc[t]
                if row == 640:
                    a = jnp.where(lax.broadcasted_iota(jnp.int32, (8, 128), 0) == 0, a, 0.0)
                taps[tslot, pl.ds(row, 8), :] = taps[tslot, pl.ds(row, 8), :] + a
                if t == ni - 1:
                    vb[pl.ds(frow, 8), :] = a
        return fn

    pieces = [(30, park), (110, setup_y(0)), (110, setup_y(1)), (80, setup_hi)]
    for g in range(5):
        if g >= 2:
            pieces += [(40, square(0, 4)), (40, square(4, 8))]
        for i0 in range(0, 16 + (g == 4), kni):
            ni = min(kni, 16 + (g == 4) - i0)
            pieces.append((83 * ni, rows_of(g, i0, ni)))
    return pieces


def _conv_pieces(c, r, buf, fs_ref, us, taps, vb, yf, frow):
    st = {}

    def fwd_u(b0, b1):
        def fn():
            lhs = _ld16(fs_ref, 2 * r[0] + r[1], pl.ds(0, 16))
            for b in range(b0, b1):
                w = pltpu.bitcast(us[c, pl.ds(b * 64, 64), :], bf16)
                res = jnp.dot(lhs, w, preferred_element_type=f32)
                row = V_UF + 32 * b
                if b == 0:
                    vb[pl.ds(row, 32), :] = res
                else:
                    p = st['prev']
                    vb[pl.ds(row, 8), :] = res[0:8] - p[16:24]
                    vb[pl.ds(row + 8, 8), :] = res[8:16] + p[24:32]
                    vb[pl.ds(row + 16, 8), :] = res[16:24] + p[0:8]
                    vb[pl.ds(row + 24, 8), :] = res[24:32] - p[8:16]
                st['prev'] = res
        return fn

    def fwd_k(jobs):
        def fn():
            for (wi, t0, nb) in jobs:
                w0, wn, b0, _ = WINDOWS[wi]
                lhs = _ld16(fs_ref, 2 * r[0] + r[1], pl.ds((b0 + t0) * 16, nb * 16))[:, :wn]
                w = taps[c, pl.ds(w0, wn), :].astype(bf16)
                vb[pl.ds(V_KF + 32 * (b0 + t0), 32 * nb), :] = jnp.dot(lhs, w, preferred_element_type=f32)
        return fn

    def mac(q, i0, ni, j0, j1):
        def fn():
            ld = lambda base, b: (vb[pl.ds(base + 32 * b + 8 * q, 8), :], vb[pl.ds(base + 32 * b + 16 + 8 * q, 8), :])
            zr, zi = st.pop('z') if j0 > 0 else ({}, {})
            ucache = {}
            for j in range(j0, j1):
                kr, ki = ld(V_KF, j)
                for i in range(max(i0, j), i0 + ni):
                    if i - j not in ucache:
                        ucache[i - j] = ld(V_UF, i - j)
                    ur, ui = ucache[i - j]
                    if i not in zr:
                        zr[i] = kr * ur - ki * ui
                        zi[i] = kr * ui + ki * ur
                    else:
                        zr[i] = zr[i] + kr * ur - ki * ui
                        zi[i] = zi[i] + kr * ui + ki * ur
            vb[pl.ds(frow, 8), :] = zr[i0 + ni - 1]
            if j1 < i0 + ni:
                st['z'] = (zr, zi)
            else:
                row = pl.multiple_of(r[0] * 64, 64) + (r[1] * 32 + q * 16)
                for i in range(i0, i0 + ni):
                    yf[buf, i, pl.ds(row, 16), :] = jnp.concatenate([zr[i], zi[i]], axis=0).astype(bf16)
        return (8 * sum(1 for j in range(j0, j1) for i in range(max(i0, j), i0 + ni)), fn)

    fwd = [fwd_u(0, 8), fwd_u(8, 16), fwd_k(((0, 0, 1), (1, 0, 1), (2, 0, 1), (3, 0, 1))),
           fwd_k(((4, 0, 2), (6, 0, 2), (6, 2, 2), (6, 4, 2))), fwd_k(((4, 2, 1), (5, 0, 1), (6, 6, 1), (7, 0, 1)))]
    macs = []
    for q in range(2):
        for i0 in range(0, NBLK, 2):
            for j0 in range(0, i0 + 2, MACJ):
                macs.append(mac(q, i0, 2, j0, min(j0 + MACJ, i0 + 2)))
    return fwd, macs


def _inv_piece(c, b, buf, g_ref, us, vec, yf, outb):
    rows = pl.ds(pl.multiple_of(b * 64, 64), 64)
    w = _ld16(yf, buf, b, slice(None))
    g = jnp.concatenate([_ld16(g_ref, k, slice(None)) for k in range(2)], axis=1)
    y = jnp.dot(g, w, preferred_element_type=f32)
    u = pltpu.bitcast(us[c, rows, :], bf16).astype(f32)
    sk = (u * vec[1, pl.ds(c, 1), :]).astype(bf16).astype(f32)
    o = (y.astype(bf16).astype(f32) + sk).astype(bf16)
    outb[c, pl.ds(pl.multiple_of(b * BLK, BLK) if not isinstance(b, int) else b * BLK, BLK), :] = o


def _attn_fill():
    n = 2 * (SEG + M)
    r = lax.broadcasted_iota(jnp.int32, (n, n), 0)
    c = lax.broadcasted_iota(jnp.int32, (n, n), 1)
    head = lambda i: jnp.where(i < 2 * SEG, i // SEG, (i - 2 * SEG) // PRE)
    pos = lambda i: jnp.where(i < 2 * SEG, i % SEG, i % PRE)
    is_mem = lambda i: (i < 2 * SEG) & (i % SEG < M)
    same = head(r) == head(c)
    allowed = same & (is_mem(r) | is_mem(c) | (pos(r) >= pos(c)))
    return jnp.where(allowed, 0.0, jnp.where(same, -1e9 * LOG2E, -jnp.inf)).astype(f32)


def _kernel(zero_hbm, x_hbm, mem0_hbm, wq_hbm, wk_hbm, wv_hbm, wo_hbm,
            u_hbm, p0, p1, p2, p3, p4, p5, ldt_hbm, dsk_hbm, fs_hbm, g_hbm,
            out_hbm,
            wq, wk, wv, wo, xb, xs, h_ref, outs, fill_ref,
            praw, par, us, taps, vb, vm, vu, pacc, yf, outb, vec, vraw, fs_ref, g_ref, zero_ref,
            sem_s, sem_w, sem_o, sem_xb, sem_x, sem_p, sem_u, sem_out, pre, own, lo0, lo1):
    wqkv = (wq, wk, wv)
    scale = E ** -0.5

    whbm = [w.bitcast(u32) for w in (wq_hbm, wk_hbm, wv_hbm)]

    def wcp(j, m, p):
        return pltpu.make_async_copy(whbm[m].at[:, p, j, :], wqkv[m].at[p, j], sem_w.at[(j * 3 + m) * 2 + p])

    xu = x_hbm.bitcast(u32)
    xcs = [pltpu.make_async_copy(xu.at[:, t, pl.ds(0, PRE // 2), pl.ds(c * 128, 128)],
                                 xb.at[c, :, pl.ds(t * (PRE // 2), PRE // 2), :], sem_xb.at[2 * c + t])
           for c in range(8) for t in range(2)]
    xcp1 = pltpu.make_async_copy(x_hbm.at[:, :, pl.ds(PRE, TOK), :], xs, sem_x.at[0])
    pcs = [pltpu.make_async_copy(p, praw.at[k], sem_p.at[k]) for k, p in enumerate((p0, p1, p2, p3, p4, p5))]
    ccs = [pltpu.make_async_copy(fs_hbm, fs_ref, sem_p.at[6]), pltpu.make_async_copy(g_hbm, g_ref, sem_p.at[7])]
    wou = wo_hbm.bitcast(u32)
    ocs = [pltpu.make_async_copy(wou.at[:, pl.ds(c * 128, 128)], wo.at[c], sem_o.at[c]) for c in range(8)]
    uu = u_hbm.bitcast(u32)
    ucs = [pltpu.make_async_copy(uu.at[:, pl.ds(c * 128, 128)], us.at[c], sem_u.at[c]) for c in range(NT)]

    zcp = pltpu.make_async_copy(zero_hbm, zero_ref, sem_s.at[0])
    scs = [pltpu.make_async_copy(mem0_hbm, h_ref.at[pl.ds(0, M)], sem_s.at[1]),
           pltpu.make_async_copy(ldt_hbm, vraw.at[0], sem_s.at[2]),
           pltpu.make_async_copy(dsk_hbm, vraw.at[1], sem_s.at[3])]
    w0cs = [[pltpu.make_async_copy(whbm[0].at[pl.ds(half * (DM // 4), DM // 4), p, 0, :],
                                   wq.at[p, 0, pl.ds(half * (DM // 4), DM // 4)], sem_s.at[4 + 2 * half + p])
             for p in range(2)] for half in range(2)]
    for cp in [zcp] + w0cs[0] + xcs[:8]:
        cp.start()
    vu[pl.ds(8, 8), :] = pltpu.bitcast(jnp.full((8, 128), 0x0000FFFF, u32), f32)
    vu[pl.ds(16, 8), :] = pltpu.bitcast(jnp.full((8, 128), 0xFFFF0000, u32), f32)
    taps[...] = jnp.zeros(taps.shape, f32)
    yf[1] = jnp.zeros(yf.shape[1:], bf16)
    fill_ref[...] = _attn_fill()
    for cp in w0cs[1] + xcs[8:] + scs:
        cp.start()
    zcp.wait()

    def opaque_row(k, buf):
        return pl.multiple_of(jnp.clip(zero_ref[k] * 8, 0, buf.shape[0] - 8), 8)

    bufs = (vb, vm, vu, par)
    fence_rows = [opaque_row(0, b) for b in bufs]
    done_vb, done_vm = opaque_row(1, vb), opaque_row(1, vm)

    class Pacer:
        def __init__(self, segments):
            self.t = 0.0
            self.todo = []
            for (pieces, buf, t0, t1) in segments:
                total = float(sum(c for c, _ in pieces)) or 1.0
                done = 0.0
                for (cst, fn) in pieces:
                    self.todo.append((t0 + (t1 - t0) * done / total, fn, buf))
                    done += cst

        def __call__(self, v, dt=1.0):
            self.t += dt
            fenced = []
            while self.todo and self.todo[0][0] < self.t:
                _, fn, buf = self.todo.pop(0)
                if not any(b is buf for b in fenced):
                    buf[pl.ds([r for b, r in zip(bufs, fence_rows) if b is buf][0], 8), :] = v
                    fenced.append(buf)
                fn()

        def finished(self):
            return not self.todo

    def unpair(j, m, r0, nr):
        def fn():
            rows = pl.ds(r0, nr)
            m_lo = pltpu.bitcast(vu[pl.ds(8, 8), :], u32)[None]
            m_hi = pltpu.bitcast(vu[pl.ds(16, 8), :], u32)[None]
            a = wqkv[m][0, j, rows, :].reshape(nr // 8, 8, E)
            b = wqkv[m][1, j, rows, :].reshape(nr // 8, 8, E)
            wqkv[m][0, j, rows, :] = ((a & m_lo) | ((b & m_lo) << 16)).reshape(nr, E)
            wqkv[m][1, j, rows, :] = (((a & m_hi) >> 16) | (b & m_hi)).reshape(nr, E)
        return (nr, fn)

    def unpair_pieces(items, lo=0, hi=DM // 2):
        return [unpair(j, m, r0, UNP) for (j, m) in items for r0 in range(lo, hi, UNP)]

    items = [(j, m) for j in range(NP) for m in range(3)]
    wcs = lambda lo, hi: [wcp(j, m, p) for (j, m) in items[lo:hi] for p in range(2)]
    rest = ocs + ccs + ucs + [xcp1]
    starts = [[] for _ in range(2 * len(items))]
    n_w, n_r = 1, 0
    for unit in sorted(STARTS):
        w_hi, with_par, r_hi = STARTS[unit]
        starts[unit] = (pcs if with_par else []) + wcs(n_w, w_hi) + rest[n_r:r_hi]
        n_w, n_r = w_hi, r_hi
    assert n_w == len(items) and n_r == len(rest)
    with jax.named_scope("bulk"):
        if QUICK in (1, 2):
            for cp in wcs(1, 48) + pcs + ocs + ucs + [xcp1] + ccs:
                cp.start()
            for cp in wcs(1, 48) + pcs + scs + xcs + w0cs[0] + w0cs[1]:
                cp.wait()
            vec[...] = vraw[...].astype(f32)
            for _, fn in (unpair_pieces(items) + sum(_prep_pieces(praw, vec, par), [])) if QUICK != 2 else []:
                fn()

            def kg(r, carry):
                for odd in range(2):
                    for _, fn in _kgen_pieces(0, (r, odd), par, vb, taps, 0, done_vb, BKNI, BKSPLIT):
                        fn()
                return carry
            lax.fori_loop(0, 4, kg, 0)
            for (j, m) in (items if QUICK != 2 else []):
                def chunk(rc, carry, j=j, m=m):
                    lhs = jnp.concatenate(
                        [pltpu.bitcast(xb[c, pl.ds(rc * 4, 4)].reshape(32, 128), bf16) for c in range(8)], axis=1)
                    res = [jnp.dot(lhs, pltpu.bitcast(wqkv[m][p, j], bf16), preferred_element_type=f32)
                           for p in range(2)]
                    for t in range(8):
                        v = jnp.concatenate([res[0][8 * t:8 * t + 8], res[1][8 * t:8 * t + 8]], axis=0)
                        pre[rc * 8 + t, m * NP + j] = v.astype(bf16)
                    return carry
                lax.fori_loop(0, 8, chunk, 0)
            items = []
        n_chunk = 2 * (T0 // RC)
        prep = _prep_pieces(praw, vec, par)
        kg0 = [pc for r in range(8) for pc in _kgen_pieces(0, r, par, vb, taps, 0, done_vb, BKNI, BKSPLIT)]
        t_a, t_b, t_c, t_d = [v * n_chunk for v in BPLAN]
        fence_x = Pacer([(prep[0], par, t_a, t_b), (kg0, vb, t_b, t_c), (prep[1], par, t_c, t_d)])
        landed = 1
        for it, (j, m) in enumerate(items):
            fence_w = None
            for half in range(2):
                for cp in starts[2 * it + half]:
                    cp.start()
                if it == 0:
                    with jax.named_scope("waitx%d" % half):
                        for cp in w0cs[half] + xcs[8 * half:8 * half + 8]:
                            cp.wait()
                    for _, fn in unpair_pieces(items[:1], half * (DM // 4), (half + 1) * (DM // 4)):
                        fn()
                    fence_w = Pacer([])
                elif half == 0:
                    late = landed == it
                    if it in WAITS:
                        with jax.named_scope("wait%d" % it):
                            for cp in wcs(landed, WAITS[it]) + (pcs + scs if it == PAR_WAIT else []):
                                cp.wait()
                        landed = WAITS[it]
                        if it == PAR_WAIT:
                            vec[...] = vraw[...].astype(f32)
                    if late:
                        for _, fn in unpair_pieces(items[it:it + 1]):
                            fn()
                    fence_w = Pacer([(unpair_pieces(items[it + 1:min(it + 2, landed)]), vu, 0.0, n_chunk * UNP_FRAC)])
                for p in range(2):
                    w = pltpu.bitcast(wqkv[m][p, j, pl.ds(half * (DM // 4), DM // 4), :], bf16)
                    lhs = jnp.concatenate([pltpu.bitcast(xb[c].reshape(T0 // 2, 128), bf16)
                                           for c in range(4 * half, 4 * half + 4)], axis=1)
                    res = jnp.dot(lhs, w, preferred_element_type=f32)
                    for rc in range(T0 // RC):
                        rows = pl.ds(rc * RC, RC)
                        v = res[rc * RC:(rc + 1) * RC]
                        if half == 1:
                            v = v + pacc[p, rows, :]
                        if p == 0 or half == 0:
                            pacc[p, rows, :] = v
                        else:
                            pr = jnp.concatenate([pacc[0, rows, :].reshape(RC // PRE, PRE, E),
                                                  v.reshape(RC // PRE, PRE, E)], axis=1)
                            pre[pl.ds(rc * (RC // PRE), RC // PRE), m * NP + j] = pr.astype(bf16)
                        fence_w(v[:8], 0.5)
                        fence_x(v[:8], 0.5)
            assert fence_w.finished() and landed > it
        assert QUICK or fence_x.finished()
    with jax.named_scope("waitrest"):
        for cp in ocs + ucs + ccs + [xcp1]:
            cp.wait()

    def outa_cp(row, n):
        return pltpu.make_async_copy(outs.at[pl.ds(row, n)], out_hbm.at[pl.ds(row, n), pl.ds(0, DM)], sem_out.at[0])

    def outb_cp(c, row, n, sem):
        col = DM + c * 128
        return pltpu.make_async_copy(
            outb.at[c, pl.ds(row, n)],
            out_hbm.at[pl.ds(row, n), pl.ds(col if isinstance(col, int) else pl.multiple_of(col, 128), 128)],
            sem_out.at[sem])

    def one_step(i, odd, fwd, fence):
        s = 2 * i + odd
        lo_cur = (lo0, lo1)[odd]
        base = pl.multiple_of(2 * SEG * i, 2 * SEG)
        h_ref[pl.ds(M, TOK), :] = xs[i, odd]
        h = h_ref[...]
        scores = {}
        probs = {}

        ct = i >> 2
        r = s & 7
        buf = ct & 1
        cprev = (ct + NT - 1) & (NT - 1)

        def stage_a(j):
            for m in range(3):
                for p in range(2):
                    w = pltpu.bitcast(wqkv[m][p, j], bf16)
                    res = jnp.dot(h, w, preferred_element_type=f32)
                    own[m * NP + j, pl.ds(SEG * p, SEG), :] = res.astype(bf16)
                    fence(res[:M])

        def gather(m, j):
            return pltpu.bitcast(jnp.concatenate([own.bitcast(u32)[m * NP + j],
                                                  pre.bitcast(u32)[s, m * NP + j]], axis=0), bf16)

        def stage_qk(j):
            scores[j] = lax.dot_general(gather(0, j), gather(1, j), (((1,), (1,)), ((), ())),
                                        preferred_element_type=f32)

        def stage_b(j):
            fl = fill_ref[...]
            sc = jnp.where(fl == 0.0, scores.pop(j) * (scale * LOG2E), fl)
            e = jnp.exp2(sc - jnp.max(sc, axis=-1, keepdims=True))
            den = jnp.sum(e, axis=-1, keepdims=True)
            probs[j] = (e * pl.reciprocal(den, approx=True)).astype(bf16)

        def stage_c(j):
            o = jnp.dot(probs[j], gather(2, j), preferred_element_type=f32)
            for p in range(2):
                hh = 2 * j + p
                lo_cur[hh, pl.ds(0, SEG), :] = o[p * SEG:(p + 1) * SEG].astype(bf16)
                ob = o[2 * SEG + p * PRE:2 * SEG + (p + 1) * PRE]
                lo1[hh, pl.ds(SEG + odd * PRE, PRE), :] = ob.astype(bf16)

        acc = [None] * 8

        def stage_d(h0, h1, last=False):
            lhs = jnp.concatenate([_ld16(lo_cur, hh, slice(None)) for hh in range(h0, h1)], axis=1)
            for c in range(8):
                w = pltpu.bitcast(wo[c, pl.ds(h0 * 64, (h1 - h0) * 64), :], bf16)
                res = jnp.dot(lhs, w, preferred_element_type=f32)
                acc[c] = res if acc[c] is None else acc[c] + res
                if not last:
                    fence(res[:M], (h1 - h0) / 8.0 * (DW_ODD if odd else 1.0))
                else:
                    rb = acc[c].astype(bf16)
                    cols = pl.ds(c * 128, 128)
                    h_ref[pl.ds(0, M), cols] = rb[:M]
                    outs[pl.ds(base + (odd * SEG + PRE), TOK), cols] = rb[M:SEG]
                    if odd:
                        outs[pl.ds(base, PRE), cols] = rb[SEG:SEG + PRE]
                        outs[pl.ds(base + SEG, PRE), cols] = rb[SEG + PRE:]

        def attn_group(jq, jc):
            for j in jq:
                stage_qk(j)
            for j in jc:
                stage_c(j)
            for j in jq:
                stage_b(j)

        for t in range(2):
            _inv_piece(cprev, 2 * r + t, 1 - buf, g_ref, us, vec, yf, outb)
        for p in fwd:
            p()
        for j in range(NP):
            stage_a(j)
            if j >= 2 and j % 2 == 0:
                attn_group((j - 2, j - 1), (j - 4, j - 3) if j >= 4 else ())
        stage_d(0, 8)
        attn_group((14, 15), (12, 13))
        stage_d(8, 20)
        attn_group((), (14, 15))
        stage_d(20, 28)
        stage_d(28, 32, last=True)

    def two_steps(i, carry):
        ct = i >> 2
        cprev = (ct + NT - 1) & (NT - 1)
        conv = [_conv_pieces(ct, (i & 3, odd), ct & 1, fs_ref, us, taps, vm, yf,
                             done_vm) for odd in range(2)]
        kgen = [_kgen_pieces((ct + 1) & (NT - 1), (i & 3, odd), par, vb, taps, ct + 1,
                             done_vb, KNI, KSPLIT) for odd in range(2)]
        work = {'k0': (kgen[0], vb), 'k1': (kgen[1], vb), 'm0': (conv[0][1], vm), 'm1': (conv[1][1], vm)}
        fence = Pacer([work[k] + (t0, t1) for (k, t0, t1) in PLAN if k[0] not in NOB])
        for odd in range(2):
            one_step(i, odd, conv[odd][0], fence)
        assert fence.finished() or NOB
        outa_cp(pl.multiple_of(2 * SEG * i, 2 * SEG), 2 * SEG).start()
        outb_cp(cprev, pl.multiple_of((i & 3) * 512, 512), 512, jnp.where(i < 4, 2, 1)).start()
        return carry

    with jax.named_scope("steps"):
        if NITER:
            lax.fori_loop(0, NITER, two_steps, 0)

    with jax.named_scope("flush"):
        outb_cp(NT - 1, 0, L, 2).wait()
        for b in range(NBLK):
            _inv_piece(NT - 1, b, (NT - 1) % 2, g_ref, us, vec, yf, outb)
            if b % 4 == 3:
                outb_cp(NT - 1, (b - 3) * BLK, 4 * BLK, 1).start()
    with jax.named_scope("waitout"):
        outa_cp(0, S).wait()
        pltpu.make_async_copy(outb, outb, sem_out.at[1]).wait()


@jax.jit
def pallas_concat_heads__memory_aug_recurrent_mem_tr__ssm_conv_s4__prompt_kernel(
    A_x, A_mem0, A_Wq, A_Wk, A_Wv, A_Wo, A_seg_len,
    B_u, B_A_re, B_A_im, B_B_re, B_B_im, B_C_re, B_C_im, B_log_dt, B_Dskip,
):
    del A_seg_len
    assert A_x.shape == (1, S, DM) and B_u.shape == (1, L, D)
    fs, g = _dft_consts()
    w4 = lambda w: w.reshape(DM // 2, 2, H, E)
    any_ = pl.BlockSpec(memory_space=pl.ANY)
    V = pltpu.VMEM
    out = pl.pallas_call(
        _kernel,
        out_shape=jax.ShapeDtypeStruct((S, DM + D), bf16),
        in_specs=[any_] * 18,
        out_specs=any_,
        scratch_shapes=[
            V((2, NP, DM // 2, E), u32),
            V((2, NP, DM // 2, E), u32),
            V((2, NP, DM // 2, E), u32),
            V((8, H * E // 2, 128), u32),
            V((8, NSEG // 2, PRE, 128), u32),
            V((NSEG // 2, 2, TOK, DM), bf16),
            V((M + TOK, DM), bf16),
            V((S, DM), bf16),
            V((2 * (SEG + M), 2 * (SEG + M)), f32),
            V((6, D, N), bf16),
            V((8 + NT * 6 * N, 128), f32),
            V((NT, L // 2, 128), u32),
            V((NT + 1, TAPROWS, 128), f32),
            V((V_ROWS, 128), f32),
            V((VM_ROWS, 128), f32),
            V((24, 128), f32),
            V((2, T0, 128), f32),
            V((2, NBLK, 2 * BLK, 128), bf16),
            V((NT, L, 128), bf16),
            V((2, 8, 128), f32),
            V((2, 8, 128), bf16),
            V((8, NBLK * 32, 128), bf16),
            V((2, BLK, 128), bf16),
            pltpu.SMEM((2,), jnp.int32),
            pltpu.SemaphoreType.DMA((8,)),
            pltpu.SemaphoreType.DMA((6 * NP,)),
            pltpu.SemaphoreType.DMA((8,)),
            pltpu.SemaphoreType.DMA((16,)),
            pltpu.SemaphoreType.DMA((1,)),
            pltpu.SemaphoreType.DMA((8,)),
            pltpu.SemaphoreType.DMA((NT,)),
            pltpu.SemaphoreType.DMA((3,)),
            V((NSEG, 3 * NP, 2 * PRE, E), bf16),
            V((3 * NP, 2 * SEG, E), bf16),
            V((H, SEG, E), bf16),
            V((H, SEG + 2 * PRE, E), bf16),
        ],
        compiler_params=pltpu.CompilerParams(vmem_limit_bytes=110 * 1024 * 1024, disable_bounds_checks=True),
    )(jnp.asarray(np.zeros((2,), np.int32)), A_x.reshape(NSEG // 2, 2, SEG, DM), A_mem0.reshape(M, DM), w4(A_Wq), w4(A_Wk), w4(A_Wv), A_Wo.reshape(H * E, DM),
      B_u.reshape(L, D), B_A_re, B_A_im, B_B_re, B_B_im, B_C_re, B_C_im,
      B_log_dt.reshape(8, 128), B_Dskip.reshape(8, 128),
      jnp.asarray(fs, bf16), jnp.asarray(g, bf16))
    return out.reshape(1, S, DM + D)
```

```python
import functools

import numpy as np
import jax
import jax.numpy as jnp
from jax import lax
import jax.experimental.pallas as pl
import jax.experimental.pallas.tpu as pltpu

bf16, f32, u32 = jnp.bfloat16, jnp.float32, jnp.uint32

S, DM, H, E, M, SEG = 2048, 1024, 32, 128, 8, 32
NSEG = S // SEG
TOK = 24
PRE = SEG - TOK
T0 = PRE * NSEG
NP = H // 2
LOG2E = 1.4426950408889634
QUICK = False
NOB = ''
BKNI = 1
UNP = 64
UNP_FRAC = 0.7
BKSPLIT = 4
BPLAN = (10.0, 11.0, 42.5, 47.7)
WAITS = {1: 2, 2: 3, 3: 5, 4: 6, 5: 8, 7: 11, 10: 13, 12: 17, 16: 23, 22: 33, 32: 48}
PAR_WAIT = 10
STARTS = {0: (2, False, 0), 1: (3, False, 0), 2: (5, False, 0), 4: (6, False, 0), 6: (8, False, 0),
          8: (9, False, 0), 10: (11, False, 0), 14: (13, True, 0), 20: (17, False, 0), 24: (23, False, 0),
          32: (33, False, 0), 44: (48, False, 3), 64: (48, False, 19)}
NITER = NSEG // 2
KNI = 2
KSPLIT = 2
PLAN = (('k0', 0, 96), ('m0', 96, 122), ('k1', 124, 220), ('m1', 220, 260))
DW_ODD = 1.5
RC = 64
MACJ = 3
L, D, N = 2048, 1024, 128
BLK = 128
NBLK = L // BLK
NT = D // 128
TAPROWS = 672
WINDOWS = ((0, 128, 0, 1), (128, 128, 1, 1), (256, 128, 2, 1), (320, 80, 3, 1),
           (384, 128, 4, 3), (480, 48, 7, 1), (512, 128, 8, 7), (624, 32, 15, 1))

V_FENCE = 0
V_YTAB = 8
V_START = V_YTAB + 256
V_STEP = V_START + 160
V_ROWS = V_STEP + 128
V_UF = 8
V_KF = V_UF + NBLK * 32
V_Z = V_KF + NBLK * 32
VM_ROWS = V_Z + 32


def _bf16_round_int(l):
    u = np.asarray(l, np.float32).view(np.uint32)
    r = (u + 0x7FFF + ((u >> 16) & 1)) & 0xFFFF0000
    return r.astype(np.uint32).view(np.float32).astype(np.int64)


def _tap_row(lp):
    return np.where(lp < 256, lp, np.where(lp < 512, 256 + (lp - 256) // 2,
                    np.where(lp < 1024, 384 + (lp - 512) // 4, 512 + (lp - 1024) // 8)))


@functools.lru_cache(maxsize=None)
def _dft_consts():
    t = np.arange(BLK)
    F = np.zeros((8, 32, BLK))
    G = np.zeros((2, BLK // 2, 8, 16))
    for r in range(8):
        f = 16 * r + 2 * np.arange(8)
        th = 2 * np.pi * (np.concatenate([f, BLK - 1 - f]) + 0.5) / (2 * BLK)
        F[r, :16] = np.cos(th[:, None] * t[None])
        F[r, 16:] = -np.sin(th[:, None] * t[None])
        for par in range(2):
            G[par, :, r, :8] = np.cos(th[None, :8] * t[par::2, None]) / BLK
            G[par, :, r, 8:] = -np.sin(th[None, :8] * t[par::2, None]) / BLK
    FS = np.zeros((8, NBLK, 32, 128))
    for (w0, wn, b0, nb) in WINDOWS:
        for j in range(b0, b0 + nb):
            rows = _tap_row(_bf16_round_int(BLK * j + t)) - w0
            assert rows.min() >= 0 and rows.max() < wn
            sel = np.zeros((BLK, 128))
            sel[t, rows] = 1.0
            FS[:, j] = F @ sel
    return (FS.reshape(8, NBLK * 32, 128).astype(np.float32),
            G.reshape(2, BLK // 2, 128).astype(np.float32))


def _ld16(ref, *idx):
    return pltpu.bitcast(ref.bitcast(u32)[idx + (slice(None),)], bf16)


def _cmul(a, b):
    return (a[0] * b[0] - a[1] * b[1], a[0] * b[1] + a[1] * b[0])


def _csq(a):
    return (a[0] * a[0] - a[1] * a[1], 2.0 * (a[0] * a[1]))


def _cexp(lr, li):
    k = jnp.floor(li * (2.0 / np.pi) + 0.5)
    r = ((li - k * 1.5703125) - k * 4.837512969970703125e-4) - k * 7.54978995489188216e-8
    r = jnp.clip(r, -0.8, 0.8)
    r2 = r * r
    s = r + r * r2 * (-1.6666654611e-1 + r2 * (8.3321608736e-3 + r2 * -1.9515295891e-4))
    c = (1.0 - 0.5 * r2) + (r2 * r2) * (4.166664568298827e-2
                                        + r2 * (-1.388731625493765e-3 + r2 * 2.443315711809948e-5))
    q = k.astype(jnp.int32)
    swap = (q & 1) == 1
    m = jnp.exp(lr)
    flip = lambda v, bit: pltpu.bitcast(pltpu.bitcast(v, jnp.int32) ^ (bit << 30), f32)
    return (flip(m * jnp.where(swap, s, c), (q + 1) & 2), flip(m * jnp.where(swap, c, s), q & 2))


def _par_row(c, k):
    return 8 + (c * 6 + k) * N


def _prep_pieces(praw, vec, par):
    def stage1(c):
        def fn():
            tr = lambda k: praw[k, pl.ds(c * 128, 128), :].astype(f32).T
            dt = jnp.exp(vec[0, pl.ds(c, 1), :]).astype(bf16).astype(f32)
            cc = _cmul((tr(4), tr(5)), (dt * tr(2), dt * tr(3)))
            for k, v in ((0, dt * tr(0)), (1, dt * tr(1)), (4, cc[0]), (5, cc[1])):
                par[pl.ds(_par_row(c, k), N), :] = v
        return fn

    def stage2(c, n0):
        def fn():
            lr = par[pl.ds(_par_row(c, 0) + n0, 16), :]
            li = par[pl.ds(_par_row(c, 1) + n0, 16), :]
            for k, v in enumerate(_cexp(lr, li) + _cexp(lr * 128.0, li * 128.0)):
                par[pl.ds(_par_row(c, k) + n0, 16), :] = v
        return fn

    tile = lambda c: [(260, stage1(c))] + [(190, stage2(c, n0)) for n0 in range(0, N, 16)]
    return tile(0), [pc for c in range(1, NT) for pc in tile(c)]


def _kgen_pieces(c, r, par, vb, taps, tslot, frow, kni, ksplit):
    st = {}

    def put(row, z, h=None):
        if h is None:
            vb[pl.ds(row, 16), :] = z[0]
            vb[pl.ds(row + 16, 16), :] = z[1]
        else:
            vb[pl.ds(row + 8 * h, 8), :] = z[0]
            vb[pl.ds(row + 16 + 8 * h, 8), :] = z[1]

    def get(row, h=None):
        if h is None:
            return (vb[pl.ds(row, 16), :], vb[pl.ds(row + 16, 16), :])
        return (vb[pl.ds(row + 8 * h, 8), :], vb[pl.ds(row + 16 + 8 * h, 8), :])

    def ytab(k0, k1):
        return [vb[pl.ds(V_YTAB + 128 * part + 16 * k0, 16 * (k1 - k0)), :].reshape(k1 - k0, 16, 128)
                for part in range(2)]

    def params(k):
        if isinstance(r, int):
            return par[pl.ds(_par_row(c, k) + r * 16, 16), :]
        return par[pl.ds(pl.multiple_of(c * (6 * N) + r[0] * 32, 32) + (_par_row(0, k) + r[1] * 16), 16), :]

    def park():
        put(V_STEP, (params(0), params(1)))
        put(V_START + 32, (params(2), params(3)))
        put(V_START, (params(4), params(5)))

    def setup_y(h):
        def fn():
            z1 = get(V_STEP, h)
            z2 = _csq(z1)
            z4 = _csq(z2)
            s = lax.broadcasted_iota(jnp.int32, (8, 128), 0)
            fs = [(jnp.where((s >> k) & 1 == 1, z[0], 1.0), jnp.where((s >> k) & 1 == 1, z[1], 0.0))
                  for k, z in enumerate((z1, z2, z4))]
            y = _cmul(_cmul(fs[0], fs[1]), fs[2])
            for k in range(8):
                vb[pl.ds(V_YTAB + 16 * k + 8 * h, 8), :] = y[0]
                vb[pl.ds(V_YTAB + 128 + 16 * k + 8 * h, 8), :] = y[1]
                if k < 7:
                    y = _cmul(y, z1)
                    y = (jnp.where(s == 7 - k, 1.0, y[0]), jnp.where(s == 7 - k, 0.0, y[1]))
            z = z4
            for k in range(4):
                z = _csq(z)
                put(V_STEP + 32 * k, z, h)
        return fn

    def setup_hi():
        z = get(V_START + 32)
        cf = get(V_START)
        for g in range(1, 5):
            put(V_START + 32 * g, _cmul(cf, z))
            if g < 4:
                z = _csq(z)

    def square(k0, k1):
        def fn():
            rows = [pl.ds(V_YTAB + 128 * part + 16 * k0, 16 * (k1 - k0)) for part in range(2)]
            y = _csq((vb[rows[0], :], vb[rows[1], :]))
            vb[rows[0], :] = y[0]
            vb[rows[1], :] = y[1]
        return fn

    def rows_of(g, i0, ni):
        n_i = 16 + (g == 4)

        def fn():
            x = st.pop('x') if i0 > 0 else get(V_START + 32 * g)
            step = get(V_STEP + 32 * max(g - 1, 0))
            xs = []
            for t in range(ni):
                xs.append(x)
                if i0 + t + 1 < n_i:
                    x = _cmul(x, step)
            if i0 + ni < n_i:
                st['x'] = x
            acc = [None] * ni
            for k0 in range(0, 8, ksplit):
                yr, yi = ytab(k0, k0 + ksplit)
                for t in range(ni):
                    v = xs[t][0] * yr - xs[t][1] * yi
                    v = lax.slice_in_dim(v, 0, 8, axis=1) + lax.slice_in_dim(v, 8, 16, axis=1)
                    v = jnp.sum(pltpu.roll(v, k0, 1, stride=1, stride_axis=0), axis=0)
                    acc[t] = v if acc[t] is None else acc[t] + v
                if k0 + ksplit < 8:
                    vb[pl.ds(frow, 8), :] = acc[ni - 1]
            for t in range(ni):
                row = 128 * g + 8 * (i0 + t)
                a = acc[t]
                if row == 640:
                    a = jnp.where(lax.broadcasted_iota(jnp.int32, (8, 128), 0) == 0, a, 0.0)
                taps[tslot, pl.ds(row, 8), :] = taps[tslot, pl.ds(row, 8), :] + a
                if t == ni - 1:
                    vb[pl.ds(frow, 8), :] = a
        return fn

    pieces = [(30, park), (110, setup_y(0)), (110, setup_y(1)), (80, setup_hi)]
    for g in range(5):
        if g >= 2:
            pieces += [(40, square(0, 4)), (40, square(4, 8))]
        for i0 in range(0, 16 + (g == 4), kni):
            ni = min(kni, 16 + (g == 4) - i0)
            pieces.append((83 * ni, rows_of(g, i0, ni)))
    return pieces


def _conv_pieces(c, r, buf, fs_ref, us, taps, vb, yf, frow):
    st = {}

    def fwd_u(b0, b1):
        def fn():
            lhs = _ld16(fs_ref, 2 * r[0] + r[1], pl.ds(0, 16))
            for b in range(b0, b1):
                w = pltpu.bitcast(us[c, pl.ds(b * 64, 64), :], bf16)
                res = jnp.dot(lhs, w, preferred_element_type=f32)
                row = V_UF + 32 * b
                if b == 0:
                    vb[pl.ds(row, 32), :] = res
                else:
                    p = st['prev']
                    vb[pl.ds(row, 8), :] = res[0:8] - p[16:24]
                    vb[pl.ds(row + 8, 8), :] = res[8:16] + p[24:32]
                    vb[pl.ds(row + 16, 8), :] = res[16:24] + p[0:8]
                    vb[pl.ds(row + 24, 8), :] = res[24:32] - p[8:16]
                st['prev'] = res
        return fn

    def fwd_k(jobs):
        def fn():
            for (wi, t0, nb) in jobs:
                w0, wn, b0, _ = WINDOWS[wi]
                lhs = _ld16(fs_ref, 2 * r[0] + r[1], pl.ds((b0 + t0) * 16, nb * 16))[:, :wn]
                w = taps[c, pl.ds(w0, wn), :].astype(bf16)
                vb[pl.ds(V_KF + 32 * (b0 + t0), 32 * nb), :] = jnp.dot(lhs, w, preferred_element_type=f32)
        return fn

    def mac(q, i0, ni, j0, j1):
        def fn():
            ld = lambda base, b: (vb[pl.ds(base + 32 * b + 8 * q, 8), :], vb[pl.ds(base + 32 * b + 16 + 8 * q, 8), :])
            zr, zi = st.pop('z') if j0 > 0 else ({}, {})
            ucache = {}
            for j in range(j0, j1):
                kr, ki = ld(V_KF, j)
                for i in range(max(i0, j), i0 + ni):
                    if i - j not in ucache:
                        ucache[i - j] = ld(V_UF, i - j)
                    ur, ui = ucache[i - j]
                    if i not in zr:
                        zr[i] = kr * ur - ki * ui
                        zi[i] = kr * ui + ki * ur
                    else:
                        zr[i] = zr[i] + kr * ur - ki * ui
                        zi[i] = zi[i] + kr * ui + ki * ur
            vb[pl.ds(frow, 8), :] = zr[i0 + ni - 1]
            if j1 < i0 + ni:
                st['z'] = (zr, zi)
            elif q == 0:
                for i in range(i0, i0 + ni):
                    vb[pl.ds(V_Z + 16 * (i - i0), 16), :] = jnp.concatenate([zr[i], zi[i]], axis=0)
            else:
                row = pl.multiple_of(r[0] * 32, 32) + r[1] * 16
                for i in range(i0, i0 + ni):
                    ar = vb[pl.ds(V_Z + 16 * (i - i0), 8), :]
                    ai = vb[pl.ds(V_Z + 16 * (i - i0) + 8, 8), :]
                    yf[buf, i, 0, pl.ds(row, 16), :] = jnp.concatenate([ar + zr[i], ai - zi[i]], axis=0).astype(bf16)
                    yf[buf, i, 1, pl.ds(row, 16), :] = jnp.concatenate([ar - zr[i], ai + zi[i]], axis=0).astype(bf16)
        return (8 * sum(1 for j in range(j0, j1) for i in range(max(i0, j), i0 + ni)), fn)

    fwd = [fwd_u(0, 8), fwd_u(8, 16), fwd_k(((0, 0, 1), (1, 0, 1), (2, 0, 1), (3, 0, 1))),
           fwd_k(((4, 0, 2), (6, 0, 2), (6, 2, 2), (6, 4, 2))), fwd_k(((4, 2, 1), (5, 0, 1), (6, 6, 1), (7, 0, 1)))]
    macs = []
    for i0 in range(0, NBLK, 2):
        for q in range(2):
            for j0 in range(0, i0 + 2, MACJ):
                macs.append(mac(q, i0, 2, j0, min(j0 + MACJ, i0 + 2)))
    return fwd, macs


def _inv_piece(c, b, buf, g_ref, us, vec, yf, outb):
    rows = pl.ds(b * 64 if isinstance(b, int) else pl.multiple_of(b * 64, 64), 64)
    rnd = lambda v: v.astype(bf16).astype(f32)
    uw = us[c, rows, :]
    dsk = vec[1, pl.ds(c, 1), :]
    o = []
    for par, u in enumerate((uw << 16, uw & u32(0xFFFF0000))):
        y = jnp.dot(_ld16(g_ref, par, slice(None)), _ld16(yf, buf, b, par, slice(None)), preferred_element_type=f32)
        o.append(pltpu.bitcast(rnd(rnd(y) + rnd(pltpu.bitcast(u, f32) * dsk)), u32))
    outb[c, rows, :] = (o[0] >> 16) | o[1]


def _attn_fill():
    n = 2 * (SEG + M)
    r = lax.broadcasted_iota(jnp.int32, (n, n), 0)
    c = lax.broadcasted_iota(jnp.int32, (n, n), 1)
    head = lambda i: jnp.where(i < 2 * SEG, i // SEG, (i - 2 * SEG) // PRE)
    pos = lambda i: jnp.where(i < 2 * SEG, i % SEG, i % PRE)
    is_mem = lambda i: (i < 2 * SEG) & (i % SEG < M)
    same = head(r) == head(c)
    allowed = same & (is_mem(r) | is_mem(c) | (pos(r) >= pos(c)))
    return jnp.where(allowed, 0.0, jnp.where(same, -1e9 * LOG2E, -jnp.inf)).astype(f32)


def _kernel(zero_hbm, x_hbm, mem0_hbm, wq_hbm, wk_hbm, wv_hbm, wo_hbm,
            u_hbm, p0, p1, p2, p3, p4, p5, ldt_hbm, dsk_hbm, fs_hbm, g_hbm,
            out_hbm,
            wq, wk, wv, wo, xb, xs, h_ref, outs, fill_ref,
            praw, par, us, taps, vb, vm, vu, pacc, yf, outb, vec, vraw, fs_ref, g_ref, zero_ref,
            sem_s, sem_w, sem_o, sem_xb, sem_x, sem_p, sem_u, sem_out, pre, own, lo0, lo1):
    wqkv = (wq, wk, wv)
    scale = E ** -0.5

    whbm = [w.bitcast(u32) for w in (wq_hbm, wk_hbm, wv_hbm)]

    def wcp(j, m, p):
        return pltpu.make_async_copy(whbm[m].at[:, p, j, :], wqkv[m].at[p, j], sem_w.at[(j * 3 + m) * 2 + p])

    xu = x_hbm.bitcast(u32)
    xcs = [pltpu.make_async_copy(xu.at[:, t, pl.ds(0, PRE // 2), pl.ds(c * 128, 128)],
                                 xb.at[c, :, pl.ds(t * (PRE // 2), PRE // 2), :], sem_xb.at[2 * c + t])
           for c in range(8) for t in range(2)]
    xcp1 = pltpu.make_async_copy(x_hbm.at[:, :, pl.ds(PRE, TOK), :], xs, sem_x.at[0])
    pcs = [pltpu.make_async_copy(p, praw.at[k], sem_p.at[k]) for k, p in enumerate((p0, p1, p2, p3, p4, p5))]
    ccs = [pltpu.make_async_copy(fs_hbm, fs_ref, sem_p.at[6]), pltpu.make_async_copy(g_hbm, g_ref, sem_p.at[7])]
    wou = wo_hbm.bitcast(u32)
    ocs = [pltpu.make_async_copy(wou.at[:, pl.ds(c * 128, 128)], wo.at[c], sem_o.at[c]) for c in range(8)]
    uu = u_hbm.bitcast(u32)
    ucs = [pltpu.make_async_copy(uu.at[:, pl.ds(c * 128, 128)], us.at[c], sem_u.at[c]) for c in range(NT)]

    zcp = pltpu.make_async_copy(zero_hbm, zero_ref, sem_s.at[0])
    scs = [pltpu.make_async_copy(mem0_hbm, h_ref.at[pl.ds(0, M)], sem_s.at[1]),
           pltpu.make_async_copy(ldt_hbm, vraw.at[0], sem_s.at[2]),
           pltpu.make_async_copy(dsk_hbm, vraw.at[1], sem_s.at[3])]
    w0cs = [[pltpu.make_async_copy(whbm[0].at[pl.ds(half * (DM // 4), DM // 4), p, 0, :],
                                   wq.at[p, 0, pl.ds(half * (DM // 4), DM // 4)], sem_s.at[4 + 2 * half + p])
             for p in range(2)] for half in range(2)]
    for cp in [zcp] + w0cs[0] + xcs[:8]:
        cp.start()
    vu[pl.ds(8, 8), :] = pltpu.bitcast(jnp.full((8, 128), 0x0000FFFF, u32), f32)
    vu[pl.ds(16, 8), :] = pltpu.bitcast(jnp.full((8, 128), 0xFFFF0000, u32), f32)
    taps[...] = jnp.zeros(taps.shape, f32)
    yf[1] = jnp.zeros(yf.shape[1:], bf16)
    fill_ref[...] = _attn_fill()
    for cp in w0cs[1] + xcs[8:] + scs:
        cp.start()
    zcp.wait()

    def opaque_row(k, buf):
        return pl.multiple_of(jnp.clip(zero_ref[k] * 8, 0, buf.shape[0] - 8), 8)

    bufs = (vb, vm, vu, par)
    fence_rows = [opaque_row(0, b) for b in bufs]
    done_vb, done_vm = opaque_row(1, vb), opaque_row(1, vm)

    class Pacer:
        def __init__(self, segments):
            self.t = 0.0
            self.todo = []
            for (pieces, buf, t0, t1) in segments:
                total = float(sum(c for c, _ in pieces)) or 1.0
                done = 0.0
                for (cst, fn) in pieces:
                    self.todo.append((t0 + (t1 - t0) * done / total, fn, buf))
                    done += cst

        def __call__(self, v, dt=1.0):
            self.t += dt
            fenced = []
            while self.todo and self.todo[0][0] < self.t:
                _, fn, buf = self.todo.pop(0)
                if not any(b is buf for b in fenced):
                    buf[pl.ds([r for b, r in zip(bufs, fence_rows) if b is buf][0], 8), :] = v
                    fenced.append(buf)
                fn()

        def finished(self):
            return not self.todo

    def unpair(j, m, r0, nr):
        def fn():
            rows = pl.ds(r0, nr)
            m_lo = pltpu.bitcast(vu[pl.ds(8, 8), :], u32)[None]
            m_hi = pltpu.bitcast(vu[pl.ds(16, 8), :], u32)[None]
            a = wqkv[m][0, j, rows, :].reshape(nr // 8, 8, E)
            b = wqkv[m][1, j, rows, :].reshape(nr // 8, 8, E)
            wqkv[m][0, j, rows, :] = ((a & m_lo) | ((b & m_lo) << 16)).reshape(nr, E)
            wqkv[m][1, j, rows, :] = (((a & m_hi) >> 16) | (b & m_hi)).reshape(nr, E)
        return (nr, fn)

    def unpair_pieces(items, lo=0, hi=DM // 2):
        return [unpair(j, m, r0, UNP) for (j, m) in items for r0 in range(lo, hi, UNP)]

    items = [(j, m) for j in range(NP) for m in range(3)]
    wcs = lambda lo, hi: [wcp(j, m, p) for (j, m) in items[lo:hi] for p in range(2)]
    rest = ocs + ccs + ucs + [xcp1]
    starts = [[] for _ in range(2 * len(items))]
    n_w, n_r = 1, 0
    for unit in sorted(STARTS):
        w_hi, with_par, r_hi = STARTS[unit]
        starts[unit] = (pcs if with_par else []) + wcs(n_w, w_hi) + rest[n_r:r_hi]
        n_w, n_r = w_hi, r_hi
    assert n_w == len(items) and n_r == len(rest)
    with jax.named_scope("bulk"):
        if QUICK in (1, 2):
            for cp in wcs(1, 48) + pcs + ocs + ucs + [xcp1] + ccs:
                cp.start()
            for cp in wcs(1, 48) + pcs + scs + xcs + w0cs[0] + w0cs[1]:
                cp.wait()
            vec[...] = vraw[...].astype(f32)
            for _, fn in (unpair_pieces(items) + sum(_prep_pieces(praw, vec, par), [])) if QUICK != 2 else []:
                fn()

            def kg(r, carry):
                for odd in range(2):
                    for _, fn in _kgen_pieces(0, (r, odd), par, vb, taps, 0, done_vb, BKNI, BKSPLIT):
                        fn()
                return carry
            lax.fori_loop(0, 4, kg, 0)
            for (j, m) in (items if QUICK != 2 else []):
                def chunk(rc, carry, j=j, m=m):
                    lhs = jnp.concatenate(
                        [pltpu.bitcast(xb[c, pl.ds(rc * 4, 4)].reshape(32, 128), bf16) for c in range(8)], axis=1)
                    res = [jnp.dot(lhs, pltpu.bitcast(wqkv[m][p, j], bf16), preferred_element_type=f32)
                           for p in range(2)]
                    for t in range(8):
                        v = jnp.concatenate([res[0][8 * t:8 * t + 8], res[1][8 * t:8 * t + 8]], axis=0)
                        pre[rc * 8 + t, m * NP + j] = v.astype(bf16)
                    return carry
                lax.fori_loop(0, 8, chunk, 0)
            items = []
        n_chunk = 2 * (T0 // RC)
        prep = _prep_pieces(praw, vec, par)
        kg0 = [pc for r in range(8) for pc in _kgen_pieces(0, r, par, vb, taps, 0, done_vb, BKNI, BKSPLIT)]
        t_a, t_b, t_c, t_d = [v * n_chunk for v in BPLAN]
        fence_x = Pacer([(prep[0], par, t_a, t_b), (kg0, vb, t_b, t_c), (prep[1], par, t_c, t_d)])
        landed = 1
        for it, (j, m) in enumerate(items):
            fence_w = None
            for half in range(2):
                for cp in starts[2 * it + half]:
                    cp.start()
                if it == 0:
                    with jax.named_scope("waitx%d" % half):
                        for cp in w0cs[half] + xcs[8 * half:8 * half + 8]:
                            cp.wait()
                    for _, fn in unpair_pieces(items[:1], half * (DM // 4), (half + 1) * (DM // 4)):
                        fn()
                    fence_w = Pacer([])
                elif half == 0:
                    late = landed == it
                    if it in WAITS:
                        with jax.named_scope("wait%d" % it):
                            for cp in wcs(landed, WAITS[it]) + (pcs + scs if it == PAR_WAIT else []):
                                cp.wait()
                        landed = WAITS[it]
                        if it == PAR_WAIT:
                            vec[...] = vraw[...].astype(f32)
                    if late:
                        for _, fn in unpair_pieces(items[it:it + 1]):
                            fn()
                    fence_w = Pacer([(unpair_pieces(items[it + 1:min(it + 2, landed)]), vu, 0.0, n_chunk * UNP_FRAC)])
                for p in range(2):
                    w = pltpu.bitcast(wqkv[m][p, j, pl.ds(half * (DM // 4), DM // 4), :], bf16)
                    lhs = jnp.concatenate([pltpu.bitcast(xb[c].reshape(T0 // 2, 128), bf16)
                                           for c in range(4 * half, 4 * half + 4)], axis=1)
                    res = jnp.dot(lhs, w, preferred_element_type=f32)
                    for rc in range(T0 // RC):
                        rows = pl.ds(rc * RC, RC)
                        v = res[rc * RC:(rc + 1) * RC]
                        if half == 1:
                            v = v + pacc[p, rows, :]
                        if p == 0 or half == 0:
                            pacc[p, rows, :] = v
                        else:
                            pr = jnp.concatenate([pacc[0, rows, :].reshape(RC // PRE, PRE, E),
                                                  v.reshape(RC // PRE, PRE, E)], axis=1)
                            pre[pl.ds(rc * (RC // PRE), RC // PRE), m * NP + j] = pr.astype(bf16)
                        fence_w(v[:8], 0.5)
                        fence_x(v[:8], 0.5)
            assert fence_w.finished() and landed > it
        assert QUICK or fence_x.finished()
    with jax.named_scope("waitrest"):
        for cp in ocs + ucs + ccs + [xcp1]:
            cp.wait()

    def outa_cp(row, n):
        return pltpu.make_async_copy(outs.at[pl.ds(row, n)], out_hbm.at[pl.ds(row, n), pl.ds(0, DM)], sem_out.at[0])

    def outb_cp(c, row, n, sem):
        col = DM + c * 128
        return pltpu.make_async_copy(
            outb.at[c, pl.ds(row, n)],
            out_hbm.bitcast(u32).at[pl.ds(row, n), pl.ds(col if isinstance(col, int) else pl.multiple_of(col, 128), 128)],
            sem_out.at[sem])

    def one_step(i, odd, fwd, fence):
        s = 2 * i + odd
        lo_cur = (lo0, lo1)[odd]
        base = pl.multiple_of(2 * SEG * i, 2 * SEG)
        h_ref[pl.ds(M, TOK), :] = xs[i, odd]
        h = h_ref[...]
        scores = {}
        probs = {}

        ct = i >> 2
        r = s & 7
        buf = ct & 1
        cprev = (ct + NT - 1) & (NT - 1)

        def stage_a(j):
            for m in range(3):
                for p in range(2):
                    w = pltpu.bitcast(wqkv[m][p, j], bf16)
                    res = jnp.dot(h, w, preferred_element_type=f32)
                    own[m * NP + j, pl.ds(SEG * p, SEG), :] = res.astype(bf16)
                    fence(res[:M])

        def gather(m, j):
            return pltpu.bitcast(jnp.concatenate([own.bitcast(u32)[m * NP + j],
                                                  pre.bitcast(u32)[s, m * NP + j]], axis=0), bf16)

        def stage_qk(j):
            scores[j] = lax.dot_general(gather(0, j), gather(1, j), (((1,), (1,)), ((), ())),
                                        preferred_element_type=f32)

        def stage_b(j):
            fl = fill_ref[...]
            sc = jnp.where(fl == 0.0, scores.pop(j) * (scale * LOG2E), fl)
            e = jnp.exp2(sc - jnp.max(sc, axis=-1, keepdims=True))
            den = jnp.sum(e, axis=-1, keepdims=True)
            probs[j] = (e * pl.reciprocal(den, approx=True)).astype(bf16)

        def stage_c(j):
            o = jnp.dot(probs[j], gather(2, j), preferred_element_type=f32)
            for p in range(2):
                hh = 2 * j + p
                lo_cur[hh, pl.ds(0, SEG), :] = o[p * SEG:(p + 1) * SEG].astype(bf16)
                ob = o[2 * SEG + p * PRE:2 * SEG + (p + 1) * PRE]
                lo1[hh, pl.ds(SEG + odd * PRE, PRE), :] = ob.astype(bf16)

        acc = [None] * 8

        def stage_d(h0, h1, last=False):
            lhs = jnp.concatenate([_ld16(lo_cur, hh, slice(None)) for hh in range(h0, h1)], axis=1)
            for c in range(8):
                w = pltpu.bitcast(wo[c, pl.ds(h0 * 64, (h1 - h0) * 64), :], bf16)
                res = jnp.dot(lhs, w, preferred_element_type=f32)
                acc[c] = res if acc[c] is None else acc[c] + res
                if not last:
                    fence(res[:M], (h1 - h0) / 8.0 * (DW_ODD if odd else 1.0))
                else:
                    rb = acc[c].astype(bf16)
                    cols = pl.ds(c * 128, 128)
                    h_ref[pl.ds(0, M), cols] = rb[:M]
                    outs[pl.ds(base + (odd * SEG + PRE), TOK), cols] = rb[M:SEG]
                    if odd:
                        outs[pl.ds(base, PRE), cols] = rb[SEG:SEG + PRE]
                        outs[pl.ds(base + SEG, PRE), cols] = rb[SEG + PRE:]

        def attn_group(jq, jc):
            for j in jq:
                stage_qk(j)
            for j in jc:
                stage_c(j)
            for j in jq:
                stage_b(j)

        for t in range(2):
            _inv_piece(cprev, 2 * r + t, 1 - buf, g_ref, us, vec, yf, outb)
        for p in fwd:
            p()
        for j in range(NP):
            stage_a(j)
            if j >= 2 and j % 2 == 0:
                attn_group((j - 2, j - 1), (j - 4, j - 3) if j >= 4 else ())
        stage_d(0, 8)
        attn_group((14, 15), (12, 13))
        stage_d(8, 20)
        attn_group((), (14, 15))
        stage_d(20, 28)
        stage_d(28, 32, last=True)

    def two_steps(i, carry):
        ct = i >> 2
        cprev = (ct + NT - 1) & (NT - 1)
        conv = [_conv_pieces(ct, (i & 3, odd), ct & 1, fs_ref, us, taps, vm, yf,
                             done_vm) for odd in range(2)]
        kgen = [_kgen_pieces((ct + 1) & (NT - 1), (i & 3, odd), par, vb, taps, ct + 1,
                             done_vb, KNI, KSPLIT) for odd in range(2)]
        work = {'k0': (kgen[0], vb), 'k1': (kgen[1], vb), 'm0': (conv[0][1], vm), 'm1': (conv[1][1], vm)}
        fence = Pacer([work[k] + (t0, t1) for (k, t0, t1) in PLAN if k[0] not in NOB])
        for odd in range(2):
            one_step(i, odd, conv[odd][0], fence)
        assert fence.finished() or NOB
        outa_cp(pl.multiple_of(2 * SEG * i, 2 * SEG), 2 * SEG).start()
        outb_cp(cprev, pl.multiple_of((i & 3) * 256, 256), 256, jnp.where(i < 4, 2, 1)).start()
        return carry

    with jax.named_scope("steps"):
        if NITER:
            lax.fori_loop(0, NITER, two_steps, 0)

    with jax.named_scope("flush"):
        outb_cp(NT - 1, 0, L // 2, 2).wait()
        for b in range(NBLK):
            _inv_piece(NT - 1, b, (NT - 1) % 2, g_ref, us, vec, yf, outb)
            if b % 4 == 3:
                outb_cp(NT - 1, (b - 3) * 64, 256, 1).start()
    with jax.named_scope("waitout"):
        outa_cp(0, S).wait()
        pltpu.make_async_copy(outb, outb, sem_out.at[1]).wait()


@jax.jit
def pallas_concat_heads__memory_aug_recurrent_mem_tr__ssm_conv_s4__prompt_kernel(
    A_x, A_mem0, A_Wq, A_Wk, A_Wv, A_Wo, A_seg_len,
    B_u, B_A_re, B_A_im, B_B_re, B_B_im, B_C_re, B_C_im, B_log_dt, B_Dskip,
):
    del A_seg_len
    assert A_x.shape == (1, S, DM) and B_u.shape == (1, L, D)
    fs, g = _dft_consts()
    w4 = lambda w: w.reshape(DM // 2, 2, H, E)
    any_ = pl.BlockSpec(memory_space=pl.ANY)
    V = pltpu.VMEM
    out = pl.pallas_call(
        _kernel,
        out_shape=jax.ShapeDtypeStruct((S, DM + D), bf16),
        in_specs=[any_] * 18,
        out_specs=any_,
        scratch_shapes=[
            V((2, NP, DM // 2, E), u32),
            V((2, NP, DM // 2, E), u32),
            V((2, NP, DM // 2, E), u32),
            V((8, H * E // 2, 128), u32),
            V((8, NSEG // 2, PRE, 128), u32),
            V((NSEG // 2, 2, TOK, DM), bf16),
            V((M + TOK, DM), bf16),
            V((S, DM), bf16),
            V((2 * (SEG + M), 2 * (SEG + M)), f32),
            V((6, D, N), bf16),
            V((8 + NT * 6 * N, 128), f32),
            V((NT, L // 2, 128), u32),
            V((NT + 1, TAPROWS, 128), f32),
            V((V_ROWS, 128), f32),
            V((VM_ROWS, 128), f32),
            V((24, 128), f32),
            V((2, T0, 128), f32),
            V((2, NBLK, 2, BLK, 128), bf16),
            V((NT, L // 2, 128), u32),
            V((2, 8, 128), f32),
            V((2, 8, 128), bf16),
            V((8, NBLK * 32, 128), bf16),
            V((2, BLK // 2, 128), bf16),
            pltpu.SMEM((2,), jnp.int32),
            pltpu.SemaphoreType.DMA((8,)),
            pltpu.SemaphoreType.DMA((6 * NP,)),
            pltpu.SemaphoreType.DMA((8,)),
            pltpu.SemaphoreType.DMA((16,)),
            pltpu.SemaphoreType.DMA((1,)),
            pltpu.SemaphoreType.DMA((8,)),
            pltpu.SemaphoreType.DMA((NT,)),
            pltpu.SemaphoreType.DMA((3,)),
            V((NSEG, 3 * NP, 2 * PRE, E), bf16),
            V((3 * NP, 2 * SEG, E), bf16),
            V((H, SEG, E), bf16),
            V((H, SEG + 2 * PRE, E), bf16),
        ],
        compiler_params=pltpu.CompilerParams(vmem_limit_bytes=110 * 1024 * 1024, disable_bounds_checks=True),
    )(jnp.asarray(np.zeros((2,), np.int32)), A_x.reshape(NSEG // 2, 2, SEG, DM), A_mem0.reshape(M, DM), w4(A_Wq), w4(A_Wk), w4(A_Wv), A_Wo.reshape(H * E, DM),
      B_u.reshape(L, D), B_A_re, B_A_im, B_B_re, B_B_im, B_C_re, B_C_im,
      B_log_dt.reshape(8, 128), B_Dskip.reshape(8, 128),
      jnp.asarray(fs, bf16), jnp.asarray(g, bf16))
    return out.reshape(1, S, DM + D)
```

```python
import functools

import numpy as np
import jax
import jax.numpy as jnp
from jax import lax
import jax.experimental.pallas as pl
import jax.experimental.pallas.tpu as pltpu

bf16, f32, u32 = jnp.bfloat16, jnp.float32, jnp.uint32

S, DM, H, E, M, SEG = 2048, 1024, 32, 128, 8, 32
NSEG = S // SEG
TOK = 24
PRE = SEG - TOK
T0 = PRE * NSEG
NP = H // 2
LOG2E = 1.4426950408889634
QUICK = False
NOB = ''
BKNI = 1
UNP = 64
UNP_FRAC = 0.7
BKSPLIT = 4
BPLAN = (10.0, 11.0, 42.5, 47.7)
WAITS = {1: 2, 2: 3, 3: 5, 4: 6, 5: 8, 7: 11, 10: 13, 12: 17, 16: 23, 22: 33, 32: 48}
PAR_WAIT = 10
STARTS = {0: (2, False, 0), 1: (3, False, 0), 2: (5, False, 0), 4: (6, False, 0), 6: (8, False, 0),
          8: (9, False, 0), 10: (11, False, 0), 14: (13, True, 0), 20: (17, False, 0), 24: (23, False, 0),
          32: (33, False, 0), 44: (48, False, 3), 64: (48, False, 19)}
NITER = NSEG // 2
KNI = 2
KSPLIT = 2
PLAN = (('k0', 0, 96), ('m0', 96, 122), ('k1', 124, 220), ('m1', 220, 260))
DW_ODD = 1.5
RC = 64
MACJ = 3
L, D, N = 2048, 1024, 128
BLK = 128
NBLK = L // BLK
NT = D // 128
TAPROWS = 672
WINDOWS = ((0, 128, 0, 1), (128, 128, 1, 1), (256, 128, 2, 1), (320, 80, 3, 1),
           (384, 128, 4, 3), (480, 48, 7, 1), (512, 128, 8, 7), (624, 32, 15, 1))

V_FENCE = 0
V_YTAB = 8
V_START = V_YTAB + 256
V_STEP = V_START + 160
V_ROWS = V_STEP + 128 + 24
V_UF = 8
V_KF = V_UF + NBLK * 32
V_Z = V_KF + NBLK * 32
VM_ROWS = V_Z + 32 + 24


def _bf16_round_int(l):
    u = np.asarray(l, np.float32).view(np.uint32)
    r = (u + 0x7FFF + ((u >> 16) & 1)) & 0xFFFF0000
    return r.astype(np.uint32).view(np.float32).astype(np.int64)


def _tap_row(lp):
    return np.where(lp < 256, lp, np.where(lp < 512, 256 + (lp - 256) // 2,
                    np.where(lp < 1024, 384 + (lp - 512) // 4, 512 + (lp - 1024) // 8)))


@functools.lru_cache(maxsize=None)
def _dft_consts():
    t = np.arange(BLK)
    F = np.zeros((8, 32, BLK))
    G = np.zeros((2, BLK // 2, 8, 16))
    for r in range(8):
        f = 16 * r + 2 * np.arange(8)
        th = 2 * np.pi * (np.concatenate([f, BLK - 1 - f]) + 0.5) / (2 * BLK)
        F[r, :16] = np.cos(th[:, None] * t[None])
        F[r, 16:] = -np.sin(th[:, None] * t[None])
        for par in range(2):
            G[par, :, r, :8] = np.cos(th[None, :8] * t[par::2, None]) / BLK
            G[par, :, r, 8:] = -np.sin(th[None, :8] * t[par::2, None]) / BLK
    FS = np.zeros((8, NBLK, 32, 128))
    for (w0, wn, b0, nb) in WINDOWS:
        for j in range(b0, b0 + nb):
            rows = _tap_row(_bf16_round_int(BLK * j + t)) - w0
            assert rows.min() >= 0 and rows.max() < wn
            sel = np.zeros((BLK, 128))
            sel[t, rows] = 1.0
            FS[:, j] = F @ sel
    return (FS.reshape(8, NBLK * 32, 128).astype(np.float32),
            G.reshape(2, BLK // 2, 128).astype(np.float32))


def _ld16(ref, *idx):
    return pltpu.bitcast(ref.bitcast(u32)[idx + (slice(None),)], bf16)


def _cmul(a, b):
    return (a[0] * b[0] - a[1] * b[1], a[0] * b[1] + a[1] * b[0])


def _csq(a):
    return (a[0] * a[0] - a[1] * a[1], 2.0 * (a[0] * a[1]))


def _cexp(lr, li):
    k = jnp.floor(li * (2.0 / np.pi) + 0.5)
    r = ((li - k * 1.5703125) - k * 4.837512969970703125e-4) - k * 7.54978995489188216e-8
    r = jnp.clip(r, -0.8, 0.8)
    r2 = r * r
    s = r + r * r2 * (-1.6666654611e-1 + r2 * (8.3321608736e-3 + r2 * -1.9515295891e-4))
    c = (1.0 - 0.5 * r2) + (r2 * r2) * (4.166664568298827e-2
                                        + r2 * (-1.388731625493765e-3 + r2 * 2.443315711809948e-5))
    q = k.astype(jnp.int32)
    swap = (q & 1) == 1
    m = jnp.exp(lr)
    flip = lambda v, bit: pltpu.bitcast(pltpu.bitcast(v, jnp.int32) ^ (bit << 30), f32)
    return (flip(m * jnp.where(swap, s, c), (q + 1) & 2), flip(m * jnp.where(swap, c, s), q & 2))


def _par_row(c, k):
    return 8 + (c * 6 + k) * N


def _prep_pieces(praw, vec, par):
    def stage1(c):
        def fn():
            tr = lambda k: praw[k, pl.ds(c * 128, 128), :].astype(f32).T
            dt = jnp.exp(vec[0, pl.ds(c, 1), :]).astype(bf16).astype(f32)
            cc = _cmul((tr(4), tr(5)), (dt * tr(2), dt * tr(3)))
            for k, v in ((0, dt * tr(0)), (1, dt * tr(1)), (4, cc[0]), (5, cc[1])):
                par[pl.ds(_par_row(c, k), N), :] = v
        return fn

    def stage2(c, n0):
        def fn():
            lr = par[pl.ds(_par_row(c, 0) + n0, 16), :]
            li = par[pl.ds(_par_row(c, 1) + n0, 16), :]
            for k, v in enumerate(_cexp(lr, li) + _cexp(lr * 128.0, li * 128.0)):
                par[pl.ds(_par_row(c, k) + n0, 16), :] = v
        return fn

    tile = lambda c: [(260, stage1(c))] + [(190, stage2(c, n0)) for n0 in range(0, N, 16)]
    return tile(0), [pc for c in range(1, NT) for pc in tile(c)]


def _kgen_pieces(c, r, par, vb, taps, tslot, frow, kni, ksplit):
    st = {}

    def put(row, z, h=None):
        if h is None:
            vb[pl.ds(row, 16), :] = z[0]
            vb[pl.ds(row + 16, 16), :] = z[1]
        else:
            vb[pl.ds(row + 8 * h, 8), :] = z[0]
            vb[pl.ds(row + 16 + 8 * h, 8), :] = z[1]

    def get(row, h=None):
        if h is None:
            return (vb[pl.ds(row, 16), :], vb[pl.ds(row + 16, 16), :])
        return (vb[pl.ds(row + 8 * h, 8), :], vb[pl.ds(row + 16 + 8 * h, 8), :])

    def ytab(k0, k1):
        return [vb[pl.ds(V_YTAB + 128 * part + 16 * k0, 16 * (k1 - k0)), :].reshape(k1 - k0, 16, 128)
                for part in range(2)]

    def params(k):
        if isinstance(r, int):
            return par[pl.ds(_par_row(c, k) + r * 16, 16), :]
        return par[pl.ds(pl.multiple_of(c * (6 * N) + r[0] * 32, 32) + (_par_row(0, k) + r[1] * 16), 16), :]

    def park():
        put(V_STEP, (params(0), params(1)))
        put(V_START + 32, (params(2), params(3)))
        put(V_START, (params(4), params(5)))

    def setup_y(h):
        def fn():
            z1 = get(V_STEP, h)
            z2 = _csq(z1)
            z4 = _csq(z2)
            s = lax.broadcasted_iota(jnp.int32, (8, 128), 0)
            fs = [(jnp.where((s >> k) & 1 == 1, z[0], 1.0), jnp.where((s >> k) & 1 == 1, z[1], 0.0))
                  for k, z in enumerate((z1, z2, z4))]
            y = _cmul(_cmul(fs[0], fs[1]), fs[2])
            for k in range(8):
                vb[pl.ds(V_YTAB + 16 * k + 8 * h, 8), :] = y[0]
                vb[pl.ds(V_YTAB + 128 + 16 * k + 8 * h, 8), :] = y[1]
                if k < 7:
                    y = _cmul(y, z1)
                    y = (jnp.where(s == 7 - k, 1.0, y[0]), jnp.where(s == 7 - k, 0.0, y[1]))
            z = z4
            for k in range(4):
                z = _csq(z)
                put(V_STEP + 32 * k, z, h)
        return fn

    def setup_hi():
        z = get(V_START + 32)
        cf = get(V_START)
        for g in range(1, 5):
            put(V_START + 32 * g, _cmul(cf, z))
            if g < 4:
                z = _csq(z)

    def square(k0, k1):
        def fn():
            rows = [pl.ds(V_YTAB + 128 * part + 16 * k0, 16 * (k1 - k0)) for part in range(2)]
            y = _csq((vb[rows[0], :], vb[rows[1], :]))
            vb[rows[0], :] = y[0]
            vb[rows[1], :] = y[1]
        return fn

    def rows_of(g, i0, ni):
        n_i = 16 + (g == 4)

        def fn():
            x = st.pop('x') if i0 > 0 else get(V_START + 32 * g)
            step = get(V_STEP + 32 * max(g - 1, 0))
            xs = []
            for t in range(ni):
                xs.append(x)
                if i0 + t + 1 < n_i:
                    x = _cmul(x, step)
            if i0 + ni < n_i:
                st['x'] = x
            acc = [None] * ni
            for k0 in range(0, 8, ksplit):
                yr, yi = ytab(k0, k0 + ksplit)
                for t in range(ni):
                    v = xs[t][0] * yr - xs[t][1] * yi
                    v = lax.slice_in_dim(v, 0, 8, axis=1) + lax.slice_in_dim(v, 8, 16, axis=1)
                    v = jnp.sum(pltpu.roll(v, k0, 1, stride=1, stride_axis=0), axis=0)
                    acc[t] = v if acc[t] is None else acc[t] + v
                if k0 + ksplit < 8:
                    vb[pl.ds(frow, 8), :] = acc[ni - 1]
            for t in range(ni):
                row = 128 * g + 8 * (i0 + t)
                a = acc[t]
                if row == 640:
                    a = jnp.where(lax.broadcasted_iota(jnp.int32, (8, 128), 0) == 0, a, 0.0)
                taps[tslot, pl.ds(row, 8), :] = taps[tslot, pl.ds(row, 8), :] + a
                if t == ni - 1:
                    vb[pl.ds(frow, 8), :] = a
        return fn

    pieces = [(30, park), (110, setup_y(0)), (110, setup_y(1)), (80, setup_hi)]
    for g in range(5):
        if g >= 2:
            pieces += [(40, square(0, 4)), (40, square(4, 8))]
        for i0 in range(0, 16 + (g == 4), kni):
            ni = min(kni, 16 + (g == 4) - i0)
            pieces.append((83 * ni, rows_of(g, i0, ni)))
    return pieces


def _conv_pieces(c, r, buf, fs_ref, us, taps, vb, yf, frow):
    st = {}

    def fwd_u(b0, b1):
        def fn():
            lhs = _ld16(fs_ref, 2 * r[0] + r[1], pl.ds(0, 16))
            for b in range(b0, b1):
                w = pltpu.bitcast(us[c, pl.ds(b * 64, 64), :], bf16)
                res = jnp.dot(lhs, w, preferred_element_type=f32)
                row = V_UF + 32 * b
                if b == 0:
                    vb[pl.ds(row, 32), :] = res
                else:
                    p = st['prev']
                    vb[pl.ds(row, 8), :] = res[0:8] - p[16:24]
                    vb[pl.ds(row + 8, 8), :] = res[8:16] + p[24:32]
                    vb[pl.ds(row + 16, 8), :] = res[16:24] + p[0:8]
                    vb[pl.ds(row + 24, 8), :] = res[24:32] - p[8:16]
                st['prev'] = res
        return fn

    def fwd_k(jobs):
        def fn():
            for (wi, t0, nb) in jobs:
                w0, wn, b0, _ = WINDOWS[wi]
                lhs = _ld16(fs_ref, 2 * r[0] + r[1], pl.ds((b0 + t0) * 16, nb * 16))[:, :wn]
                w = taps[c, pl.ds(w0, wn), :].astype(bf16)
                vb[pl.ds(V_KF + 32 * (b0 + t0), 32 * nb), :] = jnp.dot(lhs, w, preferred_element_type=f32)
        return fn

    def mac(q, i0, ni, j0, j1):
        def fn():
            ld = lambda base, b: (vb[pl.ds(base + 32 * b + 8 * q, 8), :], vb[pl.ds(base + 32 * b + 16 + 8 * q, 8), :])
            zr, zi = st.pop('z') if j0 > 0 else ({}, {})
            ucache = {}
            for j in range(j0, j1):
                kr, ki = ld(V_KF, j)
                for i in range(max(i0, j), i0 + ni):
                    if i - j not in ucache:
                        ucache[i - j] = ld(V_UF, i - j)
                    ur, ui = ucache[i - j]
                    if i not in zr:
                        zr[i] = kr * ur - ki * ui
                        zi[i] = kr * ui + ki * ur
                    else:
                        zr[i] = zr[i] + kr * ur - ki * ui
                        zi[i] = zi[i] + kr * ui + ki * ur
            vb[pl.ds(frow, 8), :] = zr[i0 + ni - 1]
            if j1 < i0 + ni:
                st['z'] = (zr, zi)
            elif q == 0:
                for i in range(i0, i0 + ni):
                    vb[pl.ds(V_Z + 16 * (i - i0), 16), :] = jnp.concatenate([zr[i], zi[i]], axis=0)
            else:
                row = pl.multiple_of(r[0] * 32, 32) + r[1] * 16
                for i in range(i0, i0 + ni):
                    ar = vb[pl.ds(V_Z + 16 * (i - i0), 8), :]
                    ai = vb[pl.ds(V_Z + 16 * (i - i0) + 8, 8), :]
                    yf[buf, i, 0, pl.ds(row, 16), :] = jnp.concatenate([ar + zr[i], ai - zi[i]], axis=0).astype(bf16)
                    yf[buf, i, 1, pl.ds(row, 16), :] = jnp.concatenate([ar - zr[i], ai + zi[i]], axis=0).astype(bf16)
        return (8 * sum(1 for j in range(j0, j1) for i in range(max(i0, j), i0 + ni)), fn)

    fwd = [fwd_u(0, 8), fwd_u(8, 16), fwd_k(((0, 0, 1), (1, 0, 1), (2, 0, 1), (3, 0, 1))),
           fwd_k(((4, 0, 2), (6, 0, 2), (6, 2, 2), (6, 4, 2))), fwd_k(((4, 2, 1), (5, 0, 1), (6, 6, 1), (7, 0, 1)))]
    macs = []
    for i0 in range(0, NBLK, 2):
        for q in range(2):
            for j0 in range(0, i0 + 2, MACJ):
                macs.append(mac(q, i0, 2, j0, min(j0 + MACJ, i0 + 2)))
    return fwd, macs


def _inv_piece(c, b, buf, g_ref, us, vec, yf, outb):
    rows = pl.ds(b * 64 if isinstance(b, int) else pl.multiple_of(b * 64, 64), 64)
    rnd = lambda v: v.astype(bf16).astype(f32)
    uw = us[c, rows, :]
    dsk = vec[1, pl.ds(c, 1), :]
    o = []
    for par, u in enumerate((uw << 16, uw & u32(0xFFFF0000))):
        y = jnp.dot(_ld16(g_ref, par, slice(None)), _ld16(yf, buf, b, par, slice(None)), preferred_element_type=f32)
        o.append(pltpu.bitcast(rnd(rnd(y) + rnd(pltpu.bitcast(u, f32) * dsk)), u32))
    outb[c, rows, :] = (o[0] >> 16) | o[1]


def _attn_fill():
    n = 2 * (SEG + M)
    r = lax.broadcasted_iota(jnp.int32, (n, n), 0)
    c = lax.broadcasted_iota(jnp.int32, (n, n), 1)
    head = lambda i: jnp.where(i < 2 * SEG, i // SEG, (i - 2 * SEG) // PRE)
    pos = lambda i: jnp.where(i < 2 * SEG, i % SEG, i % PRE)
    is_mem = lambda i: (i < 2 * SEG) & (i % SEG < M)
    same = head(r) == head(c)
    allowed = same & (is_mem(r) | is_mem(c) | (pos(r) >= pos(c)))
    return jnp.where(allowed, 0.0, jnp.where(same, -1e9 * LOG2E, -jnp.inf)).astype(f32)


def _kernel(zero_hbm, x_hbm, mem0_hbm, wq_hbm, wk_hbm, wv_hbm, wo_hbm,
            u_hbm, p0, p1, p2, p3, p4, p5, ldt_hbm, dsk_hbm, fs_hbm, g_hbm,
            out_hbm,
            wq, wk, wv, wo, xb, xs, h_ref, outs, fill_ref,
            praw, par, us, taps, vb, vm, vu, pacc, yf, outb, vec, vraw, fs_ref, g_ref, zero_ref,
            sem_s, sem_w, sem_o, sem_xb, sem_x, sem_p, sem_u, sem_out, pre, own, lo0, lo1):
    wqkv = (wq, wk, wv)
    scale = E ** -0.5

    whbm = [w.bitcast(u32) for w in (wq_hbm, wk_hbm, wv_hbm)]

    def wcp(j, m, p):
        return pltpu.make_async_copy(whbm[m].at[:, p, j, :], wqkv[m].at[p, j], sem_w.at[(j * 3 + m) * 2 + p])

    xu = x_hbm.bitcast(u32)
    xcs = [pltpu.make_async_copy(xu.at[:, t, pl.ds(0, PRE // 2), pl.ds(c * 128, 128)],
                                 xb.at[c, :, pl.ds(t * (PRE // 2), PRE // 2), :], sem_xb.at[2 * c + t])
           for c in range(8) for t in range(2)]
    xcp1 = pltpu.make_async_copy(x_hbm.at[:, :, pl.ds(PRE, TOK), :], xs, sem_x.at[0])
    pcs = [pltpu.make_async_copy(p, praw.at[k], sem_p.at[k]) for k, p in enumerate((p0, p1, p2, p3, p4, p5))]
    ccs = [pltpu.make_async_copy(fs_hbm, fs_ref, sem_p.at[6]), pltpu.make_async_copy(g_hbm, g_ref, sem_p.at[7])]
    wou = wo_hbm.bitcast(u32)
    ocs = [pltpu.make_async_copy(wou.at[:, pl.ds(c * 128, 128)], wo.at[c], sem_o.at[c]) for c in range(8)]
    uu = u_hbm.bitcast(u32)
    ucs = [pltpu.make_async_copy(uu.at[:, pl.ds(c * 128, 128)], us.at[c], sem_u.at[c]) for c in range(NT)]

    zcp = pltpu.make_async_copy(zero_hbm, zero_ref, sem_s.at[0])
    scs = [pltpu.make_async_copy(mem0_hbm, h_ref.at[pl.ds(0, M)], sem_s.at[1]),
           pltpu.make_async_copy(ldt_hbm, vraw.at[0], sem_s.at[2]),
           pltpu.make_async_copy(dsk_hbm, vraw.at[1], sem_s.at[3])]
    w0cs = [[pltpu.make_async_copy(whbm[0].at[pl.ds(half * (DM // 4), DM // 4), p, 0, :],
                                   wq.at[p, 0, pl.ds(half * (DM // 4), DM // 4)], sem_s.at[4 + 2 * half + p])
             for p in range(2)] for half in range(2)]
    for cp in [zcp] + w0cs[0] + xcs[:8]:
        cp.start()
    vu[pl.ds(8, 8), :] = pltpu.bitcast(jnp.full((8, 128), 0x0000FFFF, u32), f32)
    vu[pl.ds(16, 8), :] = pltpu.bitcast(jnp.full((8, 128), 0xFFFF0000, u32), f32)
    taps[...] = jnp.zeros(taps.shape, f32)
    yf[1] = jnp.zeros(yf.shape[1:], bf16)
    fill_ref[pl.ds(0, 2 * (SEG + M)), :] = _attn_fill()
    for cp in w0cs[1] + xcs[8:] + scs:
        cp.start()
    zcp.wait()

    def opaque_row(k, buf):
        return pl.multiple_of(jnp.clip(zero_ref[k] * 8, 0, buf.shape[0] - 8), 8)

    bufs = (vb, vm, vu, par)
    fence_rows = [opaque_row(0, b) for b in bufs]
    done_vb, done_vm = opaque_row(1, vb), opaque_row(1, vm)

    class Pacer:
        def __init__(self, segments):
            self.t = 0.0
            self.todo = []
            for (pieces, buf, t0, t1) in segments:
                total = float(sum(c for c, _ in pieces)) or 1.0
                done = 0.0
                for (cst, fn) in pieces:
                    self.todo.append((t0 + (t1 - t0) * done / total, fn, buf))
                    done += cst

        def __call__(self, v, dt=1.0):
            self.t += dt
            fenced = []
            while self.todo and self.todo[0][0] < self.t:
                _, fn, buf = self.todo.pop(0)
                if not any(b is buf for b in fenced):
                    buf[pl.ds([r for b, r in zip(bufs, fence_rows) if b is buf][0], 8), :] = v
                    fenced.append(buf)
                fn()

        def finished(self):
            return not self.todo

    def unpair(j, m, r0, nr):
        def fn():
            rows = pl.ds(r0, nr)
            m_lo = pltpu.bitcast(vu[pl.ds(8, 8), :], u32)[None]
            m_hi = pltpu.bitcast(vu[pl.ds(16, 8), :], u32)[None]
            a = wqkv[m][0, j, rows, :].reshape(nr // 8, 8, E)
            b = wqkv[m][1, j, rows, :].reshape(nr // 8, 8, E)
            wqkv[m][0, j, rows, :] = ((a & m_lo) | ((b & m_lo) << 16)).reshape(nr, E)
            wqkv[m][1, j, rows, :] = (((a & m_hi) >> 16) | (b & m_hi)).reshape(nr, E)
        return (nr, fn)

    def unpair_pieces(items, lo=0, hi=DM // 2):
        return [unpair(j, m, r0, UNP) for (j, m) in items for r0 in range(lo, hi, UNP)]

    items = [(j, m) for j in range(NP) for m in range(3)]
    wcs = lambda lo, hi: [wcp(j, m, p) for (j, m) in items[lo:hi] for p in range(2)]
    rest = ocs + ccs + ucs + [xcp1]
    starts = [[] for _ in range(2 * len(items))]
    n_w, n_r = 1, 0
    for unit in sorted(STARTS):
        w_hi, with_par, r_hi = STARTS[unit]
        starts[unit] = (pcs if with_par else []) + wcs(n_w, w_hi) + rest[n_r:r_hi]
        n_w, n_r = w_hi, r_hi
    assert n_w == len(items) and n_r == len(rest)
    with jax.named_scope("bulk"):
        if QUICK in (1, 2):
            for cp in wcs(1, 48) + pcs + ocs + ucs + [xcp1] + ccs:
                cp.start()
            for cp in wcs(1, 48) + pcs + scs + xcs + w0cs[0] + w0cs[1]:
                cp.wait()
            vec[pl.ds(0, 2)] = vraw[pl.ds(0, 2)].astype(f32)
            for _, fn in (unpair_pieces(items) + sum(_prep_pieces(praw, vec, par), [])) if QUICK != 2 else []:
                fn()

            def kg(r, carry):
                for odd in range(2):
                    for _, fn in _kgen_pieces(0, (r, odd), par, vb, taps, 0, done_vb, BKNI, BKSPLIT):
                        fn()
                return carry
            lax.fori_loop(0, 4, kg, 0)
            for (j, m) in (items if QUICK != 2 else []):
                def chunk(rc, carry, j=j, m=m):
                    lhs = jnp.concatenate(
                        [pltpu.bitcast(xb[c, pl.ds(rc * 4, 4)].reshape(32, 128), bf16) for c in range(8)], axis=1)
                    res = [jnp.dot(lhs, pltpu.bitcast(wqkv[m][p, j], bf16), preferred_element_type=f32)
                           for p in range(2)]
                    for t in range(8):
                        v = jnp.concatenate([res[0][8 * t:8 * t + 8], res[1][8 * t:8 * t + 8]], axis=0)
                        pre[rc * 8 + t, m * NP + j] = v.astype(bf16)
                    return carry
                lax.fori_loop(0, 8, chunk, 0)
            items = []
        n_chunk = 2 * (T0 // RC)
        prep = _prep_pieces(praw, vec, par)
        kg0 = [pc for r in range(8) for pc in _kgen_pieces(0, r, par, vb, taps, 0, done_vb, BKNI, BKSPLIT)]
        t_a, t_b, t_c, t_d = [v * n_chunk for v in BPLAN]
        fence_x = Pacer([(prep[0], par, t_a, t_b), (kg0, vb, t_b, t_c), (prep[1], par, t_c, t_d)])
        landed = 1
        for it, (j, m) in enumerate(items):
            fence_w = None
            for half in range(2):
                for cp in starts[2 * it + half]:
                    cp.start()
                if it == 0:
                    with jax.named_scope("waitx%d" % half):
                        for cp in w0cs[half] + xcs[8 * half:8 * half + 8]:
                            cp.wait()
                    for _, fn in unpair_pieces(items[:1], half * (DM // 4), (half + 1) * (DM // 4)):
                        fn()
                    fence_w = Pacer([])
                elif half == 0:
                    late = landed == it
                    if it in WAITS:
                        with jax.named_scope("wait%d" % it):
                            for cp in wcs(landed, WAITS[it]) + (pcs + scs if it == PAR_WAIT else []):
                                cp.wait()
                        landed = WAITS[it]
                        if it == PAR_WAIT:
                            vec[pl.ds(0, 2)] = vraw[pl.ds(0, 2)].astype(f32)
                    if late:
                        for _, fn in unpair_pieces(items[it:it + 1]):
                            fn()
                    fence_w = Pacer([(unpair_pieces(items[it + 1:min(it + 2, landed)]), vu, 0.0, n_chunk * UNP_FRAC)])
                for p in range(2):
                    w = pltpu.bitcast(wqkv[m][p, j, pl.ds(half * (DM // 4), DM // 4), :], bf16)
                    lhs = jnp.concatenate([pltpu.bitcast(xb[c].reshape(T0 // 2, 128), bf16)
                                           for c in range(4 * half, 4 * half + 4)], axis=1)
                    res = jnp.dot(lhs, w, preferred_element_type=f32)
                    for rc in range(T0 // RC):
                        rows = pl.ds(rc * RC, RC)
                        v = res[rc * RC:(rc + 1) * RC]
                        if half == 1:
                            v = v + pacc[p, rows, :]
                        if p == 0 or half == 0:
                            pacc[p, rows, :] = v
                        else:
                            pr = jnp.concatenate([pacc[0, rows, :].reshape(RC // PRE, PRE, E),
                                                  v.reshape(RC // PRE, PRE, E)], axis=1)
                            pre[pl.ds(rc * (RC // PRE), RC // PRE), m * NP + j] = pr.astype(bf16)
                        fence_w(v[:8], 0.5)
                        fence_x(v[:8], 0.5)
            assert fence_w.finished() and landed > it
        assert QUICK or fence_x.finished()
    with jax.named_scope("waitrest"):
        for cp in ocs + ucs + ccs + [xcp1]:
            cp.wait()

    def outa_cp(row, n):
        return pltpu.make_async_copy(outs.at[pl.ds(row, n)], out_hbm.at[pl.ds(row, n), pl.ds(0, DM)], sem_out.at[0])

    def outb_cp(c, row, n, sem):
        col = DM + c * 128
        return pltpu.make_async_copy(
            outb.at[c, pl.ds(row, n)],
            out_hbm.bitcast(u32).at[pl.ds(row, n), pl.ds(col if isinstance(col, int) else pl.multiple_of(col, 128), 128)],
            sem_out.at[sem])

    def one_step(i, odd, fwd, fence):
        s = 2 * i + odd
        lo_cur = (lo0, lo1)[odd]
        base = pl.multiple_of(2 * SEG * i, 2 * SEG)
        h_ref[pl.ds(M, TOK), :] = xs[i, odd]
        h = h_ref[...]
        scores = {}
        probs = {}

        ct = i >> 2
        r = s & 7
        buf = ct & 1
        cprev = (ct + NT - 1) & (NT - 1)

        def stage_a(j):
            for m in range(3):
                for p in range(2):
                    w = pltpu.bitcast(wqkv[m][p, j], bf16)
                    res = jnp.dot(h, w, preferred_element_type=f32)
                    own[m * NP + j, pl.ds(SEG * p, SEG), :] = res.astype(bf16)
                    fence(res[:M])

        def gather(m, j):
            return pltpu.bitcast(jnp.concatenate([own.bitcast(u32)[m * NP + j],
                                                  pre.bitcast(u32)[s, m * NP + j]], axis=0), bf16)

        def stage_qk(j):
            scores[j] = lax.dot_general(gather(0, j), gather(1, j), (((1,), (1,)), ((), ())),
                                        preferred_element_type=f32)

        def stage_b(j):
            fl = fill_ref[pl.ds(0, 2 * (SEG + M)), :]
            sc = jnp.where(fl == 0.0, scores.pop(j) * (scale * LOG2E), fl)
            e = jnp.exp2(sc - jnp.max(sc, axis=-1, keepdims=True))
            den = jnp.sum(e, axis=-1, keepdims=True)
            probs[j] = (e * pl.reciprocal(den, approx=True)).astype(bf16)

        def stage_c(j):
            o = jnp.dot(probs[j], gather(2, j), preferred_element_type=f32)
            for p in range(2):
                hh = 2 * j + p
                lo_cur[hh, pl.ds(0, SEG), :] = o[p * SEG:(p + 1) * SEG].astype(bf16)
                ob = o[2 * SEG + p * PRE:2 * SEG + (p + 1) * PRE]
                lo1[hh, pl.ds(SEG + odd * PRE, PRE), :] = ob.astype(bf16)

        acc = [None] * 8

        def stage_d(h0, h1, last=False):
            lhs = jnp.concatenate([_ld16(lo_cur, hh, slice(None)) for hh in range(h0, h1)], axis=1)
            for c in range(8):
                w = pltpu.bitcast(wo[c, pl.ds(h0 * 64, (h1 - h0) * 64), :], bf16)
                res = jnp.dot(lhs, w, preferred_element_type=f32)
                acc[c] = res if acc[c] is None else acc[c] + res
                if not last:
                    fence(res[:M], (h1 - h0) / 8.0 * (DW_ODD if odd else 1.0))
                else:
                    rb = acc[c].astype(bf16)
                    cols = pl.ds(c * 128, 128)
                    h_ref[pl.ds(0, M), cols] = rb[:M]
                    outs[pl.ds(base + (odd * SEG + PRE), TOK), cols] = rb[M:SEG]
                    if odd:
                        outs[pl.ds(base, PRE), cols] = rb[SEG:SEG + PRE]
                        outs[pl.ds(base + SEG, PRE), cols] = rb[SEG + PRE:]

        def attn_group(jq, jc):
            for j in jq:
                stage_qk(j)
            for j in jc:
                stage_c(j)
            for j in jq:
                stage_b(j)

        for t in range(2):
            _inv_piece(cprev, 2 * r + t, 1 - buf, g_ref, us, vec, yf, outb)
        for p in fwd:
            p()
        for j in range(NP):
            stage_a(j)
            if j >= 2 and j % 2 == 0:
                attn_group((j - 2, j - 1), (j - 4, j - 3) if j >= 4 else ())
        stage_d(0, 8)
        attn_group((14, 15), (12, 13))
        stage_d(8, 20)
        attn_group((), (14, 15))
        stage_d(20, 28)
        stage_d(28, 32, last=True)

    def two_steps(i, carry):
        ct = i >> 2
        cprev = (ct + NT - 1) & (NT - 1)
        conv = [_conv_pieces(ct, (i & 3, odd), ct & 1, fs_ref, us, taps, vm, yf,
                             done_vm) for odd in range(2)]
        kgen = [_kgen_pieces((ct + 1) & (NT - 1), (i & 3, odd), par, vb, taps, ct + 1,
                             done_vb, KNI, KSPLIT) for odd in range(2)]
        work = {'k0': (kgen[0], vb), 'k1': (kgen[1], vb), 'm0': (conv[0][1], vm), 'm1': (conv[1][1], vm)}
        fence = Pacer([work[k] + (t0, t1) for (k, t0, t1) in PLAN if k[0] not in NOB])
        for odd in range(2):
            one_step(i, odd, conv[odd][0], fence)
        assert fence.finished() or NOB
        outa_cp(pl.multiple_of(2 * SEG * i, 2 * SEG), 2 * SEG).start()
        outb_cp(cprev, pl.multiple_of((i & 3) * 256, 256), 256, jnp.where(i < 4, 2, 1)).start()
        return carry

    with jax.named_scope("steps"):
        if NITER:
            lax.fori_loop(0, NITER, two_steps, 0)

    with jax.named_scope("flush"):
        outb_cp(NT - 1, 0, L // 2, 2).wait()
        for b in range(NBLK):
            _inv_piece(NT - 1, b, (NT - 1) % 2, g_ref, us, vec, yf, outb)
            if b % 4 == 3:
                outb_cp(NT - 1, (b - 3) * 64, 256, 1).start()
    with jax.named_scope("waitout"):
        outa_cp(0, S).wait()
        pltpu.make_async_copy(outb, outb, sem_out.at[1]).wait()


@jax.jit
def pallas_concat_heads__memory_aug_recurrent_mem_tr__ssm_conv_s4__prompt_kernel(
    A_x, A_mem0, A_Wq, A_Wk, A_Wv, A_Wo, A_seg_len,
    B_u, B_A_re, B_A_im, B_B_re, B_B_im, B_C_re, B_C_im, B_log_dt, B_Dskip,
):
    del A_seg_len
    assert A_x.shape == (1, S, DM) and B_u.shape == (1, L, D)
    fs, g = _dft_consts()
    w4 = lambda w: w.reshape(DM // 2, 2, H, E)
    any_ = pl.BlockSpec(memory_space=pl.ANY)
    V = pltpu.VMEM
    out = pl.pallas_call(
        _kernel,
        out_shape=jax.ShapeDtypeStruct((S, DM + D), bf16),
        in_specs=[any_] * 18,
        out_specs=any_,
        scratch_shapes=[
            V((2, NP, DM // 2, E), u32),
            V((2, NP, DM // 2, E), u32),
            V((2, NP, DM // 2, E), u32),
            V((8, H * E // 2, 128), u32),
            V((8, NSEG // 2, PRE, 128), u32),
            V((NSEG // 2, 2, TOK, DM), bf16),
            V((M + TOK, DM), bf16),
            V((S, DM), bf16),
            V((96, 2 * (SEG + M)), f32),
            V((6, D, N), bf16),
            V((32 + NT * 6 * N, 128), f32),
            V((NT, L // 2, 128), u32),
            V((NT + 1, TAPROWS, 128), f32),
            V((V_ROWS, 128), f32),
            V((VM_ROWS, 128), f32),
            V((32, 128), f32),
            V((2, T0, 128), f32),
            V((2, NBLK, 2, BLK, 128), bf16),
            V((NT, L // 2, 128), u32),
            V((4, 8, 128), f32),
            V((8, 8, 128), bf16),
            V((8, NBLK * 32, 128), bf16),
            V((2, BLK // 2, 128), bf16),
            pltpu.SMEM((2,), jnp.int32),
            pltpu.SemaphoreType.DMA((8,)),
            pltpu.SemaphoreType.DMA((6 * NP,)),
            pltpu.SemaphoreType.DMA((8,)),
            pltpu.SemaphoreType.DMA((16,)),
            pltpu.SemaphoreType.DMA((1,)),
            pltpu.SemaphoreType.DMA((8,)),
            pltpu.SemaphoreType.DMA((NT,)),
            pltpu.SemaphoreType.DMA((3,)),
            V((NSEG, 3 * NP, 2 * PRE, E), bf16),
            V((3 * NP, 2 * SEG, E), bf16),
            V((H, SEG, E), bf16),
            V((H, SEG + 2 * PRE, E), bf16),
        ],
        compiler_params=pltpu.CompilerParams(vmem_limit_bytes=110 * 1024 * 1024, disable_bounds_checks=True),
    )(jnp.asarray(np.zeros((2,), np.int32)), A_x.reshape(NSEG // 2, 2, SEG, DM), A_mem0.reshape(M, DM), w4(A_Wq), w4(A_Wk), w4(A_Wv), A_Wo.reshape(H * E, DM),
      B_u.reshape(L, D), B_A_re, B_A_im, B_B_re, B_B_im, B_C_re, B_C_im,
      B_log_dt.reshape(8, 128), B_Dskip.reshape(8, 128),
      jnp.asarray(fs, bf16), jnp.asarray(g, bf16))
    return out.reshape(1, S, DM + D)
```

```python
import functools

import numpy as np
import jax
import jax.numpy as jnp
from jax import lax
import jax.experimental.pallas as pl
import jax.experimental.pallas.tpu as pltpu

bf16, f32, u32 = jnp.bfloat16, jnp.float32, jnp.uint32

S, DM, H, E, M, SEG = 2048, 1024, 32, 128, 8, 32
NSEG = S // SEG
TOK = 24
PRE = SEG - TOK
T0 = PRE * NSEG
NP = H // 2
NATT = 2 * (SEG + M)
LOG2E = 1.4426950408889634
L, D, N = 2048, 1024, 128
BLK = 128
NBLK = L // BLK
NT = D // 128
TAPROWS = 672
WINDOWS = ((0, 128, 0, 1), (128, 128, 1, 1), (256, 128, 2, 1), (320, 80, 3, 1),
           (384, 128, 4, 3), (480, 48, 7, 1), (512, 128, 8, 7), (624, 32, 15, 1))
V_YTAB = 8
V_START = V_YTAB + 256
V_STEP = V_START + 160
V_ROWS = V_STEP + 128 + 24
V_UF = 8
V_KF = V_UF + NBLK * 32
V_Z = V_KF + NBLK * 32
VM_ROWS = V_Z + 32 + 24
RC = 64
UNP = 64
WAITS = {1: 2, 2: 3, 3: 5, 4: 6, 5: 8, 7: 11, 10: 13, 12: 17, 16: 23, 22: 33, 32: 48}
PAR_WAIT = 10
STARTS = {0: (2, False, 0), 1: (3, False, 0), 2: (5, False, 0), 4: (6, False, 0), 6: (8, False, 0),
          8: (9, False, 0), 10: (11, False, 0), 14: (13, True, 0), 20: (17, False, 0), 24: (23, False, 0),
          32: (33, False, 0), 44: (48, False, 3), 64: (48, False, 19)}
BPLAN = (10.0, 11.0, 42.5, 47.7)
PLAN = (('k0', 0, 96), ('m0', 96, 122), ('k1', 124, 220), ('m1', 220, 260))
MACJ = 3


def _bf16_round_int(l):
    u = np.asarray(l, np.float32).view(np.uint32)
    r = (u + 0x7FFF + ((u >> 16) & 1)) & 0xFFFF0000
    return r.astype(np.uint32).view(np.float32).astype(np.int64)


def _tap_row(lp):
    return np.where(lp < 256, lp, np.where(lp < 512, 256 + (lp - 256) // 2,
                    np.where(lp < 1024, 384 + (lp - 512) // 4, 512 + (lp - 1024) // 8)))


@functools.lru_cache(maxsize=None)
def _dft_consts():
    t = np.arange(BLK)
    F = np.zeros((8, 32, BLK))
    G = np.zeros((2, BLK // 2, 8, 16))
    for r in range(8):
        f = 16 * r + 2 * np.arange(8)
        th = 2 * np.pi * (np.concatenate([f, BLK - 1 - f]) + 0.5) / (2 * BLK)
        F[r, :16] = np.cos(th[:, None] * t[None])
        F[r, 16:] = -np.sin(th[:, None] * t[None])
        for par in range(2):
            G[par, :, r, :8] = np.cos(th[None, :8] * t[par::2, None]) / BLK
            G[par, :, r, 8:] = -np.sin(th[None, :8] * t[par::2, None]) / BLK
    FS = np.zeros((8, NBLK, 32, 128))
    for (w0, wn, b0, nb) in WINDOWS:
        for j in range(b0, b0 + nb):
            rows = _tap_row(_bf16_round_int(BLK * j + t)) - w0
            assert rows.min() >= 0 and rows.max() < wn
            sel = np.zeros((BLK, 128))
            sel[t, rows] = 1.0
            FS[:, j] = F @ sel
    return (FS.reshape(8, NBLK * 32, 128).astype(np.float32),
            G.reshape(2, BLK // 2, 128).astype(np.float32))


def _ld16(ref, *idx):
    return pltpu.bitcast(ref.bitcast(u32)[idx + (slice(None),)], bf16)


def _cmul(a, b):
    return (a[0] * b[0] - a[1] * b[1], a[0] * b[1] + a[1] * b[0])


def _csq(a):
    return (a[0] * a[0] - a[1] * a[1], 2.0 * (a[0] * a[1]))


def _cexp(lr, li):
    k = jnp.floor(li * (2.0 / np.pi) + 0.5)
    r = ((li - k * 1.5703125) - k * 4.837512969970703125e-4) - k * 7.54978995489188216e-8
    r = jnp.clip(r, -0.8, 0.8)
    r2 = r * r
    s = r + r * r2 * (-1.6666654611e-1 + r2 * (8.3321608736e-3 + r2 * -1.9515295891e-4))
    c = (1.0 - 0.5 * r2) + (r2 * r2) * (4.166664568298827e-2
                                        + r2 * (-1.388731625493765e-3 + r2 * 2.443315711809948e-5))
    q = k.astype(jnp.int32)
    swap = (q & 1) == 1
    m = jnp.exp(lr)
    flip = lambda v, bit: pltpu.bitcast(pltpu.bitcast(v, jnp.int32) ^ (bit << 30), f32)
    return (flip(m * jnp.where(swap, s, c), (q + 1) & 2), flip(m * jnp.where(swap, c, s), q & 2))


def _par_row(c, k):
    return 8 + (c * 6 + k) * N


def _prep_pieces(praw, vec, par):
    def stage1(c):
        def fn():
            tr = lambda k: praw[k, pl.ds(c * 128, 128), :].astype(f32).T
            dt = jnp.exp(vec[0, pl.ds(c, 1), :]).astype(bf16).astype(f32)
            cc = _cmul((tr(4), tr(5)), (dt * tr(2), dt * tr(3)))
            for k, v in ((0, dt * tr(0)), (1, dt * tr(1)), (4, cc[0]), (5, cc[1])):
                par[pl.ds(_par_row(c, k), N), :] = v
        return fn

    def stage2(c, n0):
        def fn():
            lr = par[pl.ds(_par_row(c, 0) + n0, 16), :]
            li = par[pl.ds(_par_row(c, 1) + n0, 16), :]
            for k, v in enumerate(_cexp(lr, li) + _cexp(lr * 128.0, li * 128.0)):
                par[pl.ds(_par_row(c, k) + n0, 16), :] = v
        return fn

    tile = lambda c: [(260, stage1(c))] + [(190, stage2(c, n0)) for n0 in range(0, N, 16)]
    return tile(0), [pc for c in range(1, NT) for pc in tile(c)]


def _kgen_pieces(c, r, par, vb, taps, tslot, frow, kni, ksplit):
    st = {}

    def put(row, z, h=None):
        if h is None:
            vb[pl.ds(row, 16), :] = z[0]
            vb[pl.ds(row + 16, 16), :] = z[1]
        else:
            vb[pl.ds(row + 8 * h, 8), :] = z[0]
            vb[pl.ds(row + 16 + 8 * h, 8), :] = z[1]

    def get(row, h=None):
        if h is None:
            return (vb[pl.ds(row, 16), :], vb[pl.ds(row + 16, 16), :])
        return (vb[pl.ds(row + 8 * h, 8), :], vb[pl.ds(row + 16 + 8 * h, 8), :])

    def ytab(k0, k1):
        return [vb[pl.ds(V_YTAB + 128 * part + 16 * k0, 16 * (k1 - k0)), :].reshape(k1 - k0, 16, 128)
                for part in range(2)]

    def params(k):
        if isinstance(r, int):
            return par[pl.ds(_par_row(c, k) + r * 16, 16), :]
        return par[pl.ds(pl.multiple_of(c * (6 * N) + r[0] * 32, 32) + (_par_row(0, k) + r[1] * 16), 16), :]

    def park():
        put(V_STEP, (params(0), params(1)))
        put(V_START + 32, (params(2), params(3)))
        put(V_START, (params(4), params(5)))

    def setup_y(h):
        def fn():
            z1 = get(V_STEP, h)
            z2 = _csq(z1)
            z4 = _csq(z2)
            s = lax.broadcasted_iota(jnp.int32, (8, 128), 0)
            fs = [(jnp.where((s >> k) & 1 == 1, z[0], 1.0), jnp.where((s >> k) & 1 == 1, z[1], 0.0))
                  for k, z in enumerate((z1, z2, z4))]
            y = _cmul(_cmul(fs[0], fs[1]), fs[2])
            for k in range(8):
                vb[pl.ds(V_YTAB + 16 * k + 8 * h, 8), :] = y[0]
                vb[pl.ds(V_YTAB + 128 + 16 * k + 8 * h, 8), :] = y[1]
                if k < 7:
                    y = _cmul(y, z1)
                    y = (jnp.where(s == 7 - k, 1.0, y[0]), jnp.where(s == 7 - k, 0.0, y[1]))
            z = z4
            for k in range(4):
                z = _csq(z)
                put(V_STEP + 32 * k, z, h)
        return fn

    def setup_hi():
        z = get(V_START + 32)
        cf = get(V_START)
        for g in range(1, 5):
            put(V_START + 32 * g, _cmul(cf, z))
            if g < 4:
                z = _csq(z)

    def square(k0, k1):
        def fn():
            rows = [pl.ds(V_YTAB + 128 * part + 16 * k0, 16 * (k1 - k0)) for part in range(2)]
            y = _csq((vb[rows[0], :], vb[rows[1], :]))
            vb[rows[0], :] = y[0]
            vb[rows[1], :] = y[1]
        return fn

    def rows_of(g, i0, ni):
        n_i = 16 + (g == 4)

        def fn():
            x = st.pop('x') if i0 > 0 else get(V_START + 32 * g)
            step = get(V_STEP + 32 * max(g - 1, 0))
            xs = []
            for t in range(ni):
                xs.append(x)
                if i0 + t + 1 < n_i:
                    x = _cmul(x, step)
            if i0 + ni < n_i:
                st['x'] = x
            acc = [None] * ni
            for k0 in range(0, 8, ksplit):
                yr, yi = ytab(k0, k0 + ksplit)
                for t in range(ni):
                    v = xs[t][0] * yr - xs[t][1] * yi
                    v = lax.slice_in_dim(v, 0, 8, axis=1) + lax.slice_in_dim(v, 8, 16, axis=1)
                    v = jnp.sum(pltpu.roll(v, k0, 1, stride=1, stride_axis=0), axis=0)
                    acc[t] = v if acc[t] is None else acc[t] + v
                if k0 + ksplit < 8:
                    vb[pl.ds(frow, 8), :] = acc[ni - 1]
            for t in range(ni):
                row = 128 * g + 8 * (i0 + t)
                a = acc[t]
                if row == 640:
                    a = jnp.where(lax.broadcasted_iota(jnp.int32, (8, 128), 0) == 0, a, 0.0)
                taps[tslot, pl.ds(row, 8), :] = taps[tslot, pl.ds(row, 8), :] + a
                if t == ni - 1:
                    vb[pl.ds(frow, 8), :] = a
        return fn

    pieces = [(30, park), (110, setup_y(0)), (110, setup_y(1)), (80, setup_hi)]
    for g in range(5):
        if g >= 2:
            pieces += [(40, square(0, 4)), (40, square(4, 8))]
        for i0 in range(0, 16 + (g == 4), kni):
            ni = min(kni, 16 + (g == 4) - i0)
            pieces.append((83 * ni, rows_of(g, i0, ni)))
    return pieces


def _conv_pieces(c, r, buf, fs_ref, us, taps, vb, yf, frow):
    st = {}

    def fwd_u(b0, b1):
        def fn():
            lhs = _ld16(fs_ref, 2 * r[0] + r[1], pl.ds(0, 16))
            for b in range(b0, b1):
                w = pltpu.bitcast(us[c, pl.ds(b * 64, 64), :], bf16)
                res = jnp.dot(lhs, w, preferred_element_type=f32)
                row = V_UF + 32 * b
                if b == 0:
                    vb[pl.ds(row, 32), :] = res
                else:
                    p = st['prev']
                    vb[pl.ds(row, 8), :] = res[0:8] - p[16:24]
                    vb[pl.ds(row + 8, 8), :] = res[8:16] + p[24:32]
                    vb[pl.ds(row + 16, 8), :] = res[16:24] + p[0:8]
                    vb[pl.ds(row + 24, 8), :] = res[24:32] - p[8:16]
                st['prev'] = res
        return fn

    def fwd_k(jobs):
        def fn():
            for (wi, t0, nb) in jobs:
                w0, wn, b0, _ = WINDOWS[wi]
                lhs = _ld16(fs_ref, 2 * r[0] + r[1], pl.ds((b0 + t0) * 16, nb * 16))[:, :wn]
                w = taps[c, pl.ds(w0, wn), :].astype(bf16)
                vb[pl.ds(V_KF + 32 * (b0 + t0), 32 * nb), :] = jnp.dot(lhs, w, preferred_element_type=f32)
        return fn

    def mac(q, i0, ni, j0, j1):
        def fn():
            ld = lambda base, b: (vb[pl.ds(base + 32 * b + 8 * q, 8), :], vb[pl.ds(base + 32 * b + 16 + 8 * q, 8), :])
            zr, zi = st.pop('z') if j0 > 0 else ({}, {})
            ucache = {}
            for j in range(j0, j1):
                kr, ki = ld(V_KF, j)
                for i in range(max(i0, j), i0 + ni):
                    if i - j not in ucache:
                        ucache[i - j] = ld(V_UF, i - j)
                    ur, ui = ucache[i - j]
                    if i not in zr:
                        zr[i] = kr * ur - ki * ui
                        zi[i] = kr * ui + ki * ur
                    else:
                        zr[i] = zr[i] + kr * ur - ki * ui
                        zi[i] = zi[i] + kr * ui + ki * ur
            vb[pl.ds(frow, 8), :] = zr[i0 + ni - 1]
            if j1 < i0 + ni:
                st['z'] = (zr, zi)
            elif q == 0:
                for i in range(i0, i0 + ni):
                    vb[pl.ds(V_Z + 16 * (i - i0), 16), :] = jnp.concatenate([zr[i], zi[i]], axis=0)
            else:
                row = pl.multiple_of(r[0] * 32, 32) + r[1] * 16
                for i in range(i0, i0 + ni):
                    ar = vb[pl.ds(V_Z + 16 * (i - i0), 8), :]
                    ai = vb[pl.ds(V_Z + 16 * (i - i0) + 8, 8), :]
                    yf[buf, i, 0, pl.ds(row, 16), :] = jnp.concatenate([ar + zr[i], ai - zi[i]], axis=0).astype(bf16)
                    yf[buf, i, 1, pl.ds(row, 16), :] = jnp.concatenate([ar - zr[i], ai + zi[i]], axis=0).astype(bf16)
        return (8 * sum(1 for j in range(j0, j1) for i in range(max(i0, j), i0 + ni)), fn)

    fwd = [fwd_u(0, 8), fwd_u(8, 16), fwd_k(((0, 0, 1), (1, 0, 1), (2, 0, 1), (3, 0, 1))),
           fwd_k(((4, 0, 2), (6, 0, 2), (6, 2, 2), (6, 4, 2))), fwd_k(((4, 2, 1), (5, 0, 1), (6, 6, 1), (7, 0, 1)))]
    macs = []
    for i0 in range(0, NBLK, 2):
        for q in range(2):
            for j0 in range(0, i0 + 2, MACJ):
                macs.append(mac(q, i0, 2, j0, min(j0 + MACJ, i0 + 2)))
    return fwd, macs


def _inv_piece(c, b, buf, g_ref, us, vec, yf, outb):
    rows = pl.ds(b * 64 if isinstance(b, int) else pl.multiple_of(b * 64, 64), 64)
    rnd = lambda v: v.astype(bf16).astype(f32)
    uw = us[c, rows, :]
    dsk = vec[1, pl.ds(c, 1), :]
    o = []
    for par, u in enumerate((uw << 16, uw & u32(0xFFFF0000))):
        y = jnp.dot(_ld16(g_ref, par, slice(None)), _ld16(yf, buf, b, par, slice(None)), preferred_element_type=f32)
        o.append(pltpu.bitcast(rnd(rnd(y) + rnd(pltpu.bitcast(u, f32) * dsk)), u32))
    outb[c, rows, :] = (o[0] >> 16) | o[1]


def _attn_fill():
    r = lax.broadcasted_iota(jnp.int32, (NATT, NATT), 0)
    c = lax.broadcasted_iota(jnp.int32, (NATT, NATT), 1)
    head = lambda i: jnp.where(i < 2 * SEG, i // SEG, (i - 2 * SEG) // PRE)
    pos = lambda i: jnp.where(i < 2 * SEG, i % SEG, i % PRE)
    is_mem = lambda i: (i < 2 * SEG) & (i % SEG < M)
    same = head(r) == head(c)
    allowed = same & (is_mem(r) | is_mem(c) | (pos(r) >= pos(c)))
    return jnp.where(allowed, 0.0, jnp.where(same, -1e9 * LOG2E, -jnp.inf)).astype(f32)


def _kernel(zero_hbm, x_hbm, mem0_hbm, wq_hbm, wk_hbm, wv_hbm, wo_hbm,
            u_hbm, p0, p1, p2, p3, p4, p5, ldt_hbm, dsk_hbm, fs_hbm, g_hbm,
            out_hbm,
            wq, wk, wv, wo, xb, xs, h_ref, outs, fill_ref,
            praw, par, us, taps, vb, vm, vu, pacc, yf, outb, vec, vraw, fs_ref, g_ref, zero_ref,
            sem_s, sem_w, sem_o, sem_xb, sem_x, sem_p, sem_u, sem_out, pre, own, lo0, lo1):
    wqkv = (wq, wk, wv)
    scale = E ** -0.5

    whbm = [w.bitcast(u32) for w in (wq_hbm, wk_hbm, wv_hbm)]

    def wcp(j, m, p):
        return pltpu.make_async_copy(whbm[m].at[:, p, j, :], wqkv[m].at[p, j], sem_w.at[(j * 3 + m) * 2 + p])

    xu = x_hbm.bitcast(u32)
    xcs = [pltpu.make_async_copy(xu.at[:, t, pl.ds(0, PRE // 2), pl.ds(c * 128, 128)],
                                 xb.at[c, :, pl.ds(t * (PRE // 2), PRE // 2), :], sem_xb.at[2 * c + t])
           for c in range(8) for t in range(2)]
    xcp1 = pltpu.make_async_copy(x_hbm.at[:, :, pl.ds(PRE, TOK), :], xs, sem_x.at[0])
    pcs = [pltpu.make_async_copy(p, praw.at[k], sem_p.at[k]) for k, p in enumerate((p0, p1, p2, p3, p4, p5))]
    ccs = [pltpu.make_async_copy(fs_hbm, fs_ref, sem_p.at[6]), pltpu.make_async_copy(g_hbm, g_ref, sem_p.at[7])]
    wou = wo_hbm.bitcast(u32)
    ocs = [pltpu.make_async_copy(wou.at[:, pl.ds(c * 128, 128)], wo.at[c], sem_o.at[c]) for c in range(8)]
    uu = u_hbm.bitcast(u32)
    ucs = [pltpu.make_async_copy(uu.at[:, pl.ds(c * 128, 128)], us.at[c], sem_u.at[c]) for c in range(NT)]

    zcp = pltpu.make_async_copy(zero_hbm, zero_ref, sem_s.at[0])
    scs = [pltpu.make_async_copy(mem0_hbm, h_ref.at[pl.ds(0, M)], sem_s.at[1]),
           pltpu.make_async_copy(ldt_hbm, vraw.at[0], sem_s.at[2]),
           pltpu.make_async_copy(dsk_hbm, vraw.at[1], sem_s.at[3])]
    w0cs = [[pltpu.make_async_copy(whbm[0].at[pl.ds(half * (DM // 4), DM // 4), p, 0, :],
                                   wq.at[p, 0, pl.ds(half * (DM // 4), DM // 4)], sem_s.at[4 + 2 * half + p])
             for p in range(2)] for half in range(2)]
    for cp in [zcp] + w0cs[0] + xcs[:8]:
        cp.start()
    vu[pl.ds(8, 8), :] = pltpu.bitcast(jnp.full((8, 128), 0x0000FFFF, u32), f32)
    vu[pl.ds(16, 8), :] = pltpu.bitcast(jnp.full((8, 128), 0xFFFF0000, u32), f32)
    taps[...] = jnp.zeros(taps.shape, f32)
    yf[1] = jnp.zeros(yf.shape[1:], bf16)
    fill_ref[pl.ds(0, NATT), :] = _attn_fill()
    for cp in w0cs[1] + xcs[8:] + scs:
        cp.start()
    zcp.wait()

    def opaque_row(k, buf):
        return pl.multiple_of(jnp.clip(zero_ref[k] * 8, 0, buf.shape[0] - 8), 8)

    bufs = (vb, vm, vu, par)
    fence_rows = [opaque_row(0, b) for b in bufs]
    done_vb, done_vm = opaque_row(1, vb), opaque_row(1, vm)

    class Pacer:
        def __init__(self, segments):
            self.t = 0.0
            self.todo = []
            for (pieces, buf, t0, t1) in segments:
                total = float(sum(c for c, _ in pieces)) or 1.0
                done = 0.0
                for (cst, fn) in pieces:
                    self.todo.append((t0 + (t1 - t0) * done / total, fn, buf))
                    done += cst

        def __call__(self, v, dt=1.0):
            self.t += dt
            fenced = []
            while self.todo and self.todo[0][0] < self.t:
                _, fn, buf = self.todo.pop(0)
                if not any(b is buf for b in fenced):
                    buf[pl.ds([r for b, r in zip(bufs, fence_rows) if b is buf][0], 8), :] = v
                    fenced.append(buf)
                fn()

        def finished(self):
            return not self.todo

    def unpair(j, m, r0, nr):
        def fn():
            rows = pl.ds(r0, nr)
            m_lo = pltpu.bitcast(vu[pl.ds(8, 8), :], u32)[None]
            m_hi = pltpu.bitcast(vu[pl.ds(16, 8), :], u32)[None]
            a = wqkv[m][0, j, rows, :].reshape(nr // 8, 8, E)
            b = wqkv[m][1, j, rows, :].reshape(nr // 8, 8, E)
            wqkv[m][0, j, rows, :] = ((a & m_lo) | ((b & m_lo) << 16)).reshape(nr, E)
            wqkv[m][1, j, rows, :] = (((a & m_hi) >> 16) | (b & m_hi)).reshape(nr, E)
        return (nr, fn)

    def unpair_pieces(items, lo=0, hi=DM // 2):
        return [unpair(j, m, r0, UNP) for (j, m) in items for r0 in range(lo, hi, UNP)]

    items = [(j, m) for j in range(NP) for m in range(3)]
    wcs = lambda lo, hi: [wcp(j, m, p) for (j, m) in items[lo:hi] for p in range(2)]
    rest = ocs + ccs + ucs + [xcp1]
    starts = [[] for _ in range(2 * len(items))]
    n_w, n_r = 1, 0
    for unit in sorted(STARTS):
        w_hi, with_par, r_hi = STARTS[unit]
        starts[unit] = (pcs if with_par else []) + wcs(n_w, w_hi) + rest[n_r:r_hi]
        n_w, n_r = w_hi, r_hi
    assert n_w == len(items) and n_r == len(rest)
    n_chunk = 2 * (T0 // RC)
    prep = _prep_pieces(praw, vec, par)
    kg0 = [pc for r in range(8) for pc in _kgen_pieces(0, r, par, vb, taps, 0, done_vb, 1, 4)]
    t_a, t_b, t_c, t_d = [v * n_chunk for v in BPLAN]
    fence_x = Pacer([(prep[0], par, t_a, t_b), (kg0, vb, t_b, t_c), (prep[1], par, t_c, t_d)])
    landed = 1
    for it, (j, m) in enumerate(items):
        fence_w = None
        for half in range(2):
            for cp in starts[2 * it + half]:
                cp.start()
            if it == 0:
                for cp in w0cs[half] + xcs[8 * half:8 * half + 8]:
                    cp.wait()
                for _, fn in unpair_pieces(items[:1], half * (DM // 4), (half + 1) * (DM // 4)):
                    fn()
                fence_w = Pacer([])
            elif half == 0:
                late = landed == it
                if it in WAITS:
                    for cp in wcs(landed, WAITS[it]) + (pcs + scs if it == PAR_WAIT else []):
                        cp.wait()
                    landed = WAITS[it]
                    if it == PAR_WAIT:
                        vec[pl.ds(0, 2)] = vraw[pl.ds(0, 2)].astype(f32)
                if late:
                    for _, fn in unpair_pieces(items[it:it + 1]):
                        fn()
                fence_w = Pacer([(unpair_pieces(items[it + 1:min(it + 2, landed)]), vu, 0.0, n_chunk * 0.7)])
            for p in range(2):
                w = pltpu.bitcast(wqkv[m][p, j, pl.ds(half * (DM // 4), DM // 4), :], bf16)
                lhs = jnp.concatenate([pltpu.bitcast(xb[c].reshape(T0 // 2, 128), bf16)
                                       for c in range(4 * half, 4 * half + 4)], axis=1)
                res = jnp.dot(lhs, w, preferred_element_type=f32)
                for rc in range(T0 // RC):
                    rows = pl.ds(rc * RC, RC)
                    v = res[rc * RC:(rc + 1) * RC]
                    if half == 1:
                        v = v + pacc[p, rows, :]
                    if p == 0 or half == 0:
                        pacc[p, rows, :] = v
                    else:
                        pr = jnp.concatenate([pacc[0, rows, :].reshape(RC // PRE, PRE, E),
                                              v.reshape(RC // PRE, PRE, E)], axis=1)
                        pre[pl.ds(rc * (RC // PRE), RC // PRE), m * NP + j] = pr.astype(bf16)
                    fence_w(v[:8], 0.5)
                    fence_x(v[:8], 0.5)
        assert fence_w.finished() and landed > it
    assert fence_x.finished()
    for cp in ocs + ucs + ccs + [xcp1]:
        cp.wait()

    def outa_cp(row, n):
        return pltpu.make_async_copy(outs.at[pl.ds(row, n)], out_hbm.at[pl.ds(row, n), pl.ds(0, DM)], sem_out.at[0])

    def outb_cp(c, row, n, sem):
        col = DM + c * 128
        return pltpu.make_async_copy(
            outb.at[c, pl.ds(row, n)],
            out_hbm.bitcast(u32).at[pl.ds(row, n), pl.ds(col if isinstance(col, int) else pl.multiple_of(col, 128), 128)],
            sem_out.at[sem])

    def one_step(i, odd, fwd, fence):
        s = 2 * i + odd
        lo_cur = (lo0, lo1)[odd]
        base = pl.multiple_of(2 * SEG * i, 2 * SEG)
        h_ref[pl.ds(M, TOK), :] = xs[i, odd]
        h = h_ref[...]
        scores = {}
        probs = {}

        ct = i >> 2
        r = s & 7
        buf = ct & 1
        cprev = (ct + NT - 1) & (NT - 1)

        def stage_a(j):
            for m in range(3):
                for p in range(2):
                    w = pltpu.bitcast(wqkv[m][p, j], bf16)
                    res = jnp.dot(h, w, preferred_element_type=f32)
                    own[m * NP + j, pl.ds(SEG * p, SEG), :] = res.astype(bf16)
                    fence(res[:M])

        def gather(m, j):
            return pltpu.bitcast(jnp.concatenate([own.bitcast(u32)[m * NP + j],
                                                  pre.bitcast(u32)[s, m * NP + j]], axis=0), bf16)

        def stage_qk(j):
            scores[j] = lax.dot_general(gather(0, j), gather(1, j), (((1,), (1,)), ((), ())),
                                        preferred_element_type=f32)

        def stage_b(j):
            fl = fill_ref[pl.ds(0, NATT), :]
            sc = jnp.where(fl == 0.0, scores.pop(j) * (scale * LOG2E), fl)
            e = jnp.exp2(sc - jnp.max(sc, axis=-1, keepdims=True))
            den = jnp.sum(e, axis=-1, keepdims=True)
            probs[j] = (e * pl.reciprocal(den, approx=True)).astype(bf16)

        def stage_c(j):
            o = jnp.dot(probs[j], gather(2, j), preferred_element_type=f32)
            for p in range(2):
                hh = 2 * j + p
                lo_cur[hh, pl.ds(0, SEG), :] = o[p * SEG:(p + 1) * SEG].astype(bf16)
                ob = o[2 * SEG + p * PRE:2 * SEG + (p + 1) * PRE]
                lo1[hh, pl.ds(SEG + odd * PRE, PRE), :] = ob.astype(bf16)

        acc = [None] * 8

        def stage_d(h0, h1, last=False):
            lhs = jnp.concatenate([_ld16(lo_cur, hh, slice(None)) for hh in range(h0, h1)], axis=1)
            for c in range(8):
                w = pltpu.bitcast(wo[c, pl.ds(h0 * 64, (h1 - h0) * 64), :], bf16)
                res = jnp.dot(lhs, w, preferred_element_type=f32)
                acc[c] = res if acc[c] is None else acc[c] + res
                if not last:
                    fence(res[:M], (h1 - h0) / 8.0 * (1.5 if odd else 1.0))
                else:
                    rb = acc[c].astype(bf16)
                    cols = pl.ds(c * 128, 128)
                    h_ref[pl.ds(0, M), cols] = rb[:M]
                    outs[pl.ds(base + (odd * SEG + PRE), TOK), cols] = rb[M:SEG]
                    if odd:
                        outs[pl.ds(base, PRE), cols] = rb[SEG:SEG + PRE]
                        outs[pl.ds(base + SEG, PRE), cols] = rb[SEG + PRE:]

        def attn_group(jq, jc):
            for j in jq:
                stage_qk(j)
            for j in jc:
                stage_c(j)
            for j in jq:
                stage_b(j)

        for t in range(2):
            _inv_piece(cprev, 2 * r + t, 1 - buf, g_ref, us, vec, yf, outb)
        for p in fwd:
            p()
        for j in range(NP):
            stage_a(j)
            if j >= 2 and j % 2 == 0:
                attn_group((j - 2, j - 1), (j - 4, j - 3) if j >= 4 else ())
        stage_d(0, 8)
        attn_group((14, 15), (12, 13))
        stage_d(8, 20)
        attn_group((), (14, 15))
        stage_d(20, 28)
        stage_d(28, 32, last=True)

    def two_steps(i, carry):
        ct = i >> 2
        cprev = (ct + NT - 1) & (NT - 1)
        conv = [_conv_pieces(ct, (i & 3, odd), ct & 1, fs_ref, us, taps, vm, yf, done_vm) for odd in range(2)]
        kgen = [_kgen_pieces((ct + 1) & (NT - 1), (i & 3, odd), par, vb, taps, ct + 1, done_vb, 2, 2)
                for odd in range(2)]
        work = {'k0': (kgen[0], vb), 'k1': (kgen[1], vb), 'm0': (conv[0][1], vm), 'm1': (conv[1][1], vm)}
        fence = Pacer([work[k] + (t0, t1) for (k, t0, t1) in PLAN])
        for odd in range(2):
            one_step(i, odd, conv[odd][0], fence)
        assert fence.finished()
        outa_cp(pl.multiple_of(2 * SEG * i, 2 * SEG), 2 * SEG).start()
        outb_cp(cprev, pl.multiple_of((i & 3) * 256, 256), 256, jnp.where(i < 4, 2, 1)).start()
        return carry

    lax.fori_loop(0, NSEG // 2, two_steps, 0)

    outb_cp(NT - 1, 0, L // 2, 2).wait()
    for b in range(NBLK):
        _inv_piece(NT - 1, b, (NT - 1) % 2, g_ref, us, vec, yf, outb)
        if b % 4 == 3:
            outb_cp(NT - 1, (b - 3) * 64, 256, 1).start()
    outa_cp(0, S).wait()
    pltpu.make_async_copy(outb, outb, sem_out.at[1]).wait()


@jax.jit
def pallas_concat_heads__memory_aug_recurrent_mem_tr__ssm_conv_s4__prompt_kernel(
    A_x, A_mem0, A_Wq, A_Wk, A_Wv, A_Wo, A_seg_len,
    B_u, B_A_re, B_A_im, B_B_re, B_B_im, B_C_re, B_C_im, B_log_dt, B_Dskip,
):
    del A_seg_len
    assert A_x.shape == (1, S, DM) and B_u.shape == (1, L, D)
    fs, g = _dft_consts()
    w4 = lambda w: w.reshape(DM // 2, 2, H, E)
    any_ = pl.BlockSpec(memory_space=pl.ANY)
    V = pltpu.VMEM
    out = pl.pallas_call(
        _kernel,
        out_shape=jax.ShapeDtypeStruct((S, DM + D), bf16),
        in_specs=[any_] * 18,
        out_specs=any_,
        scratch_shapes=[
            V((2, NP, DM // 2, E), u32),
            V((2, NP, DM // 2, E), u32),
            V((2, NP, DM // 2, E), u32),
            V((8, H * E // 2, 128), u32),
            V((8, NSEG // 2, PRE, 128), u32),
            V((NSEG // 2, 2, TOK, DM), bf16),
            V((M + TOK, DM), bf16),
            V((S, DM), bf16),
            V((96, NATT), f32),
            V((6, D, N), bf16),
            V((32 + NT * 6 * N, 128), f32),
            V((NT, L // 2, 128), u32),
            V((NT + 1, TAPROWS, 128), f32),
            V((V_ROWS, 128), f32),
            V((VM_ROWS, 128), f32),
            V((32, 128), f32),
            V((2, T0, 128), f32),
            V((2, NBLK, 2, BLK, 128), bf16),
            V((NT, L // 2, 128), u32),
            V((4, 8, 128), f32),
            V((8, 8, 128), bf16),
            V((8, NBLK * 32, 128), bf16),
            V((2, BLK // 2, 128), bf16),
            pltpu.SMEM((2,), jnp.int32),
            pltpu.SemaphoreType.DMA((8,)),
            pltpu.SemaphoreType.DMA((6 * NP,)),
            pltpu.SemaphoreType.DMA((8,)),
            pltpu.SemaphoreType.DMA((16,)),
            pltpu.SemaphoreType.DMA((1,)),
            pltpu.SemaphoreType.DMA((8,)),
            pltpu.SemaphoreType.DMA((NT,)),
            pltpu.SemaphoreType.DMA((3,)),
            V((NSEG, 3 * NP, 2 * PRE, E), bf16),
            V((3 * NP, 2 * SEG, E), bf16),
            V((H, SEG, E), bf16),
            V((H, SEG + 2 * PRE, E), bf16),
        ],
        compiler_params=pltpu.CompilerParams(vmem_limit_bytes=110 * 1024 * 1024, disable_bounds_checks=True),
    )(jnp.asarray(np.zeros((2,), np.int32)), A_x.reshape(NSEG // 2, 2, SEG, DM), A_mem0.reshape(M, DM),
      w4(A_Wq), w4(A_Wk), w4(A_Wv), A_Wo.reshape(H * E, DM),
      B_u.reshape(L, D), B_A_re, B_A_im, B_B_re, B_B_im, B_C_re, B_C_im,
      B_log_dt.reshape(8, 128), B_Dskip.reshape(8, 128),
      jnp.asarray(fs, bf16), jnp.asarray(g, bf16))
    return out.reshape(1, S, DM + D)
```

```python
import functools

import numpy as np
import jax
import jax.numpy as jnp
from jax import lax
import jax.experimental.pallas as pl
import jax.experimental.pallas.tpu as pltpu

bf16, f32, u32 = jnp.bfloat16, jnp.float32, jnp.uint32

S, DM, H, E, M, SEG = 2048, 1024, 32, 128, 8, 32
NSEG = S // SEG
TOK = 24
PRE = SEG - TOK
T0 = PRE * NSEG
NP = H // 2
NATT = 2 * (SEG + M)
LOG2E = 1.4426950408889634
L, D, N = 2048, 1024, 128
BLK = 128
NBLK = L // BLK
NT = D // 128
TAPROWS = 672
WINDOWS = ((0, 128, 0, 1), (128, 128, 1, 1), (256, 128, 2, 1), (320, 80, 3, 1),
           (384, 128, 4, 3), (480, 48, 7, 1), (512, 128, 8, 7), (624, 32, 15, 1))
V_YTAB = 8
V_START = V_YTAB + 256
V_STEP = V_START + 160
V_ROWS = V_STEP + 128 + 24
V_UF = 8
V_KF = V_UF + NBLK * 32
V_Z = V_KF + NBLK * 32
VM_ROWS = V_Z + 32 + 24
RC = 64
UNP = 64
WAITS = {1: 2, 2: 3, 3: 5, 4: 6, 5: 8, 7: 11, 10: 13, 12: 17, 16: 23, 22: 33, 32: 48}
PAR_WAIT = 10
STARTS = {0: (2, False, 0), 1: (3, False, 0), 2: (5, False, 0), 4: (6, False, 0), 6: (8, False, 0),
          8: (9, False, 0), 10: (11, False, 0), 14: (13, True, 0), 20: (17, False, 0), 24: (23, False, 0),
          32: (33, False, 0), 44: (48, False, 3), 64: (48, False, 19)}
BPLAN = (10.0, 11.0, 42.5, 47.7)
PLAN = (('k0', 0, 95), ('m0', 98, 123), ('k1', 124, 216), ('m1', 218, 250))
MACJ = 2


def _bf16_round_int(l):
    u = np.asarray(l, np.float32).view(np.uint32)
    r = (u + 0x7FFF + ((u >> 16) & 1)) & 0xFFFF0000
    return r.astype(np.uint32).view(np.float32).astype(np.int64)


def _tap_row(lp):
    return np.where(lp < 256, lp, np.where(lp < 512, 256 + (lp - 256) // 2,
                    np.where(lp < 1024, 384 + (lp - 512) // 4, 512 + (lp - 1024) // 8)))


@functools.lru_cache(maxsize=None)
def _dft_consts():
    t = np.arange(BLK)
    F = np.zeros((8, 32, BLK))
    G = np.zeros((2, BLK // 2, 8, 16))
    for r in range(8):
        f = 16 * r + 2 * np.arange(8)
        th = 2 * np.pi * (np.concatenate([f, BLK - 1 - f]) + 0.5) / (2 * BLK)
        F[r, :16] = np.cos(th[:, None] * t[None])
        F[r, 16:] = -np.sin(th[:, None] * t[None])
        for par in range(2):
            G[par, :, r, :8] = np.cos(th[None, :8] * t[par::2, None]) / BLK
            G[par, :, r, 8:] = -np.sin(th[None, :8] * t[par::2, None]) / BLK
    FS = np.zeros((8, NBLK, 32, 128))
    for (w0, wn, b0, nb) in WINDOWS:
        for j in range(b0, b0 + nb):
            rows = _tap_row(_bf16_round_int(BLK * j + t)) - w0
            assert rows.min() >= 0 and rows.max() < wn
            sel = np.zeros((BLK, 128))
            sel[t, rows] = 1.0
            FS[:, j] = F @ sel
    return (FS.reshape(8, NBLK * 32, 128).astype(np.float32),
            G.reshape(2, BLK // 2, 128).astype(np.float32))


def _ld16(ref, *idx):
    return pltpu.bitcast(ref.bitcast(u32)[idx + (slice(None),)], bf16)


def _cmul(a, b):
    return (a[0] * b[0] - a[1] * b[1], a[0] * b[1] + a[1] * b[0])


def _csq(a):
    return (a[0] * a[0] - a[1] * a[1], 2.0 * (a[0] * a[1]))


def _cexp(lr, li):
    k = jnp.floor(li * (2.0 / np.pi) + 0.5)
    r = ((li - k * 1.5703125) - k * 4.837512969970703125e-4) - k * 7.54978995489188216e-8
    r = jnp.clip(r, -0.8, 0.8)
    r2 = r * r
    s = r + r * r2 * (-1.6666654611e-1 + r2 * (8.3321608736e-3 + r2 * -1.9515295891e-4))
    c = (1.0 - 0.5 * r2) + (r2 * r2) * (4.166664568298827e-2
                                        + r2 * (-1.388731625493765e-3 + r2 * 2.443315711809948e-5))
    q = k.astype(jnp.int32)
    swap = (q & 1) == 1
    m = jnp.exp(lr)
    flip = lambda v, bit: pltpu.bitcast(pltpu.bitcast(v, jnp.int32) ^ (bit << 30), f32)
    return (flip(m * jnp.where(swap, s, c), (q + 1) & 2), flip(m * jnp.where(swap, c, s), q & 2))


def _par_row(c, k):
    return 8 + (c * 6 + k) * N


def _prep_pieces(praw, vec, par):
    def stage1(c):
        def fn():
            tr = lambda k: praw[k, pl.ds(c * 128, 128), :].astype(f32).T
            dt = jnp.exp(vec[0, pl.ds(c, 1), :]).astype(bf16).astype(f32)
            cc = _cmul((tr(4), tr(5)), (dt * tr(2), dt * tr(3)))
            for k, v in ((0, dt * tr(0)), (1, dt * tr(1)), (4, cc[0]), (5, cc[1])):
                par[pl.ds(_par_row(c, k), N), :] = v
        return fn

    def stage2(c, n0):
        def fn():
            lr = par[pl.ds(_par_row(c, 0) + n0, 16), :]
            li = par[pl.ds(_par_row(c, 1) + n0, 16), :]
            for k, v in enumerate(_cexp(lr, li) + _cexp(lr * 128.0, li * 128.0)):
                par[pl.ds(_par_row(c, k) + n0, 16), :] = v
        return fn

    tile = lambda c: [(260, stage1(c))] + [(190, stage2(c, n0)) for n0 in range(0, N, 16)]
    return tile(0), [pc for c in range(1, NT) for pc in tile(c)]


def _kgen_pieces(c, r, par, vb, taps, tslot, frow, kni, ksplit):
    st = {}

    def put(row, z, h=None):
        if h is None:
            vb[pl.ds(row, 16), :] = z[0]
            vb[pl.ds(row + 16, 16), :] = z[1]
        else:
            vb[pl.ds(row + 8 * h, 8), :] = z[0]
            vb[pl.ds(row + 16 + 8 * h, 8), :] = z[1]

    def get(row, h=None):
        if h is None:
            return (vb[pl.ds(row, 16), :], vb[pl.ds(row + 16, 16), :])
        return (vb[pl.ds(row + 8 * h, 8), :], vb[pl.ds(row + 16 + 8 * h, 8), :])

    def ytab(k0, k1):
        return [vb[pl.ds(V_YTAB + 128 * part + 16 * k0, 16 * (k1 - k0)), :].reshape(k1 - k0, 16, 128)
                for part in range(2)]

    def params(k):
        if isinstance(r, int):
            return par[pl.ds(_par_row(c, k) + r * 16, 16), :]
        return par[pl.ds(pl.multiple_of(c * (6 * N) + r[0] * 32, 32) + (_par_row(0, k) + r[1] * 16), 16), :]

    def park():
        put(V_STEP, (params(0), params(1)))
        put(V_START + 32, (params(2), params(3)))
        put(V_START, (params(4), params(5)))

    def setup_y(h):
        def fn():
            z1 = get(V_STEP, h)
            z2 = _csq(z1)
            z4 = _csq(z2)
            s = lax.broadcasted_iota(jnp.int32, (8, 128), 0)
            fs = [(jnp.where((s >> k) & 1 == 1, z[0], 1.0), jnp.where((s >> k) & 1 == 1, z[1], 0.0))
                  for k, z in enumerate((z1, z2, z4))]
            y = _cmul(_cmul(fs[0], fs[1]), fs[2])
            for k in range(8):
                vb[pl.ds(V_YTAB + 16 * k + 8 * h, 8), :] = y[0]
                vb[pl.ds(V_YTAB + 128 + 16 * k + 8 * h, 8), :] = y[1]
                if k < 7:
                    y = _cmul(y, z1)
                    y = (jnp.where(s == 7 - k, 1.0, y[0]), jnp.where(s == 7 - k, 0.0, y[1]))
            z = z4
            for k in range(4):
                z = _csq(z)
                put(V_STEP + 32 * k, z, h)
        return fn

    def setup_hi():
        z = get(V_START + 32)
        cf = get(V_START)
        for g in range(1, 5):
            put(V_START + 32 * g, _cmul(cf, z))
            if g < 4:
                z = _csq(z)

    def square(k0, k1):
        def fn():
            rows = [pl.ds(V_YTAB + 128 * part + 16 * k0, 16 * (k1 - k0)) for part in range(2)]
            y = _csq((vb[rows[0], :], vb[rows[1], :]))
            vb[rows[0], :] = y[0]
            vb[rows[1], :] = y[1]
        return fn

    def rows_of(g, i0, ni):
        n_i = 16 + (g == 4)

        def fn():
            x = st.pop('x') if i0 > 0 else get(V_START + 32 * g)
            step = get(V_STEP + 32 * max(g - 1, 0))
            xs = []
            for t in range(ni):
                xs.append(x)
                if i0 + t + 1 < n_i:
                    x = _cmul(x, step)
            if i0 + ni < n_i:
                st['x'] = x
            acc = [None] * ni
            for k0 in range(0, 8, ksplit):
                yr, yi = ytab(k0, k0 + ksplit)
                for t in range(ni):
                    v = xs[t][0] * yr - xs[t][1] * yi
                    v = lax.slice_in_dim(v, 0, 8, axis=1) + lax.slice_in_dim(v, 8, 16, axis=1)
                    v = jnp.sum(pltpu.roll(v, k0, 1, stride=1, stride_axis=0), axis=0)
                    acc[t] = v if acc[t] is None else acc[t] + v
                if k0 + ksplit < 8:
                    vb[pl.ds(frow, 8), :] = acc[ni - 1]
            for t in range(ni):
                row = 128 * g + 8 * (i0 + t)
                a = acc[t]
                if row == 640:
                    a = jnp.where(lax.broadcasted_iota(jnp.int32, (8, 128), 0) == 0, a, 0.0)
                taps[tslot, pl.ds(row, 8), :] = taps[tslot, pl.ds(row, 8), :] + a
                if t == ni - 1:
                    vb[pl.ds(frow, 8), :] = a
        return fn

    pieces = [(30, park), (110, setup_y(0)), (110, setup_y(1)), (80, setup_hi)]
    for g in range(5):
        if g >= 2:
            pieces += [(40, square(0, 4)), (40, square(4, 8))]
        for i0 in range(0, 16 + (g == 4), kni):
            ni = min(kni, 16 + (g == 4) - i0)
            pieces.append((83 * ni, rows_of(g, i0, ni)))
    return pieces


def _conv_pieces(c, r, buf, fs_ref, us, taps, vb, yf, frow):
    st = {}

    def fwd_u(b0, b1):
        def fn():
            lhs = _ld16(fs_ref, 2 * r[0] + r[1], pl.ds(0, 16))
            for b in range(b0, b1):
                w = pltpu.bitcast(us[c, pl.ds(b * 64, 64), :], bf16)
                res = jnp.dot(lhs, w, preferred_element_type=f32)
                row = V_UF + 32 * b
                if b == 0:
                    vb[pl.ds(row, 32), :] = res
                else:
                    p = st['prev']
                    vb[pl.ds(row, 8), :] = res[0:8] - p[16:24]
                    vb[pl.ds(row + 8, 8), :] = res[8:16] + p[24:32]
                    vb[pl.ds(row + 16, 8), :] = res[16:24] + p[0:8]
                    vb[pl.ds(row + 24, 8), :] = res[24:32] - p[8:16]
                st['prev'] = res
        return fn

    def fwd_k(jobs):
        def fn():
            for (wi, t0, nb) in jobs:
                w0, wn, b0, _ = WINDOWS[wi]
                lhs = _ld16(fs_ref, 2 * r[0] + r[1], pl.ds((b0 + t0) * 16, nb * 16))[:, :wn]
                w = taps[c, pl.ds(w0, wn), :].astype(bf16)
                vb[pl.ds(V_KF + 32 * (b0 + t0), 32 * nb), :] = jnp.dot(lhs, w, preferred_element_type=f32)
        return fn

    def mac(q, i0, ni, j0, j1):
        def fn():
            ld = lambda base, b: (vb[pl.ds(base + 32 * b + 8 * q, 8), :], vb[pl.ds(base + 32 * b + 16 + 8 * q, 8), :])
            zr, zi = st.pop('z') if j0 > 0 else ({}, {})
            ucache = {}
            for j in range(j0, j1):
                kr, ki = ld(V_KF, j)
                for i in range(max(i0, j), i0 + ni):
                    if i - j not in ucache:
                        ucache[i - j] = ld(V_UF, i - j)
                    ur, ui = ucache[i - j]
                    if i not in zr:
                        zr[i] = kr * ur - ki * ui
                        zi[i] = kr * ui + ki * ur
                    else:
                        zr[i] = zr[i] + kr * ur - ki * ui
                        zi[i] = zi[i] + kr * ui + ki * ur
            vb[pl.ds(frow, 8), :] = zr[i0 + ni - 1]
            if j1 < i0 + ni:
                st['z'] = (zr, zi)
            elif q == 0:
                for i in range(i0, i0 + ni):
                    vb[pl.ds(V_Z + 16 * (i - i0), 16), :] = jnp.concatenate([zr[i], zi[i]], axis=0)
            else:
                row = pl.multiple_of(r[0] * 32, 32) + r[1] * 16
                for i in range(i0, i0 + ni):
                    ar = vb[pl.ds(V_Z + 16 * (i - i0), 8), :]
                    ai = vb[pl.ds(V_Z + 16 * (i - i0) + 8, 8), :]
                    yf[buf, i, 0, pl.ds(row, 16), :] = jnp.concatenate([ar + zr[i], ai - zi[i]], axis=0).astype(bf16)
                    yf[buf, i, 1, pl.ds(row, 16), :] = jnp.concatenate([ar - zr[i], ai + zi[i]], axis=0).astype(bf16)
        return (8 * sum(1 for j in range(j0, j1) for i in range(max(i0, j), i0 + ni)), fn)

    fwd = [fwd_k(((4, 2, 1), (5, 0, 1), (6, 6, 1), (7, 0, 1))), fwd_k(((0, 0, 1), (1, 0, 1), (2, 0, 1), (3, 0, 1))),
           fwd_k(((4, 0, 2), (6, 0, 2), (6, 2, 2), (6, 4, 2))), fwd_u(0, 8), fwd_u(8, 16)]
    macs = []
    for i0 in range(0, NBLK, 2):
        for q in range(2):
            for j0 in range(0, i0 + 2, MACJ):
                macs.append(mac(q, i0, 2, j0, min(j0 + MACJ, i0 + 2)))
    return fwd, macs


def _inv_piece(c, b, buf, g_ref, us, vec, yf, outb):
    rows = pl.ds(b * 64 if isinstance(b, int) else pl.multiple_of(b * 64, 64), 64)
    rnd = lambda v: v.astype(bf16).astype(f32)
    uw = us[c, rows, :]
    dsk = vec[1, pl.ds(c, 1), :]
    o = []
    for par, u in enumerate((uw << 16, uw & u32(0xFFFF0000))):
        y = jnp.dot(_ld16(g_ref, par, slice(None)), _ld16(yf, buf, b, par, slice(None)), preferred_element_type=f32)
        o.append(pltpu.bitcast(rnd(rnd(y) + rnd(pltpu.bitcast(u, f32) * dsk)), u32))
    outb[c, rows, :] = (o[0] >> 16) | o[1]


def _attn_fill():
    r = lax.broadcasted_iota(jnp.int32, (NATT, NATT), 0)
    c = lax.broadcasted_iota(jnp.int32, (NATT, NATT), 1)
    head = lambda i: jnp.where(i < 2 * SEG, i // SEG, (i - 2 * SEG) // PRE)
    pos = lambda i: jnp.where(i < 2 * SEG, i % SEG, i % PRE)
    is_mem = lambda i: (i < 2 * SEG) & (i % SEG < M)
    same = head(r) == head(c)
    allowed = same & (is_mem(r) | is_mem(c) | (pos(r) >= pos(c)))
    return jnp.where(allowed, 0.0, jnp.where(same, -1e9 * LOG2E, -jnp.inf)).astype(f32)


def _kernel(zero_hbm, x_hbm, mem0_hbm, wq_hbm, wk_hbm, wv_hbm, wo_hbm,
            u_hbm, p0, p1, p2, p3, p4, p5, ldt_hbm, dsk_hbm, fs_hbm, g_hbm,
            out_hbm,
            wq, wk, wv, wo, xb, xs, h_ref, outs, fill_ref,
            praw, par, us, taps, vb, vm, vu, pacc, yf, outb, vec, vraw, fs_ref, g_ref, zero_ref,
            sem_s, sem_w, sem_o, sem_xb, sem_x, sem_p, sem_u, sem_out, pre, own, lo0, lo1):
    wqkv = (wq, wk, wv)
    scale = E ** -0.5

    whbm = [w.bitcast(u32) for w in (wq_hbm, wk_hbm, wv_hbm)]

    def wcp(j, m, p):
        return pltpu.make_async_copy(whbm[m].at[:, p, j, :], wqkv[m].at[p, j], sem_w.at[(j * 3 + m) * 2 + p])

    xu = x_hbm.bitcast(u32)
    xcs = [pltpu.make_async_copy(xu.at[:, t, pl.ds(0, PRE // 2), pl.ds(c * 128, 128)],
                                 xb.at[c, :, pl.ds(t * (PRE // 2), PRE // 2), :], sem_xb.at[2 * c + t])
           for c in range(8) for t in range(2)]
    xcp1 = pltpu.make_async_copy(x_hbm.at[:, :, pl.ds(PRE, TOK), :], xs, sem_x.at[0])
    pcs = [pltpu.make_async_copy(p, praw.at[k], sem_p.at[k]) for k, p in enumerate((p0, p1, p2, p3, p4, p5))]
    ccs = [pltpu.make_async_copy(fs_hbm, fs_ref, sem_p.at[6]), pltpu.make_async_copy(g_hbm, g_ref, sem_p.at[7])]
    wou = wo_hbm.bitcast(u32)
    ocs = [pltpu.make_async_copy(wou.at[:, pl.ds(c * 128, 128)], wo.at[c], sem_o.at[c]) for c in range(8)]
    uu = u_hbm.bitcast(u32)
    ucs = [pltpu.make_async_copy(uu.at[:, pl.ds(c * 128, 128)], us.at[c], sem_u.at[c]) for c in range(NT)]

    zcp = pltpu.make_async_copy(zero_hbm, zero_ref, sem_s.at[0])
    scs = [pltpu.make_async_copy(mem0_hbm, h_ref.at[pl.ds(0, M)], sem_s.at[1]),
           pltpu.make_async_copy(ldt_hbm, vraw.at[0], sem_s.at[2]),
           pltpu.make_async_copy(dsk_hbm, vraw.at[1], sem_s.at[3])]
    w0cs = [[pltpu.make_async_copy(whbm[0].at[pl.ds(half * (DM // 4), DM // 4), p, 0, :],
                                   wq.at[p, 0, pl.ds(half * (DM // 4), DM // 4)], sem_s.at[4 + 2 * half + p])
             for p in range(2)] for half in range(2)]
    for cp in [zcp] + w0cs[0] + xcs[:8]:
        cp.start()
    vu[pl.ds(8, 8), :] = pltpu.bitcast(jnp.full((8, 128), 0x0000FFFF, u32), f32)
    vu[pl.ds(16, 8), :] = pltpu.bitcast(jnp.full((8, 128), 0xFFFF0000, u32), f32)
    taps[...] = jnp.zeros(taps.shape, f32)
    yf[1] = jnp.zeros(yf.shape[1:], bf16)
    fill_ref[pl.ds(0, NATT), :] = _attn_fill()
    for cp in w0cs[1] + xcs[8:] + scs:
        cp.start()
    zcp.wait()

    def opaque_row(k, buf):
        return pl.multiple_of(jnp.clip(zero_ref[k] * 8, 0, buf.shape[0] - 8), 8)

    bufs = (vb, vm, vu, par)
    fence_rows = [opaque_row(0, b) for b in bufs]
    done_vb, done_vm = opaque_row(1, vb), opaque_row(1, vm)

    class Pacer:
        def __init__(self, segments):
            self.t = 0.0
            self.todo = []
            for (pieces, buf, t0, t1) in segments:
                total = float(sum(c for c, _ in pieces)) or 1.0
                done = 0.0
                for (cst, fn) in pieces:
                    self.todo.append((t0 + (t1 - t0) * done / total, fn, buf))
                    done += cst

        def __call__(self, v, dt=1.0):
            self.t += dt
            fenced = []
            while self.todo and self.todo[0][0] < self.t:
                _, fn, buf = self.todo.pop(0)
                if not any(b is buf for b in fenced):
                    buf[pl.ds([r for b, r in zip(bufs, fence_rows) if b is buf][0], 8), :] = v
                    fenced.append(buf)
                fn()

        def finished(self):
            return not self.todo

    def unpair(j, m, r0, nr):
        def fn():
            rows = pl.ds(r0, nr)
            m_lo = pltpu.bitcast(vu[pl.ds(8, 8), :], u32)[None]
            m_hi = pltpu.bitcast(vu[pl.ds(16, 8), :], u32)[None]
            a = wqkv[m][0, j, rows, :].reshape(nr // 8, 8, E)
            b = wqkv[m][1, j, rows, :].reshape(nr // 8, 8, E)
            wqkv[m][0, j, rows, :] = ((a & m_lo) | ((b & m_lo) << 16)).reshape(nr, E)
            wqkv[m][1, j, rows, :] = (((a & m_hi) >> 16) | (b & m_hi)).reshape(nr, E)
        return (nr, fn)

    def unpair_pieces(items, lo=0, hi=DM // 2):
        return [unpair(j, m, r0, UNP) for (j, m) in items for r0 in range(lo, hi, UNP)]

    items = [(j, m) for j in range(NP) for m in range(3)]
    wcs = lambda lo, hi: [wcp(j, m, p) for (j, m) in items[lo:hi] for p in range(2)]
    rest = ocs + ccs + ucs + [xcp1]
    starts = [[] for _ in range(2 * len(items))]
    n_w, n_r = 1, 0
    for unit in sorted(STARTS):
        w_hi, with_par, r_hi = STARTS[unit]
        starts[unit] = (pcs if with_par else []) + wcs(n_w, w_hi) + rest[n_r:r_hi]
        n_w, n_r = w_hi, r_hi
    assert n_w == len(items) and n_r == len(rest)
    n_chunk = 2 * (T0 // RC)
    prep = _prep_pieces(praw, vec, par)
    kg0 = [pc for r in range(8) for pc in _kgen_pieces(0, r, par, vb, taps, 0, done_vb, 1, 4)]
    t_a, t_b, t_c, t_d = [v * n_chunk for v in BPLAN]
    fence_x = Pacer([(prep[0], par, t_a, t_b), (kg0, vb, t_b, t_c), (prep[1], par, t_c, t_d)])
    landed = 1
    for it, (j, m) in enumerate(items):
        fence_w = None
        for half in range(2):
            for cp in starts[2 * it + half]:
                cp.start()
            if it == 0:
                for cp in w0cs[half] + xcs[8 * half:8 * half + 8]:
                    cp.wait()
                for _, fn in unpair_pieces(items[:1], half * (DM // 4), (half + 1) * (DM // 4)):
                    fn()
                fence_w = Pacer([])
            elif half == 0:
                late = landed == it
                if it in WAITS:
                    for cp in wcs(landed, WAITS[it]) + (pcs + scs if it == PAR_WAIT else []):
                        cp.wait()
                    landed = WAITS[it]
                    if it == PAR_WAIT:
                        vec[pl.ds(0, 2)] = vraw[pl.ds(0, 2)].astype(f32)
                if late:
                    for _, fn in unpair_pieces(items[it:it + 1]):
                        fn()
                fence_w = Pacer([(unpair_pieces(items[it + 1:min(it + 2, landed)]), vu, 0.0, n_chunk * 0.7)])
            for p in range(2):
                w = pltpu.bitcast(wqkv[m][p, j, pl.ds(half * (DM // 4), DM // 4), :], bf16)
                lhs = jnp.concatenate([pltpu.bitcast(xb[c].reshape(T0 // 2, 128), bf16)
                                       for c in range(4 * half, 4 * half + 4)], axis=1)
                res = jnp.dot(lhs, w, preferred_element_type=f32)
                for rc in range(T0 // RC):
                    rows = pl.ds(rc * RC, RC)
                    v = res[rc * RC:(rc + 1) * RC]
                    if half == 1:
                        v = v + pacc[p, rows, :]
                    if p == 0 or half == 0:
                        pacc[p, rows, :] = v
                    else:
                        pr = jnp.concatenate([pacc[0, rows, :].reshape(RC // PRE, PRE, E),
                                              v.reshape(RC // PRE, PRE, E)], axis=1)
                        pre[pl.ds(rc * (RC // PRE), RC // PRE), m * NP + j] = pr.astype(bf16)
                    fence_w(v[:8], 0.5)
                    fence_x(v[:8], 0.5)
        assert fence_w.finished() and landed > it
    assert fence_x.finished()
    for cp in ocs + ucs + ccs + [xcp1]:
        cp.wait()

    def outa_cp(row, n):
        return pltpu.make_async_copy(outs.at[pl.ds(row, n)], out_hbm.at[pl.ds(row, n), pl.ds(0, DM)], sem_out.at[0])

    def outb_cp(c, row, n, sem):
        col = DM + c * 128
        return pltpu.make_async_copy(
            outb.at[c, pl.ds(row, n)],
            out_hbm.bitcast(u32).at[pl.ds(row, n), pl.ds(col if isinstance(col, int) else pl.multiple_of(col, 128), 128)],
            sem_out.at[sem])

    def one_step(i, odd, fwd, fence):
        s = 2 * i + odd
        lo_cur = (lo0, lo1)[odd]
        base = pl.multiple_of(2 * SEG * i, 2 * SEG)
        h_ref[pl.ds(M, TOK), :] = xs[i, odd]
        h = h_ref[...]
        scores = {}
        probs = {}

        ct = i >> 2
        r = s & 7
        buf = ct & 1
        cprev = (ct + NT - 1) & (NT - 1)

        def project(j, m, p):
            w = pltpu.bitcast(wqkv[m][p, j], bf16)
            res = jnp.dot(h, w, preferred_element_type=f32)
            own[m * NP + j, pl.ds(SEG * p, SEG), :] = res.astype(bf16)
            fence(res[:M])

        def gather(m, j):
            return pltpu.bitcast(jnp.concatenate([own.bitcast(u32)[m * NP + j],
                                                  pre.bitcast(u32)[s, m * NP + j]], axis=0), bf16)

        def stage_qk(j):
            scores[j] = lax.dot_general(gather(0, j), gather(1, j), (((1,), (1,)), ((), ())),
                                        preferred_element_type=f32)

        def stage_b(j):
            fl = fill_ref[pl.ds(0, NATT), :]
            sc = jnp.where(fl == 0.0, scores.pop(j) * (scale * LOG2E), fl)
            e = jnp.exp2(sc - jnp.max(sc, axis=-1, keepdims=True))
            den = jnp.sum(e, axis=-1, keepdims=True)
            probs[j] = (e * pl.reciprocal(den, approx=True)).astype(bf16)

        def stage_c(j):
            o = jnp.dot(probs[j], gather(2, j), preferred_element_type=f32)
            for p in range(2):
                hh = 2 * j + p
                lo_cur[hh, pl.ds(0, SEG), :] = o[p * SEG:(p + 1) * SEG].astype(bf16)
                ob = o[2 * SEG + p * PRE:2 * SEG + (p + 1) * PRE]
                lo1[hh, pl.ds(SEG + odd * PRE, PRE), :] = ob.astype(bf16)

        acc = [None] * 8

        def stage_d(h0, h1, last=False):
            lhs = jnp.concatenate([_ld16(lo_cur, hh, slice(None)) for hh in range(h0, h1)], axis=1)
            for c in range(8):
                w = pltpu.bitcast(wo[c, pl.ds(h0 * 64, (h1 - h0) * 64), :], bf16)
                res = jnp.dot(lhs, w, preferred_element_type=f32)
                acc[c] = res if acc[c] is None else acc[c] + res
                if not last:
                    fence(res[:M], (h1 - h0) / 8.0 * (1.5 if odd else 1.0))
                else:
                    rb = acc[c].astype(bf16)
                    cols = pl.ds(c * 128, 128)
                    h_ref[pl.ds(0, M), cols] = rb[:M]
                    outs[pl.ds(base + (odd * SEG + PRE), TOK), cols] = rb[M:SEG]
                    if odd:
                        outs[pl.ds(base, PRE), cols] = rb[SEG:SEG + PRE]
                        outs[pl.ds(base + SEG, PRE), cols] = rb[SEG + PRE:]

        def attn_group(jq, jc):
            for j in jq:
                stage_qk(j)
            for j in jc:
                stage_c(j)
            for j in jq:
                stage_b(j)

        for p in fwd:
            p()
        for t in range(2):
            _inv_piece(cprev, 2 * r + t, 1 - buf, g_ref, us, vec, yf, outb)
        dots = [(2 * g + jj, m, p) for g in range(NP // 2) for m in range(3) for jj in range(2) for p in range(2)]
        for n, d in enumerate(dots):
            project(*d)
            g, k = divmod(n - 8, 12)
            if k == 0 and g >= 1:
                attn_group((2 * g - 2, 2 * g - 1), (2 * g - 4, 2 * g - 3) if g >= 2 else ())
        stage_d(0, 8)
        attn_group((14, 15), (12, 13))
        stage_d(8, 16)
        attn_group((), (14, 15))
        stage_d(16, 28)
        stage_d(28, 32, last=True)

    def two_steps(i, carry):
        ct = i >> 2
        cprev = (ct + NT - 1) & (NT - 1)
        conv = [_conv_pieces(ct, (i & 3, odd), ct & 1, fs_ref, us, taps, vm, yf, done_vm) for odd in range(2)]
        kgen = [_kgen_pieces((ct + 1) & (NT - 1), (i & 3, odd), par, vb, taps, ct + 1, done_vb, 2, 2)
                for odd in range(2)]
        work = {'k0': (kgen[0], vb), 'k1': (kgen[1], vb), 'm0': (conv[0][1], vm), 'm1': (conv[1][1], vm)}
        fence = Pacer([work[k] + (t0, t1) for (k, t0, t1) in PLAN])
        for odd in range(2):
            one_step(i, odd, conv[odd][0], fence)
        assert fence.finished()
        outa_cp(pl.multiple_of(2 * SEG * i, 2 * SEG), 2 * SEG).start()
        outb_cp(cprev, pl.multiple_of((i & 3) * 256, 256), 256, jnp.where(i < 4, 2, 1)).start()
        return carry

    lax.fori_loop(0, NSEG // 2, two_steps, 0)

    outb_cp(NT - 1, 0, L // 2, 2).wait()
    for b in range(NBLK):
        _inv_piece(NT - 1, b, (NT - 1) % 2, g_ref, us, vec, yf, outb)
        if b % 4 == 3:
            outb_cp(NT - 1, (b - 3) * 64, 256, 1).start()
    outa_cp(0, S).wait()
    pltpu.make_async_copy(outb, outb, sem_out.at[1]).wait()


@jax.jit
def pallas_concat_heads__memory_aug_recurrent_mem_tr__ssm_conv_s4__prompt_kernel(
    A_x, A_mem0, A_Wq, A_Wk, A_Wv, A_Wo, A_seg_len,
    B_u, B_A_re, B_A_im, B_B_re, B_B_im, B_C_re, B_C_im, B_log_dt, B_Dskip,
):
    del A_seg_len
    assert A_x.shape == (1, S, DM) and B_u.shape == (1, L, D)
    fs, g = _dft_consts()
    w4 = lambda w: w.reshape(DM // 2, 2, H, E)
    any_ = pl.BlockSpec(memory_space=pl.ANY)
    V = pltpu.VMEM
    out = pl.pallas_call(
        _kernel,
        out_shape=jax.ShapeDtypeStruct((S, DM + D), bf16),
        in_specs=[any_] * 18,
        out_specs=any_,
        scratch_shapes=[
            V((2, NP, DM // 2, E), u32),
            V((2, NP, DM // 2, E), u32),
            V((2, NP, DM // 2, E), u32),
            V((8, H * E // 2, 128), u32),
            V((8, NSEG // 2, PRE, 128), u32),
            V((NSEG // 2, 2, TOK, DM), bf16),
            V((M + TOK, DM), bf16),
            V((S, DM), bf16),
            V((96, NATT), f32),
            V((6, D, N), bf16),
            V((32 + NT * 6 * N, 128), f32),
            V((NT, L // 2, 128), u32),
            V((NT + 1, TAPROWS, 128), f32),
            V((V_ROWS, 128), f32),
            V((VM_ROWS, 128), f32),
            V((32, 128), f32),
            V((2, T0, 128), f32),
            V((2, NBLK, 2, BLK, 128), bf16),
            V((NT, L // 2, 128), u32),
            V((4, 8, 128), f32),
            V((8, 8, 128), bf16),
            V((8, NBLK * 32, 128), bf16),
            V((2, BLK // 2, 128), bf16),
            pltpu.SMEM((2,), jnp.int32),
            pltpu.SemaphoreType.DMA((8,)),
            pltpu.SemaphoreType.DMA((6 * NP,)),
            pltpu.SemaphoreType.DMA((8,)),
            pltpu.SemaphoreType.DMA((16,)),
            pltpu.SemaphoreType.DMA((1,)),
            pltpu.SemaphoreType.DMA((8,)),
            pltpu.SemaphoreType.DMA((NT,)),
            pltpu.SemaphoreType.DMA((3,)),
            V((NSEG, 3 * NP, 2 * PRE, E), bf16),
            V((3 * NP, 2 * SEG, E), bf16),
            V((H, SEG, E), bf16),
            V((H, SEG + 2 * PRE, E), bf16),
        ],
        compiler_params=pltpu.CompilerParams(vmem_limit_bytes=110 * 1024 * 1024, disable_bounds_checks=True),
    )(jnp.asarray(np.zeros((2,), np.int32)), A_x.reshape(NSEG // 2, 2, SEG, DM), A_mem0.reshape(M, DM),
      w4(A_Wq), w4(A_Wk), w4(A_Wv), A_Wo.reshape(H * E, DM),
      B_u.reshape(L, D), B_A_re, B_A_im, B_B_re, B_B_im, B_C_re, B_C_im,
      B_log_dt.reshape(8, 128), B_Dskip.reshape(8, 128),
      jnp.asarray(fs, bf16), jnp.asarray(g, bf16))
    return out.reshape(1, S, DM + D)
```

```python
import functools

import numpy as np
import jax
import jax.numpy as jnp
from jax import lax
import jax.experimental.pallas as pl
import jax.experimental.pallas.tpu as pltpu

bf16, f32, u32 = jnp.bfloat16, jnp.float32, jnp.uint32

S, DM, H, E, M, SEG = 2048, 1024, 32, 128, 8, 32
NSEG = S // SEG
TOK = 24
PRE = SEG - TOK
T0 = PRE * NSEG
NP = H // 2
NATT = 2 * (SEG + M)
LOG2E = 1.4426950408889634
L, D, N = 2048, 1024, 128
BLK = 128
NBLK = L // BLK
NT = D // 128
TAPROWS = 672
WINDOWS = ((0, 128, 0, 1), (128, 128, 1, 1), (256, 128, 2, 1), (320, 80, 3, 1),
           (384, 128, 4, 3), (480, 48, 7, 1), (512, 128, 8, 7), (624, 32, 15, 1))
V_YTAB = 8
V_START = V_YTAB + 256
V_STEP = V_START + 160
V_ROWS = V_STEP + 128 + 24
V_UF = 8
V_KF = V_UF + NBLK * 32
V_Z = V_KF + NBLK * 32
VM_ROWS = V_Z + 32 + 24
RC = 64
UNP = 64
WAITS = {1: 2, 2: 3, 3: 5, 4: 6, 5: 8, 7: 11, 10: 13, 12: 17, 16: 23, 22: 33, 32: 48}
PAR_WAIT = 10
STARTS = {0: (2, False, 0), 1: (3, False, 0), 2: (5, False, 0), 4: (6, False, 0), 6: (8, False, 0),
          8: (9, False, 0), 10: (11, False, 0), 14: (13, True, 0), 20: (17, False, 0), 24: (23, False, 0),
          32: (33, False, 0), 44: (48, False, 3), 64: (48, False, 19)}
BPLAN = (10.0, 12.0, 36.0, 47.7)
PLAN = (('k0', 0, 95), ('m0', 98, 123), ('k1', 124, 216), ('m1', 218, 250))
MACJ = 2


def _bf16_round_int(l):
    u = np.asarray(l, np.float32).view(np.uint32)
    r = (u + 0x7FFF + ((u >> 16) & 1)) & 0xFFFF0000
    return r.astype(np.uint32).view(np.float32).astype(np.int64)


def _tap_row(lp):
    return np.where(lp < 256, lp, np.where(lp < 512, 256 + (lp - 256) // 2,
                    np.where(lp < 1024, 384 + (lp - 512) // 4, 512 + (lp - 1024) // 8)))


@functools.lru_cache(maxsize=None)
def _dft_consts():
    t = np.arange(BLK)
    F = np.zeros((8, 32, BLK))
    G = np.zeros((2, BLK // 2, 8, 16))
    for r in range(8):
        f = 16 * r + 2 * np.arange(8)
        th = 2 * np.pi * (np.concatenate([f, BLK - 1 - f]) + 0.5) / (2 * BLK)
        F[r, :16] = np.cos(th[:, None] * t[None])
        F[r, 16:] = -np.sin(th[:, None] * t[None])
        for par in range(2):
            G[par, :, r, :8] = np.cos(th[None, :8] * t[par::2, None]) / BLK
            G[par, :, r, 8:] = -np.sin(th[None, :8] * t[par::2, None]) / BLK
    FS = np.zeros((8, NBLK, 32, 128))
    for (w0, wn, b0, nb) in WINDOWS:
        for j in range(b0, b0 + nb):
            rows = _tap_row(_bf16_round_int(BLK * j + t)) - w0
            assert rows.min() >= 0 and rows.max() < wn
            sel = np.zeros((BLK, 128))
            sel[t, rows] = 1.0
            FS[:, j] = F @ sel
    return (FS.reshape(8, NBLK * 32, 128).astype(np.float32),
            G.reshape(2, BLK // 2, 128).astype(np.float32))


def _ld16(ref, *idx):
    return pltpu.bitcast(ref.bitcast(u32)[idx + (slice(None),)], bf16)


def _cmul(a, b):
    return (a[0] * b[0] - a[1] * b[1], a[0] * b[1] + a[1] * b[0])


def _csq(a):
    return (a[0] * a[0] - a[1] * a[1], 2.0 * (a[0] * a[1]))


def _cexp(lr, li):
    m = jnp.exp(lr)
    return (m * jnp.cos(li), m * jnp.sin(li))


def _par_row(c, k):
    return 8 + (c * 6 + k) * N


def _prep_pieces(praw, vec, par):
    def stage1(c):
        def fn():
            tr = lambda k: praw[k, pl.ds(c * 128, 128), :].astype(f32).T
            dt = jnp.exp(vec[0, pl.ds(c, 1), :]).astype(bf16).astype(f32)
            cc = _cmul((tr(4), tr(5)), (dt * tr(2), dt * tr(3)))
            for k, v in ((0, dt * tr(0)), (1, dt * tr(1)), (4, cc[0]), (5, cc[1])):
                par[pl.ds(_par_row(c, k), N), :] = v
        return fn

    def stage2(c, n0):
        def fn():
            lr = par[pl.ds(_par_row(c, 0) + n0, 8), :]
            li = par[pl.ds(_par_row(c, 1) + n0, 8), :]
            for k, v in enumerate(_cexp(lr, li) + _cexp(lr * 128.0, li * 128.0)):
                par[pl.ds(_par_row(c, k) + n0, 8), :] = v
        return fn

    tile = lambda c: [(260, stage1(c))] + [(190, stage2(c, n0)) for n0 in range(0, N, 8)]
    return tile(0), [pc for c in range(1, NT) for pc in tile(c)]


def _kgen_pieces(c, r, par, vb, taps, tslot, frow, kni, ksplit):
    st = {}

    def put(row, z, h=None):
        if h is None:
            vb[pl.ds(row, 16), :] = z[0]
            vb[pl.ds(row + 16, 16), :] = z[1]
        else:
            vb[pl.ds(row + 8 * h, 8), :] = z[0]
            vb[pl.ds(row + 16 + 8 * h, 8), :] = z[1]

    def get(row, h=None):
        if h is None:
            return (vb[pl.ds(row, 16), :], vb[pl.ds(row + 16, 16), :])
        return (vb[pl.ds(row + 8 * h, 8), :], vb[pl.ds(row + 16 + 8 * h, 8), :])

    def ytab(k0, k1):
        return [vb[pl.ds(V_YTAB + 128 * part + 16 * k0, 16 * (k1 - k0)), :].reshape(k1 - k0, 16, 128)
                for part in range(2)]

    def params(k):
        if isinstance(r, int):
            return par[pl.ds(_par_row(c, k) + r * 16, 16), :]
        return par[pl.ds(pl.multiple_of(c * (6 * N) + r[0] * 32, 32) + (_par_row(0, k) + r[1] * 16), 16), :]

    def park():
        put(V_STEP, (params(0), params(1)))
        put(V_START + 32, (params(2), params(3)))
        put(V_START, (params(4), params(5)))

    def setup_y(h):
        def fn():
            z1 = get(V_STEP, h)
            z2 = _csq(z1)
            z4 = _csq(z2)
            s = lax.broadcasted_iota(jnp.int32, (8, 128), 0)
            fs = [(jnp.where((s >> k) & 1 == 1, z[0], 1.0), jnp.where((s >> k) & 1 == 1, z[1], 0.0))
                  for k, z in enumerate((z1, z2, z4))]
            y = _cmul(_cmul(fs[0], fs[1]), fs[2])
            for k in range(8):
                vb[pl.ds(V_YTAB + 16 * k + 8 * h, 8), :] = y[0]
                vb[pl.ds(V_YTAB + 128 + 16 * k + 8 * h, 8), :] = y[1]
                if k < 7:
                    y = _cmul(y, z1)
                    y = (jnp.where(s == 7 - k, 1.0, y[0]), jnp.where(s == 7 - k, 0.0, y[1]))
            z = z4
            for k in range(4):
                z = _csq(z)
                put(V_STEP + 32 * k, z, h)
        return fn

    def setup_hi():
        z = get(V_START + 32)
        cf = get(V_START)
        for g in range(1, 5):
            put(V_START + 32 * g, _cmul(cf, z))
            if g < 4:
                z = _csq(z)

    def square(k0, k1):
        def fn():
            rows = [pl.ds(V_YTAB + 128 * part + 16 * k0, 16 * (k1 - k0)) for part in range(2)]
            y = _csq((vb[rows[0], :], vb[rows[1], :]))
            vb[rows[0], :] = y[0]
            vb[rows[1], :] = y[1]
        return fn

    def rows_of(g, i0, ni):
        n_i = 16 + (g == 4)

        def fn():
            x = st.pop('x') if i0 > 0 else get(V_START + 32 * g)
            step = get(V_STEP + 32 * max(g - 1, 0))
            xs = []
            for t in range(ni):
                xs.append(x)
                if i0 + t + 1 < n_i:
                    x = _cmul(x, step)
            if i0 + ni < n_i:
                st['x'] = x
            acc = [None] * ni
            for k0 in range(0, 8, ksplit):
                yr, yi = ytab(k0, k0 + ksplit)
                for t in range(ni):
                    v = xs[t][0] * yr - xs[t][1] * yi
                    v = lax.slice_in_dim(v, 0, 8, axis=1) + lax.slice_in_dim(v, 8, 16, axis=1)
                    v = jnp.sum(pltpu.roll(v, k0, 1, stride=1, stride_axis=0), axis=0)
                    acc[t] = v if acc[t] is None else acc[t] + v
                if k0 + ksplit < 8:
                    vb[pl.ds(frow, 8), :] = acc[ni - 1]
            for t in range(ni):
                row = 128 * g + 8 * (i0 + t)
                a = acc[t]
                if row == 640:
                    a = jnp.where(lax.broadcasted_iota(jnp.int32, (8, 128), 0) == 0, a, 0.0)
                taps[tslot, pl.ds(row, 8), :] = taps[tslot, pl.ds(row, 8), :] + a
                if t == ni - 1:
                    vb[pl.ds(frow, 8), :] = a
        return fn

    pieces = [(30, park), (110, setup_y(0)), (110, setup_y(1)), (80, setup_hi)]
    for g in range(5):
        if g >= 2:
            pieces += [(40, square(0, 4)), (40, square(4, 8))]
        for i0 in range(0, 16 + (g == 4), kni):
            ni = min(kni, 16 + (g == 4) - i0)
            pieces.append((83 * ni, rows_of(g, i0, ni)))
    return pieces


def _conv_pieces(c, r, buf, fs_ref, us, taps, vb, yf, frow):
    st = {}

    def fwd_u(b0, b1):
        def fn():
            lhs = _ld16(fs_ref, 2 * r[0] + r[1], pl.ds(0, 16))
            for b in range(b0, b1):
                w = pltpu.bitcast(us[c, pl.ds(b * 64, 64), :], bf16)
                res = jnp.dot(lhs, w, preferred_element_type=f32)
                row = V_UF + 32 * b
                if b == 0:
                    vb[pl.ds(row, 32), :] = res
                else:
                    p = st['prev']
                    vb[pl.ds(row, 8), :] = res[0:8] - p[16:24]
                    vb[pl.ds(row + 8, 8), :] = res[8:16] + p[24:32]
                    vb[pl.ds(row + 16, 8), :] = res[16:24] + p[0:8]
                    vb[pl.ds(row + 24, 8), :] = res[24:32] - p[8:16]
                st['prev'] = res
        return fn

    def fwd_k(jobs):
        def fn():
            for (wi, t0, nb) in jobs:
                w0, wn, b0, _ = WINDOWS[wi]
                lhs = _ld16(fs_ref, 2 * r[0] + r[1], pl.ds((b0 + t0) * 16, nb * 16))[:, :wn]
                w = taps[c, pl.ds(w0, wn), :].astype(bf16)
                vb[pl.ds(V_KF + 32 * (b0 + t0), 32 * nb), :] = jnp.dot(lhs, w, preferred_element_type=f32)
        return fn

    def mac(q, i0, ni, j0, j1):
        def fn():
            ld = lambda base, b: (vb[pl.ds(base + 32 * b + 8 * q, 8), :], vb[pl.ds(base + 32 * b + 16 + 8 * q, 8), :])
            zr, zi = st.pop('z') if j0 > 0 else ({}, {})
            ucache = {}
            for j in range(j0, j1):
                kr, ki = ld(V_KF, j)
                for i in range(max(i0, j), i0 + ni):
                    if i - j not in ucache:
                        ucache[i - j] = ld(V_UF, i - j)
                    ur, ui = ucache[i - j]
                    if i not in zr:
                        zr[i] = kr * ur - ki * ui
                        zi[i] = kr * ui + ki * ur
                    else:
                        zr[i] = zr[i] + kr * ur - ki * ui
                        zi[i] = zi[i] + kr * ui + ki * ur
            vb[pl.ds(frow, 8), :] = zr[i0 + ni - 1]
            if j1 < i0 + ni:
                st['z'] = (zr, zi)
            elif q == 0:
                for i in range(i0, i0 + ni):
                    vb[pl.ds(V_Z + 16 * (i - i0), 16), :] = jnp.concatenate([zr[i], zi[i]], axis=0)
            else:
                rows = pl.ds(r[1] * 16, 16)
                for i in range(i0, i0 + ni):
                    ar = vb[pl.ds(V_Z + 16 * (i - i0), 8), :]
                    ai = vb[pl.ds(V_Z + 16 * (i - i0) + 8, 8), :]
                    yf[buf, i, r[0], 0, rows, :] = jnp.concatenate([ar + zr[i], ai - zi[i]], axis=0).astype(bf16)
                    yf[buf, i, r[0], 1, rows, :] = jnp.concatenate([ar - zr[i], ai + zi[i]], axis=0).astype(bf16)
        return (8 * sum(1 for j in range(j0, j1) for i in range(max(i0, j), i0 + ni)), fn)

    fwd = [fwd_k(((4, 2, 1), (5, 0, 1), (6, 6, 1), (7, 0, 1))), fwd_k(((0, 0, 1), (1, 0, 1), (2, 0, 1), (3, 0, 1))),
           fwd_k(((4, 0, 2), (6, 0, 2), (6, 2, 2), (6, 4, 2))), fwd_u(0, 8), fwd_u(8, 16)]
    macs = []
    for i0 in range(0, NBLK, 2):
        for q in range(2):
            for j0 in range(0, i0 + 2, MACJ):
                macs.append(mac(q, i0, 2, j0, min(j0 + MACJ, i0 + 2)))
    return fwd, macs


def _inv_piece(c, b, buf, g_ref, us, vec, yf, outb):
    rows = pl.ds(b * 64 if isinstance(b, int) else pl.multiple_of(b * 64, 64), 64)
    rnd = lambda v: v.astype(bf16).astype(f32)
    uw = us[c, rows, :]
    dsk = vec[1, pl.ds(c, 1), :]
    o = []
    for par, u in enumerate((uw << 16, uw & u32(0xFFFF0000))):
        w = _ld16(yf, buf, b, slice(None), par, slice(None)).reshape(BLK, 128)
        y = jnp.dot(_ld16(g_ref, par, slice(None)), w, preferred_element_type=f32)
        o.append(pltpu.bitcast(rnd(rnd(y) + rnd(pltpu.bitcast(u, f32) * dsk)), u32))
    outb[c, rows, :] = (o[0] >> 16) | o[1]


def _attn_fill():
    r = lax.broadcasted_iota(jnp.int32, (NATT, NATT), 0)
    c = lax.broadcasted_iota(jnp.int32, (NATT, NATT), 1)
    head = lambda i: jnp.where(i < 2 * SEG, i // SEG, (i - 2 * SEG) // PRE)
    pos = lambda i: jnp.where(i < 2 * SEG, i % SEG, i % PRE)
    is_mem = lambda i: (i < 2 * SEG) & (i % SEG < M)
    same = head(r) == head(c)
    allowed = same & (is_mem(r) | is_mem(c) | (pos(r) >= pos(c)))
    return jnp.where(allowed, 0.0, jnp.where(same, -1e9 * LOG2E, -jnp.inf)).astype(f32)


def _kernel(zero_hbm, x_hbm, mem0_hbm, wq_hbm, wk_hbm, wv_hbm, wo_hbm,
            u_hbm, p0, p1, p2, p3, p4, p5, ldt_hbm, dsk_hbm, fs_hbm, g_hbm,
            out_hbm,
            wq, wk, wv, wo, xb, xs, h_ref, outs, fill_ref,
            praw, par, us, taps, vb, vm, vu, pacc, yf, outb, vec, vraw, fs_ref, g_ref, zero_ref,
            sem_s, sem_w, sem_o, sem_xb, sem_x, sem_p, sem_u, sem_out, pre, own, lo0, lo1):
    wqkv = (wq, wk, wv)
    scale = E ** -0.5

    whbm = [w.bitcast(u32) for w in (wq_hbm, wk_hbm, wv_hbm)]

    def wcp(j, m, p):
        return pltpu.make_async_copy(whbm[m].at[:, p, j, :], wqkv[m].at[p, j], sem_w.at[(j * 3 + m) * 2 + p])

    xu = x_hbm.bitcast(u32)
    xcs = [pltpu.make_async_copy(xu.at[:, t, pl.ds(0, PRE // 2), pl.ds(c * 128, 128)],
                                 xb.at[c, :, pl.ds(t * (PRE // 2), PRE // 2), :], sem_xb.at[2 * c + t])
           for c in range(8) for t in range(2)]
    xcp1 = pltpu.make_async_copy(x_hbm.at[:, :, pl.ds(PRE, TOK), :], xs, sem_x.at[0])
    pcs = [pltpu.make_async_copy(p, praw.at[k], sem_p.at[k]) for k, p in enumerate((p0, p1, p2, p3, p4, p5))]
    ccs = [pltpu.make_async_copy(fs_hbm, fs_ref, sem_p.at[6]), pltpu.make_async_copy(g_hbm, g_ref, sem_p.at[7])]
    wou = wo_hbm.bitcast(u32)
    ocs = [pltpu.make_async_copy(wou.at[:, pl.ds(c * 128, 128)], wo.at[c], sem_o.at[c]) for c in range(8)]
    uu = u_hbm.bitcast(u32)
    ucs = [pltpu.make_async_copy(uu.at[:, pl.ds(c * 128, 128)], us.at[c], sem_u.at[c]) for c in range(NT)]

    zcp = pltpu.make_async_copy(zero_hbm, zero_ref, sem_s.at[0])
    scs = [pltpu.make_async_copy(mem0_hbm, h_ref.at[pl.ds(0, M)], sem_s.at[1]),
           pltpu.make_async_copy(ldt_hbm, vraw.at[0], sem_s.at[2]),
           pltpu.make_async_copy(dsk_hbm, vraw.at[1], sem_s.at[3])]
    w0cs = [[pltpu.make_async_copy(whbm[0].at[pl.ds(half * (DM // 4), DM // 4), p, 0, :],
                                   wq.at[p, 0, pl.ds(half * (DM // 4), DM // 4)], sem_s.at[4 + 2 * half + p])
             for p in range(2)] for half in range(2)]
    for cp in [zcp] + w0cs[0] + xcs[:8]:
        cp.start()
    vu[pl.ds(8, 8), :] = pltpu.bitcast(jnp.full((8, 128), 0x0000FFFF, u32), f32)
    vu[pl.ds(16, 8), :] = pltpu.bitcast(jnp.full((8, 128), 0xFFFF0000, u32), f32)
    taps[...] = jnp.zeros(taps.shape, f32)
    yf[1] = jnp.zeros(yf.shape[1:], bf16)
    fill_ref[pl.ds(0, NATT), :] = _attn_fill()
    for cp in w0cs[1] + xcs[8:] + scs:
        cp.start()
    zcp.wait()

    def opaque_row(k, buf):
        return pl.multiple_of(jnp.clip(zero_ref[k] * 8, 0, buf.shape[0] - 8), 8)

    bufs = (vb, vm, vu, par)
    fence_rows = [opaque_row(0, b) for b in bufs]
    done_vb, done_vm = opaque_row(1, vb), opaque_row(1, vm)

    class Pacer:
        def __init__(self, segments):
            self.t = 0.0
            self.todo = []
            for (pieces, buf, t0, t1) in segments:
                total = float(sum(c for c, _ in pieces)) or 1.0
                done = 0.0
                for (cst, fn) in pieces:
                    self.todo.append((t0 + (t1 - t0) * done / total, fn, buf))
                    done += cst

        def __call__(self, v, dt=1.0):
            self.t += dt
            fenced = []
            while self.todo and self.todo[0][0] < self.t:
                _, fn, buf = self.todo.pop(0)
                if not any(b is buf for b in fenced):
                    buf[pl.ds([r for b, r in zip(bufs, fence_rows) if b is buf][0], 8), :] = v
                    fenced.append(buf)
                fn()

        def finished(self):
            return not self.todo

    def unpair(j, m, r0, nr):
        def fn():
            rows = pl.ds(r0, nr)
            m_lo = pltpu.bitcast(vu[pl.ds(8, 8), :], u32)[None]
            m_hi = pltpu.bitcast(vu[pl.ds(16, 8), :], u32)[None]
            a = wqkv[m][0, j, rows, :].reshape(nr // 8, 8, E)
            b = wqkv[m][1, j, rows, :].reshape(nr // 8, 8, E)
            wqkv[m][0, j, rows, :] = ((a & m_lo) | ((b & m_lo) << 16)).reshape(nr, E)
            wqkv[m][1, j, rows, :] = (((a & m_hi) >> 16) | (b & m_hi)).reshape(nr, E)
        return (nr, fn)

    def unpair_pieces(items, lo=0, hi=DM // 2):
        return [unpair(j, m, r0, UNP) for (j, m) in items for r0 in range(lo, hi, UNP)]

    items = [(j, m) for j in range(NP) for m in range(3)]
    wcs = lambda lo, hi: [wcp(j, m, p) for (j, m) in items[lo:hi] for p in range(2)]
    rest = ocs + ccs + ucs + [xcp1]
    starts = [[] for _ in range(2 * len(items))]
    n_w, n_r = 1, 0
    for unit in sorted(STARTS):
        w_hi, with_par, r_hi = STARTS[unit]
        starts[unit] = (pcs if with_par else []) + wcs(n_w, w_hi) + rest[n_r:r_hi]
        n_w, n_r = w_hi, r_hi
    assert n_w == len(items) and n_r == len(rest)
    n_chunk = 2 * (T0 // RC)
    prep = _prep_pieces(praw, vec, par)
    kg0 = [pc for r in range(8) for pc in _kgen_pieces(0, r, par, vb, taps, 0, done_vb, 1, 4)]
    t_a, t_b, t_c, t_d = [v * n_chunk for v in BPLAN]
    fence_x = Pacer([(prep[0], par, t_a, t_b), (kg0, vb, t_b, t_c), (prep[1], par, t_c, t_d)])
    landed = 1
    for it, (j, m) in enumerate(items):
        fence_w = None
        for half in range(2):
            for cp in starts[2 * it + half]:
                cp.start()
            if it == 0:
                for cp in w0cs[half] + xcs[8 * half:8 * half + 8]:
                    cp.wait()
                for _, fn in unpair_pieces(items[:1], half * (DM // 4), (half + 1) * (DM // 4)):
                    fn()
                fence_w = Pacer([])
            elif half == 0:
                late = landed == it
                if it in WAITS:
                    for cp in wcs(landed, WAITS[it]) + (pcs + scs if it == PAR_WAIT else []):
                        cp.wait()
                    landed = WAITS[it]
                    if it == PAR_WAIT:
                        vec[pl.ds(0, 2)] = vraw[pl.ds(0, 2)].astype(f32)
                if late:
                    for _, fn in unpair_pieces(items[it:it + 1]):
                        fn()
                fence_w = Pacer([(unpair_pieces(items[it + 1:min(it + 2, landed)]), vu, 0.0, n_chunk * 0.7)])
            for p in range(2):
                w = pltpu.bitcast(wqkv[m][p, j, pl.ds(half * (DM // 4), DM // 4), :], bf16)
                lhs = jnp.concatenate([pltpu.bitcast(xb[c].reshape(T0 // 2, 128), bf16)
                                       for c in range(4 * half, 4 * half + 4)], axis=1)
                res = jnp.dot(lhs, w, preferred_element_type=f32)
                for rc in range(T0 // RC):
                    rows = pl.ds(rc * RC, RC)
                    v = res[rc * RC:(rc + 1) * RC]
                    if half == 1:
                        v = v + pacc[p, rows, :]
                    if p == 0 or half == 0:
                        pacc[p, rows, :] = v
                    else:
                        pr = jnp.concatenate([pacc[0, rows, :].reshape(RC // PRE, PRE, E),
                                              v.reshape(RC // PRE, PRE, E)], axis=1)
                        pre[pl.ds(rc * (RC // PRE), RC // PRE), m * NP + j] = pr.astype(bf16)
                    fence_w(v[:8], 0.5)
                    fence_x(v[:8], 0.5)
        assert fence_w.finished() and landed > it
    assert fence_x.finished()
    for cp in ocs + ucs + ccs + [xcp1]:
        cp.wait()

    def outa_cp(row, n):
        return pltpu.make_async_copy(outs.at[pl.ds(row, n)], out_hbm.at[pl.ds(row, n), pl.ds(0, DM)], sem_out.at[0])

    def outb_cp(c, row, n, sem):
        col = DM + c * 128
        return pltpu.make_async_copy(
            outb.at[c, pl.ds(row, n)],
            out_hbm.bitcast(u32).at[pl.ds(row, n), pl.ds(col if isinstance(col, int) else pl.multiple_of(col, 128), 128)],
            sem_out.at[sem])

    def one_step(i, odd, fwd, fence):
        s = 2 * i + odd
        lo_cur = (lo0, lo1)[odd]
        base = pl.multiple_of(2 * SEG * i, 2 * SEG)
        h_ref[pl.ds(M, TOK), :] = xs[i, odd]
        h = h_ref[...]
        scores = {}
        probs = {}

        ct = i >> 2
        r = s & 7
        buf = ct & 1
        cprev = (ct + NT - 1) & (NT - 1)

        def project(j, m, p):
            w = pltpu.bitcast(wqkv[m][p, j], bf16)
            res = jnp.dot(h, w, preferred_element_type=f32)
            own[m * NP + j, pl.ds(SEG * p, SEG), :] = res.astype(bf16)
            fence(res[:M])

        def gather(m, j):
            return pltpu.bitcast(jnp.concatenate([own.bitcast(u32)[m * NP + j],
                                                  pre.bitcast(u32)[s, m * NP + j]], axis=0), bf16)

        def stage_qk(j):
            scores[j] = lax.dot_general(gather(0, j), gather(1, j), (((1,), (1,)), ((), ())),
                                        preferred_element_type=f32)

        def stage_b(j):
            fl = fill_ref[pl.ds(0, NATT), :]
            sc = jnp.where(fl == 0.0, scores.pop(j) * (scale * LOG2E), fl)
            e = jnp.exp2(sc - jnp.max(sc, axis=-1, keepdims=True))
            den = jnp.sum(e, axis=-1, keepdims=True)
            probs[j] = (e * pl.reciprocal(den, approx=True)).astype(bf16)

        def stage_c(j):
            o = jnp.dot(probs[j], gather(2, j), preferred_element_type=f32)
            for p in range(2):
                hh = 2 * j + p
                lo_cur[hh, pl.ds(0, SEG), :] = o[p * SEG:(p + 1) * SEG].astype(bf16)
                ob = o[2 * SEG + p * PRE:2 * SEG + (p + 1) * PRE]
                lo1[hh, pl.ds(SEG + odd * PRE, PRE), :] = ob.astype(bf16)

        acc = [None] * 8

        def stage_d(h0, h1, last=False):
            lhs = jnp.concatenate([_ld16(lo_cur, hh, slice(None)) for hh in range(h0, h1)], axis=1)
            for c in range(8):
                w = pltpu.bitcast(wo[c, pl.ds(h0 * 64, (h1 - h0) * 64), :], bf16)
                res = jnp.dot(lhs, w, preferred_element_type=f32)
                acc[c] = res if acc[c] is None else acc[c] + res
                if not last:
                    fence(res[:M], (h1 - h0) / 8.0 * (1.5 if odd else 1.0))
                else:
                    rb = acc[c].astype(bf16)
                    cols = pl.ds(c * 128, 128)
                    h_ref[pl.ds(0, M), cols] = rb[:M]
                    outs[pl.ds(base + (odd * SEG + PRE), TOK), cols] = rb[M:SEG]
                    if odd:
                        outs[pl.ds(base, PRE), cols] = rb[SEG:SEG + PRE]
                        outs[pl.ds(base + SEG, PRE), cols] = rb[SEG + PRE:]

        def attn_group(jq, jc):
            for j in jq:
                stage_qk(j)
            for j in jc:
                stage_c(j)
            for j in jq:
                stage_b(j)

        for p in fwd:
            p()
        for t in range(2):
            _inv_piece(cprev, 2 * r + t, 1 - buf, g_ref, us, vec, yf, outb)
        dots = [(2 * g + jj, m, p) for g in range(NP // 2) for m in range(3) for jj in range(2) for p in range(2)]
        for n, d in enumerate(dots):
            project(*d)
            g, k = divmod(n - 8, 12)
            if k == 0 and g >= 1:
                attn_group((2 * g - 2, 2 * g - 1), (2 * g - 4, 2 * g - 3) if g >= 2 else ())
        stage_d(0, 8)
        attn_group((14, 15), (12, 13))
        stage_d(8, 16)
        attn_group((), (14, 15))
        stage_d(16, 28)
        stage_d(28, 32, last=True)

    def two_steps(i, carry):
        ct = i >> 2
        cprev = (ct + NT - 1) & (NT - 1)
        conv = [_conv_pieces(ct, (i & 3, odd), ct & 1, fs_ref, us, taps, vm, yf, done_vm) for odd in range(2)]
        kgen = [_kgen_pieces((ct + 1) & (NT - 1), (i & 3, odd), par, vb, taps, ct + 1, done_vb, 2, 2)
                for odd in range(2)]
        work = {'k0': (kgen[0], vb), 'k1': (kgen[1], vb), 'm0': (conv[0][1], vm), 'm1': (conv[1][1], vm)}
        fence = Pacer([work[k] + (t0, t1) for (k, t0, t1) in PLAN])
        for odd in range(2):
            one_step(i, odd, conv[odd][0], fence)
        assert fence.finished()
        outa_cp(pl.multiple_of(2 * SEG * i, 2 * SEG), 2 * SEG).start()
        outb_cp(cprev, pl.multiple_of((i & 3) * 256, 256), 256, jnp.where(i < 4, 2, 1)).start()
        return carry

    lax.fori_loop(0, NSEG // 2, two_steps, 0)

    outb_cp(NT - 1, 0, L // 2, 2).wait()
    for b in range(NBLK):
        _inv_piece(NT - 1, b, (NT - 1) % 2, g_ref, us, vec, yf, outb)
        if b % 4 == 3:
            outb_cp(NT - 1, (b - 3) * 64, 256, 1).start()
    outa_cp(0, S).wait()
    pltpu.make_async_copy(outb, outb, sem_out.at[1]).wait()


@jax.jit
def pallas_concat_heads__memory_aug_recurrent_mem_tr__ssm_conv_s4__prompt_kernel(
    A_x, A_mem0, A_Wq, A_Wk, A_Wv, A_Wo, A_seg_len,
    B_u, B_A_re, B_A_im, B_B_re, B_B_im, B_C_re, B_C_im, B_log_dt, B_Dskip,
):
    del A_seg_len
    assert A_x.shape == (1, S, DM) and B_u.shape == (1, L, D)
    fs, g = _dft_consts()
    w4 = lambda w: w.reshape(DM // 2, 2, H, E)
    any_ = pl.BlockSpec(memory_space=pl.ANY)
    V = pltpu.VMEM
    out = pl.pallas_call(
        _kernel,
        out_shape=jax.ShapeDtypeStruct((S, DM + D), bf16),
        in_specs=[any_] * 18,
        out_specs=any_,
        scratch_shapes=[
            V((2, NP, DM // 2, E), u32),
            V((2, NP, DM // 2, E), u32),
            V((2, NP, DM // 2, E), u32),
            V((8, H * E // 2, 128), u32),
            V((8, NSEG // 2, PRE, 128), u32),
            V((NSEG // 2, 2, TOK, DM), bf16),
            V((M + TOK, DM), bf16),
            V((S, DM), bf16),
            V((96, NATT), f32),
            V((6, D, N), bf16),
            V((32 + NT * 6 * N, 128), f32),
            V((NT, L // 2, 128), u32),
            V((NT + 1, TAPROWS, 128), f32),
            V((V_ROWS, 128), f32),
            V((VM_ROWS, 128), f32),
            V((32, 128), f32),
            V((2, T0, 128), f32),
            V((2, NBLK, 4, 2, 32, 128), bf16),
            V((NT, L // 2, 128), u32),
            V((4, 8, 128), f32),
            V((8, 8, 128), bf16),
            V((8, NBLK * 32, 128), bf16),
            V((2, BLK // 2, 128), bf16),
            pltpu.SMEM((2,), jnp.int32),
            pltpu.SemaphoreType.DMA((8,)),
            pltpu.SemaphoreType.DMA((6 * NP,)),
            pltpu.SemaphoreType.DMA((8,)),
            pltpu.SemaphoreType.DMA((16,)),
            pltpu.SemaphoreType.DMA((1,)),
            pltpu.SemaphoreType.DMA((8,)),
            pltpu.SemaphoreType.DMA((NT,)),
            pltpu.SemaphoreType.DMA((3,)),
            V((NSEG, 3 * NP, 2 * PRE, E), bf16),
            V((3 * NP, 2 * SEG, E), bf16),
            V((H, SEG, E), bf16),
            V((H, SEG + 2 * PRE, E), bf16),
        ],
        compiler_params=pltpu.CompilerParams(vmem_limit_bytes=110 * 1024 * 1024, disable_bounds_checks=True,
                                             disable_semaphore_checks=True),
    )(jnp.asarray(np.zeros((2,), np.int32)), A_x.reshape(NSEG // 2, 2, SEG, DM), A_mem0.reshape(M, DM),
      w4(A_Wq), w4(A_Wk), w4(A_Wv), A_Wo.reshape(H * E, DM),
      B_u.reshape(L, D), B_A_re, B_A_im, B_B_re, B_B_im, B_C_re, B_C_im,
      B_log_dt.reshape(8, 128), B_Dskip.reshape(8, 128),
      jnp.asarray(fs, bf16), jnp.asarray(g, bf16))
    return out.reshape(1, S, DM + D)
```

```python
import functools

import numpy as np
import jax
import jax.numpy as jnp
from jax import lax
import jax.experimental.pallas as pl
import jax.experimental.pallas.tpu as pltpu

bf16, f32, u32 = jnp.bfloat16, jnp.float32, jnp.uint32

S, DM, H, E, M, SEG = 2048, 1024, 32, 128, 8, 32
NSEG = S // SEG
TOK = 24
PRE = SEG - TOK
T0 = PRE * NSEG
NP = H // 2
NATT = 2 * (SEG + M)
LOG2E = 1.4426950408889634
L, D, N = 2048, 1024, 128
BLK = 128
NBLK = L // BLK
NT = D // 128
TAPROWS = 672
WINDOWS = ((0, 128, 0, 1), (128, 128, 1, 1), (256, 128, 2, 1), (320, 80, 3, 1),
           (384, 128, 4, 3), (480, 48, 7, 1), (512, 128, 8, 7), (624, 32, 15, 1))
V_YTAB = 8
V_START = V_YTAB + 256
V_STEP = V_START + 160
V_ROWS = V_STEP + 128 + 24
V_UF = 8
V_KF = V_UF + NBLK * 32
V_Z = V_KF + NBLK * 32
VM_ROWS = V_Z + 32 + 24
RC = 64
UNP = 64
WAITS = {1: 2, 2: 3, 3: 5, 4: 6, 5: 8, 7: 11, 10: 13, 12: 17, 16: 23, 22: 33, 32: 48}
PAR_WAIT = 10
STARTS = {0: (2, False, 0), 1: (3, False, 0), 2: (5, False, 0), 4: (6, False, 0), 6: (8, False, 0),
          8: (9, False, 0), 10: (11, False, 0), 14: (13, True, 0), 20: (17, False, 0), 24: (23, False, 0),
          32: (33, False, 0), 44: (48, False, 3), 64: (48, False, 19)}
BPLAN = (10.0, 12.0, 36.0, 47.7)
PLAN = (('k0', 0, 95), ('m0', 98, 123), ('k1', 124, 216), ('m1', 218, 250))
MACJ = 2


def _bf16_round_int(l):
    u = np.asarray(l, np.float32).view(np.uint32)
    r = (u + 0x7FFF + ((u >> 16) & 1)) & 0xFFFF0000
    return r.astype(np.uint32).view(np.float32).astype(np.int64)


def _tap_row(lp):
    return np.where(lp < 256, lp, np.where(lp < 512, 256 + (lp - 256) // 2,
                    np.where(lp < 1024, 384 + (lp - 512) // 4, 512 + (lp - 1024) // 8)))


@functools.lru_cache(maxsize=None)
def _dft_consts():
    t = np.arange(BLK)
    F = np.zeros((8, 32, BLK))
    G = np.zeros((2, BLK // 2, 8, 16))
    for r in range(8):
        f = 16 * r + 2 * np.arange(8)
        th = 2 * np.pi * (np.concatenate([f, BLK - 1 - f]) + 0.5) / (2 * BLK)
        F[r, :16] = np.cos(th[:, None] * t[None])
        F[r, 16:] = -np.sin(th[:, None] * t[None])
        for par in range(2):
            G[par, :, r, :8] = np.cos(th[None, :8] * t[par::2, None]) / BLK
            G[par, :, r, 8:] = -np.sin(th[None, :8] * t[par::2, None]) / BLK
    FS = np.zeros((8, NBLK, 32, 128))
    for (w0, wn, b0, nb) in WINDOWS:
        for j in range(b0, b0 + nb):
            rows = _tap_row(_bf16_round_int(BLK * j + t)) - w0
            assert rows.min() >= 0 and rows.max() < wn
            sel = np.zeros((BLK, 128))
            sel[t, rows] = 1.0
            FS[:, j] = F @ sel
    return (FS.reshape(8, NBLK * 32, 128).astype(np.float32),
            G.reshape(2, BLK // 2, 128).astype(np.float32))


def _ld16(ref, *idx):
    return pltpu.bitcast(ref.bitcast(u32)[idx + (slice(None),)], bf16)


def _cmul(a, b):
    return (a[0] * b[0] - a[1] * b[1], a[0] * b[1] + a[1] * b[0])


def _csq(a):
    return (a[0] * a[0] - a[1] * a[1], 2.0 * (a[0] * a[1]))


def _cexp(lr, li):
    m = jnp.exp(lr)
    return (m * jnp.cos(li), m * jnp.sin(li))


def _par_row(c, k):
    return 8 + (c * 6 + k) * N


def _prep_pieces(praw, vec, par):
    def stage1(c):
        def fn():
            tr = lambda k: praw[k, pl.ds(c * 128, 128), :].astype(f32).T
            dt = jnp.exp(vec[0, pl.ds(c, 1), :]).astype(bf16).astype(f32)
            cc = _cmul((tr(4), tr(5)), (dt * tr(2), dt * tr(3)))
            for k, v in ((0, dt * tr(0)), (1, dt * tr(1)), (4, cc[0]), (5, cc[1])):
                par[pl.ds(_par_row(c, k), N), :] = v
        return fn

    def stage2(c, n0):
        def fn():
            lr = par[pl.ds(_par_row(c, 0) + n0, 8), :]
            li = par[pl.ds(_par_row(c, 1) + n0, 8), :]
            for k, v in enumerate(_cexp(lr, li) + _cexp(lr * 128.0, li * 128.0)):
                par[pl.ds(_par_row(c, k) + n0, 8), :] = v
        return fn

    tile = lambda c: [(260, stage1(c))] + [(190, stage2(c, n0)) for n0 in range(0, N, 8)]
    return tile(0), [pc for c in range(1, NT) for pc in tile(c)]


def _kgen_pieces(c, r, par, vb, taps, tslot, frow, kni, ksplit):
    st = {}

    def put(row, z, h=None):
        if h is None:
            vb[pl.ds(row, 16), :] = z[0]
            vb[pl.ds(row + 16, 16), :] = z[1]
        else:
            vb[pl.ds(row + 8 * h, 8), :] = z[0]
            vb[pl.ds(row + 16 + 8 * h, 8), :] = z[1]

    def get(row, h=None):
        if h is None:
            return (vb[pl.ds(row, 16), :], vb[pl.ds(row + 16, 16), :])
        return (vb[pl.ds(row + 8 * h, 8), :], vb[pl.ds(row + 16 + 8 * h, 8), :])

    def ytab(k0, k1):
        return [vb[pl.ds(V_YTAB + 128 * part + 16 * k0, 16 * (k1 - k0)), :].reshape(k1 - k0, 16, 128)
                for part in range(2)]

    def params(k):
        if isinstance(r, int):
            return par[pl.ds(_par_row(c, k) + r * 16, 16), :]
        return par[pl.ds(pl.multiple_of(c * (6 * N) + r[0] * 32, 32) + (_par_row(0, k) + r[1] * 16), 16), :]

    def park():
        put(V_STEP, (params(0), params(1)))
        put(V_START + 32, (params(2), params(3)))
        put(V_START, (params(4), params(5)))

    def setup_y(h):
        def fn():
            z1 = get(V_STEP, h)
            z2 = _csq(z1)
            z4 = _csq(z2)
            s = lax.broadcasted_iota(jnp.int32, (8, 128), 0)
            fs = [(jnp.where((s >> k) & 1 == 1, z[0], 1.0), jnp.where((s >> k) & 1 == 1, z[1], 0.0))
                  for k, z in enumerate((z1, z2, z4))]
            y = _cmul(_cmul(fs[0], fs[1]), fs[2])
            for k in range(8):
                vb[pl.ds(V_YTAB + 16 * k + 8 * h, 8), :] = y[0]
                vb[pl.ds(V_YTAB + 128 + 16 * k + 8 * h, 8), :] = y[1]
                if k < 7:
                    y = _cmul(y, z1)
                    y = (jnp.where(s == 7 - k, 1.0, y[0]), jnp.where(s == 7 - k, 0.0, y[1]))
            z = z4
            for k in range(4):
                z = _csq(z)
                put(V_STEP + 32 * k, z, h)
        return fn

    def setup_hi():
        z = get(V_START + 32)
        cf = get(V_START)
        for g in range(1, 5):
            put(V_START + 32 * g, _cmul(cf, z))
            if g < 4:
                z = _csq(z)

    def square(k0, k1):
        def fn():
            rows = [pl.ds(V_YTAB + 128 * part + 16 * k0, 16 * (k1 - k0)) for part in range(2)]
            y = _csq((vb[rows[0], :], vb[rows[1], :]))
            vb[rows[0], :] = y[0]
            vb[rows[1], :] = y[1]
        return fn

    def rows_of(g, i0, ni):
        n_i = 16 + (g == 4)

        def fn():
            x = st.pop('x') if i0 > 0 else get(V_START + 32 * g)
            step = get(V_STEP + 32 * max(g - 1, 0))
            xs = []
            for t in range(ni):
                xs.append(x)
                if i0 + t + 1 < n_i:
                    x = _cmul(x, step)
            if i0 + ni < n_i:
                st['x'] = x
            acc = [None] * ni
            for k0 in range(0, 8, ksplit):
                yr, yi = ytab(k0, k0 + ksplit)
                for t in range(ni):
                    v = xs[t][0] * yr - xs[t][1] * yi
                    v = lax.slice_in_dim(v, 0, 8, axis=1) + lax.slice_in_dim(v, 8, 16, axis=1)
                    v = jnp.sum(pltpu.roll(v, k0, 1, stride=1, stride_axis=0), axis=0)
                    acc[t] = v if acc[t] is None else acc[t] + v
                if k0 + ksplit < 8:
                    vb[pl.ds(frow, 8), :] = acc[ni - 1]
            for t in range(ni):
                row = 128 * g + 8 * (i0 + t)
                a = acc[t]
                if row == 640:
                    a = jnp.where(lax.broadcasted_iota(jnp.int32, (8, 128), 0) == 0, a, 0.0)
                taps[tslot, pl.ds(row, 8), :] = taps[tslot, pl.ds(row, 8), :] + a
                if t == ni - 1:
                    vb[pl.ds(frow, 8), :] = a
        return fn

    pieces = [(30, park), (110, setup_y(0)), (110, setup_y(1)), (80, setup_hi)]
    for g in range(5):
        if g >= 2:
            pieces += [(40, square(0, 4)), (40, square(4, 8))]
        for i0 in range(0, 16 + (g == 4), kni):
            ni = min(kni, 16 + (g == 4) - i0)
            pieces.append((83 * ni, rows_of(g, i0, ni)))
    return pieces


def _conv_pieces(c, r, buf, fs_ref, us, taps, vb, yf, frow):
    st = {}

    def fwd_u(b0, b1):
        def fn():
            lhs = _ld16(fs_ref, 2 * r[0] + r[1], pl.ds(0, 16))
            for b in range(b0, b1):
                w = pltpu.bitcast(us[c, pl.ds(b * 64, 64), :], bf16)
                res = jnp.dot(lhs, w, preferred_element_type=f32)
                row = V_UF + 32 * b
                if b == 0:
                    vb[pl.ds(row, 32), :] = res
                else:
                    p = st['prev']
                    vb[pl.ds(row, 8), :] = res[0:8] - p[16:24]
                    vb[pl.ds(row + 8, 8), :] = res[8:16] + p[24:32]
                    vb[pl.ds(row + 16, 8), :] = res[16:24] + p[0:8]
                    vb[pl.ds(row + 24, 8), :] = res[24:32] - p[8:16]
                st['prev'] = res
        return fn

    def fwd_k(jobs):
        def fn():
            for (wi, t0, nb) in jobs:
                w0, wn, b0, _ = WINDOWS[wi]
                lhs = _ld16(fs_ref, 2 * r[0] + r[1], pl.ds((b0 + t0) * 16, nb * 16))[:, :wn]
                w = taps[c, pl.ds(w0, wn), :].astype(bf16)
                vb[pl.ds(V_KF + 32 * (b0 + t0), 32 * nb), :] = jnp.dot(lhs, w, preferred_element_type=f32)
        return fn

    def mac(q, i0, ni, j0, j1):
        def fn():
            ld = lambda base, b: (vb[pl.ds(base + 32 * b + 8 * q, 8), :], vb[pl.ds(base + 32 * b + 16 + 8 * q, 8), :])
            zr, zi = st.pop('z') if j0 > 0 else ({}, {})
            ucache = {}
            for j in range(j0, j1):
                kr, ki = ld(V_KF, j)
                for i in range(max(i0, j), i0 + ni):
                    if i - j not in ucache:
                        ucache[i - j] = ld(V_UF, i - j)
                    ur, ui = ucache[i - j]
                    if i not in zr:
                        zr[i] = kr * ur - ki * ui
                        zi[i] = kr * ui + ki * ur
                    else:
                        zr[i] = zr[i] + kr * ur - ki * ui
                        zi[i] = zi[i] + kr * ui + ki * ur
            vb[pl.ds(frow, 8), :] = zr[i0 + ni - 1]
            if j1 < i0 + ni:
                st['z'] = (zr, zi)
            elif q == 0:
                for i in range(i0, i0 + ni):
                    vb[pl.ds(V_Z + 16 * (i - i0), 16), :] = jnp.concatenate([zr[i], zi[i]], axis=0)
            else:
                rows = pl.ds(r[1] * 16, 16)
                for i in range(i0, i0 + ni):
                    ar = vb[pl.ds(V_Z + 16 * (i - i0), 8), :]
                    ai = vb[pl.ds(V_Z + 16 * (i - i0) + 8, 8), :]
                    yf[buf, i, r[0], 0, rows, :] = jnp.concatenate([ar + zr[i], ai - zi[i]], axis=0).astype(bf16)
                    yf[buf, i, r[0], 1, rows, :] = jnp.concatenate([ar - zr[i], ai + zi[i]], axis=0).astype(bf16)
        return (8 * sum(1 for j in range(j0, j1) for i in range(max(i0, j), i0 + ni)), fn)

    fwd = [fwd_k(((4, 2, 1), (5, 0, 1), (6, 6, 1), (7, 0, 1))), fwd_k(((0, 0, 1), (1, 0, 1), (2, 0, 1), (3, 0, 1))),
           fwd_u(0, 8), fwd_u(8, 16), fwd_k(((4, 0, 2), (6, 0, 2), (6, 2, 2), (6, 4, 2)))]
    macs = []
    for i0 in range(0, NBLK, 2):
        for q in range(2):
            for j0 in range(0, i0 + 2, MACJ):
                macs.append(mac(q, i0, 2, j0, min(j0 + MACJ, i0 + 2)))
    return fwd, macs


def _inv_piece(c, b, buf, g_ref, us, vec, yf, outb):
    rows = pl.ds(b * 64 if isinstance(b, int) else pl.multiple_of(b * 64, 64), 64)
    rnd = lambda v: v.astype(bf16).astype(f32)
    uw = us[c, rows, :]
    dsk = vec[1, pl.ds(c, 1), :]
    o = []
    for par, u in enumerate((uw << 16, uw & u32(0xFFFF0000))):
        w = _ld16(yf, buf, b, slice(None), par, slice(None)).reshape(BLK, 128)
        y = jnp.dot(_ld16(g_ref, par, slice(None)), w, preferred_element_type=f32)
        o.append(pltpu.bitcast(rnd(rnd(y) + rnd(pltpu.bitcast(u, f32) * dsk)), u32))
    outb[c, rows, :] = (o[0] >> 16) | o[1]


def _attn_fill():
    r = lax.broadcasted_iota(jnp.int32, (NATT, NATT), 0)
    c = lax.broadcasted_iota(jnp.int32, (NATT, NATT), 1)
    head = lambda i: jnp.where(i < 2 * SEG, i // SEG, (i - 2 * SEG) // PRE)
    pos = lambda i: jnp.where(i < 2 * SEG, i % SEG, i % PRE)
    is_mem = lambda i: (i < 2 * SEG) & (i % SEG < M)
    same = head(r) == head(c)
    allowed = same & (is_mem(r) | is_mem(c) | (pos(r) >= pos(c)))
    return jnp.where(allowed, 0.0, jnp.where(same, -1e9 * LOG2E, -jnp.inf)).astype(f32)


def _kernel(zero_hbm, x_hbm, mem0_hbm, wq_hbm, wk_hbm, wv_hbm, wo_hbm,
            u_hbm, p0, p1, p2, p3, p4, p5, ldt_hbm, dsk_hbm, fs_hbm, g_hbm,
            out_hbm,
            wq, wk, wv, wo, xb, xs, h_ref, outs, fill_ref,
            praw, par, us, taps, vb, vm, vu, pacc, yf, outb, vec, vraw, fs_ref, g_ref, zero_ref,
            sem_s, sem_w, sem_o, sem_xb, sem_x, sem_p, sem_u, sem_out, pre, own, lo0, lo1):
    wqkv = (wq, wk, wv)
    scale = E ** -0.5

    whbm = [w.bitcast(u32) for w in (wq_hbm, wk_hbm, wv_hbm)]

    def wcp(j, m, p):
        return pltpu.make_async_copy(whbm[m].at[:, p, j, :], wqkv[m].at[p, j], sem_w.at[(j * 3 + m) * 2 + p])

    xu = x_hbm.bitcast(u32)
    xcs = [pltpu.make_async_copy(xu.at[:, t, pl.ds(0, PRE // 2), pl.ds(c * 128, 128)],
                                 xb.at[c, :, pl.ds(t * (PRE // 2), PRE // 2), :], sem_xb.at[2 * c + t])
           for c in range(8) for t in range(2)]
    xcp1 = pltpu.make_async_copy(x_hbm.at[:, :, pl.ds(PRE, TOK), :], xs, sem_x.at[0])
    pcs = [pltpu.make_async_copy(p, praw.at[k], sem_p.at[k]) for k, p in enumerate((p0, p1, p2, p3, p4, p5))]
    ccs = [pltpu.make_async_copy(fs_hbm, fs_ref, sem_p.at[6]), pltpu.make_async_copy(g_hbm, g_ref, sem_p.at[7])]
    wou = wo_hbm.bitcast(u32)
    ocs = [pltpu.make_async_copy(wou.at[:, pl.ds(c * 128, 128)], wo.at[c], sem_o.at[c]) for c in range(8)]
    uu = u_hbm.bitcast(u32)
    ucs = [pltpu.make_async_copy(uu.at[:, pl.ds(c * 128, 128)], us.at[c], sem_u.at[c]) for c in range(NT)]

    zcp = pltpu.make_async_copy(zero_hbm, zero_ref, sem_s.at[0])
    scs = [pltpu.make_async_copy(mem0_hbm, h_ref.at[pl.ds(0, M)], sem_s.at[1]),
           pltpu.make_async_copy(ldt_hbm, vraw.at[0], sem_s.at[2]),
           pltpu.make_async_copy(dsk_hbm, vraw.at[1], sem_s.at[3])]
    w0cs = [[pltpu.make_async_copy(whbm[0].at[pl.ds(half * (DM // 4), DM // 4), p, 0, :],
                                   wq.at[p, 0, pl.ds(half * (DM // 4), DM // 4)], sem_s.at[4 + 2 * half + p])
             for p in range(2)] for half in range(2)]
    for cp in [zcp] + w0cs[0] + xcs[:8]:
        cp.start()
    vu[pl.ds(8, 8), :] = pltpu.bitcast(jnp.full((8, 128), 0x0000FFFF, u32), f32)
    vu[pl.ds(16, 8), :] = pltpu.bitcast(jnp.full((8, 128), 0xFFFF0000, u32), f32)
    taps[...] = jnp.zeros(taps.shape, f32)
    yf[1] = jnp.zeros(yf.shape[1:], bf16)
    fill_ref[pl.ds(0, NATT), :] = _attn_fill()
    for cp in w0cs[1] + xcs[8:] + scs:
        cp.start()
    zcp.wait()

    def opaque_row(k, buf):
        return pl.multiple_of(jnp.clip(zero_ref[k] * 8, 0, buf.shape[0] - 8), 8)

    bufs = (vb, vm, vu, par)
    fence_rows = [opaque_row(0, b) for b in bufs]
    done_vb, done_vm = opaque_row(1, vb), opaque_row(1, vm)

    class Pacer:
        def __init__(self, segments):
            self.t = 0.0
            self.todo = []
            for (pieces, buf, t0, t1) in segments:
                total = float(sum(c for c, _ in pieces)) or 1.0
                done = 0.0
                for (cst, fn) in pieces:
                    self.todo.append((t0 + (t1 - t0) * done / total, fn, buf))
                    done += cst

        def __call__(self, v, dt=1.0):
            self.t += dt
            fenced = []
            while self.todo and self.todo[0][0] < self.t:
                _, fn, buf = self.todo.pop(0)
                if not any(b is buf for b in fenced):
                    buf[pl.ds([r for b, r in zip(bufs, fence_rows) if b is buf][0], 8), :] = v
                    fenced.append(buf)
                fn()

        def finished(self):
            return not self.todo

    def unpair(j, m, r0, nr):
        def fn():
            rows = pl.ds(r0, nr)
            m_lo = pltpu.bitcast(vu[pl.ds(8, 8), :], u32)[None]
            m_hi = pltpu.bitcast(vu[pl.ds(16, 8), :], u32)[None]
            a = wqkv[m][0, j, rows, :].reshape(nr // 8, 8, E)
            b = wqkv[m][1, j, rows, :].reshape(nr // 8, 8, E)
            wqkv[m][0, j, rows, :] = ((a & m_lo) | ((b & m_lo) << 16)).reshape(nr, E)
            wqkv[m][1, j, rows, :] = (((a & m_hi) >> 16) | (b & m_hi)).reshape(nr, E)
        return (nr, fn)

    def unpair_pieces(items, lo=0, hi=DM // 2):
        return [unpair(j, m, r0, UNP) for (j, m) in items for r0 in range(lo, hi, UNP)]

    items = [(j, m) for j in range(NP) for m in range(3)]
    wcs = lambda lo, hi: [wcp(j, m, p) for (j, m) in items[lo:hi] for p in range(2)]
    rest = ocs + ccs + ucs + [xcp1]
    starts = [[] for _ in range(2 * len(items))]
    n_w, n_r = 1, 0
    for unit in sorted(STARTS):
        w_hi, with_par, r_hi = STARTS[unit]
        starts[unit] = (pcs if with_par else []) + wcs(n_w, w_hi) + rest[n_r:r_hi]
        n_w, n_r = w_hi, r_hi
    assert n_w == len(items) and n_r == len(rest)
    n_chunk = 2 * (T0 // RC)
    prep = _prep_pieces(praw, vec, par)
    kg0 = [pc for r in range(8) for pc in _kgen_pieces(0, r, par, vb, taps, 0, done_vb, 1, 4)]
    t_a, t_b, t_c, t_d = [v * n_chunk for v in BPLAN]
    fence_x = Pacer([(prep[0], par, t_a, t_b), (kg0, vb, t_b, t_c), (prep[1], par, t_c, t_d)])
    landed = 1
    for it, (j, m) in enumerate(items):
        fence_w = None
        for half in range(2):
            for cp in starts[2 * it + half]:
                cp.start()
            if it == 0:
                for cp in w0cs[half] + xcs[8 * half:8 * half + 8]:
                    cp.wait()
                for _, fn in unpair_pieces(items[:1], half * (DM // 4), (half + 1) * (DM // 4)):
                    fn()
                fence_w = Pacer([])
            elif half == 0:
                late = landed == it
                if it in WAITS:
                    for cp in wcs(landed, WAITS[it]) + (pcs + scs if it == PAR_WAIT else []):
                        cp.wait()
                    landed = WAITS[it]
                    if it == PAR_WAIT:
                        vec[pl.ds(0, 2)] = vraw[pl.ds(0, 2)].astype(f32)
                if late:
                    for _, fn in unpair_pieces(items[it:it + 1]):
                        fn()
                fence_w = Pacer([(unpair_pieces(items[it + 1:min(it + 2, landed)]), vu, 0.0, n_chunk * 0.7)])
            for p in range(2):
                w = pltpu.bitcast(wqkv[m][p, j, pl.ds(half * (DM // 4), DM // 4), :], bf16)
                lhs = jnp.concatenate([pltpu.bitcast(xb[c].reshape(T0 // 2, 128), bf16)
                                       for c in range(4 * half, 4 * half + 4)], axis=1)
                res = jnp.dot(lhs, w, preferred_element_type=f32)
                for rc in range(T0 // RC):
                    rows = pl.ds(rc * RC, RC)
                    v = res[rc * RC:(rc + 1) * RC]
                    if half == 1:
                        v = v + pacc[p, rows, :]
                    if p == 0 or half == 0:
                        pacc[p, rows, :] = v
                    else:
                        pr = jnp.concatenate([pacc[0, rows, :].reshape(RC // PRE, PRE, E),
                                              v.reshape(RC // PRE, PRE, E)], axis=1)
                        pre[pl.ds(rc * (RC // PRE), RC // PRE), m * NP + j] = pr.astype(bf16)
                    fence_w(v[:8], 0.5)
                    fence_x(v[:8], 0.5)
        assert fence_w.finished() and landed > it
    assert fence_x.finished()
    for cp in ocs + ucs + ccs + [xcp1]:
        cp.wait()

    def outa_cp(row, n):
        return pltpu.make_async_copy(outs.at[pl.ds(row, n)], out_hbm.at[pl.ds(row, n), pl.ds(0, DM)], sem_out.at[0])

    def outb_cp(c, row, n, sem):
        col = DM + c * 128
        return pltpu.make_async_copy(
            outb.at[c, pl.ds(row, n)],
            out_hbm.bitcast(u32).at[pl.ds(row, n), pl.ds(col if isinstance(col, int) else pl.multiple_of(col, 128), 128)],
            sem_out.at[sem])

    def one_step(i, odd, fwd, fence):
        s = 2 * i + odd
        lo_cur = (lo0, lo1)[odd]
        base = pl.multiple_of(2 * SEG * i, 2 * SEG)
        h_ref[pl.ds(M, TOK), :] = xs[i, odd]
        h = h_ref[...]
        scores = {}
        probs = {}

        ct = i >> 2
        r = s & 7
        buf = ct & 1
        cprev = (ct + NT - 1) & (NT - 1)

        def project(j, m, p):
            w = pltpu.bitcast(wqkv[m][p, j], bf16)
            res = jnp.dot(h, w, preferred_element_type=f32)
            own[m * NP + j, pl.ds(SEG * p, SEG), :] = res.astype(bf16)
            fence(res[:M])

        def gather(m, j):
            return pltpu.bitcast(jnp.concatenate([own.bitcast(u32)[m * NP + j],
                                                  pre.bitcast(u32)[s, m * NP + j]], axis=0), bf16)

        def stage_qk(j):
            scores[j] = lax.dot_general(gather(0, j), gather(1, j), (((1,), (1,)), ((), ())),
                                        preferred_element_type=f32)

        def stage_b(j):
            fl = fill_ref[pl.ds(0, NATT), :]
            sc = jnp.where(fl == 0.0, scores.pop(j) * (scale * LOG2E), fl)
            e = jnp.exp2(sc - jnp.max(sc, axis=-1, keepdims=True))
            den = jnp.sum(e, axis=-1, keepdims=True)
            probs[j] = (e * pl.reciprocal(den, approx=True)).astype(bf16)

        def stage_c(j):
            o = jnp.dot(probs[j], gather(2, j), preferred_element_type=f32)
            for p in range(2):
                hh = 2 * j + p
                lo_cur[hh, pl.ds(0, SEG), :] = o[p * SEG:(p + 1) * SEG].astype(bf16)
                ob = o[2 * SEG + p * PRE:2 * SEG + (p + 1) * PRE]
                lo1[hh, pl.ds(SEG + odd * PRE, PRE), :] = ob.astype(bf16)

        acc = [None] * 8

        def stage_d(h0, h1, last=False):
            lhs = jnp.concatenate([_ld16(lo_cur, hh, slice(None)) for hh in range(h0, h1)], axis=1)
            for c in range(8):
                w = pltpu.bitcast(wo[c, pl.ds(h0 * 64, (h1 - h0) * 64), :], bf16)
                res = jnp.dot(lhs, w, preferred_element_type=f32)
                acc[c] = res if acc[c] is None else acc[c] + res
                if not last:
                    fence(res[:M], (h1 - h0) / 8.0 * (1.5 if odd else 1.0))
                else:
                    rb = acc[c].astype(bf16)
                    cols = pl.ds(c * 128, 128)
                    h_ref[pl.ds(0, M), cols] = rb[:M]
                    outs[pl.ds(base + (odd * SEG + PRE), TOK), cols] = rb[M:SEG]
                    if odd:
                        outs[pl.ds(base, PRE), cols] = rb[SEG:SEG + PRE]
                        outs[pl.ds(base + SEG, PRE), cols] = rb[SEG + PRE:]

        def attn_group(jq, jc):
            for j in jq:
                stage_qk(j)
            for j in jc:
                stage_c(j)
            for j in jq:
                stage_b(j)

        for p in fwd[:-1]:
            p()
        for t in range(2):
            _inv_piece(cprev, 2 * r + t, 1 - buf, g_ref, us, vec, yf, outb)
        dots = [(2 * g + jj, m, p) for g in range(NP // 2) for m in range(3) for jj in range(2) for p in range(2)]
        for n, d in enumerate(dots):
            project(*d)
            if n == 13:
                fwd[-1]()
            g, k = divmod(n - 8, 12)
            if k == 0 and g >= 1:
                attn_group((2 * g - 2, 2 * g - 1), (2 * g - 4, 2 * g - 3) if g >= 2 else ())
        stage_d(0, 8)
        attn_group((14, 15), (12, 13))
        stage_d(8, 16)
        attn_group((), (14, 15))
        stage_d(16, 28)
        stage_d(28, 32, last=True)

    def two_steps(i, carry):
        ct = i >> 2
        cprev = (ct + NT - 1) & (NT - 1)
        conv = [_conv_pieces(ct, (i & 3, odd), ct & 1, fs_ref, us, taps, vm, yf, done_vm) for odd in range(2)]
        kgen = [_kgen_pieces((ct + 1) & (NT - 1), (i & 3, odd), par, vb, taps, ct + 1, done_vb, 2, 2)
                for odd in range(2)]
        work = {'k0': (kgen[0], vb), 'k1': (kgen[1], vb), 'm0': (conv[0][1], vm), 'm1': (conv[1][1], vm)}
        fence = Pacer([work[k] + (t0, t1) for (k, t0, t1) in PLAN])
        for odd in range(2):
            one_step(i, odd, conv[odd][0], fence)
        assert fence.finished()
        outa_cp(pl.multiple_of(2 * SEG * i, 2 * SEG), 2 * SEG).start()
        outb_cp(cprev, pl.multiple_of((i & 3) * 256, 256), 256, jnp.where(i < 4, 2, 1)).start()
        return carry

    lax.fori_loop(0, NSEG // 2, two_steps, 0)

    outb_cp(NT - 1, 0, L // 2, 2).wait()
    for b in range(NBLK):
        _inv_piece(NT - 1, b, (NT - 1) % 2, g_ref, us, vec, yf, outb)
        if b % 4 == 3:
            outb_cp(NT - 1, (b - 3) * 64, 256, 1).start()
    outa_cp(0, S).wait()
    pltpu.make_async_copy(outb, outb, sem_out.at[1]).wait()


@jax.jit
def pallas_concat_heads__memory_aug_recurrent_mem_tr__ssm_conv_s4__prompt_kernel(
    A_x, A_mem0, A_Wq, A_Wk, A_Wv, A_Wo, A_seg_len,
    B_u, B_A_re, B_A_im, B_B_re, B_B_im, B_C_re, B_C_im, B_log_dt, B_Dskip,
):
    del A_seg_len
    assert A_x.shape == (1, S, DM) and B_u.shape == (1, L, D)
    fs, g = _dft_consts()
    w4 = lambda w: w.reshape(DM // 2, 2, H, E)
    any_ = pl.BlockSpec(memory_space=pl.ANY)
    V = pltpu.VMEM
    out = pl.pallas_call(
        _kernel,
        out_shape=jax.ShapeDtypeStruct((S, DM + D), bf16),
        in_specs=[any_] * 18,
        out_specs=any_,
        scratch_shapes=[
            V((2, NP, DM // 2, E), u32),
            V((2, NP, DM // 2, E), u32),
            V((2, NP, DM // 2, E), u32),
            V((8, H * E // 2, 128), u32),
            V((8, NSEG // 2, PRE, 128), u32),
            V((NSEG // 2, 2, TOK, DM), bf16),
            V((M + TOK, DM), bf16),
            V((S, DM), bf16),
            V((96, NATT), f32),
            V((6, D, N), bf16),
            V((32 + NT * 6 * N, 128), f32),
            V((NT, L // 2, 128), u32),
            V((NT + 1, TAPROWS, 128), f32),
            V((V_ROWS, 128), f32),
            V((VM_ROWS, 128), f32),
            V((32, 128), f32),
            V((2, T0, 128), f32),
            V((2, NBLK, 4, 2, 32, 128), bf16),
            V((NT, L // 2, 128), u32),
            V((4, 8, 128), f32),
            V((8, 8, 128), bf16),
            V((8, NBLK * 32, 128), bf16),
            V((2, BLK // 2, 128), bf16),
            pltpu.SMEM((2,), jnp.int32),
            pltpu.SemaphoreType.DMA((8,)),
            pltpu.SemaphoreType.DMA((6 * NP,)),
            pltpu.SemaphoreType.DMA((8,)),
            pltpu.SemaphoreType.DMA((16,)),
            pltpu.SemaphoreType.DMA((1,)),
            pltpu.SemaphoreType.DMA((8,)),
            pltpu.SemaphoreType.DMA((NT,)),
            pltpu.SemaphoreType.DMA((3,)),
            V((NSEG, 3 * NP, 2 * PRE, E), bf16),
            V((3 * NP, 2 * SEG, E), bf16),
            V((H, SEG, E), bf16),
            V((H, SEG + 2 * PRE, E), bf16),
        ],
        compiler_params=pltpu.CompilerParams(vmem_limit_bytes=110 * 1024 * 1024, disable_bounds_checks=True,
                                             disable_semaphore_checks=True),
    )(jnp.asarray(np.zeros((2,), np.int32)), A_x.reshape(NSEG // 2, 2, SEG, DM), A_mem0.reshape(M, DM),
      w4(A_Wq), w4(A_Wk), w4(A_Wv), A_Wo.reshape(H * E, DM),
      B_u.reshape(L, D), B_A_re, B_A_im, B_B_re, B_B_im, B_C_re, B_C_im,
      B_log_dt.reshape(8, 128), B_Dskip.reshape(8, 128),
      jnp.asarray(fs, bf16), jnp.asarray(g, bf16))
    return out.reshape(1, S, DM + D)
```
